```python
import jax
import jax.numpy as jnp

def _softmax(x, axis=-1):
    return jax.nn.softmax(x, axis=axis)
def _gelu(x):
    return jax.nn.gelu(x, approximate=True)
def _silu(x):
    return jax.nn.silu(x)
def _sigmoid(x):
    return jax.nn.sigmoid(x)
def _layernorm(x, axis=-1, eps=1e-5):
    m = jnp.mean(x, axis=axis, keepdims=True)
    v = jnp.var(x, axis=axis, keepdims=True)
    return (x - m) / jnp.sqrt(v + eps)
def _scatter_add(tgt, idx, src, axis=0):
    return tgt.at[idx].add(src)
def _segment_sum(src, seg, n):
    return jax.ops.segment_sum(src, seg, n)
class _Rng:
    def __init__(self, key):
        self._k = key
    def _next(self):
        self._k, sub = jax.random.split(self._k)
        return sub
    def normal(self, shape):
        return jax.random.normal(self._next(), shape, dtype=jnp.bfloat16)
    def randint(self, lo, hi, shape):
        return jax.random.randint(self._next(), shape, lo, hi, dtype=jnp.int32)
    def uniform(self, shape, lo=0.0, hi=1.0):
        return jax.random.uniform(self._next(), shape, jnp.bfloat16, lo, hi)
    def permutation(self, n):
        return jax.random.permutation(self._next(), n)


kernel_name = 'concat_heads__sliding_local_dilated__spectral_gfnet__prompt'

def setup_inputs():
    _rng = _Rng(jax.random.key(int.from_bytes(__import__("os").urandom(4), "little")))
    _w = (lambda a: (lambda t: t.astype(jnp.bfloat16) if jnp.issubdtype(t.dtype, jnp.floating) else t)(jnp.asarray(a)))
    def _A_setup():
        B, S, D = 1, 2048, 576
        return {
            "x": _w((lambda *s: _rng.normal(s) * 0.05)(B, S, D)),
            "wqkv": _w((lambda *s: _rng.normal(s) * 0.05)(D, 3 * D)),
            "wo": _w((lambda *s: _rng.normal(s) * 0.05)(D, D)),
        }
    _A_in = _A_setup()

    def _B_setup():
        B, S, D = 1, 2048, 576
        Df = D // 2 + 1
        return {
            "x": _w((lambda *s: _rng.normal(s) * 0.05)(B, S, D)),
            "w_r": _w((lambda *s: _rng.normal(s) * 0.05)(S, Df) * 0.02),
            "w_i": _w((lambda *s: _rng.normal(s) * 0.05)(S, Df) * 0.02),
        }
    _B_in = _B_setup()

    return {
        "A_x": _A_in["x"],
        "A_wqkv": _A_in["wqkv"],
        "A_wo": _A_in["wo"],
        "B_x": _B_in["x"],
        "B_w_r": _B_in["w_r"],
        "B_w_i": _B_in["w_i"],
    }

def reference(A_x, A_wqkv, A_wo, B_x, B_w_r, B_w_i):
    def _A_ref(x, wqkv, wo):
        B, S, D = x.shape
        H = 32; Dh = D // H
        W, dil = 8, 2
        qkv = (lambda x, *d: x.transpose(*d))((x @ wqkv).reshape(B, S, 3, H, Dh), 2, 0, 3, 1, 4)
        q, k, v = qkv[0], qkv[1], qkv[2]
        scale = Dh ** -0.5
        pos = jnp.arange(S)
        off = jnp.arange(W) * dil
        idx = pos[:, None] - off[None, :]
        mask = idx >= 0
        idx_c = jnp.where(mask, idx, 0).reshape(-1)
        kg = k[:, :, idx_c, :].reshape(B, H, S, W, Dh)
        vg = v[:, :, idx_c, :].reshape(B, H, S, W, Dh)
        logits = jnp.einsum("bhsd,bhswd->bhsw", q, kg) * scale
        logits = jnp.where(mask[None, None, :, :], logits, -1e9)
        attn = _softmax(logits, axis=-1)
        o = jnp.einsum("bhsw,bhswd->bhsd", attn, vg)
        return (lambda x, *d: x.transpose(*d))(o, 0, 2, 1, 3).reshape(B, S, D) @ wo

    def _B_ref(x, w_r, w_i):
        B, S, D = x.shape
        X = (lambda x, axes=(-2,-1): jnp.fft.rfft2(x.astype(jnp.float32), axes=axes))(x, axes=(-2, -1))
        W = w_r + 1j * w_i
        X = X * W
        y = (lambda x, s, axes=(-2,-1): jnp.fft.irfft2(x, s=s, axes=axes).astype(jnp.bfloat16))(X, (S, D), axes=(-2, -1))
        return y

    a = _A_ref(A_x, A_wqkv, A_wo)
    b = _B_ref(B_x, B_w_r, B_w_i)
    return jnp.concatenate([a, b], axis=-1)
```

```python
import numpy as np

import jax
import jax.numpy as jnp
from jax import lax
import jax.experimental.pallas as pl
import jax.experimental.pallas.tpu as pltpu

S = 2048
D = 576
H = 32
DH = 18
W = 8
DF = D // 2 + 1
NR = 296

F32 = jnp.float32
BF16 = jnp.bfloat16
U32 = jnp.uint32

_C3 = float(np.sqrt(3.0) / 2)
_C1, _S1 = float(np.cos(2 * np.pi / 9)), float(np.sin(2 * np.pi / 9))
_C2, _S2 = float(np.cos(4 * np.pi / 9)), float(np.sin(4 * np.pi / 9))


def _bfly9_fwd(x):
    a0, ar, ai = [], [], []
    for j in range(3):
        t = x[j + 3] + x[j + 6]
        a0.append(x[j] + t)
        ar.append(x[j] - 0.5 * t)
        ai.append(x[j + 6] - x[j + 3])
    t = a0[1] + a0[2]
    u0 = a0[0] + t
    u3r = a0[0] - 0.5 * t
    u3i = a0[2] - a0[1]
    b1r = ar[1] * _C1 + ai[1] * (_C3 * _S1)
    b1i = ai[1] * (_C3 * _C1) - ar[1] * _S1
    b2r = ar[2] * _C2 + ai[2] * (_C3 * _S2)
    b2i = ai[2] * (_C3 * _C2) - ar[2] * _S2
    a_r, a_i = ar[0], ai[0] * _C3
    tr, ti = b1r + b2r, b1i + b2i
    dr, di = (b1r - b2r) * _C3, (b1i - b2i) * _C3
    u1r, u1i = a_r + tr, a_i + ti
    mr, mi = a_r - 0.5 * tr, a_i - 0.5 * ti
    return [u0, u1r, u1i, mr - di, mi + dr, u3r, u3i, mr + di, mi - dr]


def _bfly9_inv(v):
    u0, u1r, u1i, u7r, u7i, u3r, u3i, u4r, u4i = v
    mr, mi = u4r + u7r, u4i + u7i
    di, dr = (u4r - u7r) * _C3, (u7i - u4i) * _C3
    a_r, a_i = u1r + mr, u1i + mi
    tr, ti = u1r - 0.5 * mr, u1i - 0.5 * mi
    b1r, b2r, b1i, b2i = tr + dr, tr - dr, ti + di, ti - di
    ar = [a_r, b1r * _C1 - b1i * _S1, b2r * _C2 - b2i * _S2]
    ai = [a_i * _C3, b1r * (_C3 * _S1) + b1i * (_C3 * _C1),
          b2r * (_C3 * _S2) + b2i * (_C3 * _C2)]
    t = u0 - 0.5 * u3r
    a0 = [u0 + u3r, t - u3i, t + u3i]
    y = [None] * 9
    for j in range(3):
        t = a0[j] - 0.5 * ar[j]
        y[j] = a0[j] + ar[j]
        y[j + 3] = t - ai[j]
        y[j + 6] = t + ai[j]
    return y


def _bfly4(x, inverse):
    (ar, ai), (br, bi), (cr, ci), (dr, di) = x
    pr, pi, qr, qi = ar + cr, ai + ci, ar - cr, ai - ci
    sr, si, tr, ti = br + dr, bi + di, br - dr, bi - di
    y1, y3 = (qr + ti, qi - tr), (qr - ti, qi + tr)
    if inverse:
        y1, y3 = y3, y1
    return [(pr + sr, pi + si), y1, (pr - sr, pi - si), y3]


def _twiddle16(z, e, inverse):
    zr, zi = z
    e = (-e if inverse else e) % 16
    h = float(np.sqrt(0.5))
    if e == 0:
        return z
    if e == 4:
        return zi, -zr
    if e == 12:
        return -zi, zr
    if e == 2:
        return (zr + zi) * h, (zi - zr) * h
    if e == 14:
        return (zr - zi) * h, (zr + zi) * h
    if e == 6:
        return (zi - zr) * h, (zr + zi) * (-h)
    if e == 10:
        return (zr + zi) * (-h), (zr - zi) * h
    c, s = float(np.cos(2 * np.pi * e / 16)), float(np.sin(2 * np.pi * e / 16))
    return zr * c + zi * s, zi * c - zr * s


_GROUPS = (1, 2, 3, 4, 0)


def _group_classes(g):
    return sorted({g, g + 9, 9 - g, 18 - g}) if g else [0, 9]


_ROWGROUPS = [(k0, h) for g in _GROUPS for k0 in _group_classes(g) for h in range(2)]


def _to_words(m):
    u = np.ascontiguousarray(m, dtype=np.float32).view(np.uint32)
    u = (u + 0x7FFF + ((u >> 16) & 1)) >> 16
    return (u[0::2] | (u[1::2] << 16)).astype(np.uint32)


def _make_tables():
    basis = np.array(_bfly9_fwd(list(np.eye(9))))
    m_fwd = np.array([2 * (r % 32) + r // 32 for r in range(64)])
    lf, li = [], []
    for g in _GROUPS:
        rows = [k0 + 18 * i for k0 in _group_classes(g) for i in range(16)]
        if g == 0:
            rows += [DF - 1] + [-1] * 7
        cols = [2 * g - 1, 2 * g] if g else [0]
        a = basis[cols].T.astype(complex)
        n = len(rows)
        f = np.zeros((2 * n, 128))
        b = np.zeros((64 * len(cols), 128))
        for r, k in enumerate(rows):
            if k < 0:
                continue
            ck = np.exp(-2j * np.pi * ((np.arange(9) * k) % 9) / 9)
            lam = np.linalg.solve(a.conj().T @ a, a.conj().T @ ck)
            wk = (1.0 if k in (0, DF - 1) else 2.0) / (S * D)
            for c in range(len(cols)):
                e = lam[c] * np.exp(-2j * np.pi * ((m_fwd * k) % D) / D)
                f[r, 64 * c:64 * c + 64] = e.real
                f[n + r, 64 * c:64 * c + 64] = e.imag
                e = wk * lam[c] * np.exp(-2j * np.pi * ((np.arange(64) * k) % D) / D)
                b[64 * c:64 * c + 64, r] = e.real
                b[64 * c:64 * c + 64, n + r] = e.imag
        lf.append(_to_words(f))
        li.append(_to_words(b))
    n = np.arange(128)
    b_of_n = 16 * (n // 16) + 8 * (n % 2) + (n % 16) // 2
    f128 = np.exp(-2j * np.pi * (np.outer(b_of_n, n) % 128) / 128)
    tw = np.exp(-2j * np.pi * np.outer(np.arange(16), n) / S)
    f32w = lambda m: np.ascontiguousarray(m, dtype=np.float32).view(np.uint32)
    parts = [f32w(f128.real), f32w(f128.imag), f32w(tw.real), f32w(tw.imag)] + lf + li
    offs = np.cumsum([0] + [p.shape[0] for p in parts])
    return np.concatenate(parts, axis=0), [int(o) for o in offs]


_TABLE, _OFF = _make_tables()
_OFF_FR, _OFF_FI, _OFF_TR, _OFF_TI = _OFF[0:4]
_OFF_LF = _OFF[4:10]
_OFF_LI = _OFF[9:15]


def _pack(lo, hi):
    return pltpu.pack_elementwise([lo, hi], packed_dtype=BF16)


def _unpack(w, index):
    return pltpu.unpack_elementwise(w, index=index, packed_dtype=BF16, unpacked_dtype=F32)


def _bf(words):
    return pltpu.bitcast(words, BF16)


def _dot(a, b):
    return lax.dot_general(a, b, (((1,), (0,)), ((), ())), preferred_element_type=F32)


def _dot_nt(a, b):
    return lax.dot_general(a, b, (((1,), (1,)), ((), ())), preferred_element_type=F32)


def _kernel(xa_hbm, wqkv_hbm, wo_hbm, xb_hbm, wr_hbm, wi_hbm, tab_hbm, out_hbm,
            tab, xb_raw, xa_raw, wq_raw, wo_raw, wr_raw, wi_raw, wlast,
            gmat, u_nat, t_buf, x_nat, x_perm, wt_nat, wt, wo_nat, wo_perm,
            k_buf, v_buf, q_buf, o_t, o_nat, stage,
            sem_xb, sem_xa, sem_w, sem_f, sem_out):
    def cp_tab():
        return pltpu.make_async_copy(tab_hbm, tab, sem_w.at[0])

    def cp_xb(t):
        return pltpu.make_async_copy(
            xb_hbm.at[:, pl.ds(t * 128, 128)], xb_raw.at[t].bitcast(BF16), sem_xb.at[t])

    def cp_xa(t):
        return pltpu.make_async_copy(
            xa_hbm.at[:, pl.ds(t * 128, 128)], xa_raw.at[t].bitcast(BF16), sem_xa.at[t])

    def cp_wq():
        return pltpu.make_async_copy(wqkv_hbm, wq_raw, sem_w.at[1])

    def cp_wo():
        return pltpu.make_async_copy(wo_hbm, wo_raw, sem_w.at[2])

    def cp_f(i, t):
        src, dst = ((wr_hbm, wr_raw), (wi_hbm, wi_raw))[i]
        return pltpu.make_async_copy(
            src.at[pl.ds(0, DF - 1), pl.ds(t * 128, 128)], dst.at[t].bitcast(BF16),
            sem_f.at[16 * i + t])

    def cp_flast(i):
        src = (wr_hbm, wi_hbm)[i]
        return pltpu.make_async_copy(src.at[pl.ds(DF - 1, 1), :], wlast.at[i], sem_w.at[3 + i])

    def cp_out(ct, row0, rows, sem):
        return pltpu.make_async_copy(
            stage.at[ct, pl.ds(row0, rows), :].bitcast(BF16),
            out_hbm.at[pl.ds(2 * row0, 2 * rows), pl.ds(ct * 128, 128)], sem)

    cp_tab().start()
    for t in range(16):
        cp_xb(t).start()
    for t in range(16):
        cp_xa(t).start()
    cp_wq().start()
    for i in range(2):
        for t in range(16):
            cp_f(i, t).start()
        cp_flast(i).start()
    cp_wo().start()

    zeros_w = lambda rows: jnp.zeros((rows, 128), U32)

    cp_tab().wait()

    @pl.loop(0, 16)
    def _(a):
        twr = jnp.broadcast_to(pltpu.bitcast(tab[pl.ds(_OFF_TR + a, 1), :], F32), (8, 128))
        twi = jnp.broadcast_to(pltpu.bitcast(tab[pl.ds(_OFF_TI + a, 1), :], F32), (8, 128))
        for i in range(16):
            fr = pltpu.bitcast(tab[pl.ds(_OFF_FR + 8 * i, 8), :], F32)
            fi = pltpu.bitcast(tab[pl.ds(_OFF_FI + 8 * i, 8), :], F32)
            gmat[a, 0, pl.ds(8 * i, 8), :] = fr * twr - fi * twi
            gmat[a, 1, pl.ds(8 * i, 8), :] = fr * twi + fi * twr

    @pl.loop(0, 8)
    def _(tau):
        cp_xb(2 * tau).wait()
        cp_xb(2 * tau + 1).wait()
        pieces = [[None] * 8 for _ in range(9)]
        for i in range(4):
            words = [[xb_raw[2 * tau + z, pl.ds(32 * j + 8 * i, 8), :] for j in range(9)]
                     for z in range(2)]
            for e in range(2):
                u = [_bfly9_fwd([_unpack(w, e) for w in words[z]]) for z in range(2)]
                for o in range(9):
                    pieces[o][4 * e + i] = _pack(u[0][o], u[1][o])
        for gi, g in enumerate(_GROUPS):
            if g:
                v = jnp.concatenate(pieces[2 * g - 1] + pieces[2 * g], axis=0)
            else:
                v = jnp.concatenate(pieces[0] + [zeros_w(64)], axis=0)
            vt = v.T
            for r in range(16):
                u_nat[gi, pl.ds(136 * tau + 17 * (r // 2) + 8 * (r % 2), 8), :] = (
                    vt[8 * r:8 * r + 8])

    @pl.loop(0, 16)
    def _(a):
        re, im = [], []
        for gi in range(5):
            lf = _bf(tab[pl.ds(_OFF_LF[gi], _OFF_LF[gi + 1] - _OFF_LF[gi]), :])
            x1 = _dot_nt(lf, _bf(u_nat[gi, pl.ds(a, 128 // 2, stride=17), :]))
            n = x1.shape[0] // 2
            re.append(x1[:n])
            im.append(x1[n:])
        g = jnp.concatenate([gmat[a, 0], gmat[a, 1]], axis=1)
        p = _dot(jnp.concatenate(re + im, axis=0), g)
        t_buf[a, 0] = p[:NR, :128] - p[NR:, 128:]
        t_buf[a, 1] = p[:NR, 128:] + p[NR:, :128]

    for i in range(2):
        for t in range(16):
            cp_f(i, t).wait()
        cp_flast(i).wait()

    def mid(row0, load_w):
        rows = pl.ds(row0, 8)
        y = [[None] * 4 for _ in range(4)]
        for a0 in range(4):
            z = _bfly4([(t_buf[4 * a1 + a0, 0, rows, :], t_buf[4 * a1 + a0, 1, rows, :])
                        for a1 in range(4)], False)
            for g0 in range(4):
                y[g0][a0] = _twiddle16(z[g0], a0 * g0, False)
        for g0 in range(4):
            z = _bfly4(y[g0], False)
            for g1 in range(4):
                wr, wi = load_w(g0 + 4 * g1)
                zr, zi = z[g1]
                z[g1] = (zr * wr - zi * wi, zr * wi + zi * wr)
            z = _bfly4(z, True)
            for a0 in range(4):
                y[g0][a0] = _twiddle16(z[a0], a0 * g0, True)
        for a0 in range(4):
            z = _bfly4([y[g0][a0] for g0 in range(4)], True)
            for a1 in range(4):
                t_buf[4 * a1 + a0, 0, rows, :] = z[a1][0]
                t_buf[4 * a1 + a0, 1, rows, :] = z[a1][1]

    @pl.loop(0, 2)
    def _(h):
        for ci in range(18):
            k0 = _ROWGROUPS[2 * ci][0]

            def load_w(f1, k0=k0):
                rows = pl.ds(k0 // 2 + 72 * h, 8, stride=9)
                return _unpack(wr_raw[f1, rows, :], k0 % 2), _unpack(wi_raw[f1, rows, :], k0 % 2)

            mid(pl.multiple_of(16 * ci + 8 * h, 8), load_w)

    def load_w_last(f1):
        return tuple(
            jnp.broadcast_to(wlast[i, :, pl.ds(128 * f1, 128)].astype(F32), (8, 128))
            for i in range(2))

    mid(NR - 8, load_w_last)

    def inv_tile(a):
        lhs = jnp.concatenate([t_buf[a, 0], t_buf[a, 1]], axis=0)
        g = jnp.concatenate(
            [gmat[a, c, pl.ds(16 * tau + e, 8, stride=2), :]
             for c in range(2) for tau in range(8) for e in range(2)], axis=0)
        p = _dot_nt(lhs, g)
        zr = p[:NR, :128] + p[NR:, 128:]
        zi = p[NR:, :128] - p[:NR, 128:]
        v = [None] * 9
        for gi, g_ in enumerate(_GROUPS):
            li = _bf(tab[pl.ds(_OFF_LI[gi], _OFF_LI[gi + 1] - _OFF_LI[gi]), :])
            if g_:
                rows = slice(64 * gi, 64 * gi + 64)
                o = _dot(li, jnp.concatenate([zr[rows], zi[rows]], axis=0))
                v[2 * g_ - 1], v[2 * g_] = o[:64], o[64:]
            else:
                v[0] = _dot(li, jnp.concatenate(
                    [zr[256:], zi[256:], jnp.zeros((48, 128), F32)], axis=0))
        ys = [_bfly9_inv([vo[8 * i:8 * i + 8] for vo in v]) for i in range(8)]
        return ys

    @pl.loop(0, 8)
    def _(c):
        y0, y1 = inv_tile(2 * c), inv_tile(2 * c + 1)
        slab = [[_pack(y0[i][j], y1[i][j]) for i in range(8)] for j in range(9)]
        blocks = [[zeros_w(64)] + slab[0]] + [slab[2 * q - 1] + slab[2 * q] for q in range(1, 5)]
        for q in range(5):
            stage[4 + q, pl.ds(c, 128, stride=8), :] = jnp.concatenate(blocks[q], axis=0).T

    for ct in range(5, 9):
        cp_out(ct, 0, S // 2, sem_out.at[ct - 5]).start()

    @pl.loop(0, 16)
    def _(t):
        cp_xa(t).wait()
        for q in range(3):
            if q < 2:
                v = xa_raw[t, pl.ds(128 * q, 128), :]
            else:
                v = jnp.concatenate([xa_raw[t, pl.ds(256, 32), :], zeros_w(96)], axis=0)
            vt = v.T
            for r in range(16):
                x_nat[q, pl.ds(136 * t + 17 * (r // 2) + 8 * (r % 2), 8), :] = vt[8 * r:8 * r + 8]

    @pl.loop(0, 16)
    def _(a):
        for q in range(3):
            vt = x_nat[q, pl.ds(a, 128, stride=17), :].T
            n = 128 if q < 2 else 64
            x_perm[a, pl.ds(128 * q, n), :] = vt[:n]

    cp_wq().wait()
    for kt in range(5):
        for nt in range(14):
            nk, nn = min(128, D - 128 * kt), min(128, 3 * D - 128 * nt)
            blk = wq_raw[pl.ds(128 * kt, nk), pl.ds(128 * nt, nn)]
            if nk < 128:
                blk = jnp.concatenate([blk, jnp.zeros((128 - nk, nn), BF16)], axis=0)
            wt_nat[kt, pl.ds(64 * nt, nn // 2), :] = pltpu.bitcast(blk.T, U32)

    @pl.loop(0, 3)
    def _(part):
        for kt in range(5):
            for i in range(2):
                for dl in range(9):
                    base = 288 * part + 144 * i + dl
                    wa = wt_nat[kt, pl.ds(base, 8, stride=18), :]
                    wb = wt_nat[kt, pl.ds(base + 9, 8, stride=18), :]
                    for e in range(2):
                        wt[part, pl.ds(16 * (2 * dl + e) + 8 * i, 8), pl.ds(128 * kt, 128)] = (
                            _pack(_unpack(wa, e), _unpack(wb, e)))

    cp_wo().wait()
    for nt in range(5):
        nn = min(128, D - 128 * nt)
        blk = wo_raw[:, pl.ds(128 * nt, nn)]
        if nn < 128:
            blk = jnp.concatenate([blk, jnp.zeros((D, 128 - nn), BF16)], axis=1)
        wo_nat[nt] = pltpu.bitcast(blk, U32)
    for nt in range(5):
        for i in range(2):
            for dl in range(9):
                wa = wo_nat[nt, pl.ds(144 * i + dl, 8, stride=18), :]
                wb = wo_nat[nt, pl.ds(144 * i + dl + 9, 8, stride=18), :]
                for e in range(2):
                    wo_perm[pl.ds(16 * (2 * dl + e) + 8 * i, 8), pl.ds(128 * nt, 128)] = (
                        _pack(_unpack(wa, e), _unpack(wb, e)))
    wo_perm[pl.ds(288, 32), :] = jnp.zeros((32, 640), U32)

    def proj(part, p, gam):
        x = jnp.concatenate([_bf(x_perm[4 * gam + p]), _bf(x_perm[4 * gam + 2 + p])], axis=1)
        return _dot(_bf(wt[part]), x)

    @pl.loop(0, 8)
    def _(it):
        p, gam = it // 4, it % 4
        for part, buf in ((1, k_buf), (2, v_buf)):
            r = proj(part, p, gam)
            for e in range(2):
                tile = r[:, 128 * e:128 * e + 128]
                buf[p, 8 + 2 * gam + e] = tile
                buf[p, 2 * gam + e] = pltpu.roll(tile, 1, 1)

    scale = float(DH) ** -0.5
    lane = lax.broadcasted_iota(jnp.int32, (8, 128), 1)

    @pl.loop(0, 8)
    def _(it):
        p, gam = it // 4, it % 4
        r = proj(0, p, gam)
        q_buf[0] = r[:, :128]
        q_buf[1] = r[:, 128:]
        base = 2 * gam + 1
        invalid = [lane < jnp.where(l < 7 - 2 * gam, 1, 0) for l in range(7)]
        for hg in range(4):
            acc = [[None] * W for _ in range(2)]
            for d in range(DH):
                rows = pl.ds(32 * d + 8 * hg, 8)
                kk = [k_buf[p, base + l, rows, :] for l in range(9)]
                for e in range(2):
                    q = q_buf[e, rows, :]
                    for w in range(W):
                        t = q * kk[7 + e - w]
                        acc[e][w] = t if d == 0 else acc[e][w] + t
            prob = []
            for e in range(2):
                lg = [jnp.where(invalid[7 + e - w], -1e9 / scale, acc[e][w])
                      if 7 + e - w < 7 else acc[e][w] for w in range(W)]
                m = lg[0]
                for w in range(1, W):
                    m = jnp.maximum(m, lg[w])
                ex = [jnp.exp2((l_ - m) * (scale * float(np.log2(np.e)))) for l_ in lg]
                tot = ex[0]
                for w in range(1, W):
                    tot = tot + ex[w]
                inv = 1.0 / tot
                prob.append([x_ * inv for x_ in ex])
            for d in range(DH):
                rows = pl.ds(32 * d + 8 * hg, 8)
                vv = [v_buf[p, base + l, rows, :] for l in range(9)]
                o = []
                for e in range(2):
                    t = prob[e][0] * vv[7 + e]
                    for w in range(1, W):
                        t = t + prob[e][w] * vv[7 + e - w]
                    o.append(t)
                o_t[rows, :] = _pack(o[0], o[1])
        for kt in range(5):
            if kt < 4:
                v = o_t[pl.ds(128 * kt, 128), :]
            else:
                v = jnp.concatenate([o_t[pl.ds(512, 64), :], zeros_w(64)], axis=0)
            o_nat[p, kt, pl.ds(gam, 128, stride=4), :] = v.T

    n_chunks = 8
    cw = 512 // n_chunks

    @pl.loop(0, n_chunks)
    def _(ch):
        row0 = pl.multiple_of(ch * cw, cw)
        lhs = jnp.concatenate(
            [jnp.concatenate([_bf(o_nat[p, kt, pl.ds(row0, cw), :]) for kt in range(5)], axis=1)
             for p in range(2)], axis=0)
        r = _dot(lhs, _bf(wo_perm[...]))
        words = _pack(r[:2 * cw], r[2 * cw:])
        rows = pl.ds(pl.multiple_of(2 * row0, 2 * cw), 2 * cw)
        for ct in range(4):
            stage[ct, rows, :] = words[:, 128 * ct:128 * ct + 128]
        lane_c = lax.broadcasted_iota(jnp.int32, (2 * cw, 128), 1)
        stage[4, rows, :] = jnp.where(lane_c < 64, words[:, 512:], stage[4, rows, :])
        for ct in range(5):
            cp_out(ct, pl.multiple_of(2 * row0, 2 * cw), 2 * cw, sem_out.at[4 + 5 * ch + ct]).start()

    for ct in range(5, 9):
        cp_out(ct, 0, S // 2, sem_out.at[ct - 5]).wait()
    for ch in range(n_chunks):
        for ct in range(5):
            cp_out(ct, 2 * cw * ch, 2 * cw, sem_out.at[4 + 5 * ch + ct]).wait()


@jax.jit
def pallas_concat_heads__sliding_local_dilated__spectral_gfnet__prompt_kernel(
    A_x: jax.Array,
    A_wqkv: jax.Array,
    A_wo: jax.Array,
    B_x: jax.Array,
    B_w_r: jax.Array,
    B_w_i: jax.Array,
):
    assert A_x.shape == (1, S, D) and B_x.shape == (1, S, D)
    any_spec = pl.BlockSpec(memory_space=pl.ANY)
    scratch = [
        pltpu.VMEM(_TABLE.shape, U32),
        pltpu.VMEM((16, 288, 128), U32),
        pltpu.VMEM((16, 288, 128), U32),
        pltpu.VMEM((D, 3 * D), BF16),
        pltpu.VMEM((D, D), BF16),
        pltpu.VMEM((16, 144, 128), U32),
        pltpu.VMEM((16, 144, 128), U32),
        pltpu.VMEM((2, 1, S), BF16),
        pltpu.VMEM((16, 2, 128, 128), F32),
        pltpu.VMEM((5, 8 * 136, 128), U32),
        pltpu.VMEM((16, 2, NR, 128), F32),
        pltpu.VMEM((3, 16 * 136, 128), U32),
        pltpu.VMEM((16, 320, 128), U32),
        pltpu.VMEM((5, 864, 128), U32),
        pltpu.VMEM((3, 288, 640), U32),
        pltpu.VMEM((5, 288, 128), U32),
        pltpu.VMEM((320, 640), U32),
        pltpu.VMEM((2, 16, D, 128), F32),
        pltpu.VMEM((2, 16, D, 128), F32),
        pltpu.VMEM((2, D, 128), F32),
        pltpu.VMEM((D, 128), U32),
        pltpu.VMEM((2, 5, 512, 128), U32),
        pltpu.VMEM((9, S // 2, 128), U32),
        pltpu.SemaphoreType.DMA((16,)),
        pltpu.SemaphoreType.DMA((16,)),
        pltpu.SemaphoreType.DMA((5,)),
        pltpu.SemaphoreType.DMA((32,)),
        pltpu.SemaphoreType.DMA((44,)),
    ]
    out = pl.pallas_call(
        _kernel,
        out_shape=jax.ShapeDtypeStruct((S, 2 * D), BF16),
        in_specs=[any_spec] * 7,
        out_specs=any_spec,
        scratch_shapes=scratch,
        compiler_params=pltpu.CompilerParams(vmem_limit_bytes=110 * 1024 * 1024),
        name="attn_gfnet",
    )(A_x[0].T, A_wqkv, A_wo, B_x[0].T, B_w_r.T, B_w_i.T, _TABLE)
    return out[None]
```

```python
import numpy as np

import jax
import jax.numpy as jnp
from jax import lax
import jax.experimental.pallas as pl
import jax.experimental.pallas.tpu as pltpu

S = 2048
D = 576
H = 32
DH = 18
W = 8
DF = D // 2 + 1
NR = 296

F32 = jnp.float32
BF16 = jnp.bfloat16
U32 = jnp.uint32

_C3 = float(np.sqrt(3.0) / 2)
_C1, _S1 = float(np.cos(2 * np.pi / 9)), float(np.sin(2 * np.pi / 9))
_C2, _S2 = float(np.cos(4 * np.pi / 9)), float(np.sin(4 * np.pi / 9))


def _bfly9_fwd(x):
    a0, ar, ai = [], [], []
    for j in range(3):
        t = x[j + 3] + x[j + 6]
        a0.append(x[j] + t)
        ar.append(x[j] - 0.5 * t)
        ai.append(x[j + 6] - x[j + 3])
    t = a0[1] + a0[2]
    u0 = a0[0] + t
    u3r = a0[0] - 0.5 * t
    u3i = a0[2] - a0[1]
    b1r = ar[1] * _C1 + ai[1] * (_C3 * _S1)
    b1i = ai[1] * (_C3 * _C1) - ar[1] * _S1
    b2r = ar[2] * _C2 + ai[2] * (_C3 * _S2)
    b2i = ai[2] * (_C3 * _C2) - ar[2] * _S2
    a_r, a_i = ar[0], ai[0] * _C3
    tr, ti = b1r + b2r, b1i + b2i
    dr, di = (b1r - b2r) * _C3, (b1i - b2i) * _C3
    u1r, u1i = a_r + tr, a_i + ti
    mr, mi = a_r - 0.5 * tr, a_i - 0.5 * ti
    return [u0, u1r, u1i, mr - di, mi + dr, u3r, u3i, mr + di, mi - dr]


def _bfly9_inv(v):
    u0, u1r, u1i, u7r, u7i, u3r, u3i, u4r, u4i = v
    mr, mi = u4r + u7r, u4i + u7i
    di, dr = (u4r - u7r) * _C3, (u7i - u4i) * _C3
    a_r, a_i = u1r + mr, u1i + mi
    tr, ti = u1r - 0.5 * mr, u1i - 0.5 * mi
    b1r, b2r, b1i, b2i = tr + dr, tr - dr, ti + di, ti - di
    ar = [a_r, b1r * _C1 - b1i * _S1, b2r * _C2 - b2i * _S2]
    ai = [a_i * _C3, b1r * (_C3 * _S1) + b1i * (_C3 * _C1),
          b2r * (_C3 * _S2) + b2i * (_C3 * _C2)]
    t = u0 - 0.5 * u3r
    a0 = [u0 + u3r, t - u3i, t + u3i]
    y = [None] * 9
    for j in range(3):
        t = a0[j] - 0.5 * ar[j]
        y[j] = a0[j] + ar[j]
        y[j + 3] = t - ai[j]
        y[j + 6] = t + ai[j]
    return y


def _bfly4(x, inverse):
    (ar, ai), (br, bi), (cr, ci), (dr, di) = x
    pr, pi, qr, qi = ar + cr, ai + ci, ar - cr, ai - ci
    sr, si, tr, ti = br + dr, bi + di, br - dr, bi - di
    y1, y3 = (qr + ti, qi - tr), (qr - ti, qi + tr)
    if inverse:
        y1, y3 = y3, y1
    return [(pr + sr, pi + si), y1, (pr - sr, pi - si), y3]


def _twiddle16(z, e, inverse):
    zr, zi = z
    e = (-e if inverse else e) % 16
    h = float(np.sqrt(0.5))
    if e == 0:
        return z
    if e == 4:
        return zi, -zr
    if e == 12:
        return -zi, zr
    if e == 2:
        return (zr + zi) * h, (zi - zr) * h
    if e == 14:
        return (zr - zi) * h, (zr + zi) * h
    if e == 6:
        return (zi - zr) * h, (zr + zi) * (-h)
    if e == 10:
        return (zr + zi) * (-h), (zr - zi) * h
    c, s = float(np.cos(2 * np.pi * e / 16)), float(np.sin(2 * np.pi * e / 16))
    return zr * c + zi * s, zi * c - zr * s


_GROUPS = (1, 2, 3, 4, 0)


def _group_classes(g):
    return sorted({g, g + 9, 9 - g, 18 - g}) if g else [0, 9]


_ROWGROUPS = [(k0, h) for g in _GROUPS for k0 in _group_classes(g) for h in range(2)]


def _to_words(m):
    u = np.ascontiguousarray(m, dtype=np.float32).view(np.uint32)
    u = (u + 0x7FFF + ((u >> 16) & 1)) >> 16
    return (u[0::2] | (u[1::2] << 16)).astype(np.uint32)


def _make_tables():
    basis = np.array(_bfly9_fwd(list(np.eye(9))))
    m_fwd = np.array([2 * (r % 32) + r // 32 for r in range(64)])
    lf, li = [], []
    for g in _GROUPS:
        rows = [k0 + 18 * i for k0 in _group_classes(g) for i in range(16)]
        if g == 0:
            rows += [DF - 1] + [-1] * 7
        cols = [2 * g - 1, 2 * g] if g else [0]
        a = basis[cols].T.astype(complex)
        n = len(rows)
        f = np.zeros((2 * n, 128))
        b = np.zeros((64 * len(cols), 128))
        for r, k in enumerate(rows):
            if k < 0:
                continue
            ck = np.exp(-2j * np.pi * ((np.arange(9) * k) % 9) / 9)
            lam = np.linalg.solve(a.conj().T @ a, a.conj().T @ ck)
            wk = (1.0 if k in (0, DF - 1) else 2.0) / (S * D)
            for c in range(len(cols)):
                e = lam[c] * np.exp(-2j * np.pi * ((m_fwd * k) % D) / D)
                f[r, 64 * c:64 * c + 64] = e.real
                f[n + r, 64 * c:64 * c + 64] = e.imag
                e = wk * lam[c] * np.exp(-2j * np.pi * ((np.arange(64) * k) % D) / D)
                b[64 * c:64 * c + 64, r] = e.real
                b[64 * c:64 * c + 64, n + r] = e.imag
        lf.append(_to_words(f))
        li.append(_to_words(b))
    n = np.arange(128)
    b_of_n = 16 * (n // 16) + 8 * (n % 2) + (n % 16) // 2
    f128 = np.exp(-2j * np.pi * (np.outer(b_of_n, n) % 128) / 128)
    tw = np.exp(-2j * np.pi * np.outer(np.arange(16), n) / S)
    f32w = lambda m: np.ascontiguousarray(m, dtype=np.float32).view(np.uint32)
    parts = [f32w(f128.real), f32w(f128.imag), f32w(tw.real), f32w(tw.imag)] + lf + li
    offs = np.cumsum([0] + [p.shape[0] for p in parts])
    return np.concatenate(parts, axis=0), [int(o) for o in offs]


_TABLE, _OFF = _make_tables()
_OFF_FR, _OFF_FI, _OFF_TR, _OFF_TI = _OFF[0:4]
_OFF_LF = _OFF[4:10]
_OFF_LI = _OFF[9:15]


def _pack(lo, hi):
    return pltpu.pack_elementwise([lo, hi], packed_dtype=BF16)


def _unpack(w, index):
    return pltpu.unpack_elementwise(w, index=index, packed_dtype=BF16, unpacked_dtype=F32)


def _bf(words):
    return pltpu.bitcast(words, BF16)


def _dot(a, b):
    return lax.dot_general(a, b, (((1,), (0,)), ((), ())), preferred_element_type=F32)


def _dot_nt(a, b):
    return lax.dot_general(a, b, (((1,), (1,)), ((), ())), preferred_element_type=F32)


def _zeros_w(rows):
    return jnp.zeros((rows, 128), U32)


class _SideWork:
    LINK = 7.0
    MIN_LINKS = 4

    def __init__(self, zero_ref):
        self.zero_ref = zero_ref
        self.zero = zero_ref[0]
        self.lead = 0.0

    def start(self, seed, sink):
        self.chain = pltpu.bitcast(seed, F32)
        self.sink = sink
        self.jobs = []
        self.credit = 0.0
        self.delay = 0.0
        self.blocks = 0
        self.now = 0.0
        self.pending = []

    def set_load(self, load, stretch):
        self.load = load
        self.zero = self.zero_ref[0]
        self.lead = -100.0
        self.stretch = stretch

    def add(self, name, gen, first=False):
        self.jobs.insert(0 if first else len(self.jobs), (name, gen))

    def _tick(self, cycles):
        self.now += cycles
        self.delay += cycles
        while self.pending and self.pending[0][0] <= self.now:
            self.chain = self.pending.pop(0)[1] + self.chain
            self.delay -= 2.0
        n = int(self.delay / self.LINK)
        if n >= self.MIN_LINKS:
            for _ in range(n):
                self.chain = pl.reciprocal(self.chain, approx=True)
            self.delay -= n * self.LINK

    def _step(self):
        item = next(self.jobs[0][1], None)
        if item is None:
            self.jobs.pop(0)
            return
        values, cycles, latency = (item + (0.0,))[:3]
        values = values if isinstance(values, list) else [values]
        values = [pltpu.bitcast(v, F32) for v in values]
        while len(values) > 1:
            values = [values[i] + values[i + 1] if i + 1 < len(values) else values[i]
                      for i in range(0, len(values), 2)]
        self.pending.append((self.now + latency, values[0]))
        self.pending.sort(key=lambda x: x[0])
        self.credit -= cycles / self.load
        self.lead += cycles / self.load
        while self.lead >= 6.0:
            self.zero = self.zero_ref[self.zero]
            self.lead -= 6.0
        self._tick(self.stretch * cycles / self.load)

    def run(self, cycles):
        self.credit += cycles
        while self.jobs and self.credit > 0:
            self._step()
        if not self.jobs and self.credit > 0:
            self._tick(self.stretch * self.credit)
            self.credit = 0.0

    def finish(self, name):
        while any(n == name for n, _ in self.jobs):
            self._step()

    def close(self):
        while self.jobs:
            self._step()
        while self.pending:
            self.chain = self.pending.pop(0)[1] + self.chain
        self.sink[pl.ds(8 * self.blocks, 8), :] = self.chain
        self.blocks += 1
        self.credit = self.delay = 0.0


def _drain(gen):
    for _ in gen:
        pass


_W_COLS = ((0, 512), (512, 640), (1152, 576))


def _kernel(xa_hbm, wqkv_hbm, wo_hbm, xb_hbm, wr_hbm, wi_hbm, tab_hbm, zero_ref, out_hbm,
            tab, xb_raw, xa_raw, wq_raw, wo_raw, wr_raw, wi_raw, wlast,
            gmat, u_t, y_t, u_nat, x1_buf, t_buf, z_buf, x_nat, x_perm, wt_nat, wt_q, wt_k, wt_v,
            wo_nat, wo_perm, q_buf, k_buf, v_buf, o_t, o_nat, out0, stage,
            sem_xa, sem_in, sem_out):
    side = _SideWork(zero_ref)
    zero = side.zero

    def now(ref):
        return ref.at[side.zero]

    (u_r, y_r, t_r, wn_r, won_r, q_r, k_r, v_r, o_r) = (
        u_t, y_t, t_buf, wt_nat, wo_nat, q_buf, k_buf, v_buf, o_t)
    (gmat, u_t, y_t, x1_buf, t_buf, z_buf, x_perm, wt_nat, wt_q, wt_k, wt_v, wo_nat, wo_perm,
     q_buf, k_buf, v_buf, o_t, o_nat, out0) = jax.tree.map(
        lambda r: r.at[zero],
        (gmat, u_t, y_t, x1_buf, t_buf, z_buf, x_perm, wt_nat, wt_q, wt_k, wt_v, wo_nat, wo_perm,
         q_buf, k_buf, v_buf, o_t, o_nat, out0))
    wt = (wt_q, wt_k, wt_v)

    SEM_XB, SEM_TAB, SEM_WQ, SEM_WK, SEM_WV, SEM_WO, SEM_WR, SEM_WI, SEM_LAST = range(9)

    def cp_tab(row0, rows):
        return pltpu.make_async_copy(
            tab_hbm.at[pl.ds(row0, rows)], tab.at[pl.ds(row0, rows)], sem_in.at[SEM_TAB])

    def cp_xb(t):
        return pltpu.make_async_copy(
            xb_hbm.at[:, pl.ds(t * 128, 128)], xb_raw.at[t].bitcast(BF16), sem_in.at[SEM_XB])

    def cp_xa(t):
        return pltpu.make_async_copy(
            xa_hbm.at[:, pl.ds(pl.multiple_of(t * 128, 128), 128)],
            xa_raw.at[t].bitcast(BF16), sem_xa.at[t // 2])

    def cp_wq(part, row0=0, rows=D):
        rows, cols = pl.ds(row0, rows), pl.ds(*_W_COLS[part])
        return pltpu.make_async_copy(
            wqkv_hbm.at[rows, cols], wq_raw.at[rows, cols], sem_in.at[SEM_WQ + part])

    def cp_wo(row0=0, rows=D):
        return pltpu.make_async_copy(
            wo_hbm.at[pl.ds(row0, rows)], wo_raw.at[pl.ds(row0, rows)], sem_in.at[SEM_WO])

    def cp_f(i, t):
        src, dst = ((wr_hbm, wr_raw), (wi_hbm, wi_raw))[i]
        return pltpu.make_async_copy(
            src.at[pl.ds(0, DF - 1), pl.ds(t * 128, 128)], dst.at[t].bitcast(BF16),
            sem_in.at[SEM_WR + i])

    def cp_flast(i):
        src = (wr_hbm, wi_hbm)[i]
        return pltpu.make_async_copy(src.at[pl.ds(DF - 1, 1), :], wlast.at[i], sem_in.at[SEM_LAST])

    def cp_out(ct, row0, rows):
        return pltpu.make_async_copy(
            stage.at[ct, pl.ds(row0, rows), :].bitcast(BF16),
            out_hbm.at[pl.ds(2 * row0, 2 * rows), pl.ds(ct * 128, 128)], sem_out)

    def fetch_xb(t):
        def go(v):
            xb_raw[t, pl.ds(0, 8), :] = v
            cp_xb(t).start()
        return go

    def fetch_wq(part, piece):
        def go(v):
            wq_raw[pl.ds(144 * piece, 16), pl.ds(_W_COLS[part][0], 128)] = _bf(v)
            cp_wq(part, 144 * piece, 144).start()
        return go

    def fetch_wo(piece):
        def go(v):
            wo_raw[pl.ds(144 * piece, 16), pl.ds(0, 128)] = _bf(v)
            cp_wo(144 * piece, 144).start()
        return go

    def fetch_tab(row0, rows):
        def go(v):
            tab[pl.ds(row0, 8), :] = v
            cp_tab(row0, rows).start()
        return go

    def fetch_f(t):
        def go(v):
            wr_raw[t, pl.ds(0, 8), :] = v
            cp_f(0, t).start()
            wi_raw[t, pl.ds(0, 8), :] = v
            cp_f(1, t).start()
            if t == 0:
                cp_flast(0).start()
                cp_flast(1).start()
        return go

    n_tab = _TABLE.shape[0]
    fetches = ([fetch_xb(t) for t in range(4, 16)]
               + [fetch_tab(r, min(296, n_tab - r)) for r in range(0, n_tab, 296)]
               + [fetch_wq(2, i) for i in range(4)]
               + [fetch_f(t) for t in range(16)]
               + [fetch_wo(i) for i in range(4)])

    def fetch_next(value):
        if fetches:
            fetches.pop(0)(pltpu.bitcast(value[:8, :128], U32))

    def store_pitched(dst, row0, vt):
        for r in range(16):
            dst[pl.ds(row0 + 17 * (r // 2) + 8 * (r % 2), 8), :] = vt[8 * r:8 * r + 8]

    def radix9(tau):
        for i in range(4):
            words = [[xb_raw[side.zero + 2 * tau + z, pl.ds(32 * j + 8 * i, 8), :] for j in range(9)]
                     for z in range(2)]
            for e in range(2):
                u = []
                for z in range(2):
                    u.append(_bfly9_fwd([_unpack(w, e) for w in words[z]]))
                    yield u[z][8], 14
                out = [_pack(u[0][o], u[1][o]) for o in range(9)]
                for o in range(9):
                    u_t[tau, pl.ds(64 * o + 32 * e + 8 * i, 8), :] = out[o]
                yield out, 5

    def u_to_token_major(tau, cost):
        for gi, g in enumerate(_GROUPS):
            if g:
                v = now(u_r)[tau, pl.ds(64 * (2 * g - 1), 128), :]
            else:
                v = jnp.concatenate([now(u_r)[tau, pl.ds(0, 64), :], _zeros_w(64)], axis=0)
            vt = v.T
            store_pitched(u_nat.at[gi], 136 * tau, vt)
            yield vt[120:], cost, 240

    def dft_matrix(a):
        twr = jnp.broadcast_to(pltpu.bitcast(tab[pl.ds(_OFF_TR + a, 1), :], F32), (8, 128))
        twi = jnp.broadcast_to(pltpu.bitcast(tab[pl.ds(_OFF_TI + a, 1), :], F32), (8, 128))
        for i in range(16):
            fr = pltpu.bitcast(tab[pl.ds(side.zero + _OFF_FR + 8 * i, 8), :], F32)
            fi = pltpu.bitcast(tab[pl.ds(side.zero + _OFF_FI + 8 * i, 8), :], F32)
            gr, gi = fr * twr - fi * twi, fr * twi + fi * twr
            gmat[a, 0, pl.ds(8 * i, 8), :] = gr
            out = [gr + gi, gi - gr]
            gmat[a, 1, pl.ds(8 * i, 8), :] = out[0]
            gmat[a, 2, pl.ds(8 * i, 8), :] = out[1]
            yield out, 3

    def filter_rows(row0, load_w):
        rows = pl.ds(row0, 8)
        y = [[None] * 4 for _ in range(4)]
        for a0 in range(4):
            src = now(t_r)
            z = _bfly4([(src[4 * a1 + a0, 0, rows, :], src[4 * a1 + a0, 1, rows, :])
                        for a1 in range(4)], False)
            for g0 in range(4):
                y[g0][a0] = _twiddle16(z[g0], a0 * g0, False)
            yield y[3][a0][0], 7
        for g0 in range(4):
            z = _bfly4(y[g0], False)
            yield z[3][1], 4
            for g1 in range(4):
                wr, wi = load_w(g0 + 4 * g1)
                zr, zi = z[g1]
                z[g1] = (zr * wr - zi * wi, zr * wi + zi * wr)
                if g1 % 2:
                    yield z[g1][1], 4
            z = _bfly4(z, True)
            for a0 in range(4):
                y[g0][a0] = _twiddle16(z[a0], a0 * g0, True)
            yield y[g0][3][0], 6
        for a0 in range(4):
            z = _bfly4([y[g0][a0] for g0 in range(4)], True)
            for a1 in range(4):
                t_buf[4 * a1 + a0, 0, rows, :] = z[a1][0]
                t_buf[4 * a1 + a0, 1, rows, :] = z[a1][1]
            yield [v for pair in z for v in pair], 6

    def filter_all():
        for n, (k0, h) in enumerate(_ROWGROUPS):
            rows = pl.ds(k0 // 2 + 72 * h, 8, stride=9)
            yield from filter_rows(8 * n, lambda f1: (
                _unpack(wr_raw[side.zero + f1, rows, :], k0 % 2),
                _unpack(wi_raw[side.zero + f1, rows, :], k0 % 2)))
        yield from filter_rows(NR - 8, lambda f1: tuple(
            jnp.broadcast_to(wlast[i, :, pl.ds(128 * f1, 128)].astype(F32), (8, 128))
            for i in range(2)))

    def radix9_inv(c):
        for i in range(8):
            y = []
            for e in range(2):
                y.append(_bfly9_inv(
                    [now(t_r)[2 * c + e, i // 4, pl.ds(256 + 8 * (i % 4), 8), :]]
                    + [now(t_r)[2 * c + e, o % 2, pl.ds(64 * (o // 2) + 8 * i, 8), :]
                       for o in range(8)]))
                yield (y[e] if 0 else y[e][8]), 12
            out = [_pack(y[0][j], y[1][j]) for j in range(9)]
            for j in range(9):
                y_t[c, pl.ds(64 * j + 8 * i, 8), :] = out[j]
            yield out, 5

    def y_to_token_major(c, cost):
        for q in range(5):
            if q:
                v = now(y_r)[c, pl.ds(128 * q - 64, 128), :]
            else:
                v = jnp.concatenate([_zeros_w(64), now(y_r)[c, pl.ds(0, 64), :]], axis=0)
            vt = v.T
            stage[4 + q, pl.ds(c, 128, stride=8), :] = vt
            yield vt[120:], cost, 240

    def x_to_token_major(t):
        for q in range(3):
            if q < 2:
                v = xa_raw[t, pl.ds(128 * q, 128), :]
            else:
                v = jnp.concatenate([xa_raw[t, pl.ds(256, 32), :], _zeros_w(96)], axis=0)
            store_pitched(x_nat.at[q], 136 * t, v.T)

    def x_tile(a):
        for q in range(3):
            vt = x_nat[side.zero + q, pl.ds(a, 128, stride=17), :].T
            n = 128 if q < 2 else 64
            x_perm[a, pl.ds(128 * q, n), :] = vt[:n]
            yield vt[n - 8:n], 43, 240

    def w_prep(part):
        col0, _ = _W_COLS[part]
        first = 288 * part - col0 // 2
        for kt in range(5):
            for nt in range(5):
                nn = min(128, 3 * D - col0 - 128 * nt)
                rows = pl.ds(pl.multiple_of(side.zero + 128 * kt, 128), 128)
                vt = wq_raw[rows, pl.ds(col0 + 128 * nt, nn)].T
                vt = pltpu.bitcast(vt, U32)
                wt_nat[kt, pl.ds(64 * nt, nn // 2), :] = vt
                yield vt[-8:], 22, 180
        for kt in range(5):
            for i in range(2):
                for dl in range(9):
                    base = first + 144 * i + dl
                    wa = now(wn_r)[kt, pl.ds(base, 8, stride=18), :]
                    wb = now(wn_r)[kt, pl.ds(base + 9, 8, stride=18), :]
                    out = [_pack(_unpack(wa, e), _unpack(wb, e)) for e in range(2)]
                    for e in range(2):
                        wt[part][kt, pl.ds(16 * (2 * dl + e) + 8 * i, 8), :] = out[e]
                    yield out, 2

    def wo_prep():
        for nt in range(5):
            nn = min(128, D - 128 * nt)
            blk = wo_raw[:, pl.ds(128 * nt, nn)]
            if nn < 128:
                blk = jnp.concatenate([blk, jnp.zeros((D, 128 - nn), BF16)], axis=1)
            blk = pltpu.bitcast(blk, U32)
            wo_nat[nt] = blk
            wo_perm[nt, pl.ds(288, 32), :] = _zeros_w(32)
            yield blk[-8:], 20
            for i in range(2):
                for dl in range(9):
                    wa = now(won_r)[nt, pl.ds(144 * i + dl, 8, stride=18), :]
                    wb = now(won_r)[nt, pl.ds(144 * i + dl + 9, 8, stride=18), :]
                    out = [_pack(_unpack(wa, e), _unpack(wb, e)) for e in range(2)]
                    for e in range(2):
                        wo_perm[nt, pl.ds(16 * (2 * dl + e) + 8 * i, 8), :] = out[e]
                    yield out, 2

    scale = float(DH) ** -0.5
    QB = 6

    def attend(p, units):
        lane0 = lax.broadcasted_iota(jnp.int32, (8, 128), 1) == 0
        for unit in units:
            gam, hg = divmod(unit, 4)
            base = 2 * gam + 1
            acc = [[None] * W for _ in range(2)]
            for d0 in range(0, DH, QB):
                rows = [pl.ds(32 * d + 8 * hg, 8) for d in range(d0, d0 + QB)]
                q = [[now(q_r[4 * p + gam])[e, r, :] for r in rows] for e in range(2)]
                for l in range(9):
                    for n, r in enumerate(rows):
                        k = now(k_r[p])[base + l, r, :]
                        for e in range(2):
                            w = 7 + e - l
                            if 0 <= w < W:
                                t = q[e][n] * k
                                acc[e][w] = t if acc[e][w] is None else acc[e][w] + t
                    done = [acc[e][7 + e - l] for e in range(2) if 0 <= 7 + e - l < W]
                    yield done, QB / 2 * len(done)
            prob = []
            for e in range(2):
                lg = [jnp.where(lane0, -1e9 / scale, acc[e][w]) if 2 * gam + e < w else acc[e][w]
                      for w in range(W)]
                m = lg[0]
                for w in range(1, W):
                    m = jnp.maximum(m, lg[w])
                ex = [jnp.exp2((l_ - m) * (scale * float(np.log2(np.e)))) for l_ in lg]
                tot = ex[0]
                for w in range(1, W):
                    tot = tot + ex[w]
                inv = 1.0 / tot
                prob.append([x_ * inv for x_ in ex])
                yield prob[e][W - 1], 13, 30
            for d in range(DH):
                rows = pl.ds(32 * d + 8 * hg, 8)
                vv = [now(v_r[p])[base + l, rows, :] for l in range(9)]
                o = []
                for e in range(2):
                    t = prob[e][0] * vv[7 + e]
                    for w in range(1, W):
                        t = t + prob[e][w] * vv[7 + e - w]
                    o.append(t)
                word = _pack(o[0], o[1])
                o_t[p][gam, rows, :] = word
                yield word, 8

    def o_to_token_major(p, cost, gams):
        for gam in gams:
            for kt in range(5):
                if kt < 4:
                    v = now(o_r[p])[gam, pl.ds(128 * kt, 128), :]
                else:
                    v = jnp.concatenate([now(o_r[p])[gam, pl.ds(512, 64), :], _zeros_w(64)], axis=0)
                vt = v.T
                o_nat[p][kt, pl.ds(gam, 128, stride=4), :] = vt
                yield vt[120:], cost, 240

    def table(off, i):
        return _bf(tab[pl.ds(off[i], off[i + 1] - off[i]), :])

    def dft64(a):
        side.run(148)
        for gi in range(5):
            x1 = _dot_nt(table(_OFF_LF, gi), _bf(u_nat[gi, pl.ds(a, 64, stride=17), :]))
            n = x1.shape[0] // 2
            x1_buf[a % 2, 0, pl.ds(64 * gi, n), :] = x1[:n]
            x1_buf[a % 2, 1, pl.ds(64 * gi, n), :] = x1[n:]

    def dft128(a):
        side.run(222)
        xr, xi = x1_buf[a % 2, 0], x1_buf[a % 2, 1]
        k1 = _dot(xr + xi, gmat[a, 0])
        t_buf[a, 0] = k1 - _dot(xi, gmat[a, 1])
        ti = k1 + _dot(xr, gmat[a, 2])
        t_buf[a, 1] = ti
        fetch_next(ti)

    def idft128(a):
        side.run(222)
        g = [jnp.concatenate([gmat[a, c, pl.ds(16 * tau + e, 8, stride=2), :]
                              for tau in range(8) for e in range(2)], axis=0) for c in range(3)]
        tr, ti = t_buf[a, 0], t_buf[a, 1]
        k1 = _dot_nt(tr + ti, g[0])
        z_buf[a % 2, 0] = k1 + _dot_nt(ti, g[2])
        z_buf[a % 2, 1] = k1 - _dot_nt(tr, g[1])

    def idft64(a):
        side.run(144)
        for gi in range(5):
            n = 64 if gi < 4 else NR - 256
            parts = [z_buf[a % 2, c, pl.ds(64 * gi, n), :] for c in range(2)]
            if n < 64:
                parts.append(jnp.zeros((128 - 2 * n, 128), F32))
            o = _dot(table(_OFF_LI, gi), jnp.concatenate(parts, axis=0))
            if gi < 4:
                t_buf[a, 0, pl.ds(64 * gi, 64), :] = o[:64]
                t_buf[a, 1, pl.ds(64 * gi, 64), :] = o[64:]
            else:
                t_buf[a, 0, pl.ds(256, 32), :] = o[:32]
                t_buf[a, 1, pl.ds(256, 32), :] = o[32:]

    def proj(part, p, gam, chunks=4):
        a = 4 * gam + p
        m = 288 // chunks
        for ch in range(chunks):
            side.run(5 * m)
            w = jnp.concatenate(
                [_bf(wt[part][kt, pl.ds(m * ch, m), :]) for kt in range(5)], axis=1)
            x = jnp.concatenate([_bf(x_perm[a]), _bf(x_perm[a + 2])], axis=1)
            r = _dot(w, x)
            rows = pl.ds(2 * m * ch, 2 * m)
            for e in range(2):
                tile = r[:, 128 * e:128 * e + 128]
                c = 2 * gam + e
                if part == 0:
                    q_buf[4 * p + gam][e, rows, :] = tile
                else:
                    buf = (k_buf, v_buf)[part - 1][p]
                    buf[8 + c, rows, :] = tile
                    if c:
                        buf[c, rows, :] = pltpu.roll(tile, 1, 1)
            fetch_next(r)

    def out_proj(p, row0, cw):
        side.run(12.5 * cw)
        lhs = jnp.concatenate([_bf(o_nat[p][kt, pl.ds(row0, cw), :]) for kt in range(5)], axis=1)
        r = _dot(lhs, jnp.concatenate([_bf(wo_perm[nt]) for nt in range(5)], axis=1))
        rows = pl.ds(2 * row0, 2 * cw)
        for ct in range(5):
            tile = r[:, 128 * ct:128 * ct + 128]
            if p == 0:
                out0[ct, rows, :] = tile
                continue
            word = _pack(out0[ct, rows, :], tile)
            if ct == 4:
                lane = lax.broadcasted_iota(jnp.int32, word.shape, 1)
                word = jnp.where(lane < 64, word, stage[4, rows, :])
            stage[ct, rows, :] = word
            cp_out(ct, 2 * row0, 2 * cw).start()

    cp_wq(1).start()
    for t in range(4):
        cp_xa(t).start()
    wq_raw[pl.ds(D, 64), :] = jnp.zeros((64, 3 * D), BF16)
    cp_wq(1).wait()
    _drain(w_prep(1))

    @pl.loop(0, 8)
    def _(tau):
        @pl.when(tau < 6)
        def _():
            cp_xa(2 * tau + 4).start()
            cp_xa(2 * tau + 5).start()

        @pl.when(tau == 6)
        def _():
            cp_wq(0).start()

        @pl.when(tau == 7)
        def _():
            for t in range(4):
                cp_xb(t).start()

        cp_xa(2 * tau).wait()
        cp_xa(2 * tau + 1).wait()
        x_to_token_major(2 * tau)
        x_to_token_major(2 * tau + 1)

    _drain(x_tile(0))
    _drain(x_tile(2))

    side.start(xa_raw[0, pl.ds(0, 8), :], x1_buf.at[2, 0])

    side.set_load(14 * 129 / 5760, 1.0)
    order = [4, 6, 8, 10, 12, 14, 1, 3, 5, 7, 9, 11, 13, 15]
    for gam in range(4):
        for a in order[2 * gam:2 * gam + 2]:
            side.add("next", x_tile(a), first=True)
        for a in order[8 + 2 * gam:10 + 2 * gam]:
            side.add("later", x_tile(a))
        proj(1, 0, gam)
        side.finish("next")
    side.close()

    def barrier():
        side.close()
        _barrier(sem_in.at[SEM_LAST], wr_hbm, wlast)

    pltpu.make_async_copy(xb_raw, xb_raw, sem_in.at[SEM_XB]).wait()
    cp_wq(0).wait()
    side.set_load((8 * 264 + 730) / 5760, 0.95)
    side.add("w", w_prep(0))
    for tau in range(8):
        side.add("r9", radix9(tau))
    for gam in range(4):
        proj(1, 1, gam)
    barrier()

    side.set_load(40 * 43 / 2500, 1.0)
    for tau in range(8):
        side.add("t", u_to_token_major(tau, 43))
    proj(0, 0, 0)
    proj(0, 0, 1)
    side.close()

    cp_tab(0, n_tab).wait()
    cp_wq(2).wait()
    side.set_load((15 * 48 + 730) / 5920, 1.0)
    side.add("w", w_prep(2))
    _drain(dft_matrix(0))
    dft64(0)
    for a in range(16):
        if a < 15:
            side.add("g", dft_matrix(a + 1), first=True)
            dft64(a + 1)
        dft128(a)
        side.finish("g")
    side.close()

    pltpu.make_async_copy(wr_raw, wr_raw, sem_in.at[SEM_WR]).wait()
    pltpu.make_async_copy(wi_raw, wi_raw, sem_in.at[SEM_WI]).wait()
    cp_flast(0).wait()
    cp_flast(1).wait()
    cp_wo().wait()
    assert not fetches
    side.set_load((37 * 120 + 280) / 8640, 0.9)
    side.add("f", filter_all())
    side.add("wo", wo_prep())
    for gam in range(4):
        proj(2, 0, gam)
    proj(0, 0, 2)
    proj(0, 0, 3)
    barrier()

    n6, n8 = 8, 4
    side.set_load(n6 * 319 / 5856, 1.0)
    side.add("att", attend(0, range(n6)))
    idft128(0)
    for a in range(16):
        if a < 15:
            idft128(a + 1)
        idft64(a)
    barrier()

    side.set_load(((16 - n6) * 319 + 8 * 232) / 7200, 1.0)
    side.add("att", attend(0, range(n6, 16)))
    for c in range(8):
        side.add("r9", radix9_inv(c))
    for gam in range(4):
        proj(2, 1, gam)
    proj(0, 1, 0)
    barrier()

    tc = 42.0
    load = n8 * 319 / (4320 - 60 * tc)
    side.set_load(load, 1.0)
    side.add("att", attend(1, range(n8)))
    side.add("o", o_to_token_major(0, tc * load, range(4)))
    for c in range(8):
        side.add("y", y_to_token_major(c, tc * load))
    for gam in range(1, 4):
        proj(0, 1, gam)
    side.close()
    for ct in range(5, 9):
        cp_out(ct, 0, S // 2).start()
    _barrier(sem_in.at[SEM_LAST], wr_hbm, wlast)

    keep = 64
    side.set_load((16 - n8) * 319 / (12.5 * (512 - keep)), 1.0)
    side.add("att", attend(1, range(n8, 16)))
    for row0 in range(0, 512 - keep, 64):
        out_proj(0, row0, min(64, 512 - keep - row0))
    barrier()

    side.set_load(1.0, 0.0)
    out_proj(0, 512 - keep, keep)
    _drain(o_to_token_major(1, 0, range(4)))
    row0 = 0
    for cw in (128, 128, 96, 64, 48, 32, 16):
        out_proj(1, row0, cw)
        row0 += cw
    pltpu.make_async_copy(out_hbm, out_hbm, sem_out).wait()


def _barrier(sem, src, dst):
    if 1:
        cp = pltpu.make_async_copy(src.at[pl.ds(DF - 1, 1), :], dst.at[0], sem)
        cp.start()
        cp.wait()


@jax.jit
def pallas_concat_heads__sliding_local_dilated__spectral_gfnet__prompt_kernel(
    A_x: jax.Array,
    A_wqkv: jax.Array,
    A_wo: jax.Array,
    B_x: jax.Array,
    B_w_r: jax.Array,
    B_w_i: jax.Array,
):
    assert A_x.shape == (1, S, D) and B_x.shape == (1, S, D)
    any_spec = pl.BlockSpec(memory_space=pl.ANY)
    scratch = [
        pltpu.VMEM(_TABLE.shape, U32),
        pltpu.VMEM((16, 288, 128), U32),
        pltpu.VMEM((16, 288, 128), U32),
        pltpu.VMEM((D + 64, 3 * D), BF16),
        pltpu.VMEM((D, D), BF16),
        pltpu.VMEM((16, 144, 128), U32),
        pltpu.VMEM((16, 144, 128), U32),
        pltpu.VMEM((2, 1, S), BF16),
        pltpu.VMEM((1, 16, 3, 128, 128), F32),
        pltpu.VMEM((1, 8, D, 128), U32),
        pltpu.VMEM((1, 8, D, 128), U32),
        pltpu.VMEM((5, 8 * 136, 128), U32),
        pltpu.VMEM((1, 3, 2, NR, 128), F32),
        pltpu.VMEM((1, 16, 2, NR, 128), F32),
        pltpu.VMEM((1, 2, 2, NR, 128), F32),
        pltpu.VMEM((3, 16 * 136, 128), U32),
        pltpu.VMEM((1, 16, 320, 128), U32),
        pltpu.VMEM((1, 5, 320, 128), U32),
        pltpu.VMEM((1, 5, 288, 128), U32),
        pltpu.VMEM((1, 5, 288, 128), U32),
        pltpu.VMEM((1, 5, 288, 128), U32),
        pltpu.VMEM((1, 5, 288, 128), U32),
        pltpu.VMEM((1, 5, 320, 128), U32),
        [pltpu.VMEM((1, 2, D, 128), F32)] * 8,
        [pltpu.VMEM((1, 16, D, 128), F32)] * 2,
        [pltpu.VMEM((1, 16, D, 128), F32)] * 2,
        [pltpu.VMEM((1, 4, D, 128), U32)] * 2,
        [pltpu.VMEM((1, 5, 512, 128), U32)] * 2,
        pltpu.VMEM((1, 5, S // 2, 128), F32),
        pltpu.VMEM((9, S // 2, 128), U32),
        pltpu.SemaphoreType.DMA((8,)),
        pltpu.SemaphoreType.DMA((9,)),
        pltpu.SemaphoreType.DMA(()),
    ]
    out = pl.pallas_call(
        _kernel,
        out_shape=jax.ShapeDtypeStruct((S, 2 * D), BF16),
        in_specs=[any_spec] * 7 + [pl.BlockSpec(memory_space=pltpu.SMEM)],
        out_specs=any_spec,
        scratch_shapes=scratch,
        compiler_params=pltpu.CompilerParams(vmem_limit_bytes=120 * 1024 * 1024),
        name="attn_gfnet",
    )(A_x[0].T, A_wqkv, A_wo, B_x[0].T, B_w_r.T, B_w_i.T, _TABLE, np.zeros((2,), np.int32))
    return out[None]
```

```python
from functools import partial

import numpy as np

import jax
import jax.numpy as jnp
from jax import lax
import jax.experimental.pallas as pl
import jax.experimental.pallas.tpu as pltpu

S = 2048
D = 576
H = 32
DH = 18
W = 8
DF = D // 2 + 1
NR = 296

F32 = jnp.float32
BF16 = jnp.bfloat16
U32 = jnp.uint32

_C3 = float(np.sqrt(3.0) / 2)
_C1, _S1 = float(np.cos(2 * np.pi / 9)), float(np.sin(2 * np.pi / 9))
_C2, _S2 = float(np.cos(4 * np.pi / 9)), float(np.sin(4 * np.pi / 9))


def _bfly9_fwd(x):
    a0, ar, ai = [], [], []
    for j in range(3):
        t = x[j + 3] + x[j + 6]
        a0.append(x[j] + t)
        ar.append(x[j] - 0.5 * t)
        ai.append(x[j + 6] - x[j + 3])
    t = a0[1] + a0[2]
    u0 = a0[0] + t
    u3r = a0[0] - 0.5 * t
    u3i = a0[2] - a0[1]
    b1r = ar[1] * _C1 + ai[1] * (_C3 * _S1)
    b1i = ai[1] * (_C3 * _C1) - ar[1] * _S1
    b2r = ar[2] * _C2 + ai[2] * (_C3 * _S2)
    b2i = ai[2] * (_C3 * _C2) - ar[2] * _S2
    a_r, a_i = ar[0], ai[0] * _C3
    tr, ti = b1r + b2r, b1i + b2i
    dr, di = (b1r - b2r) * _C3, (b1i - b2i) * _C3
    u1r, u1i = a_r + tr, a_i + ti
    mr, mi = a_r - 0.5 * tr, a_i - 0.5 * ti
    return [u0, u1r, u1i, mr - di, mi + dr, u3r, u3i, mr + di, mi - dr]


def _bfly9_inv(v):
    u0, u1r, u1i, u7r, u7i, u3r, u3i, u4r, u4i = v
    mr, mi = u4r + u7r, u4i + u7i
    di, dr = (u4r - u7r) * _C3, (u7i - u4i) * _C3
    a_r, a_i = u1r + mr, u1i + mi
    tr, ti = u1r - 0.5 * mr, u1i - 0.5 * mi
    b1r, b2r, b1i, b2i = tr + dr, tr - dr, ti + di, ti - di
    ar = [a_r, b1r * _C1 - b1i * _S1, b2r * _C2 - b2i * _S2]
    ai = [a_i * _C3, b1r * (_C3 * _S1) + b1i * (_C3 * _C1),
          b2r * (_C3 * _S2) + b2i * (_C3 * _C2)]
    t = u0 - 0.5 * u3r
    a0 = [u0 + u3r, t - u3i, t + u3i]
    y = [None] * 9
    for j in range(3):
        t = a0[j] - 0.5 * ar[j]
        y[j] = a0[j] + ar[j]
        y[j + 3] = t - ai[j]
        y[j + 6] = t + ai[j]
    return y


def _bfly4(x, inverse):
    (ar, ai), (br, bi), (cr, ci), (dr, di) = x
    pr, pi, qr, qi = ar + cr, ai + ci, ar - cr, ai - ci
    sr, si, tr, ti = br + dr, bi + di, br - dr, bi - di
    y1, y3 = (qr + ti, qi - tr), (qr - ti, qi + tr)
    if inverse:
        y1, y3 = y3, y1
    return [(pr + sr, pi + si), y1, (pr - sr, pi - si), y3]


def _twiddle16(z, e, inverse):
    zr, zi = z
    e = (-e if inverse else e) % 16
    h = float(np.sqrt(0.5))
    if e == 0:
        return z
    if e == 4:
        return zi, -zr
    if e == 12:
        return -zi, zr
    if e == 2:
        return (zr + zi) * h, (zi - zr) * h
    if e == 14:
        return (zr - zi) * h, (zr + zi) * h
    if e == 6:
        return (zi - zr) * h, (zr + zi) * (-h)
    if e == 10:
        return (zr + zi) * (-h), (zr - zi) * h
    c, s = float(np.cos(2 * np.pi * e / 16)), float(np.sin(2 * np.pi * e / 16))
    return zr * c + zi * s, zi * c - zr * s


_GROUPS = (1, 2, 3, 4, 0)


def _group_classes(g):
    return sorted({g, g + 9, 9 - g, 18 - g}) if g else [0, 9]


_ROWGROUPS = [(k0, h) for g in _GROUPS for k0 in _group_classes(g) for h in range(2)]


def _to_words(m):
    u = np.ascontiguousarray(m, dtype=np.float32).view(np.uint32)
    u = (u + 0x7FFF + ((u >> 16) & 1)) >> 16
    return (u[0::2] | (u[1::2] << 16)).astype(np.uint32)


def _make_tables():
    basis = np.array(_bfly9_fwd(list(np.eye(9))))
    m_fwd = np.array([2 * (r % 32) + r // 32 for r in range(64)])
    lf, li = [], []
    for g in _GROUPS:
        rows = [k0 + 18 * i for k0 in _group_classes(g) for i in range(16)]
        if g == 0:
            rows += [DF - 1] + [-1] * 7
        cols = [2 * g - 1, 2 * g] if g else [0]
        a = basis[cols].T.astype(complex)
        n = len(rows)
        f = np.zeros((2 * n, 128))
        b = np.zeros((64 * len(cols), 128))
        for r, k in enumerate(rows):
            if k < 0:
                continue
            ck = np.exp(-2j * np.pi * ((np.arange(9) * k) % 9) / 9)
            lam = np.linalg.solve(a.conj().T @ a, a.conj().T @ ck)
            wk = (1.0 if k in (0, DF - 1) else 2.0) / (S * D)
            for c in range(len(cols)):
                e = lam[c] * np.exp(-2j * np.pi * ((m_fwd * k) % D) / D)
                f[r, 64 * c:64 * c + 64] = e.real
                f[n + r, 64 * c:64 * c + 64] = e.imag
                e = wk * lam[c] * np.exp(-2j * np.pi * ((np.arange(64) * k) % D) / D)
                b[64 * c:64 * c + 64, r] = e.real
                b[64 * c:64 * c + 64, n + r] = e.imag
        lf.append(_to_words(f))
        li.append(_to_words(b))
    n = np.arange(128)
    b_of_n = 16 * (n // 16) + 8 * (n % 2) + (n % 16) // 2
    f128 = np.exp(-2j * np.pi * (np.outer(b_of_n, n) % 128) / 128)
    tw = np.exp(-2j * np.pi * np.outer(np.arange(16), n) / S)
    f32w = lambda m: np.ascontiguousarray(m, dtype=np.float32).view(np.uint32)
    parts = [f32w(f128.real), f32w(f128.imag), f32w(tw.real), f32w(tw.imag)] + lf + li
    offs = np.cumsum([0] + [p.shape[0] for p in parts])
    parts.append(np.zeros((-offs[-1] % 32, 128), np.uint32))
    return np.concatenate(parts, axis=0), [int(o) for o in offs]


_TABLE, _OFF = _make_tables()
_OFF_FR, _OFF_FI, _OFF_TR, _OFF_TI = _OFF[0:4]
_OFF_LF = _OFF[4:10]
_OFF_LI = _OFF[9:15]


def _pack(lo, hi):
    return pltpu.pack_elementwise([lo, hi], packed_dtype=BF16)


def _unpack(w, index):
    return pltpu.unpack_elementwise(w, index=index, packed_dtype=BF16, unpacked_dtype=F32)


def _bf(words):
    return pltpu.bitcast(words, BF16)


def _dot(a, b):
    return lax.dot_general(a, b, (((1,), (0,)), ((), ())), preferred_element_type=F32)


def _dot_nt(a, b):
    return lax.dot_general(a, b, (((1,), (1,)), ((), ())), preferred_element_type=F32)


def _zeros_w(rows):
    return jnp.zeros((rows, 128), U32)


class _SideWork:
    LINK = 7.0
    MIN_LINKS = 4

    def __init__(self, zero_ref):
        self.zero_ref = zero_ref
        self.zero = zero_ref[0]
        self.lead = 0.0

    def start(self, seed, sink):
        self.chain = pltpu.bitcast(seed, F32)
        self.sink = sink
        self.jobs = []
        self.credit = 0.0
        self.delay = 0.0
        self.blocks = 0
        self.now = 0.0
        self.pending = []

    def set_load(self, load, stretch):
        self.load = load
        self.zero = self.zero_ref[0]
        self.lead = -100.0
        self.stretch = stretch

    def add(self, name, gen, first=False):
        self.jobs.insert(0 if first else len(self.jobs), (name, gen))

    def _advance(self, cycles):
        self.lead += cycles
        while self.lead >= 6.0:
            self.zero = self.zero_ref[self.zero]
            self.lead -= 6.0

    def _tick(self, cycles):
        self.now += cycles
        self.delay += cycles
        while self.pending and self.pending[0][0] <= self.now:
            self.chain = self.pending.pop(0)[1] + self.chain
            self.delay -= 2.0
        n = int(self.delay / self.LINK)
        if n >= self.MIN_LINKS:
            for _ in range(n):
                self.chain = pl.reciprocal(self.chain, approx=True)
            self.delay -= n * self.LINK

    def _step(self):
        item = next(self.jobs[0][1], None)
        if item is None:
            self.jobs.pop(0)
            return
        values, cycles, latency = (item + (0.0,))[:3]
        values = values if isinstance(values, list) else [values]
        values = [pltpu.bitcast(v, F32) for v in values]
        while len(values) > 1:
            values = [values[i] + values[i + 1] if i + 1 < len(values) else values[i]
                      for i in range(0, len(values), 2)]
        self.pending.append((self.now + latency, values[0]))
        self.pending.sort(key=lambda x: x[0])
        self.credit -= cycles / self.load
        self._advance(cycles / self.load)
        self._tick(self.stretch * cycles / self.load)

    def run(self, cycles):
        self.credit += cycles
        while self.jobs and self.credit > 0:
            self._step()
        if not self.jobs and self.credit > 0:
            self._tick(self.stretch * self.credit)
            self.credit = 0.0

    def finish(self, name):
        while any(n == name for n, _ in self.jobs):
            self._step()

    def close(self):
        while self.jobs:
            self._step()
        while self.pending:
            self.chain = self.pending.pop(0)[1] + self.chain
        self.sink[pl.ds(8 * self.blocks, 8), :] = self.chain
        self.blocks += 1
        self.credit = self.delay = 0.0


def _drain(gen):
    for _ in gen:
        pass


_W_COLS = ((0, 512), (512, 640), (1152, 576))


def _kernel(xa_hbm, wqkv_hbm, wo_hbm, xb_hbm, wr_hbm, wi_hbm, tab_hbm, zero_ref, out_hbm,
            tab, xb_raw, xa_raw, wq_raw, wo_raw, wr_raw, wi_raw, wlast,
            gmat, u_t, y_t, u_nat, x1_buf, t_buf, z_buf, x_nat, x_perm, wt_nat, wt_q, wt_k, wt_v,
            wo_nat, wo_perm, q_buf, k_buf, v_buf, o_t, o_nat, out0, stage,
            sem_xa, sem_in, sem_out, sem_bar):
    side = _SideWork(zero_ref)
    zero = side.zero

    def now(ref):
        return ref.at[side.zero]

    tab_r, wr_r, wi_r = tab, wr_raw, wi_raw
    tab, wr_raw, wi_raw = tab.at[0], wr_raw.at[0], wi_raw.at[0]
    (u_r, y_r, t_r, wn_r, won_r, q_r, k_r, v_r, o_r) = (
        u_t, y_t, t_buf, wt_nat, wo_nat, q_buf, k_buf, v_buf, o_t)
    (gmat, u_t, y_t, x1_buf, t_buf, z_buf, x_perm, wt_nat, wt_q, wt_k, wt_v, wo_nat, wo_perm,
     q_buf, k_buf, v_buf, o_t, o_nat, out0) = jax.tree.map(
        lambda r: r.at[zero],
        (gmat, u_t, y_t, x1_buf, t_buf, z_buf, x_perm, wt_nat, wt_q, wt_k, wt_v, wo_nat, wo_perm,
         q_buf, k_buf, v_buf, o_t, o_nat, out0))
    wt = (wt_q, wt_k, wt_v)

    SEM_XB, SEM_TAB, SEM_WQ, SEM_WK, SEM_WV, SEM_WO, SEM_WR, SEM_WI, SEM_LAST = range(9)

    def cp_tab(row0, rows, z=0):
        return pltpu.make_async_copy(
            tab_hbm.at[pl.ds(row0, rows)], tab.at[pl.ds(pl.multiple_of(z + row0, 8), rows)],
            sem_in.at[SEM_TAB])

    def cp_xb(t, z=0):
        return pltpu.make_async_copy(
            xb_hbm.at[:, pl.ds(t * 128, 128)], xb_raw.at[z + t].bitcast(BF16), sem_in.at[SEM_XB])

    def cp_xa(t, late):
        rows = pl.ds(256, D - 256) if late else pl.ds(0, 256)
        return pltpu.make_async_copy(
            xa_hbm.at[rows, pl.ds(pl.multiple_of(t * 128, 128), 128)],
            xa_raw.at[t].bitcast(BF16).at[rows], sem_xa.at[4 if late else t // 4])

    def cp_wq(part, row0=0, rows=D, z=0):
        cols = pl.ds(*_W_COLS[part])
        return pltpu.make_async_copy(
            wqkv_hbm.at[pl.ds(row0, rows), cols],
            wq_raw.at[pl.ds(pl.multiple_of(z + row0, 16), rows), cols], sem_in.at[SEM_WQ + part])

    def cp_wo(row0=0, rows=D, z=0):
        return pltpu.make_async_copy(
            wo_hbm.at[pl.ds(row0, rows)], wo_raw.at[pl.ds(pl.multiple_of(z + row0, 16), rows)],
            sem_in.at[SEM_WO])

    def cp_f(i, t, z=0):
        src, dst = ((wr_hbm, wr_raw), (wi_hbm, wi_raw))[i]
        return pltpu.make_async_copy(
            src.at[pl.ds(0, DF - 1), pl.ds(t * 128, 128)], dst.at[z + t].bitcast(BF16),
            sem_in.at[SEM_WR + i])

    def cp_flast(i):
        src = (wr_hbm, wi_hbm)[i]
        return pltpu.make_async_copy(src.at[pl.ds(DF - 1, 1), :], wlast.at[i], sem_in.at[SEM_LAST])

    def cp_out(ct, row0, rows):
        return pltpu.make_async_copy(
            stage.at[ct, pl.ds(row0, rows), :].bitcast(BF16),
            out_hbm.at[pl.ds(2 * row0, 2 * rows), pl.ds(ct * 128, 128)], sem_out)

    def fetch_xb(t, v):
        xb_raw[t, pl.ds(0, 8), :] = v
        cp_xb(t).start()

    def fetch_wq(part, piece, v):
        wq_raw[pl.ds(144 * piece, 16), pl.ds(_W_COLS[part][0], 128)] = _bf(v)
        cp_wq(part, 144 * piece, 144).start()

    def fetch_wo(piece, v):
        wo_raw[pl.ds(144 * piece, 16), pl.ds(0, 128)] = _bf(v)
        cp_wo(144 * piece, 144).start()

    def wo_settle(v):
        wo_raw[pl.ds(D, 16), pl.ds(0, 128)] = _bf(v)

    def fetch_tab(row0, rows, v):
        tab[pl.ds(row0, 8), :] = v
        cp_tab(row0, rows).start()

    def fetch_f(t, v):
        wr_raw[t, pl.ds(0, 8), :] = v
        cp_f(0, t).start()
        wi_raw[t, pl.ds(0, 8), :] = v
        cp_f(1, t).start()
        if t == 0:
            cp_flast(0).start()
            cp_flast(1).start()

    n_tab = _TABLE.shape[0]
    fetches = []

    def fetch_next(value):
        if fetches:
            for fetch in fetches.pop(0):
                fetch(pltpu.bitcast(value[:8, :128], U32))

    def store_pitched(dst, row0, vt):
        for r in range(16):
            dst[pl.ds(row0 + 17 * (r // 2) + 8 * (r % 2), 8), :] = vt[8 * r:8 * r + 8]

    def radix9(tau):
        for i in range(4):
            words = [[xb_raw[side.zero + 2 * tau + z, pl.ds(32 * j + 8 * i, 8), :] for j in range(9)]
                     for z in range(2)]
            for e in range(2):
                u = []
                for z in range(2):
                    u.append(_bfly9_fwd([_unpack(w, e) for w in words[z]]))
                    yield u[z][8], 14
                out = [_pack(u[0][o], u[1][o]) for o in range(9)]
                for o in range(9):
                    u_t[tau, pl.ds(64 * o + 32 * e + 8 * i, 8), :] = out[o]
                yield out, 5

    def u_to_token_major(tau, cost):
        for gi, g in enumerate(_GROUPS):
            if g:
                v = (u_t if 1 else now(u_r))[tau, pl.ds(64 * (2 * g - 1), 128), :]
            else:
                v = jnp.concatenate([(u_t if 1 else now(u_r))[tau, pl.ds(0, 64), :], _zeros_w(64)], axis=0)
            vt = v.T
            store_pitched(u_nat.at[gi], 136 * tau, vt)
            yield vt[120:], cost, 240

    def dft_matrix(a):
        twr = jnp.broadcast_to(pltpu.bitcast(tab[pl.ds(_OFF_TR + a, 1), :], F32), (8, 128))
        twi = jnp.broadcast_to(pltpu.bitcast(tab[pl.ds(_OFF_TI + a, 1), :], F32), (8, 128))
        for i in range(16):
            fr = pltpu.bitcast(now(tab_r)[pl.ds(_OFF_FR + 8 * i, 8), :], F32)
            fi = pltpu.bitcast(now(tab_r)[pl.ds(_OFF_FI + 8 * i, 8), :], F32)
            gr, gi = fr * twr - fi * twi, fr * twi + fi * twr
            gmat[a, 0, pl.ds(8 * i, 8), :] = gr
            out = [gr + gi, gi - gr]
            gmat[a, 1, pl.ds(8 * i, 8), :] = out[0]
            gmat[a, 2, pl.ds(8 * i, 8), :] = out[1]
            yield out, 3

    def filter_rows(row0, load_w):
        rows = pl.ds(row0, 8)
        y = [[None] * 4 for _ in range(4)]
        for a0 in range(4):
            src = now(t_r)
            z = _bfly4([(src[4 * a1 + a0, 0, rows, :], src[4 * a1 + a0, 1, rows, :])
                        for a1 in range(4)], False)
            for g0 in range(4):
                y[g0][a0] = _twiddle16(z[g0], a0 * g0, False)
            yield y[3][a0][0], 7
        for g0 in range(4):
            z = _bfly4(y[g0], False)
            yield z[3][1], 4
            for g1 in range(4):
                wr, wi = load_w(g0 + 4 * g1)
                zr, zi = z[g1]
                z[g1] = (zr * wr - zi * wi, zr * wi + zi * wr)
                if g1 % 2:
                    yield z[g1][1], 4
            z = _bfly4(z, True)
            for a0 in range(4):
                y[g0][a0] = _twiddle16(z[a0], a0 * g0, True)
            yield y[g0][3][0], 6
        for a0 in range(4):
            z = _bfly4([y[g0][a0] for g0 in range(4)], True)
            for a1 in range(4):
                t_buf[4 * a1 + a0, 0, rows, :] = z[a1][0]
                t_buf[4 * a1 + a0, 1, rows, :] = z[a1][1]
            yield [v for pair in z for v in pair], 6

    def filter_all():
        for n, (k0, h) in enumerate(_ROWGROUPS):
            rows = pl.ds(k0 // 2 + 72 * h, 8, stride=9)
            yield from filter_rows(8 * n, lambda f1: (
                _unpack(now(wr_r)[f1, rows, :], k0 % 2),
                _unpack(now(wi_r)[f1, rows, :], k0 % 2)))
        yield from filter_rows(NR - 8, lambda f1: tuple(
            jnp.broadcast_to(wlast[i, :, pl.ds(128 * f1, 128)].astype(F32), (8, 128))
            for i in range(2)))

    def radix9_inv(c):
        for i in range(8):
            y = []
            for e in range(2):
                y.append(_bfly9_inv(
                    [now(t_r)[2 * c + e, i // 4, pl.ds(256 + 8 * (i % 4), 8), :]]
                    + [now(t_r)[2 * c + e, o % 2, pl.ds(64 * (o // 2) + 8 * i, 8), :]
                       for o in range(8)]))
                yield (y[e] if 0 else y[e][8]), 12
            out = [_pack(y[0][j], y[1][j]) for j in range(9)]
            for j in range(9):
                y_t[c, pl.ds(64 * j + 8 * i, 8), :] = out[j]
            yield out, 5

    def y_to_token_major(c, cost):
        for q in range(5):
            if q:
                v = (y_t if 1 else now(y_r))[c, pl.ds(128 * q - 64, 128), :]
            else:
                v = jnp.concatenate([_zeros_w(64), (y_t if 1 else now(y_r))[c, pl.ds(0, 64), :]], axis=0)
            vt = v.T
            stage[4 + q, pl.ds(c, 128, stride=8), :] = vt
            yield vt[120:], cost, 240

    def x_to_token_major(t, qs):
        for q in qs:
            if q < 2:
                v = xa_raw[t, pl.ds(128 * q, 128), :]
            else:
                v = jnp.concatenate([xa_raw[t, pl.ds(256, 32), :], _zeros_w(96)], axis=0)
            store_pitched(x_nat.at[q], 136 * t, v.T)

    def x_tile(a, qs):
        for q in qs:
            vt = x_nat[q, pl.ds(a, 128, stride=17), :].T
            n = 128 if q < 2 else 64
            x_perm[q][a] = vt[:n]
            yield vt[n - 8:n], 43, 240

    def w_prep(part, kts=range(5)):
        col0, _ = _W_COLS[part]
        first = 288 * part - col0 // 2
        for kt in kts:
            for nt in range(5):
                nn = min(128, 3 * D - col0 - 128 * nt)
                vt = wq_raw[pl.ds(128 * kt, 128), pl.ds(col0 + 128 * nt, nn)].T
                vt = pltpu.bitcast(vt, U32)
                wt_nat[kt, pl.ds(64 * nt, nn // 2), :] = vt
                yield vt[-8:], 22, 180
        for kt in kts:
            for i in range(2):
                for dl in range(9):
                    base = first + 144 * i + dl
                    wa = now(wn_r)[kt, pl.ds(base, 8, stride=18), :]
                    wb = now(wn_r)[kt, pl.ds(base + 9, 8, stride=18), :]
                    out = [_pack(_unpack(wa, e), _unpack(wb, e)) for e in range(2)]
                    for e in range(2):
                        wt[part][kt, pl.ds(16 * (2 * dl + e) + 8 * i, 8), :] = out[e]
                    yield out, 2

    def wo_prep():
        for nt in range(5):
            nn = min(128, D - 128 * nt)
            blk = wo_raw[pl.ds(0, D), pl.ds(128 * nt, nn)]
            if nn < 128:
                blk = jnp.concatenate([blk, jnp.zeros((D, 128 - nn), BF16)], axis=1)
            blk = pltpu.bitcast(blk, U32)
            wo_nat[nt] = blk
            wo_perm[nt, pl.ds(288, 32), :] = _zeros_w(32)
            yield blk[-8:], 20
            for i in range(2):
                for dl in range(9):
                    wa = now(won_r)[nt, pl.ds(144 * i + dl, 8, stride=18), :]
                    wb = now(won_r)[nt, pl.ds(144 * i + dl + 9, 8, stride=18), :]
                    out = [_pack(_unpack(wa, e), _unpack(wb, e)) for e in range(2)]
                    for e in range(2):
                        wo_perm[nt, pl.ds(16 * (2 * dl + e) + 8 * i, 8), :] = out[e]
                    yield out, 2

    scale = float(DH) ** -0.5
    QB = 6

    def attend(p, units):
        lane0 = lax.broadcasted_iota(jnp.int32, (8, 128), 1) == 0
        for unit in units:
            gam, hg = divmod(unit, 4)
            base = 2 * gam + 1
            acc = [[None] * W for _ in range(2)]
            for d0 in range(0, DH, QB):
                rows = [pl.ds(144 * hg + 8 * d, 8) for d in range(d0, d0 + QB)]
                q = [[now(q_r[4 * p + gam])[e, r, :] for r in rows] for e in range(2)]
                for l in range(9):
                    for n, r in enumerate(rows):
                        k = now(k_r[p])[base + l, r, :]
                        for e in range(2):
                            w = 7 + e - l
                            if 0 <= w < W:
                                t = q[e][n] * k
                                acc[e][w] = t if acc[e][w] is None else acc[e][w] + t
                    done = [acc[e][7 + e - l] for e in range(2) if 0 <= 7 + e - l < W]
                    yield done, QB / 2 * len(done)
            prob = []
            for e in range(2):
                lg = [jnp.where(lane0, -1e9 / scale, acc[e][w]) if 2 * gam + e < w else acc[e][w]
                      for w in range(W)]
                m = lg[0]
                for w in range(1, W):
                    m = jnp.maximum(m, lg[w])
                ex = [jnp.exp2((l_ - m) * (scale * float(np.log2(np.e)))) for l_ in lg]
                tot = ex[0]
                for w in range(1, W):
                    tot = tot + ex[w]
                inv = 1.0 / tot
                prob.append([x_ * inv for x_ in ex])
                yield prob[e][W - 1], 13, 30
            for d in range(DH):
                rows = pl.ds(32 * d + 8 * hg, 8)
                vv = [now(v_r[p])[base + l, pl.ds(144 * hg + 8 * d, 8), :] for l in range(9)]
                o = []
                for e in range(2):
                    t = prob[e][0] * vv[7 + e]
                    for w in range(1, W):
                        t = t + prob[e][w] * vv[7 + e - w]
                    o.append(t)
                word = _pack(o[0], o[1])
                o_t[p][gam, rows, :] = word
                yield word, 8

    def o_to_token_major(p, cost, gams):
        for gam in gams:
            for kt in range(5):
                if kt < 4:
                    v = (o_t[p] if 1 else now(o_r[p]))[gam, pl.ds(128 * kt, 128), :]
                else:
                    v = jnp.concatenate([(o_t[p] if 1 else now(o_r[p]))[gam, pl.ds(512, 64), :], _zeros_w(64)], axis=0)
                vt = v.T
                o_nat[p][kt, pl.ds(gam, 128, stride=4), :] = vt
                yield vt[120:], cost, 240

    def table(off, i):
        return _bf(tab[pl.ds(off[i], off[i + 1] - off[i]), :])

    def dft64(a):
        side.run(148)
        for gi in range(5):
            x1 = _dot_nt(table(_OFF_LF, gi), _bf(u_nat[gi, pl.ds(a, 64, stride=17), :]))
            n = x1.shape[0] // 2
            x1_buf[a % 2, 0, pl.ds(64 * gi, n), :] = x1[:n]
            x1_buf[a % 2, 1, pl.ds(64 * gi, n), :] = x1[n:]

    def dft128(a):
        side.run(222)
        xr, xi = x1_buf[a % 2, 0], x1_buf[a % 2, 1]
        k1 = _dot(xr + xi, gmat[a, 0])
        t_buf[a, 0] = k1 - _dot(xi, gmat[a, 1])
        ti = k1 + _dot(xr, gmat[a, 2])
        t_buf[a, 1] = ti
        fetch_next(ti)

    def idft128(a):
        side.run(222)
        g = [jnp.concatenate([gmat[a, c, pl.ds(16 * tau + e, 8, stride=2), :]
                              for tau in range(8) for e in range(2)], axis=0) for c in range(3)]
        tr, ti = t_buf[a, 0], t_buf[a, 1]
        k1 = _dot_nt(tr + ti, g[0])
        z_buf[a % 2, 0] = k1 + _dot_nt(ti, g[2])
        z_buf[a % 2, 1] = k1 - _dot_nt(tr, g[1])

    def idft64(a):
        side.run(144)
        for gi in range(5):
            n = 64 if gi < 4 else NR - 256
            parts = [z_buf[a % 2, c, pl.ds(64 * gi, n), :] for c in range(2)]
            if n < 64:
                parts.append(jnp.zeros((128 - 2 * n, 128), F32))
            o = _dot(table(_OFF_LI, gi), jnp.concatenate(parts, axis=0))
            if gi < 4:
                t_buf[a, 0, pl.ds(64 * gi, 64), :] = o[:64]
                t_buf[a, 1, pl.ds(64 * gi, 64), :] = o[64:]
            else:
                t_buf[a, 0, pl.ds(256, 32), :] = o[:32]
                t_buf[a, 1, pl.ds(256, 32), :] = o[32:]

    def proj(part, p, gam, qs=(0, 1, 2), chunks=4):
        a = 4 * gam + p
        m = 288 // chunks
        kts = [kt for q in qs for kt in (2 * q, 2 * q + 1) if kt < 5]
        for ch in range(chunks):
            side.run(len(kts) * m)
            w = jnp.concatenate(
                [_bf(wt[part][kt, pl.ds(m * ch, m), :]) for kt in kts], axis=1)
            x = jnp.concatenate(
                [jnp.concatenate([_bf(x_perm[q][a + 2 * e]) for e in range(2)], axis=1)
                 for q in qs], axis=0)
            r = _dot(w, x)
            for e in range(2):
                c = 2 * gam + e
                buf, slot = (q_buf[4 * p + gam], e) if part == 0 else (
                    (k_buf, v_buf)[part - 1][p], 8 + c)
                rows = []
                for i in range(m // 4):
                    d, hg = divmod(m // 4 * ch + i, 4)
                    rows.append(pl.ds(144 * hg + 8 * d, 8))
                tile = r[:, 128 * e:128 * e + 128]
                if qs[0]:
                    tile = tile + jnp.concatenate([buf[slot, r_, :] for r_ in rows], axis=0)
                shifted = part and c and qs[-1] == 2
                rolled = pltpu.roll(tile, 1, 1) if shifted else None
                for i, r_ in enumerate(rows):
                    buf[slot, r_, :] = tile[8 * i:8 * i + 8]
                    if shifted:
                        buf[c, r_, :] = rolled[8 * i:8 * i + 8]
            fetch_next(r)

    def out_proj(p, row0, cw):
        side.run(12.5 * cw)
        lhs = jnp.concatenate([_bf(o_nat[p][kt, pl.ds(row0, cw), :]) for kt in range(5)], axis=1)
        r = _dot(lhs, jnp.concatenate([_bf(wo_perm[nt]) for nt in range(5)], axis=1))
        rows = pl.ds(2 * row0, 2 * cw)
        for ct in range(5):
            tile = r[:, 128 * ct:128 * ct + 128]
            if p == 0:
                out0[ct, rows, :] = tile
                continue
            word = _pack(out0[ct, rows, :], tile)
            if ct == 4:
                lane = lax.broadcasted_iota(jnp.int32, word.shape, 1)
                word = jnp.where(lane < 64, word, stage[4, rows, :])
            stage[ct, rows, :] = word
            cp_out(ct, 2 * row0, 2 * cw).start()

    cp_wq(1, 0, 256).start()
    for t in range(8):
        cp_xa(t, False).start()
    wq_raw[pl.ds(D, 64), :] = jnp.zeros((64, 3 * D), BF16)
    cp_wq(1, 0, 256).wait()
    _drain(w_prep(1, range(2)))

    @pl.loop(0, 4)
    def _(i):
        @pl.when(i < 2)
        def _():
            for t in range(4):
                cp_xa(4 * i + 8 + t, False).start()

        @pl.when(i == 2)
        def _():
            cp_wq(1, 256, D - 256).start()

        @pl.when(i == 3)
        def _():
            for t in range(6):
                cp_xa(t, True).start()

        for t in range(4):
            cp_xa(4 * i + t, False).wait()
        for t in range(4):
            x_to_token_major(4 * i + t, (0,))

    _drain(x_tile(0, (0,)))
    _drain(x_tile(2, (0,)))

    side.start(xa_raw[0, pl.ds(0, 8), :], x1_buf.at[2, 0])
    pairs = [(p, gam) for p in range(2) for gam in range(4)]

    def barrier():
        side.close()
        _barrier(sem_bar)

    def pair_tiles(name, n, qs, first=False):
        p, gam = pairs[n]
        for e in (1, 0) if first else (0, 1):
            side.add(name, x_tile(4 * gam + p + 2 * e, qs), first=first)

    def fetch_xa(t, v):
        xa_raw[t, pl.ds(128, 8), :] = v
        cp_xa(t, True).start()

    side.set_load(0.5, 0.0)
    fetches += [[partial(fetch_xa, t), partial(fetch_xa, t + 1)] for t in range(6, 16, 2)]
    fetches += [[partial(fetch_xb, t)] for t in range(16)]
    fetches += [[partial(fetch_wq, part, i) for part in (0, 2)] for i in range(4)]
    for i, r in enumerate(range(0, n_tab, 304)):
        fetches[-1 - i].append(partial(fetch_tab, r, min(304, n_tab - r)))
    n_early = 2
    fetches[-1] += [partial(fetch_f, t) for t in range(n_early)]
    for n in range(5):
        pair_tiles("next", n + 1, (0,), first=True)
        if n < 2:
            pair_tiles("later", n + 6, (0,))
        proj(1, *pairs[n], qs=(0,), chunks=2)
        side.finish("next")
    side.close()

    for t in range(16):
        cp_xa(t, True).wait()
    cp_wq(1, 256, D - 256).wait()
    side.set_load(0.6, 0.0)
    for n in range(5, 8):
        proj(1, *pairs[n], qs=(0,), chunks=2)
    for t in range(16):
        x_to_token_major(t, (1, 2))
    pair_tiles("next", 0, (1, 2))
    side.add("next", w_prep(1, range(2, 5)))
    side.finish("next")
    for n in range(3):
        pair_tiles("next", n + 1, (1, 2))
        proj(1, *pairs[n], qs=(1, 2), chunks=3)
        side.finish("next")
    side.close()

    assert not fetches
    pltpu.make_async_copy(xb_raw, xb_raw, sem_in.at[SEM_XB]).wait()
    side.set_load((8 * 264 + 4 * 172) / 3456, 1.1)
    for tau in range(8):
        side.add("r9", radix9(tau))
    for n in range(3, 7):
        pair_tiles("next", n + 1, (1, 2), first=True)
        proj(1, *pairs[n], qs=(1, 2), chunks=3)
        side.finish("next")
    side.close()

    cp_tab(0, n_tab).wait()
    cp_wq(0).wait()
    cp_wq(2).wait()
    side.set_load((40 * 43 + 16 * 48 + 2 * 730) / 9664 * 1.6, 0.5)
    side.add("q", w_prep(0))
    proj(1, *pairs[7], qs=(1, 2), chunks=3)
    side.finish("q")
    for tau in range(8):
        side.add("t", u_to_token_major(tau, 43))
    side.add("t", dft_matrix(0))
    side.add("w", w_prep(2))
    fetches += [[partial(fetch_f, t)] for t in range(2, 16)]
    fetches += [[partial(fetch_wo, i)] for i in range(4)]
    fetches.append([wo_settle])
    proj(0, 0, 0)
    proj(0, 0, 1)
    side.finish("t")
    dft64(0)
    for a in range(16):
        if a < 15:
            side.add("g", dft_matrix(a + 1), first=True)
            dft64(a + 1)
        dft128(a)
        side.finish("g")
    side.close()

    pltpu.make_async_copy(wr_raw, wr_raw, sem_in.at[SEM_WR]).wait()
    pltpu.make_async_copy(wi_raw, wi_raw, sem_in.at[SEM_WI]).wait()
    cp_flast(0).wait()
    cp_flast(1).wait()
    cp_wo().wait()
    assert not fetches
    side.set_load((37 * 120 + 280) / 8640, 0.95)
    side.add("f", filter_all())
    side.add("wo", wo_prep())
    for gam in range(4):
        proj(2, 0, gam)
    proj(0, 0, 2)
    proj(0, 0, 3)
    barrier()

    n6, n8, keep = 8, 4, 64
    side.set_load(n6 * 319 / 5856, 1.0)
    side.add("att", attend(0, range(n6)))
    idft128(0)
    for a in range(16):
        if a < 15:
            idft128(a + 1)
        idft64(a)
    barrier()

    side.set_load(((16 - n6) * 319 + 8 * 232) / 7200, 1.0)
    side.add("att", attend(0, range(n6, 16)))
    for c in range(8):
        side.add("r9", radix9_inv(c))
    for gam in range(4):
        proj(2, 1, gam)
    proj(0, 1, 0)
    barrier()

    tc = 34.0
    load = n8 * 319 / (4320 - 60 * tc)
    side.set_load(load, 1.0)
    side.add("att", attend(1, range(n8)))
    side.add("o", o_to_token_major(0, tc * load, range(4)))
    for c in range(8):
        side.add("y", y_to_token_major(c, tc * load))
    for gam in range(1, 4):
        proj(0, 1, gam)
    side.close()
    for ct in range(5, 9):
        cp_out(ct, 0, S // 2).start()
    _barrier(sem_bar)

    side.set_load((16 - n8) * 319 / (12.5 * (512 - keep)), 1.0)
    side.add("att", attend(1, range(n8, 16)))
    for row0 in range(0, 512 - keep, 64):
        out_proj(0, row0, min(64, 512 - keep - row0))
    barrier()

    side.set_load(1.0, 0.0)
    out_proj(0, 512 - keep, keep)
    _drain(o_to_token_major(1, 0, range(4)))
    row0 = 0
    for cw in (128, 128, 96, 64, 48, 32, 16):
        out_proj(1, row0, cw)
        row0 += cw
    pltpu.make_async_copy(out_hbm, out_hbm, sem_out).wait()


def _barrier(sem):
    pl.semaphore_signal(sem)
    pl.semaphore_wait(sem)


@jax.jit
def pallas_concat_heads__sliding_local_dilated__spectral_gfnet__prompt_kernel(
    A_x: jax.Array,
    A_wqkv: jax.Array,
    A_wo: jax.Array,
    B_x: jax.Array,
    B_w_r: jax.Array,
    B_w_i: jax.Array,
):
    assert A_x.shape == (1, S, D) and B_x.shape == (1, S, D)
    any_spec = pl.BlockSpec(memory_space=pl.ANY)
    scratch = [
        pltpu.VMEM((1,) + _TABLE.shape, U32),
        pltpu.VMEM((16, 288, 128), U32),
        pltpu.VMEM((16, 288, 128), U32),
        pltpu.VMEM((D + 64, 3 * D), BF16),
        pltpu.VMEM((D + 64, D), BF16),
        pltpu.VMEM((1, 16, 144, 128), U32),
        pltpu.VMEM((1, 16, 144, 128), U32),
        pltpu.VMEM((2, 1, S), BF16),
        pltpu.VMEM((1, 16, 3, 128, 128), F32),
        pltpu.VMEM((1, 8, D, 128), U32),
        pltpu.VMEM((1, 8, D, 128), U32),
        pltpu.VMEM((5, 8 * 136, 128), U32),
        pltpu.VMEM((1, 4, 2, NR, 128), F32),
        pltpu.VMEM((1, 16, 2, NR, 128), F32),
        pltpu.VMEM((1, 2, 2, NR, 128), F32),
        pltpu.VMEM((3, 16 * 136, 128), U32),
        [pltpu.VMEM((1, 16, n, 128), U32) for n in (128, 128, 64)],
        pltpu.VMEM((1, 5, 320, 128), U32),
        pltpu.VMEM((1, 5, 288, 128), U32),
        pltpu.VMEM((1, 5, 288, 128), U32),
        pltpu.VMEM((1, 5, 288, 128), U32),
        pltpu.VMEM((1, 5, 288, 128), U32),
        pltpu.VMEM((1, 5, 320, 128), U32),
        [pltpu.VMEM((1, 2, D + 16, 128), F32)] * 8,
        [pltpu.VMEM((1, 16, D + 8, 128), F32)] * 2,
        [pltpu.VMEM((1, 16, D + 8, 128), F32)] * 2,
        [pltpu.VMEM((1, 4, D, 128), U32)] * 2,
        [pltpu.VMEM((1, 5, 512, 128), U32)] * 2,
        pltpu.VMEM((1, 5, S // 2, 128), F32),
        pltpu.VMEM((9, S // 2, 128), U32),
        pltpu.SemaphoreType.DMA((5,)),
        pltpu.SemaphoreType.DMA((9,)),
        pltpu.SemaphoreType.DMA(()),
        pltpu.SemaphoreType.REGULAR,
    ]
    out = pl.pallas_call(
        _kernel,
        out_shape=jax.ShapeDtypeStruct((S, 2 * D), BF16),
        in_specs=[any_spec] * 7 + [pl.BlockSpec(memory_space=pltpu.SMEM)],
        out_specs=any_spec,
        scratch_shapes=scratch,
        compiler_params=pltpu.CompilerParams(vmem_limit_bytes=120 * 1024 * 1024),
        name="attn_gfnet",
    )(A_x[0].T, A_wqkv, A_wo, B_x[0].T, B_w_r.T, B_w_i.T, _TABLE, np.zeros((2,), np.int32))
    return out[None]
```

```python
from functools import partial

import numpy as np

import jax
import jax.numpy as jnp
from jax import lax
import jax.experimental.pallas as pl
import jax.experimental.pallas.tpu as pltpu

S = 2048
D = 576
H = 32
DH = 18
W = 8
DF = D // 2 + 1
NR = 296

F32 = jnp.float32
BF16 = jnp.bfloat16
U32 = jnp.uint32

_C3 = float(np.sqrt(3.0) / 2)
_C1, _S1 = float(np.cos(2 * np.pi / 9)), float(np.sin(2 * np.pi / 9))
_C2, _S2 = float(np.cos(4 * np.pi / 9)), float(np.sin(4 * np.pi / 9))


def _bfly9_fwd(x):
    a0, ar, ai = [], [], []
    for j in range(3):
        t = x[j + 3] + x[j + 6]
        a0.append(x[j] + t)
        ar.append(x[j] - 0.5 * t)
        ai.append(x[j + 6] - x[j + 3])
    t = a0[1] + a0[2]
    u0 = a0[0] + t
    u3r = a0[0] - 0.5 * t
    u3i = a0[2] - a0[1]
    b1r = ar[1] * _C1 + ai[1] * (_C3 * _S1)
    b1i = ai[1] * (_C3 * _C1) - ar[1] * _S1
    b2r = ar[2] * _C2 + ai[2] * (_C3 * _S2)
    b2i = ai[2] * (_C3 * _C2) - ar[2] * _S2
    a_r, a_i = ar[0], ai[0] * _C3
    tr, ti = b1r + b2r, b1i + b2i
    dr, di = (b1r - b2r) * _C3, (b1i - b2i) * _C3
    u1r, u1i = a_r + tr, a_i + ti
    mr, mi = a_r - 0.5 * tr, a_i - 0.5 * ti
    return [u0, u1r, u1i, mr - di, mi + dr, u3r, u3i, mr + di, mi - dr]


def _bfly9_inv(v):
    u0, u1r, u1i, u7r, u7i, u3r, u3i, u4r, u4i = v
    mr, mi = u4r + u7r, u4i + u7i
    di, dr = (u4r - u7r) * _C3, (u7i - u4i) * _C3
    a_r, a_i = u1r + mr, u1i + mi
    tr, ti = u1r - 0.5 * mr, u1i - 0.5 * mi
    b1r, b2r, b1i, b2i = tr + dr, tr - dr, ti + di, ti - di
    ar = [a_r, b1r * _C1 - b1i * _S1, b2r * _C2 - b2i * _S2]
    ai = [a_i * _C3, b1r * (_C3 * _S1) + b1i * (_C3 * _C1),
          b2r * (_C3 * _S2) + b2i * (_C3 * _C2)]
    t = u0 - 0.5 * u3r
    a0 = [u0 + u3r, t - u3i, t + u3i]
    y = [None] * 9
    for j in range(3):
        t = a0[j] - 0.5 * ar[j]
        y[j] = a0[j] + ar[j]
        y[j + 3] = t - ai[j]
        y[j + 6] = t + ai[j]
    return y


def _bfly4(x, inverse):
    (ar, ai), (br, bi), (cr, ci), (dr, di) = x
    pr, pi, qr, qi = ar + cr, ai + ci, ar - cr, ai - ci
    sr, si, tr, ti = br + dr, bi + di, br - dr, bi - di
    y1, y3 = (qr + ti, qi - tr), (qr - ti, qi + tr)
    if inverse:
        y1, y3 = y3, y1
    return [(pr + sr, pi + si), y1, (pr - sr, pi - si), y3]


def _twiddle16(z, e, inverse):
    zr, zi = z
    e = (-e if inverse else e) % 16
    h = float(np.sqrt(0.5))
    if e == 0:
        return z
    if e == 4:
        return zi, -zr
    if e == 12:
        return -zi, zr
    if e == 2:
        return (zr + zi) * h, (zi - zr) * h
    if e == 14:
        return (zr - zi) * h, (zr + zi) * h
    if e == 6:
        return (zi - zr) * h, (zr + zi) * (-h)
    if e == 10:
        return (zr + zi) * (-h), (zr - zi) * h
    c, s = float(np.cos(2 * np.pi * e / 16)), float(np.sin(2 * np.pi * e / 16))
    return zr * c + zi * s, zi * c - zr * s


_GROUPS = (1, 2, 3, 4, 0)


def _group_classes(g):
    return sorted({g, g + 9, 9 - g, 18 - g}) if g else [0, 9]


_ROWGROUPS = [(k0, h) for g in _GROUPS for k0 in _group_classes(g) for h in range(2)]


def _to_words(m):
    u = np.ascontiguousarray(m, dtype=np.float32).view(np.uint32)
    u = (u + 0x7FFF + ((u >> 16) & 1)) >> 16
    return (u[0::2] | (u[1::2] << 16)).astype(np.uint32)


def _make_tables():
    basis = np.array(_bfly9_fwd(list(np.eye(9))))
    m_fwd = np.array([2 * (r % 32) + r // 32 for r in range(64)])
    lf, li = [], []
    for g in _GROUPS:
        rows = [k0 + 18 * i for k0 in _group_classes(g) for i in range(16)]
        if g == 0:
            rows += [DF - 1] + [-1] * 7
        cols = [2 * g - 1, 2 * g] if g else [0]
        a = basis[cols].T.astype(complex)
        n = len(rows)
        f = np.zeros((2 * n, 128))
        b = np.zeros((64 * len(cols), 128))
        for r, k in enumerate(rows):
            if k < 0:
                continue
            ck = np.exp(-2j * np.pi * ((np.arange(9) * k) % 9) / 9)
            lam = np.linalg.solve(a.conj().T @ a, a.conj().T @ ck)
            wk = (1.0 if k in (0, DF - 1) else 2.0) / (S * D)
            for c in range(len(cols)):
                e = lam[c] * np.exp(-2j * np.pi * ((m_fwd * k) % D) / D)
                f[r, 64 * c:64 * c + 64] = e.real
                f[n + r, 64 * c:64 * c + 64] = e.imag
                e = wk * lam[c] * np.exp(-2j * np.pi * ((np.arange(64) * k) % D) / D)
                b[64 * c:64 * c + 64, r] = e.real
                b[64 * c:64 * c + 64, n + r] = e.imag
        lf.append(_to_words(f))
        li.append(_to_words(b))
    n = np.arange(128)
    b_of_n = 16 * (n // 16) + 8 * (n % 2) + (n % 16) // 2
    f128 = np.exp(-2j * np.pi * (np.outer(b_of_n, n) % 128) / 128)
    tw = np.exp(-2j * np.pi * np.outer(np.arange(16), n) / S)
    f32w = lambda m: np.ascontiguousarray(m, dtype=np.float32).view(np.uint32)
    parts = [f32w(f128.real), f32w(f128.imag), f32w(tw.real), f32w(tw.imag)] + lf + li
    offs = np.cumsum([0] + [p.shape[0] for p in parts])
    parts.append(np.zeros((-offs[-1] % 32, 128), np.uint32))
    return np.concatenate(parts, axis=0), [int(o) for o in offs]


_TABLE, _OFF = _make_tables()
_OFF_FR, _OFF_FI, _OFF_TR, _OFF_TI = _OFF[0:4]
_OFF_LF = _OFF[4:10]
_OFF_LI = _OFF[9:15]


def _pack(lo, hi):
    return pltpu.pack_elementwise([lo, hi], packed_dtype=BF16)


def _unpack(w, index):
    return pltpu.unpack_elementwise(w, index=index, packed_dtype=BF16, unpacked_dtype=F32)


def _bf(words):
    return pltpu.bitcast(words, BF16)


def _dot(a, b):
    return lax.dot_general(a, b, (((1,), (0,)), ((), ())), preferred_element_type=F32)


def _dot_nt(a, b):
    return lax.dot_general(a, b, (((1,), (1,)), ((), ())), preferred_element_type=F32)


def _zeros_w(rows):
    return jnp.zeros((rows, 128), U32)


class _SideWork:
    LINK = 7.0

    def __init__(self, zero_ref):
        self.zero_ref = zero_ref
        self.zero = zero_ref[0]
        self.lead = 0.0

    def start(self, seed, sink):
        self.chain = pltpu.bitcast(seed, F32)
        self.sink = sink
        self.jobs = []
        self.credit = 0.0
        self.delay = 0.0
        self.blocks = 0
        self.now = 0.0
        self.pending = []

    def open(self, stretch=1.0, slack=100.0, links=4):
        self.min_links = links
        self.zero = self.zero_ref[0]
        self.lead = -slack
        self.stretch = stretch

    def add(self, name, gen, load, first=False):
        self.jobs.insert(0 if first else len(self.jobs), (name, gen, load * 1.0))

    def _advance(self, cycles):
        self.lead += cycles
        while self.lead >= 6.0:
            self.zero = self.zero_ref[self.zero]
            self.lead -= 6.0

    def _tick(self, cycles):
        self.now += cycles
        self.delay += cycles
        while self.pending and self.pending[0][0] <= self.now:
            self.chain = self.pending.pop(0)[1] + self.chain
            self.delay -= 2.0
        n = int(self.delay / self.LINK)
        if n >= self.min_links:
            for _ in range(n):
                self.chain = pl.reciprocal(self.chain, approx=True)
            self.delay -= n * self.LINK

    def _step(self):
        item = next(self.jobs[0][1], None)
        if item is None:
            self.jobs.pop(0)
            return
        values, cycles, latency = (item + (0.0,))[:3]
        values = values if isinstance(values, list) else [values]
        values = [pltpu.bitcast(v, F32) for v in values]
        while len(values) > 1:
            values = [values[i] + values[i + 1] if i + 1 < len(values) else values[i]
                      for i in range(0, len(values), 2)]
        self.pending.append((self.now + latency, values[0]))
        self.pending.sort(key=lambda x: x[0])
        cycles = cycles / self.jobs[0][2]
        self.credit -= cycles
        self._advance(cycles)
        self._tick(self.stretch * cycles)

    def run(self, cycles):
        self.credit += cycles
        while self.jobs and self.credit > 0:
            self._step()
        if not self.jobs and self.credit > 0:
            self._tick(self.stretch * self.credit)
            self.credit = 0.0

    def finish(self, name):
        while any(job[0] == name for job in self.jobs):
            self._step()

    def close(self):
        while self.jobs:
            self._step()
        while self.pending:
            self.chain = self.pending.pop(0)[1] + self.chain
        self.sink[pl.ds(8 * self.blocks, 8), :] = self.chain
        self.blocks += 1
        self.credit = self.delay = 0.0


def _drain(gen):
    for _ in gen:
        pass


_W_COLS = ((0, 512), (512, 640), (1152, 576))


def _kernel(xa_hbm, wqkv_hbm, wo_hbm, xb_hbm, wr_hbm, wi_hbm, tab_hbm, zero_ref, out_hbm,
            tab, xb_raw, xa_raw, xa_rest, wq_raw, wo_raw, wr_raw, wi_raw, wlast,
            gmat, u_t, y_t, u_nat, x1_buf, t_buf, z_buf, x_nat, x_perm, wt_nat, wt_q, wt_k, wt_v,
            wo_nat, wo_perm, wo_tail, q_buf, k_buf, v_buf, o_t, o_nat, out0, a_tail, stage,
            sem_xa, sem_in, sem_out, sem_bar):
    side = _SideWork(zero_ref)
    zero = side.zero

    def now(ref):
        return ref.at[side.zero]

    tab_r, wr_r, wi_r = tab, wr_raw, wi_raw
    tab, wr_raw, wi_raw = tab.at[0], wr_raw.at[0], wi_raw.at[0]
    (u_r, y_r, t_r, wn_r, won_r, q_r, k_r, v_r, o_r) = (
        u_t, y_t, t_buf, wt_nat, wo_nat, q_buf, k_buf, v_buf, o_t)
    (gmat, u_t, y_t, x1_buf, t_buf, z_buf, x_perm, wt_nat, wt_q, wt_k, wt_v, wo_nat, wo_perm,
     wo_tail, q_buf, k_buf, v_buf, o_t, o_nat, out0, a_tail) = jax.tree.map(
        lambda r: r.at[zero],
        (gmat, u_t, y_t, x1_buf, t_buf, z_buf, x_perm, wt_nat, wt_q, wt_k, wt_v, wo_nat, wo_perm,
         wo_tail, q_buf, k_buf, v_buf, o_t, o_nat, out0, a_tail))
    wt = (wt_q, wt_k, wt_v)

    SEM_XB, SEM_TAB, SEM_WQ, SEM_WK, SEM_WV, SEM_WO, SEM_WR, SEM_WI, SEM_LAST = range(9)

    def cp_tab(row0, rows, z=0):
        return pltpu.make_async_copy(
            tab_hbm.at[pl.ds(row0, rows)], tab.at[pl.ds(pl.multiple_of(z + row0, 8), rows)],
            sem_in.at[SEM_TAB])

    def cp_xb(t, z=0):
        return pltpu.make_async_copy(
            xb_hbm.at[:, pl.ds(t * 128, 128)], xb_raw.at[z + t].bitcast(BF16), sem_in.at[SEM_XB])

    def cp_xa(t):
        return pltpu.make_async_copy(
            xa_hbm.at[pl.ds(0, 256), pl.ds(t * 128, 128)], xa_raw.at[t].bitcast(BF16),
            sem_xa.at[sum(t >= s for s in (6, 11, 14))])

    def cp_xa_rest():
        return pltpu.make_async_copy(xa_hbm.at[pl.ds(256, D - 256)], xa_rest, sem_xa.at[4])

    def cp_wq(part, row0=0, rows=D, z=0):
        cols = pl.ds(*_W_COLS[part])
        return pltpu.make_async_copy(
            wqkv_hbm.at[pl.ds(row0, rows), cols],
            wq_raw.at[pl.ds(pl.multiple_of(z + row0, 16), rows), cols], sem_in.at[SEM_WQ + part])

    def cp_wo(row0=0, rows=D, z=0):
        return pltpu.make_async_copy(
            wo_hbm.at[pl.ds(row0, rows)], wo_raw.at[pl.ds(pl.multiple_of(z + row0, 16), rows)],
            sem_in.at[SEM_WO])

    def cp_f(i, t, z=0):
        src, dst = ((wr_hbm, wr_raw), (wi_hbm, wi_raw))[i]
        return pltpu.make_async_copy(
            src.at[pl.ds(0, DF - 1), pl.ds(t * 128, 128)], dst.at[z + t].bitcast(BF16),
            sem_in.at[SEM_WR + i])

    def cp_flast(i):
        src = (wr_hbm, wi_hbm)[i]
        return pltpu.make_async_copy(src.at[pl.ds(DF - 1, 1), :], wlast.at[i], sem_in.at[SEM_LAST])

    def cp_out(ct, row0, rows):
        return pltpu.make_async_copy(
            stage.at[ct, pl.ds(row0, rows), :].bitcast(BF16),
            out_hbm.at[pl.ds(2 * row0, 2 * rows), pl.ds(ct * 128, 128)], sem_out)

    def fetch_xb(t, v):
        xb_raw[t, pl.ds(0, 8), :] = v
        cp_xb(t).start()

    def fetch_wq(part, piece, v):
        wq_raw[pl.ds(144 * piece, 16), pl.ds(_W_COLS[part][0], 128)] = _bf(v)
        cp_wq(part, 144 * piece, 144).start()

    def fetch_wo(piece, v):
        wo_raw[pl.ds(144 * piece, 16), pl.ds(0, 128)] = _bf(v)
        cp_wo(144 * piece, 144).start()

    def wo_settle(v):
        wo_raw[pl.ds(D, 16), pl.ds(0, 128)] = _bf(v)

    def fetch_tab(row0, rows, v):
        tab[pl.ds(row0, 8), :] = v
        cp_tab(row0, rows).start()

    def fetch_f(t, v):
        wr_raw[t, pl.ds(0, 8), :] = v
        cp_f(0, t).start()
        wi_raw[t, pl.ds(0, 8), :] = v
        cp_f(1, t).start()
        if t == 0:
            cp_flast(0).start()
            cp_flast(1).start()

    n_tab = _TABLE.shape[0]
    fetches = []

    def fetch_next(value):
        if fetches:
            for fetch in fetches.pop(0):
                fetch(pltpu.bitcast(value[:8, :128], U32))

    def store_pitched(dst, row0, vt):
        for r in range(16):
            dst[pl.ds(row0 + 17 * (r // 2) + 8 * (r % 2), 8), :] = vt[8 * r:8 * r + 8]

    def radix9(tau):
        for i in range(4):
            words = [[xb_raw[side.zero + 2 * tau + z, pl.ds(32 * j + 8 * i, 8), :] for j in range(9)]
                     for z in range(2)]
            for e in range(2):
                u = []
                for z in range(2):
                    u.append(_bfly9_fwd([_unpack(w, e) for w in words[z]]))
                    yield u[z][8], 14
                out = [_pack(u[0][o], u[1][o]) for o in range(9)]
                for o in range(9):
                    u_t[tau, pl.ds(64 * o + 32 * e + 8 * i, 8), :] = out[o]
                yield out, 5

    def u_to_token_major(tau, cost):
        for gi, g in enumerate(_GROUPS):
            if g:
                v = (u_t if 1 else now(u_r))[tau, pl.ds(64 * (2 * g - 1), 128), :]
            else:
                v = jnp.concatenate([(u_t if 1 else now(u_r))[tau, pl.ds(0, 64), :], _zeros_w(64)], axis=0)
            vt = v.T
            store_pitched(u_nat.at[gi], 136 * tau, vt)
            yield vt[120:], cost, 240

    def dft_matrix(a):
        twr = jnp.broadcast_to(pltpu.bitcast(tab[pl.ds(_OFF_TR + a, 1), :], F32), (8, 128))
        twi = jnp.broadcast_to(pltpu.bitcast(tab[pl.ds(_OFF_TI + a, 1), :], F32), (8, 128))
        for i in range(16):
            fr = pltpu.bitcast(now(tab_r)[pl.ds(_OFF_FR + 8 * i, 8), :], F32)
            fi = pltpu.bitcast(now(tab_r)[pl.ds(_OFF_FI + 8 * i, 8), :], F32)
            gr, gi = fr * twr - fi * twi, fr * twi + fi * twr
            gmat[a, 0, pl.ds(8 * i, 8), :] = gr
            out = [gr + gi, gi - gr]
            gmat[a, 1, pl.ds(8 * i, 8), :] = out[0]
            gmat[a, 2, pl.ds(8 * i, 8), :] = out[1]
            yield out, 3

    def filter_rows(row0, load_w):
        rows = pl.ds(row0, 8)
        y = [[None] * 4 for _ in range(4)]
        for a0 in range(4):
            src = now(t_r)
            z = _bfly4([(src[4 * a1 + a0, 0, rows, :], src[4 * a1 + a0, 1, rows, :])
                        for a1 in range(4)], False)
            for g0 in range(4):
                y[g0][a0] = _twiddle16(z[g0], a0 * g0, False)
            yield y[3][a0][0], 7
        for g0 in range(4):
            z = _bfly4(y[g0], False)
            yield z[3][1], 4
            for g1 in range(4):
                wr, wi = load_w(g0 + 4 * g1)
                zr, zi = z[g1]
                z[g1] = (zr * wr - zi * wi, zr * wi + zi * wr)
                if g1 % 2:
                    yield z[g1][1], 4
            z = _bfly4(z, True)
            for a0 in range(4):
                y[g0][a0] = _twiddle16(z[a0], a0 * g0, True)
            yield y[g0][3][0], 6
        for a0 in range(4):
            z = _bfly4([y[g0][a0] for g0 in range(4)], True)
            for a1 in range(4):
                t_buf[4 * a1 + a0, 0, rows, :] = z[a1][0]
                t_buf[4 * a1 + a0, 1, rows, :] = z[a1][1]
            yield [v for pair in z for v in pair], 6

    def filter_all():
        for n, (k0, h) in enumerate(_ROWGROUPS):
            rows = pl.ds(k0 // 2 + 72 * h, 8, stride=9)
            yield from filter_rows(8 * n, lambda f1: (
                _unpack(now(wr_r)[f1, rows, :], k0 % 2),
                _unpack(now(wi_r)[f1, rows, :], k0 % 2)))
        yield from filter_rows(NR - 8, lambda f1: tuple(
            jnp.broadcast_to(wlast[i, :, pl.ds(128 * f1, 128)].astype(F32), (8, 128))
            for i in range(2)))

    def radix9_inv(c):
        for i in range(8):
            y = []
            for e in range(2):
                y.append(_bfly9_inv(
                    [now(t_r)[2 * c + e, i // 4, pl.ds(256 + 8 * (i % 4), 8), :]]
                    + [now(t_r)[2 * c + e, o % 2, pl.ds(64 * (o // 2) + 8 * i, 8), :]
                       for o in range(8)]))
                yield (y[e] if 0 else y[e][8]), 12
            out = [_pack(y[0][j], y[1][j]) for j in range(9)]
            for j in range(9):
                y_t[c, pl.ds(64 * j + 8 * i, 8), :] = out[j]
            yield out, 5

    def y_to_token_major(c, cost):
        for q in range(4):
            vt = y_t[c, pl.ds(64 + 128 * q, 128), :].T
            stage[5 + q, pl.ds(c, 128, stride=8), :] = vt
            yield vt[120:], cost, 240

    def seam_to_token_major(c):
        top = _pack(a_tail[0, c], a_tail[1, c])
        stage[4, pl.ds(c, 128, stride=8), :] = jnp.concatenate(
            [top, y_t[c, pl.ds(0, 64), :]], axis=0).T

    def wo_tail_prep():
        for kt in range(5):
            vt = pltpu.bitcast(_bf(wo_perm[4, pl.ds(64 * kt, 64), :]).T, U32)
            wo_tail[kt] = vt[:32]
            yield vt[24:32], 22, 180

    def x_to_token_major(t, qs):
        lanes = pl.ds(128 * t, 128)
        for q in qs:
            if q == 0:
                v = xa_raw[t]
            elif q == 1:
                v = pltpu.bitcast(xa_rest[pl.ds(0, 256), lanes], U32)
            else:
                v = pltpu.bitcast(xa_rest[pl.ds(256, 64), lanes], U32)
                v = jnp.concatenate([v, _zeros_w(96)], axis=0)
            store_pitched(x_nat.at[q], 136 * t, v.T)

    def x_tile(a, qs):
        for q in qs:
            vt = x_nat[q, pl.ds(a, 128, stride=17), :].T
            n = 128 if q < 2 else 64
            x_perm[q][a] = vt[:n]
            yield vt[n - 8:n], 43, 240

    def w_prep(part, kts=range(5)):
        col0, _ = _W_COLS[part]
        first = 288 * part - col0 // 2
        for kt in kts:
            for nt in range(5):
                nn = min(128, 3 * D - col0 - 128 * nt)
                vt = wq_raw[pl.ds(128 * kt, 128), pl.ds(col0 + 128 * nt, nn)].T
                vt = pltpu.bitcast(vt, U32)
                wt_nat[kt, pl.ds(64 * nt, nn // 2), :] = vt
                yield vt[-8:], 22, 180
        for kt in kts:
            for i in range(2):
                for dl in range(9):
                    base = first + 144 * i + dl
                    wa = now(wn_r)[kt, pl.ds(base, 8, stride=18), :]
                    wb = now(wn_r)[kt, pl.ds(base + 9, 8, stride=18), :]
                    out = [_pack(_unpack(wa, e), _unpack(wb, e)) for e in range(2)]
                    for e in range(2):
                        wt[part][kt, pl.ds(16 * (2 * dl + e) + 8 * i, 8), :] = out[e]
                    yield out, 2

    def wo_prep():
        for nt in range(5):
            nn = min(128, D - 128 * nt)
            blk = wo_raw[pl.ds(0, D), pl.ds(128 * nt, nn)]
            if nn < 128:
                blk = jnp.concatenate([blk, jnp.zeros((D, 128 - nn), BF16)], axis=1)
            blk = pltpu.bitcast(blk, U32)
            wo_nat[nt] = blk
            wo_perm[nt, pl.ds(288, 32), :] = _zeros_w(32)
            yield blk[-8:], 20
            for i in range(2):
                for dl in range(9):
                    wa = now(won_r)[nt, pl.ds(144 * i + dl, 8, stride=18), :]
                    wb = now(won_r)[nt, pl.ds(144 * i + dl + 9, 8, stride=18), :]
                    out = [_pack(_unpack(wa, e), _unpack(wb, e)) for e in range(2)]
                    for e in range(2):
                        wo_perm[nt, pl.ds(16 * (2 * dl + e) + 8 * i, 8), :] = out[e]
                    yield out, 2

    scale = float(DH) ** -0.5
    QB = 6

    def attend(p, units):
        lane0 = lax.broadcasted_iota(jnp.int32, (8, 128), 1) == 0
        for unit in units:
            gam, hg = divmod(unit, 4)
            base = 2 * gam + 1
            acc = [[None] * W for _ in range(2)]
            for d0 in range(0, DH, QB):
                rows = [pl.ds(144 * hg + 8 * d, 8) for d in range(d0, d0 + QB)]
                q = [[now(q_r[4 * p + gam])[e, r, :] for r in rows] for e in range(2)]
                for l in range(9):
                    for n, r in enumerate(rows):
                        k = now(k_r[p])[base + l, r, :]
                        for e in range(2):
                            w = 7 + e - l
                            if 0 <= w < W:
                                t = q[e][n] * k
                                acc[e][w] = t if acc[e][w] is None else acc[e][w] + t
                    done = [acc[e][7 + e - l] for e in range(2) if 0 <= 7 + e - l < W]
                    yield done, QB / 2 * len(done)
            prob = []
            for e in range(2):
                lg = [jnp.where(lane0, -1e9 / scale, acc[e][w]) if 2 * gam + e < w else acc[e][w]
                      for w in range(W)]
                m = lg[0]
                for w in range(1, W):
                    m = jnp.maximum(m, lg[w])
                ex = [jnp.exp2((l_ - m) * (scale * float(np.log2(np.e)))) for l_ in lg]
                tot = ex[0]
                for w in range(1, W):
                    tot = tot + ex[w]
                inv = 1.0 / tot
                prob.append([x_ * inv for x_ in ex])
                yield prob[e][W - 1], 13, 30
            for d in range(DH):
                rows = pl.ds(32 * d + 8 * hg, 8)
                vv = [now(v_r[p])[base + l, pl.ds(144 * hg + 8 * d, 8), :] for l in range(9)]
                o = []
                for e in range(2):
                    t = prob[e][0] * vv[7 + e]
                    for w in range(1, W):
                        t = t + prob[e][w] * vv[7 + e - w]
                    o.append(t)
                word = _pack(o[0], o[1])
                o_t[p][gam, rows, :] = word
                yield word, 8

    def o_to_token_major(p, cost, gams):
        for gam in gams:
            for kt in range(5):
                if kt < 4:
                    v = (o_t[p] if 1 else now(o_r[p]))[gam, pl.ds(128 * kt, 128), :]
                else:
                    v = jnp.concatenate([(o_t[p] if 1 else now(o_r[p]))[gam, pl.ds(512, 64), :], _zeros_w(64)], axis=0)
                vt = v.T
                o_nat[p][kt, pl.ds(gam, 128, stride=4), :] = vt
                yield vt[120:], cost, 240

    def table(off, i):
        return _bf(tab[pl.ds(off[i], off[i + 1] - off[i]), :])

    def dft64(a):
        side.run(148)
        for gi in range(5):
            x1 = _dot_nt(table(_OFF_LF, gi), _bf(u_nat[gi, pl.ds(a, 64, stride=17), :]))
            n = x1.shape[0] // 2
            x1_buf[a % 2, 0, pl.ds(64 * gi, n), :] = x1[:n]
            x1_buf[a % 2, 1, pl.ds(64 * gi, n), :] = x1[n:]

    def dft128(a):
        side.run(222)
        xr, xi = x1_buf[a % 2, 0], x1_buf[a % 2, 1]
        k1 = _dot(xr + xi, gmat[a, 0])
        t_buf[a, 0] = k1 - _dot(xi, gmat[a, 1])
        ti = k1 + _dot(xr, gmat[a, 2])
        t_buf[a, 1] = ti
        fetch_next(ti)

    def idft128(a):
        side.run(222)
        g = [jnp.concatenate([gmat[a, c, pl.ds(16 * tau + e, 8, stride=2), :]
                              for tau in range(8) for e in range(2)], axis=0) for c in range(3)]
        tr, ti = t_buf[a, 0], t_buf[a, 1]
        k1 = _dot_nt(tr + ti, g[0])
        z_buf[a % 2, 0] = k1 + _dot_nt(ti, g[2])
        z_buf[a % 2, 1] = k1 - _dot_nt(tr, g[1])

    def idft64(a):
        side.run(144)
        for gi in range(5):
            n = 64 if gi < 4 else NR - 256
            parts = [z_buf[a % 2, c, pl.ds(64 * gi, n), :] for c in range(2)]
            if n < 64:
                parts.append(jnp.zeros((128 - 2 * n, 128), F32))
            o = _dot(table(_OFF_LI, gi), jnp.concatenate(parts, axis=0))
            if gi < 4:
                t_buf[a, 0, pl.ds(64 * gi, 64), :] = o[:64]
                t_buf[a, 1, pl.ds(64 * gi, 64), :] = o[64:]
            else:
                t_buf[a, 0, pl.ds(256, 32), :] = o[:32]
                t_buf[a, 1, pl.ds(256, 32), :] = o[32:]

    def proj(part, p, gam, qs=(0, 1, 2), chunks=4):
        a = 4 * gam + p
        m = 288 // chunks
        kts = [kt for q in qs for kt in (2 * q, 2 * q + 1) if kt < 5]
        for ch in range(chunks):
            side.run(len(kts) * m)
            w = jnp.concatenate(
                [_bf(wt[part][kt, pl.ds(m * ch, m), :]) for kt in kts], axis=1)
            x = jnp.concatenate(
                [jnp.concatenate([_bf(x_perm[q][a + 2 * e]) for e in range(2)], axis=1)
                 for q in qs], axis=0)
            r = _dot(w, x)
            for e in range(2):
                c = 2 * gam + e
                buf, slot = (q_buf[4 * p + gam], e) if part == 0 else (
                    (k_buf, v_buf)[part - 1][p], 8 + c)
                rows = []
                for i in range(m // 4):
                    d, hg = divmod(m // 4 * ch + i, 4)
                    rows.append(pl.ds(144 * hg + 8 * d, 8))
                tile = r[:, 128 * e:128 * e + 128]
                if qs[0]:
                    tile = tile + jnp.concatenate([buf[slot, r_, :] for r_ in rows], axis=0)
                shifted = part and c and qs[-1] == 2
                rolled = pltpu.roll(tile, 1, 1) if shifted else None
                for i, r_ in enumerate(rows):
                    buf[slot, r_, :] = tile[8 * i:8 * i + 8]
                    if shifted:
                        buf[c, r_, :] = rolled[8 * i:8 * i + 8]
            fetch_next(r)

    def out_proj(p, row0, cw):
        side.run(10 * cw)
        lhs = jnp.concatenate([_bf(o_nat[p][kt, pl.ds(row0, cw), :]) for kt in range(5)], axis=1)
        r = _dot(lhs, jnp.concatenate([_bf(wo_perm[nt]) for nt in range(4)], axis=1))
        rows = pl.ds(2 * row0, 2 * cw)
        for ct in range(4):
            tile = r[:, 128 * ct:128 * ct + 128]
            if p == 0:
                out0[ct, rows, :] = tile
            else:
                stage[ct, rows, :] = _pack(out0[ct, rows, :], tile)
                cp_out(ct, 2 * row0, 2 * cw).start()

    def out_tail(p, gam):
        side.run(160)
        words = o_t[p][gam]
        o = jnp.concatenate([_unpack(words, e) for e in range(2)], axis=1)
        o = jnp.concatenate([o, jnp.zeros((64, 256), F32)], axis=0)
        r = _dot(jnp.concatenate([_bf(wo_tail[kt]) for kt in range(5)], axis=1), o)
        for e in range(2):
            a_tail[p, 2 * gam + e] = r[:, 128 * e:128 * e + 128]

    cp_wq(1, 0, 256).start()
    for t in range(8):
        cp_xa(t).start()
    wq_raw[pl.ds(D, 64), :] = jnp.zeros((64, 3 * D), BF16)
    cp_wq(1, 0, 256).wait()
    _drain(w_prep(1, range(2)))

    for t0, t1 in ((0, 6), (6, 11), (11, 14), (14, 16)):
        if t0 == 0:
            for t in range(8, 16):
                cp_xa(t).start()
        elif t0 == 6:
            cp_wq(1, 256, D - 256).start()
        elif t0 == 11:
            cp_xa_rest().start()
        for t in range(t0, t1):
            cp_xa(t).wait()
        for t in range(t0, t1):
            x_to_token_major(t, (0,))

    _drain(x_tile(0, (0,)))
    _drain(x_tile(2, (0,)))

    side.start(xa_raw[0, pl.ds(0, 8), :], x1_buf.at[2, 0])
    pairs = [(p, gam) for p in range(2) for gam in range(4)]

    def barrier():
        side.close()
        _barrier(sem_bar)

    def pair_tiles(name, n, qs, load, first=False):
        p, gam = pairs[n]
        for e in (1, 0) if first else (0, 1):
            side.add(name, x_tile(4 * gam + p + 2 * e, qs), load, first=first)

    side.open(0.0)
    fetches += [[]] * 3
    fetches += [[partial(fetch_wq, 0, i)] for i in range(4)]
    fetches += [[partial(fetch_xb, t)] for t in range(16)]
    fetches += [[partial(fetch_wq, 2, i) for i in range(4)]]
    fetches += [[partial(fetch_tab, r, min(304, n_tab - r)) for r in range(0, n_tab, 304)]]
    fetches += [[partial(fetch_f, t) for t in range(4)]]
    n_a = 5
    for n in range(n_a):
        pair_tiles("next", n + 1, (0,), 0.5, first=True)
        if n + n_a + 1 < 8:
            pair_tiles("later", n + n_a + 1, (0,), 0.5)
        proj(1, *pairs[n], qs=(0,), chunks=2)
        side.finish("next")
    side.close()

    cp_xa_rest().wait()
    cp_wq(1, 256, D - 256).wait()
    side.open(0.0)
    for n in range(5, 8):
        proj(1, *pairs[n], qs=(0,), chunks=2)
    for t in range(16):
        x_to_token_major(t, (1, 2))
    pair_tiles("next", 0, (1, 2), 0.6)
    side.add("next", w_prep(1, range(2, 5)), 0.6)
    side.finish("next")
    for n in range(5):
        pair_tiles("next", n + 1, (1, 2), 0.6)
        proj(1, *pairs[n], qs=(1, 2), chunks=3)
        side.finish("next")
    side.close()

    assert not fetches
    pltpu.make_async_copy(xb_raw, xb_raw, sem_in.at[SEM_XB]).wait()
    cp_wq(0).wait()
    side.open()
    n_b = 5
    load = (8 * 264 + (7 - n_b) * 172 + 730) / (864 * (8 - n_b) + 1440)
    side.add("w", w_prep(0), load)
    for tau in range(8):
        side.add("r9", radix9(tau), load)
    for n in range(n_b, 8):
        if n < 7:
            pair_tiles("next", n + 1, (1, 2), load, first=True)
        proj(1, *pairs[n], qs=(1, 2), chunks=3)
        side.finish("next")
    side.finish("w")
    proj(0, 0, 0)
    side.finish("r9")
    for tau in range(0):
        _drain(u_to_token_major(tau, 0))
    side.close()

    cp_tab(0, n_tab).wait()
    cp_wq(2).wait()
    side.open(0.75)
    side.add("t", dft_matrix(0), 1.0)
    for tau in range(0, 8):
        side.add("t", u_to_token_major(tau, 43), 1.0)
    side.add("w", w_prep(2), 1.0)
    fetches += [[partial(fetch_f, t)] for t in range(4, 16)]
    fetches += [[partial(fetch_wo, i)] for i in range(4)]
    fetches.append([wo_settle])
    proj(0, 0, 1, chunks=6)
    side.finish("t")
    dft64(0)
    for a in range(16):
        if a < 15:
            side.add("g", dft_matrix(a + 1), 1.0, first=True)
            dft64(a + 1)
        dft128(a)
        side.finish("g")
    side.close()

    n6, n8 = 8, 4
    cuts = '56789'

    def cut(i):
        if str(i) in cuts or -1 == i:
            barrier()
            side.open()

    pltpu.make_async_copy(wr_raw, wr_raw, sem_in.at[SEM_WR]).wait()
    pltpu.make_async_copy(wi_raw, wi_raw, sem_in.at[SEM_WI]).wait()
    cp_flast(0).wait()
    cp_flast(1).wait()
    cp_wo().wait()
    assert not fetches
    side.open(0.95, 400.0)
    load = (37 * 120 + 280) / (8640 if '5' in cuts else 8400)
    side.add("f", filter_all(), load)
    side.add("wo", wo_prep(), load)
    for gam in range(4):
        proj(2, 0, gam, chunks=1)
    proj(0, 0, 2, chunks=1)
    proj(0, 0, 3, chunks=1)
    side.finish("f")
    cut(5)

    if -1 >= 0:
        side.open()

    side.add("att", attend(0, range(n6)), n6 * 319 / 5856)
    idft128(0)
    for a in range(16):
        if a < 15:
            idft128(a + 1)
        idft64(a)
    cut(6)

    load = ((16 - n6) * 319 + 8 * 232) / 7200
    side.add("att", attend(0, range(n6, 16)), load)
    for c in range(8):
        side.add("r9", radix9_inv(c), load)
    for gam in range(4):
        proj(2, 1, gam, chunks=2)
    proj(0, 1, 0, chunks=2)
    side.finish("att")
    side.finish("r9")
    cut(7)

    tc = 34.0
    side.add("att", attend(1, range(n8)), n8 * 319 / (4320 - 52 * tc))
    side.add("o", o_to_token_major(0, tc, range(4)), 1.0)
    for c in range(8):
        side.add("y", y_to_token_major(c, tc), 1.0)
    side.add("y", wo_tail_prep(), 1.0)
    for gam in range(1, 4):
        proj(0, 1, gam, chunks=1)
    side.finish("y")
    for ct in range(5, 9):
        cp_out(ct, 0, S // 2).start()
    cut(8)

    side.add("att", attend(1, range(n8, 16)), (16 - n8) * 319 / 5120)
    for row0 in range(0, 512, 64):
        out_proj(0, row0, 64)
    side.finish("att")
    cut(9)

    side.close()
    side.open(0.0)
    for p, gam in pairs:
        out_tail(p, gam)
    _drain(o_to_token_major(1, 0, range(4)))
    for c in range(8):
        seam_to_token_major(c)
    cp_out(4, 0, S // 2).start()
    row0 = 0
    for cw in (16, 32, 64, 128, 128, 64, 32, 32, 16):
        out_proj(1, row0, cw)
        row0 += cw
    pltpu.make_async_copy(out_hbm, out_hbm, sem_out).wait()


def _barrier(sem):
    pl.semaphore_signal(sem)
    pl.semaphore_wait(sem)


@jax.jit
def pallas_concat_heads__sliding_local_dilated__spectral_gfnet__prompt_kernel(
    A_x: jax.Array,
    A_wqkv: jax.Array,
    A_wo: jax.Array,
    B_x: jax.Array,
    B_w_r: jax.Array,
    B_w_i: jax.Array,
):
    assert A_x.shape == (1, S, D) and B_x.shape == (1, S, D)
    any_spec = pl.BlockSpec(memory_space=pl.ANY)
    scratch = [
        pltpu.VMEM((1,) + _TABLE.shape, U32),
        pltpu.VMEM((16, 288, 128), U32),
        pltpu.VMEM((16, 128, 128), U32),
        pltpu.VMEM((D - 256, S), BF16),
        pltpu.VMEM((D + 64, 3 * D), BF16),
        pltpu.VMEM((D + 64, D), BF16),
        pltpu.VMEM((1, 16, 144, 128), U32),
        pltpu.VMEM((1, 16, 144, 128), U32),
        pltpu.VMEM((2, 1, S), BF16),
        pltpu.VMEM((1, 16, 3, 128, 128), F32),
        pltpu.VMEM((1, 8, D, 128), U32),
        pltpu.VMEM((1, 8, D, 128), U32),
        pltpu.VMEM((5, 8 * 136, 128), U32),
        pltpu.VMEM((1, 4, 2, NR, 128), F32),
        pltpu.VMEM((1, 16, 2, NR, 128), F32),
        pltpu.VMEM((1, 2, 2, NR, 128), F32),
        pltpu.VMEM((3, 16 * 136, 128), U32),
        [pltpu.VMEM((1, 16, n, 128), U32) for n in (128, 128, 64)],
        pltpu.VMEM((1, 5, 320, 128), U32),
        pltpu.VMEM((1, 5, 288, 128), U32),
        pltpu.VMEM((1, 5, 288, 128), U32),
        pltpu.VMEM((1, 5, 288, 128), U32),
        pltpu.VMEM((1, 5, 288, 128), U32),
        pltpu.VMEM((1, 5, 320, 128), U32),
        pltpu.VMEM((1, 5, 32, 128), U32),
        [pltpu.VMEM((1, 2, D + 16, 128), F32)] * 8,
        [pltpu.VMEM((1, 16, D + 8, 128), F32)] * 2,
        [pltpu.VMEM((1, 16, D + 8, 128), F32)] * 2,
        [pltpu.VMEM((1, 4, D, 128), U32)] * 2,
        [pltpu.VMEM((1, 5, 512, 128), U32)] * 2,
        pltpu.VMEM((1, 4, S // 2, 128), F32),
        pltpu.VMEM((1, 2, 8, 64, 128), F32),
        pltpu.VMEM((9, S // 2, 128), U32),
        pltpu.SemaphoreType.DMA((5,)),
        pltpu.SemaphoreType.DMA((9,)),
        pltpu.SemaphoreType.DMA(()),
        pltpu.SemaphoreType.REGULAR,
    ]
    out = pl.pallas_call(
        _kernel,
        out_shape=jax.ShapeDtypeStruct((S, 2 * D), BF16),
        in_specs=[any_spec] * 7 + [pl.BlockSpec(memory_space=pltpu.SMEM)],
        out_specs=any_spec,
        scratch_shapes=scratch,
        compiler_params=pltpu.CompilerParams(vmem_limit_bytes=120 * 1024 * 1024),
        name="attn_gfnet",
    )(A_x[0].T, A_wqkv, A_wo, B_x[0].T, B_w_r.T, B_w_i.T, _TABLE, np.zeros((2,), np.int32))
    return out[None]
```

```python
from functools import partial

import numpy as np

import jax
import jax.numpy as jnp
from jax import lax
import jax.experimental.pallas as pl
import jax.experimental.pallas.tpu as pltpu

S = 2048
D = 576
H = 32
DH = 18
W = 8
DF = D // 2 + 1
NR = 296

F32 = jnp.float32
BF16 = jnp.bfloat16
U32 = jnp.uint32

_C3 = float(np.sqrt(3.0) / 2)
_C1, _S1 = float(np.cos(2 * np.pi / 9)), float(np.sin(2 * np.pi / 9))
_C2, _S2 = float(np.cos(4 * np.pi / 9)), float(np.sin(4 * np.pi / 9))


def _bfly9_fwd(x):
    a0, ar, ai = [], [], []
    for j in range(3):
        t = x[j + 3] + x[j + 6]
        a0.append(x[j] + t)
        ar.append(x[j] - 0.5 * t)
        ai.append(x[j + 6] - x[j + 3])
    t = a0[1] + a0[2]
    u0 = a0[0] + t
    u3r = a0[0] - 0.5 * t
    u3i = a0[2] - a0[1]
    b1r = ar[1] * _C1 + ai[1] * (_C3 * _S1)
    b1i = ai[1] * (_C3 * _C1) - ar[1] * _S1
    b2r = ar[2] * _C2 + ai[2] * (_C3 * _S2)
    b2i = ai[2] * (_C3 * _C2) - ar[2] * _S2
    a_r, a_i = ar[0], ai[0] * _C3
    tr, ti = b1r + b2r, b1i + b2i
    dr, di = (b1r - b2r) * _C3, (b1i - b2i) * _C3
    u1r, u1i = a_r + tr, a_i + ti
    mr, mi = a_r - 0.5 * tr, a_i - 0.5 * ti
    return [u0, u1r, u1i, mr - di, mi + dr, u3r, u3i, mr + di, mi - dr]


def _bfly9_inv(v):
    u0, u1r, u1i, u7r, u7i, u3r, u3i, u4r, u4i = v
    mr, mi = u4r + u7r, u4i + u7i
    di, dr = (u4r - u7r) * _C3, (u7i - u4i) * _C3
    a_r, a_i = u1r + mr, u1i + mi
    tr, ti = u1r - 0.5 * mr, u1i - 0.5 * mi
    b1r, b2r, b1i, b2i = tr + dr, tr - dr, ti + di, ti - di
    ar = [a_r, b1r * _C1 - b1i * _S1, b2r * _C2 - b2i * _S2]
    ai = [a_i * _C3, b1r * (_C3 * _S1) + b1i * (_C3 * _C1),
          b2r * (_C3 * _S2) + b2i * (_C3 * _C2)]
    t = u0 - 0.5 * u3r
    a0 = [u0 + u3r, t - u3i, t + u3i]
    y = [None] * 9
    for j in range(3):
        t = a0[j] - 0.5 * ar[j]
        y[j] = a0[j] + ar[j]
        y[j + 3] = t - ai[j]
        y[j + 6] = t + ai[j]
    return y


def _bfly4(x, inverse):
    (ar, ai), (br, bi), (cr, ci), (dr, di) = x
    pr, pi, qr, qi = ar + cr, ai + ci, ar - cr, ai - ci
    sr, si, tr, ti = br + dr, bi + di, br - dr, bi - di
    y1, y3 = (qr + ti, qi - tr), (qr - ti, qi + tr)
    if inverse:
        y1, y3 = y3, y1
    return [(pr + sr, pi + si), y1, (pr - sr, pi - si), y3]


def _twiddle16(z, e, inverse):
    zr, zi = z
    e = (-e if inverse else e) % 16
    h = float(np.sqrt(0.5))
    if e == 0:
        return z
    if e == 4:
        return zi, -zr
    if e == 12:
        return -zi, zr
    if e == 2:
        return (zr + zi) * h, (zi - zr) * h
    if e == 14:
        return (zr - zi) * h, (zr + zi) * h
    if e == 6:
        return (zi - zr) * h, (zr + zi) * (-h)
    if e == 10:
        return (zr + zi) * (-h), (zr - zi) * h
    c, s = float(np.cos(2 * np.pi * e / 16)), float(np.sin(2 * np.pi * e / 16))
    return zr * c + zi * s, zi * c - zr * s


_GROUPS = (1, 2, 3, 4, 0)


def _group_classes(g):
    return sorted({g, g + 9, 9 - g, 18 - g}) if g else [0, 9]


_ROWGROUPS = [(k0, h) for g in _GROUPS for k0 in _group_classes(g) for h in range(2)]


def _to_words(m):
    u = np.ascontiguousarray(m, dtype=np.float32).view(np.uint32)
    u = (u + 0x7FFF + ((u >> 16) & 1)) >> 16
    return (u[0::2] | (u[1::2] << 16)).astype(np.uint32)


def _make_tables():
    basis = np.array(_bfly9_fwd(list(np.eye(9))))
    m_fwd = np.array([2 * (r % 32) + r // 32 for r in range(64)])
    lf, li = [], []
    for g in _GROUPS:
        rows = [k0 + 18 * i for k0 in _group_classes(g) for i in range(16)]
        if g == 0:
            rows += [DF - 1] + [-1] * 7
        cols = [2 * g - 1, 2 * g] if g else [0]
        a = basis[cols].T.astype(complex)
        n = len(rows)
        f = np.zeros((2 * n, 128))
        b = np.zeros((64 * len(cols), 128))
        for r, k in enumerate(rows):
            if k < 0:
                continue
            ck = np.exp(-2j * np.pi * ((np.arange(9) * k) % 9) / 9)
            lam = np.linalg.solve(a.conj().T @ a, a.conj().T @ ck)
            wk = (1.0 if k in (0, DF - 1) else 2.0) / (S * D)
            for c in range(len(cols)):
                e = lam[c] * np.exp(-2j * np.pi * ((m_fwd * k) % D) / D)
                f[r, 64 * c:64 * c + 64] = e.real
                f[n + r, 64 * c:64 * c + 64] = e.imag
                e = wk * lam[c] * np.exp(-2j * np.pi * ((np.arange(64) * k) % D) / D)
                b[64 * c:64 * c + 64, r] = e.real
                b[64 * c:64 * c + 64, n + r] = e.imag
        lf.append(_to_words(f))
        li.append(_to_words(b))
    n = np.arange(128)
    b_of_n = 16 * (n // 16) + 8 * (n % 2) + (n % 16) // 2
    f128 = np.exp(-2j * np.pi * (np.outer(b_of_n, n) % 128) / 128)
    tw = np.exp(-2j * np.pi * np.outer(np.arange(16), n) / S)
    f32w = lambda m: np.ascontiguousarray(m, dtype=np.float32).view(np.uint32)
    parts = [f32w(f128.real), f32w(f128.imag), f32w(tw.real), f32w(tw.imag)] + lf + li
    offs = np.cumsum([0] + [p.shape[0] for p in parts])
    parts.append(np.zeros((-offs[-1] % 32, 128), np.uint32))
    return np.concatenate(parts, axis=0), [int(o) for o in offs]


_TABLE, _OFF = _make_tables()
_OFF_FR, _OFF_FI, _OFF_TR, _OFF_TI = _OFF[0:4]
_OFF_LF = _OFF[4:10]
_OFF_LI = _OFF[9:15]


def _pack(lo, hi):
    return pltpu.pack_elementwise([lo, hi], packed_dtype=BF16)


def _unpack(w, index):
    return pltpu.unpack_elementwise(w, index=index, packed_dtype=BF16, unpacked_dtype=F32)


def _bf(words):
    return pltpu.bitcast(words, BF16)


def _dot(a, b):
    return lax.dot_general(a, b, (((1,), (0,)), ((), ())), preferred_element_type=F32)


def _dot_nt(a, b):
    return lax.dot_general(a, b, (((1,), (1,)), ((), ())), preferred_element_type=F32)


def _zeros_w(rows):
    return jnp.zeros((rows, 128), U32)


class _SideWork:
    LINK = 7.0

    def __init__(self, zero_ref):
        self.zero_ref = zero_ref
        self.zero = zero_ref[0]
        self.lead = 0.0

    def start(self, seed, sink):
        self.chain = pltpu.bitcast(seed, F32)
        self.sink = sink
        self.jobs = []
        self.credit = 0.0
        self.delay = 0.0
        self.blocks = 0
        self.now = 0.0
        self.pending = []

    def open(self, stretch=1.0, slack=100.0, links=4):
        self.min_links = links
        self.zero = self.zero_ref[0]
        self.lead = -slack
        self.stretch = stretch

    def add(self, name, gen, load, first=False):
        self.jobs.insert(0 if first else len(self.jobs), (name, gen, load * 1.0))

    def _advance(self, cycles):
        self.lead += cycles
        while self.lead >= 6.0:
            self.zero = self.zero_ref[self.zero]
            self.lead -= 6.0

    def _tick(self, cycles):
        self.now += cycles
        self.delay += cycles
        while self.pending and self.pending[0][0] <= self.now:
            self.chain = self.pending.pop(0)[1] + self.chain
            self.delay -= 2.0
        n = int(self.delay / self.LINK)
        if n >= self.min_links:
            for _ in range(n):
                self.chain = pl.reciprocal(self.chain, approx=True)
            self.delay -= n * self.LINK

    def _step(self):
        item = next(self.jobs[0][1], None)
        if item is None:
            self.jobs.pop(0)
            return
        values, cycles, latency = (item + (0.0,))[:3]
        values = values if isinstance(values, list) else [values]
        values = [pltpu.bitcast(v, F32) for v in values]
        while len(values) > 1:
            values = [values[i] + values[i + 1] if i + 1 < len(values) else values[i]
                      for i in range(0, len(values), 2)]
        self.pending.append((self.now + latency, values[0]))
        self.pending.sort(key=lambda x: x[0])
        cycles = cycles / self.jobs[0][2]
        self.credit -= cycles
        self._advance(cycles)
        self._tick(self.stretch * cycles)

    def run(self, cycles):
        self.credit += cycles
        while self.jobs and self.credit > 0:
            self._step()
        if not self.jobs and self.credit > 0:
            self._tick(self.stretch * self.credit)
            self.credit = 0.0

    def finish(self, name):
        while any(job[0] == name for job in self.jobs):
            self._step()

    def close(self):
        while self.jobs:
            self._step()
        while self.pending:
            self.chain = self.pending.pop(0)[1] + self.chain
        self.sink[pl.ds(8 * self.blocks, 8), :] = self.chain
        self.blocks += 1
        self.credit = self.delay = 0.0


def _drain(gen):
    for _ in gen:
        pass


_W_COLS = ((0, 512), (512, 640), (1152, 576))


def _kernel(xa_hbm, wqkv_hbm, wo_hbm, xb_hbm, wr_hbm, wi_hbm, tab_hbm, zero_ref, out_hbm,
            tab, xb_raw, xa_raw, xa_rest, wq_raw, wo_raw, wr_raw, wi_raw, wlast,
            gmat, u_t, y_t, u_nat, x1_buf, t_buf, z_buf, x_nat, x_perm, wt_nat, wt_q, wt_k, wt_v,
            wo_nat, wo_perm, wo_tail, q_buf, k_buf, v_buf, o_t, o_nat, out0, a_tail, stage,
            sem_xa, sem_in, sem_out, sem_bar):
    side = _SideWork(zero_ref)
    zero = side.zero

    def now(ref):
        return ref.at[side.zero]

    tab_r, wr_r, wi_r = tab, wr_raw, wi_raw
    tab, wr_raw, wi_raw = tab.at[0], wr_raw.at[0], wi_raw.at[0]
    (u_r, y_r, t_r, wn_r, won_r, q_r, k_r, v_r, o_r) = (
        u_t, y_t, t_buf, wt_nat, wo_nat, q_buf, k_buf, v_buf, o_t)
    (gmat, u_t, y_t, x1_buf, t_buf, z_buf, x_perm, wt_nat, wt_q, wt_k, wt_v, wo_nat, wo_perm,
     wo_tail, q_buf, k_buf, v_buf, o_t, o_nat, out0, a_tail) = jax.tree.map(
        lambda r: r.at[zero],
        (gmat, u_t, y_t, x1_buf, t_buf, z_buf, x_perm, wt_nat, wt_q, wt_k, wt_v, wo_nat, wo_perm,
         wo_tail, q_buf, k_buf, v_buf, o_t, o_nat, out0, a_tail))
    wt = (wt_q, wt_k, wt_v)

    SEM_XB, SEM_TAB, SEM_WQ, SEM_WK, SEM_WV, SEM_WO, SEM_WR, SEM_WI, SEM_LAST = range(9)

    def cp_tab(row0, rows, z=0):
        return pltpu.make_async_copy(
            tab_hbm.at[pl.ds(row0, rows)], tab.at[pl.ds(pl.multiple_of(z + row0, 8), rows)],
            sem_in.at[SEM_TAB])

    def cp_xb(t, z=0):
        return pltpu.make_async_copy(
            xb_hbm.at[:, pl.ds(t * 128, 128)], xb_raw.at[z + t].bitcast(BF16), sem_in.at[SEM_XB])

    def cp_xa(t):
        return pltpu.make_async_copy(
            xa_hbm.at[pl.ds(0, 256), pl.ds(t * 128, 128)], xa_raw.at[t].bitcast(BF16),
            sem_xa.at[sum(t >= s for s in (6, 11, 14))])

    def cp_xa_rest():
        return pltpu.make_async_copy(xa_hbm.at[pl.ds(256, D - 256)], xa_rest, sem_xa.at[4])

    def cp_wq(part, row0=0, rows=D, z=0):
        cols = pl.ds(*_W_COLS[part])
        return pltpu.make_async_copy(
            wqkv_hbm.at[pl.ds(row0, rows), cols],
            wq_raw.at[pl.ds(pl.multiple_of(z + row0, 16), rows), cols], sem_in.at[SEM_WQ + part])

    def cp_wo(row0=0, rows=D, z=0):
        return pltpu.make_async_copy(
            wo_hbm.at[pl.ds(row0, rows)], wo_raw.at[pl.ds(pl.multiple_of(z + row0, 16), rows)],
            sem_in.at[SEM_WO])

    def cp_f(i, t, z=0):
        src, dst = ((wr_hbm, wr_raw), (wi_hbm, wi_raw))[i]
        return pltpu.make_async_copy(
            src.at[pl.ds(0, DF - 1), pl.ds(t * 128, 128)], dst.at[z + t].bitcast(BF16),
            sem_in.at[SEM_WR + i])

    def cp_flast(i):
        src = (wr_hbm, wi_hbm)[i]
        return pltpu.make_async_copy(src.at[pl.ds(DF - 1, 1), :], wlast.at[i], sem_in.at[SEM_LAST])

    def cp_out(ct, row0, rows):
        return pltpu.make_async_copy(
            stage.at[ct, pl.ds(row0, rows), :].bitcast(BF16),
            out_hbm.at[pl.ds(2 * row0, 2 * rows), pl.ds(ct * 128, 128)], sem_out)

    def fetch_xb(t, v):
        xb_raw[t, pl.ds(0, 8), :] = v
        cp_xb(t).start()

    def fetch_wq(part, piece, v):
        wq_raw[pl.ds(144 * piece, 16), pl.ds(_W_COLS[part][0], 128)] = _bf(v)
        cp_wq(part, 144 * piece, 144).start()

    def fetch_wo(piece, v):
        wo_raw[pl.ds(144 * piece, 16), pl.ds(0, 128)] = _bf(v)
        cp_wo(144 * piece, 144).start()

    def wo_settle(v):
        wo_raw[pl.ds(D, 16), pl.ds(0, 128)] = _bf(v)

    def fetch_tab(row0, rows, v):
        tab[pl.ds(row0, 8), :] = v
        cp_tab(row0, rows).start()

    def fetch_f(t, v):
        wr_raw[t, pl.ds(0, 8), :] = v
        cp_f(0, t).start()
        wi_raw[t, pl.ds(0, 8), :] = v
        cp_f(1, t).start()
        if t == 0:
            cp_flast(0).start()
            cp_flast(1).start()

    n_tab = _TABLE.shape[0]
    fetches = []

    def fetch_next(value):
        if fetches:
            for fetch in fetches.pop(0):
                fetch(pltpu.bitcast(value[:8, :128], U32))

    def store_pitched(dst, row0, vt):
        for r in range(16):
            dst[pl.ds(row0 + 17 * (r // 2) + 8 * (r % 2), 8), :] = vt[8 * r:8 * r + 8]

    def radix9(tau):
        for i in range(4):
            words = [[xb_raw[side.zero + 2 * tau + z, pl.ds(32 * j + 8 * i, 8), :] for j in range(9)]
                     for z in range(2)]
            for e in range(2):
                u = []
                for z in range(2):
                    u.append(_bfly9_fwd([_unpack(w, e) for w in words[z]]))
                    yield u[z][8], 14
                out = [_pack(u[0][o], u[1][o]) for o in range(9)]
                for o in range(9):
                    u_t[tau, pl.ds(64 * o + 32 * e + 8 * i, 8), :] = out[o]
                yield out, 5

    def u_to_token_major(gi, cost):
        g = _GROUPS[gi]
        for tau in range(8):
            if g:
                v = u_t[tau, pl.ds(64 * (2 * g - 1), 128), :]
            else:
                v = jnp.concatenate([u_t[tau, pl.ds(0, 64), :], _zeros_w(64)], axis=0)
            vt = v.T
            store_pitched(u_nat.at[gi], 136 * tau, vt)
            yield vt[120:], cost, 240

    def dft_matrix(a):
        twr = jnp.broadcast_to(pltpu.bitcast(tab[pl.ds(_OFF_TR + a, 1), :], F32), (8, 128))
        twi = jnp.broadcast_to(pltpu.bitcast(tab[pl.ds(_OFF_TI + a, 1), :], F32), (8, 128))
        for i in range(16):
            fr = pltpu.bitcast(now(tab_r)[pl.ds(_OFF_FR + 8 * i, 8), :], F32)
            fi = pltpu.bitcast(now(tab_r)[pl.ds(_OFF_FI + 8 * i, 8), :], F32)
            gr, gi = fr * twr - fi * twi, fr * twi + fi * twr
            gmat[a, 0, pl.ds(8 * i, 8), :] = gr
            out = [gr + gi, gi - gr]
            gmat[a, 1, pl.ds(8 * i, 8), :] = out[0]
            gmat[a, 2, pl.ds(8 * i, 8), :] = out[1]
            yield out, 3

    def filter_rows(row0, load_w):
        rows = pl.ds(row0, 8)
        y = [[None] * 4 for _ in range(4)]
        for a0 in range(4):
            src = now(t_r)
            z = _bfly4([(src[4 * a1 + a0, 0, rows, :], src[4 * a1 + a0, 1, rows, :])
                        for a1 in range(4)], False)
            for g0 in range(4):
                y[g0][a0] = _twiddle16(z[g0], a0 * g0, False)
            yield y[3][a0][0], 7
        for g0 in range(4):
            z = _bfly4(y[g0], False)
            yield z[3][1], 4
            for g1 in range(4):
                wr, wi = load_w(g0 + 4 * g1)
                zr, zi = z[g1]
                z[g1] = (zr * wr - zi * wi, zr * wi + zi * wr)
                if g1 % 2:
                    yield z[g1][1], 4
            z = _bfly4(z, True)
            for a0 in range(4):
                y[g0][a0] = _twiddle16(z[a0], a0 * g0, True)
            yield y[g0][3][0], 6
        for a0 in range(4):
            z = _bfly4([y[g0][a0] for g0 in range(4)], True)
            for a1 in range(4):
                t_buf[4 * a1 + a0, 0, rows, :] = z[a1][0]
                t_buf[4 * a1 + a0, 1, rows, :] = z[a1][1]
            yield [v for pair in z for v in pair], 6

    def filter_all():
        for n, (k0, h) in enumerate(_ROWGROUPS):
            rows = pl.ds(k0 // 2 + 72 * h, 8, stride=9)
            yield from filter_rows(8 * n, lambda f1: (
                _unpack(now(wr_r)[f1, rows, :], k0 % 2),
                _unpack(now(wi_r)[f1, rows, :], k0 % 2)))
        yield from filter_rows(NR - 8, lambda f1: tuple(
            jnp.broadcast_to(wlast[i, :, pl.ds(128 * f1, 128)].astype(F32), (8, 128))
            for i in range(2)))

    def radix9_inv(c):
        for i in range(8):
            y = []
            for e in range(2):
                y.append(_bfly9_inv(
                    [now(t_r)[2 * c + e, i // 4, pl.ds(256 + 8 * (i % 4), 8), :]]
                    + [now(t_r)[2 * c + e, o % 2, pl.ds(64 * (o // 2) + 8 * i, 8), :]
                       for o in range(8)]))
                yield (y[e] if 0 else y[e][8]), 12
            out = [_pack(y[0][j], y[1][j]) for j in range(9)]
            for j in range(9):
                y_t[c, pl.ds(64 * j + 8 * i, 8), :] = out[j]
            yield out, 5

    def y_to_token_major(c, cost):
        for q in range(4):
            vt = y_t[c, pl.ds(64 + 128 * q, 128), :].T
            stage[5 + q, pl.ds(c, 128, stride=8), :] = vt
            yield vt[120:], cost, 240

    def seam_to_token_major(c):
        top = _pack(a_tail[0, c], a_tail[1, c])
        stage[4, pl.ds(c, 128, stride=8), :] = jnp.concatenate(
            [top, y_t[c, pl.ds(0, 64), :]], axis=0).T

    def wo_tail_prep():
        for kt in range(5):
            vt = pltpu.bitcast(_bf(wo_perm[4, pl.ds(64 * kt, 64), :]).T, U32)
            wo_tail[kt] = vt[:32]
            yield vt[24:32], 22, 180

    def x_to_token_major(t, qs):
        lanes = pl.ds(128 * t, 128)
        for q in qs:
            if q == 0:
                v = xa_raw[t]
            elif q == 1:
                v = pltpu.bitcast(xa_rest[pl.ds(0, 256), lanes], U32)
            else:
                v = pltpu.bitcast(xa_rest[pl.ds(256, 64), lanes], U32)
                v = jnp.concatenate([v, _zeros_w(96)], axis=0)
            store_pitched(x_nat.at[q], 136 * t, v.T)

    def x_tile(a, qs):
        for q in qs:
            vt = x_nat[q, pl.ds(a, 128, stride=17), :].T
            n = 128 if q < 2 else 64
            x_perm[q][a] = vt[:n]
            yield vt[n - 8:n], 43, 240

    def w_prep(part, kts=range(5)):
        col0, _ = _W_COLS[part]
        first = 288 * part - col0 // 2
        for kt in kts:
            for nt in range(5):
                nn = min(128, 3 * D - col0 - 128 * nt)
                vt = wq_raw[pl.ds(128 * kt, 128), pl.ds(col0 + 128 * nt, nn)].T
                vt = pltpu.bitcast(vt, U32)
                wt_nat[kt, pl.ds(64 * nt, nn // 2), :] = vt
                yield vt[-8:], 22, 180
        for kt in kts:
            for i in range(2):
                for dl in range(9):
                    base = first + 144 * i + dl
                    wa = now(wn_r)[kt, pl.ds(base, 8, stride=18), :]
                    wb = now(wn_r)[kt, pl.ds(base + 9, 8, stride=18), :]
                    out = [_pack(_unpack(wa, e), _unpack(wb, e)) for e in range(2)]
                    for e in range(2):
                        wt[part][kt, pl.ds(16 * (2 * dl + e) + 8 * i, 8), :] = out[e]
                    yield out, 2

    def wo_prep():
        for nt in range(5):
            nn = min(128, D - 128 * nt)
            blk = wo_raw[pl.ds(0, D), pl.ds(128 * nt, nn)]
            if nn < 128:
                blk = jnp.concatenate([blk, jnp.zeros((D, 128 - nn), BF16)], axis=1)
            blk = pltpu.bitcast(blk, U32)
            wo_nat[nt] = blk
            wo_perm[nt, pl.ds(288, 32), :] = _zeros_w(32)
            yield blk[-8:], 20
            for i in range(2):
                for dl in range(9):
                    wa = now(won_r)[nt, pl.ds(144 * i + dl, 8, stride=18), :]
                    wb = now(won_r)[nt, pl.ds(144 * i + dl + 9, 8, stride=18), :]
                    out = [_pack(_unpack(wa, e), _unpack(wb, e)) for e in range(2)]
                    for e in range(2):
                        wo_perm[nt, pl.ds(16 * (2 * dl + e) + 8 * i, 8), :] = out[e]
                    yield out, 2

    scale = float(DH) ** -0.5
    QB = 6

    def attend(p, units):
        lane0 = lax.broadcasted_iota(jnp.int32, (8, 128), 1) == 0
        for unit in units:
            gam, hg = divmod(unit, 4)
            base = 2 * gam + 1
            acc = [[None] * W for _ in range(2)]
            for d0 in range(0, DH, QB):
                rows = [pl.ds(144 * hg + 8 * d, 8) for d in range(d0, d0 + QB)]
                q = [[now(q_r[4 * p + gam])[e, r, :] for r in rows] for e in range(2)]
                for l in range(9):
                    for n, r in enumerate(rows):
                        k = now(k_r[p])[base + l, r, :]
                        for e in range(2):
                            w = 7 + e - l
                            if 0 <= w < W:
                                t = q[e][n] * k
                                acc[e][w] = t if acc[e][w] is None else acc[e][w] + t
                    done = [acc[e][7 + e - l] for e in range(2) if 0 <= 7 + e - l < W]
                    yield done, QB / 2 * len(done)
            prob = []
            for e in range(2):
                lg = [jnp.where(lane0, -1e9 / scale, acc[e][w]) if 2 * gam + e < w else acc[e][w]
                      for w in range(W)]
                m = lg[0]
                for w in range(1, W):
                    m = jnp.maximum(m, lg[w])
                ex = [jnp.exp2((l_ - m) * (scale * float(np.log2(np.e)))) for l_ in lg]
                tot = ex[0]
                for w in range(1, W):
                    tot = tot + ex[w]
                inv = 1.0 / tot
                prob.append([x_ * inv for x_ in ex])
                yield prob[e][W - 1], 13, 30
            for d in range(DH):
                rows = pl.ds(32 * d + 8 * hg, 8)
                vv = [now(v_r[p])[base + l, pl.ds(144 * hg + 8 * d, 8), :] for l in range(9)]
                o = []
                for e in range(2):
                    t = prob[e][0] * vv[7 + e]
                    for w in range(1, W):
                        t = t + prob[e][w] * vv[7 + e - w]
                    o.append(t)
                word = _pack(o[0], o[1])
                o_t[p][gam, rows, :] = word
                yield word, 8

    def o_to_token_major(p, cost, gams):
        for gam in gams:
            for kt in range(5):
                if kt < 4:
                    v = (o_t[p] if 1 else now(o_r[p]))[gam, pl.ds(128 * kt, 128), :]
                else:
                    v = jnp.concatenate([(o_t[p] if 1 else now(o_r[p]))[gam, pl.ds(512, 64), :], _zeros_w(64)], axis=0)
                vt = v.T
                o_nat[p][kt, pl.ds(gam, 128, stride=4), :] = vt
                yield vt[120:], cost, 240

    def table(off, i):
        return _bf(tab[pl.ds(off[i], off[i + 1] - off[i]), :])

    def dft64(a, gi):
        x1 = _dot_nt(table(_OFF_LF, gi), _bf(u_nat[gi, pl.ds(a, 64, stride=17), :]))
        n = x1.shape[0] // 2
        side.run(n / 2)
        x1_buf[a, 0, pl.ds(64 * gi, n), :] = x1[:n]
        x1_buf[a, 1, pl.ds(64 * gi, n), :] = x1[n:]
        if a % 4 == 3:
            fetch_next(x1)

    def dft128(a):
        side.run(222)
        xr, xi = x1_buf[a, 0], x1_buf[a, 1]
        k1 = _dot(xr + xi, gmat[a, 0])
        t_buf[a, 0] = k1 - _dot(xi, gmat[a, 1])
        t_buf[a, 1] = k1 + _dot(xr, gmat[a, 2])

    def idft128(a):
        side.run(222)
        g = [jnp.concatenate([gmat[a, c, pl.ds(16 * tau + e, 8, stride=2), :]
                              for tau in range(8) for e in range(2)], axis=0) for c in range(3)]
        tr, ti = t_buf[a, 0], t_buf[a, 1]
        k1 = _dot_nt(tr + ti, g[0])
        z_buf[a % 2, 0] = k1 + _dot_nt(ti, g[2])
        z_buf[a % 2, 1] = k1 - _dot_nt(tr, g[1])

    def idft64(a):
        side.run(144)
        for gi in range(5):
            n = 64 if gi < 4 else NR - 256
            parts = [z_buf[a % 2, c, pl.ds(64 * gi, n), :] for c in range(2)]
            if n < 64:
                parts.append(jnp.zeros((128 - 2 * n, 128), F32))
            o = _dot(table(_OFF_LI, gi), jnp.concatenate(parts, axis=0))
            if gi < 4:
                t_buf[a, 0, pl.ds(64 * gi, 64), :] = o[:64]
                t_buf[a, 1, pl.ds(64 * gi, 64), :] = o[64:]
            else:
                t_buf[a, 0, pl.ds(256, 32), :] = o[:32]
                t_buf[a, 1, pl.ds(256, 32), :] = o[32:]

    def proj(part, p, gam, qs=(0, 1, 2), chunks=4, only=None):
        a = 4 * gam + p
        m = 288 // chunks
        kts = [kt for q in qs for kt in (2 * q, 2 * q + 1) if kt < 5]
        for ch in only or range(chunks):
            side.run(len(kts) * m)
            w = jnp.concatenate(
                [_bf(wt[part][kt, pl.ds(m * ch, m), :]) for kt in kts], axis=1)
            x = jnp.concatenate(
                [jnp.concatenate([_bf(x_perm[q][a + 2 * e]) for e in range(2)], axis=1)
                 for q in qs], axis=0)
            r = _dot(w, x)
            for e in range(2):
                c = 2 * gam + e
                buf, slot = (q_buf[4 * p + gam], e) if part == 0 else (
                    (k_buf, v_buf)[part - 1][p], 8 + c)
                rows = []
                for i in range(m // 4):
                    d, hg = divmod(m // 4 * ch + i, 4)
                    rows.append(pl.ds(144 * hg + 8 * d, 8))
                tile = r[:, 128 * e:128 * e + 128]
                if qs[0]:
                    tile = tile + jnp.concatenate([buf[slot, r_, :] for r_ in rows], axis=0)
                shifted = part and c and qs[-1] == 2
                rolled = pltpu.roll(tile, 1, 1) if shifted else None
                for i, r_ in enumerate(rows):
                    buf[slot, r_, :] = tile[8 * i:8 * i + 8]
                    if shifted:
                        buf[c, r_, :] = rolled[8 * i:8 * i + 8]
            fetch_next(r)

    def out_proj(p, row0, cw):
        side.run(10 * cw)
        lhs = jnp.concatenate([_bf(o_nat[p][kt, pl.ds(row0, cw), :]) for kt in range(5)], axis=1)
        r = _dot(lhs, jnp.concatenate([_bf(wo_perm[nt]) for nt in range(4)], axis=1))
        rows = pl.ds(2 * row0, 2 * cw)
        for ct in range(4):
            tile = r[:, 128 * ct:128 * ct + 128]
            if p == 0:
                out0[ct, rows, :] = tile
            else:
                stage[ct, rows, :] = _pack(out0[ct, rows, :], tile)
                cp_out(ct, 2 * row0, 2 * cw).start()

    def out_tail(p, gam):
        side.run(160)
        words = o_t[p][gam]
        o = jnp.concatenate([_unpack(words, e) for e in range(2)], axis=1)
        o = jnp.concatenate([o, jnp.zeros((64, 256), F32)], axis=0)
        r = _dot(jnp.concatenate([_bf(wo_tail[kt]) for kt in range(5)], axis=1), o)
        for e in range(2):
            a_tail[p, 2 * gam + e] = r[:, 128 * e:128 * e + 128]

    cp_wq(1, 0, 256).start()
    for t in range(8):
        cp_xa(t).start()
    wq_raw[pl.ds(D, 64), :] = jnp.zeros((64, 3 * D), BF16)
    cp_wq(1, 0, 256).wait()
    _drain(w_prep(1, range(2)))

    for t0, t1 in ((0, 6), (6, 11), (11, 14), (14, 16)):
        if t0 == 0:
            for t in range(8, 16):
                cp_xa(t).start()
        elif t0 == 6:
            cp_wq(1, 256, D - 256).start()
        elif t0 == 11:
            cp_xa_rest().start()
        for t in range(t0, t1):
            cp_xa(t).wait()
        for t in range(t0, t1):
            x_to_token_major(t, (0,))

    _drain(x_tile(0, (0,)))
    _drain(x_tile(2, (0,)))

    side.start(xa_raw[0, pl.ds(0, 8), :], x1_buf.at[16, 0])
    pairs = [(p, gam) for p in range(2) for gam in range(4)]

    def barrier():
        side.close()
        _barrier(sem_bar)

    def pair_tiles(name, n, qs, load, first=False):
        p, gam = pairs[n]
        for e in (1, 0) if first else (0, 1):
            side.add(name, x_tile(4 * gam + p + 2 * e, qs), load, first=first)

    side.open(0.0)
    fetches += [[]] * 3
    fetches += [[partial(fetch_wq, 0, i)] for i in range(4)]
    fetches += [[partial(fetch_xb, t)] for t in range(16)]
    fetches += [[partial(fetch_wq, 2, i) for i in range(4)]]
    fetches += [[partial(fetch_tab, r, min(304, n_tab - r)) for r in range(0, n_tab, 304)]]
    fetches += [[partial(fetch_f, t) for t in range(4)]]
    n_a = 5
    for n in range(n_a):
        pair_tiles("next", n + 1, (0,), 0.5, first=True)
        if n + n_a + 1 < 8:
            pair_tiles("later", n + n_a + 1, (0,), 0.5)
        proj(1, *pairs[n], qs=(0,), chunks=2)
        side.finish("next")
    side.close()

    cp_xa_rest().wait()
    cp_wq(1, 256, D - 256).wait()
    side.open(0.0)
    for n in range(5, 8):
        proj(1, *pairs[n], qs=(0,), chunks=2)
    for q in (1, 2):
        for t in range(16):
            x_to_token_major(t, (q,))
        for n in range(2):
            pair_tiles("next", n, (q,), 0.6)
        side.add("next", w_prep(1, (2, 3) if q == 1 else (4,)), 0.6)
        if q == 2:
            pair_tiles("next", 2, (1, 2), 0.6)
        side.finish("next")
        for n in range(2):
            proj(1, *pairs[n], qs=(q,), chunks=2)
    for n in range(2, 5):
        pair_tiles("next", n + 1, (1, 2), 0.6)
        proj(1, *pairs[n], qs=(1, 2), chunks=3)
        side.finish("next")
    side.close()

    assert not fetches
    pltpu.make_async_copy(xb_raw, xb_raw, sem_in.at[SEM_XB]).wait()
    cp_wq(0).wait()
    side.open(0.9, 300.0)
    load = (8 * 264 + 2 * 172 + 730) / 4752
    side.add("w", w_prep(0), load)
    for tau in range(8):
        side.add("r9", radix9(tau), load)
    for n in range(5, 8):
        if n < 7:
            pair_tiles("next", n + 1, (1, 2), load, first=True)
        proj(1, *pairs[n], qs=(1, 2), chunks=3)
        side.finish("next")
    side.finish("w")
    proj(0, 0, 0)
    proj(0, 0, 1, chunks=4, only=(0, 1))
    side.close()

    cp_tab(0, n_tab).wait()
    cp_wq(2).wait()
    side.open(0.75)
    fetches += [[partial(fetch_f, t)] for t in range(4, 16)]
    fetches += [[partial(fetch_wo, i)] for i in range(4)]
    fetches.append([wo_settle])
    side.add("t", u_to_token_major(0, 43), 1.0)
    for a in range(16):
        side.add("g%d" % a, dft_matrix(a), 0.3)
    proj(0, 0, 1, chunks=4, only=(2, 3))
    side.finish("t")
    for gi in range(5):
        if gi < 4:
            side.add("t", u_to_token_major(gi + 1, 43), 1.0, first=True)
        for a in range(16):
            dft64(a, gi)
        side.finish("t")
    side.add("w", w_prep(2), 0.5)
    for a in range(16):
        side.finish("g%d" % a)
        dft128(a)
    side.close()

    n6, n8 = 8, 4

    pltpu.make_async_copy(wr_raw, wr_raw, sem_in.at[SEM_WR]).wait()
    pltpu.make_async_copy(wi_raw, wi_raw, sem_in.at[SEM_WI]).wait()
    cp_flast(0).wait()
    cp_flast(1).wait()
    cp_wo().wait()
    assert not fetches
    side.open(0.95, 400.0)
    load = (37 * 120 + 280) / 8640
    side.add("f", filter_all(), load)
    side.add("wo", wo_prep(), load)
    for gam in range(4):
        proj(2, 0, gam, chunks=1)
    proj(0, 0, 2, chunks=1)
    proj(0, 0, 3, chunks=1)
    side.finish("f")
    barrier()
    side.open()

    if -1 >= 0:
        side.open()

    side.add("att", attend(0, range(n6)), n6 * 319 / 5856)
    idft128(0)
    for a in range(16):
        if a < 15:
            idft128(a + 1)
        idft64(a)
    barrier()
    side.open()

    load = ((16 - n6) * 319 + 8 * 232) / 7200
    side.add("att", attend(0, range(n6, 16)), load)
    for c in range(8):
        side.add("r9", radix9_inv(c), load)
    for gam in range(4):
        proj(2, 1, gam, chunks=2)
    proj(0, 1, 0, chunks=2)
    side.finish("att")
    side.finish("r9")
    barrier()
    side.open()

    tc = 34.0
    side.add("att", attend(1, range(n8)), n8 * 319 / (4320 - 52 * tc))
    side.add("o", o_to_token_major(0, tc, range(4)), 1.0)
    for c in range(8):
        side.add("y", y_to_token_major(c, tc), 1.0)
    side.add("y", wo_tail_prep(), 1.0)
    for gam in range(1, 4):
        proj(0, 1, gam, chunks=1)
    side.close()
    for ct in range(5, 9):
        cp_out(ct, 0, S // 2).start()
    _barrier(sem_bar)
    side.open()

    side.add("att", attend(1, range(n8, 16)), (16 - n8) * 319 / 5120)
    for row0 in range(0, 512, 64):
        out_proj(0, row0, 64)
    side.finish("att")
    barrier()
    side.open()

    side.open(0.0)
    for p, gam in pairs:
        out_tail(p, gam)
    _drain(o_to_token_major(1, 0, range(4)))
    for c in range(8):
        seam_to_token_major(c)
    cp_out(4, 0, S // 2).start()
    row0 = 0
    for cw in (16, 32, 64, 128, 128, 64, 32, 32, 16):
        out_proj(1, row0, cw)
        row0 += cw
    pltpu.make_async_copy(out_hbm, out_hbm, sem_out).wait()


def _barrier(sem):
    pl.semaphore_signal(sem)
    pl.semaphore_wait(sem)


@jax.jit
def pallas_concat_heads__sliding_local_dilated__spectral_gfnet__prompt_kernel(
    A_x: jax.Array,
    A_wqkv: jax.Array,
    A_wo: jax.Array,
    B_x: jax.Array,
    B_w_r: jax.Array,
    B_w_i: jax.Array,
):
    assert A_x.shape == (1, S, D) and B_x.shape == (1, S, D)
    any_spec = pl.BlockSpec(memory_space=pl.ANY)
    scratch = [
        pltpu.VMEM((1,) + _TABLE.shape, U32),
        pltpu.VMEM((16, 288, 128), U32),
        pltpu.VMEM((16, 128, 128), U32),
        pltpu.VMEM((D - 256, S), BF16),
        pltpu.VMEM((D + 64, 3 * D), BF16),
        pltpu.VMEM((D + 64, D), BF16),
        pltpu.VMEM((1, 16, 144, 128), U32),
        pltpu.VMEM((1, 16, 144, 128), U32),
        pltpu.VMEM((2, 1, S), BF16),
        pltpu.VMEM((1, 16, 3, 128, 128), F32),
        pltpu.VMEM((1, 8, D, 128), U32),
        pltpu.VMEM((1, 8, D, 128), U32),
        pltpu.VMEM((5, 8 * 136, 128), U32),
        pltpu.VMEM((1, 18, 2, NR, 128), F32),
        pltpu.VMEM((1, 16, 2, NR, 128), F32),
        pltpu.VMEM((1, 2, 2, NR, 128), F32),
        pltpu.VMEM((3, 16 * 136, 128), U32),
        [pltpu.VMEM((1, 16, n, 128), U32) for n in (128, 128, 64)],
        pltpu.VMEM((1, 5, 320, 128), U32),
        pltpu.VMEM((1, 5, 288, 128), U32),
        pltpu.VMEM((1, 5, 288, 128), U32),
        pltpu.VMEM((1, 5, 288, 128), U32),
        pltpu.VMEM((1, 5, 288, 128), U32),
        pltpu.VMEM((1, 5, 320, 128), U32),
        pltpu.VMEM((1, 5, 32, 128), U32),
        [pltpu.VMEM((1, 2, D + 16, 128), F32)] * 8,
        [pltpu.VMEM((1, 16, D + 8, 128), F32)] * 2,
        [pltpu.VMEM((1, 16, D + 8, 128), F32)] * 2,
        [pltpu.VMEM((1, 4, D, 128), U32)] * 2,
        [pltpu.VMEM((1, 5, 512, 128), U32)] * 2,
        pltpu.VMEM((1, 4, S // 2, 128), F32),
        pltpu.VMEM((1, 2, 8, 64, 128), F32),
        pltpu.VMEM((9, S // 2, 128), U32),
        pltpu.SemaphoreType.DMA((5,)),
        pltpu.SemaphoreType.DMA((9,)),
        pltpu.SemaphoreType.DMA(()),
        pltpu.SemaphoreType.REGULAR,
    ]
    out = pl.pallas_call(
        _kernel,
        out_shape=jax.ShapeDtypeStruct((S, 2 * D), BF16),
        in_specs=[any_spec] * 7 + [pl.BlockSpec(memory_space=pltpu.SMEM)],
        out_specs=any_spec,
        scratch_shapes=scratch,
        compiler_params=pltpu.CompilerParams(vmem_limit_bytes=120 * 1024 * 1024),
        name="attn_gfnet",
    )(A_x[0].T, A_wqkv, A_wo, B_x[0].T, B_w_r.T, B_w_i.T, _TABLE, np.zeros((2,), np.int32))
    return out[None]
```

```python
from functools import partial

import numpy as np

import jax
import jax.numpy as jnp
from jax import lax
import jax.experimental.pallas as pl
import jax.experimental.pallas.tpu as pltpu

S = 2048
D = 576
H = 32
DH = 18
W = 8
DF = D // 2 + 1
NR = 296

F32 = jnp.float32
BF16 = jnp.bfloat16
U32 = jnp.uint32

_C3 = float(np.sqrt(3.0) / 2)
_C1, _S1 = float(np.cos(2 * np.pi / 9)), float(np.sin(2 * np.pi / 9))
_C2, _S2 = float(np.cos(4 * np.pi / 9)), float(np.sin(4 * np.pi / 9))


def _bfly9_fwd(x):
    a0, ar, ai = [], [], []
    for j in range(3):
        t = x[j + 3] + x[j + 6]
        a0.append(x[j] + t)
        ar.append(x[j] - 0.5 * t)
        ai.append(x[j + 6] - x[j + 3])
    t = a0[1] + a0[2]
    u0 = a0[0] + t
    u3r = a0[0] - 0.5 * t
    u3i = a0[2] - a0[1]
    b1r = ar[1] * _C1 + ai[1] * (_C3 * _S1)
    b1i = ai[1] * (_C3 * _C1) - ar[1] * _S1
    b2r = ar[2] * _C2 + ai[2] * (_C3 * _S2)
    b2i = ai[2] * (_C3 * _C2) - ar[2] * _S2
    a_r, a_i = ar[0], ai[0] * _C3
    tr, ti = b1r + b2r, b1i + b2i
    dr, di = (b1r - b2r) * _C3, (b1i - b2i) * _C3
    u1r, u1i = a_r + tr, a_i + ti
    mr, mi = a_r - 0.5 * tr, a_i - 0.5 * ti
    return [u0, u1r, u1i, mr - di, mi + dr, u3r, u3i, mr + di, mi - dr]


def _bfly9_inv(v):
    u0, u1r, u1i, u7r, u7i, u3r, u3i, u4r, u4i = v
    mr, mi = u4r + u7r, u4i + u7i
    di, dr = (u4r - u7r) * _C3, (u7i - u4i) * _C3
    a_r, a_i = u1r + mr, u1i + mi
    tr, ti = u1r - 0.5 * mr, u1i - 0.5 * mi
    b1r, b2r, b1i, b2i = tr + dr, tr - dr, ti + di, ti - di
    ar = [a_r, b1r * _C1 - b1i * _S1, b2r * _C2 - b2i * _S2]
    ai = [a_i * _C3, b1r * (_C3 * _S1) + b1i * (_C3 * _C1),
          b2r * (_C3 * _S2) + b2i * (_C3 * _C2)]
    t = u0 - 0.5 * u3r
    a0 = [u0 + u3r, t - u3i, t + u3i]
    y = [None] * 9
    for j in range(3):
        t = a0[j] - 0.5 * ar[j]
        y[j] = a0[j] + ar[j]
        y[j + 3] = t - ai[j]
        y[j + 6] = t + ai[j]
    return y


def _bfly4(x, inverse):
    (ar, ai), (br, bi), (cr, ci), (dr, di) = x
    pr, pi, qr, qi = ar + cr, ai + ci, ar - cr, ai - ci
    sr, si, tr, ti = br + dr, bi + di, br - dr, bi - di
    y1, y3 = (qr + ti, qi - tr), (qr - ti, qi + tr)
    if inverse:
        y1, y3 = y3, y1
    return [(pr + sr, pi + si), y1, (pr - sr, pi - si), y3]


def _twiddle16(z, e, inverse):
    zr, zi = z
    e = (-e if inverse else e) % 16
    h = float(np.sqrt(0.5))
    if e == 0:
        return z
    if e == 4:
        return zi, -zr
    if e == 12:
        return -zi, zr
    if e == 2:
        return (zr + zi) * h, (zi - zr) * h
    if e == 14:
        return (zr - zi) * h, (zr + zi) * h
    if e == 6:
        return (zi - zr) * h, (zr + zi) * (-h)
    if e == 10:
        return (zr + zi) * (-h), (zr - zi) * h
    c, s = float(np.cos(2 * np.pi * e / 16)), float(np.sin(2 * np.pi * e / 16))
    return zr * c + zi * s, zi * c - zr * s


_GROUPS = (1, 2, 3, 4, 0)


def _group_classes(g):
    return sorted({g, g + 9, 9 - g, 18 - g}) if g else [0, 9]


_ROWGROUPS = [(k0, h) for g in _GROUPS for k0 in _group_classes(g) for h in range(2)]


def _to_words(m):
    u = np.ascontiguousarray(m, dtype=np.float32).view(np.uint32)
    u = (u + 0x7FFF + ((u >> 16) & 1)) >> 16
    return (u[0::2] | (u[1::2] << 16)).astype(np.uint32)


def _make_tables():
    basis = np.array(_bfly9_fwd(list(np.eye(9))))
    m_fwd = np.array([2 * (r % 32) + r // 32 for r in range(64)])
    lf, li = [], []
    for g in _GROUPS:
        rows = [k0 + 18 * i for k0 in _group_classes(g) for i in range(16)]
        if g == 0:
            rows += [DF - 1] + [-1] * 7
        cols = [2 * g - 1, 2 * g] if g else [0]
        a = basis[cols].T.astype(complex)
        n = len(rows)
        f = np.zeros((2 * n, 128))
        b = np.zeros((64 * len(cols), 128))
        for r, k in enumerate(rows):
            if k < 0:
                continue
            ck = np.exp(-2j * np.pi * ((np.arange(9) * k) % 9) / 9)
            lam = np.linalg.solve(a.conj().T @ a, a.conj().T @ ck)
            wk = (1.0 if k in (0, DF - 1) else 2.0) / (S * D)
            for c in range(len(cols)):
                e = lam[c] * np.exp(-2j * np.pi * ((m_fwd * k) % D) / D)
                f[r, 64 * c:64 * c + 64] = e.real
                f[n + r, 64 * c:64 * c + 64] = e.imag
                e = wk * lam[c] * np.exp(-2j * np.pi * ((np.arange(64) * k) % D) / D)
                b[64 * c:64 * c + 64, r] = e.real
                b[64 * c:64 * c + 64, n + r] = e.imag
        lf.append(_to_words(f))
        li.append(_to_words(b))
    n = np.arange(128)
    b_of_n = 16 * (n // 16) + 8 * (n % 2) + (n % 16) // 2
    f128 = np.exp(-2j * np.pi * (np.outer(b_of_n, n) % 128) / 128)
    tw = np.exp(-2j * np.pi * np.outer(np.arange(16), n) / S)
    f32w = lambda m: np.ascontiguousarray(m, dtype=np.float32).view(np.uint32)
    parts = [f32w(f128.real), f32w(f128.imag), f32w(tw.real), f32w(tw.imag)] + lf + li
    offs = np.cumsum([0] + [p.shape[0] for p in parts])
    parts.append(np.zeros((-offs[-1] % 32, 128), np.uint32))
    return np.concatenate(parts, axis=0), [int(o) for o in offs]


_TABLE, _OFF = _make_tables()
_OFF_FR, _OFF_FI, _OFF_TR, _OFF_TI = _OFF[0:4]
_OFF_LF = _OFF[4:10]
_OFF_LI = _OFF[9:15]


def _pack(lo, hi):
    return pltpu.pack_elementwise([lo, hi], packed_dtype=BF16)


def _unpack(w, index):
    return pltpu.unpack_elementwise(w, index=index, packed_dtype=BF16, unpacked_dtype=F32)


def _bf(words):
    return pltpu.bitcast(words, BF16)


def _dot(a, b):
    return lax.dot_general(a, b, (((1,), (0,)), ((), ())), preferred_element_type=F32)


def _dot_nt(a, b):
    return lax.dot_general(a, b, (((1,), (1,)), ((), ())), preferred_element_type=F32)


def _zeros_w(rows):
    return jnp.zeros((rows, 128), U32)


class _SideWork:
    LINK = 7.0

    def __init__(self, zero_ref):
        self.zero_ref = zero_ref
        self.zero = zero_ref[0]
        self.lead = 0.0

    def start(self, seed, sink):
        self.chain = pltpu.bitcast(seed, F32)
        self.sink = sink
        self.jobs = []
        self.credit = 0.0
        self.delay = 0.0
        self.blocks = 0
        self.now = 0.0
        self.pending = []

    def open(self, stretch=1.0, slack=100.0, links=4):
        self.min_links = links
        self.zero = self.zero_ref[0]
        self.lead = -slack
        self.stretch = stretch

    def add(self, name, gen, load, first=False):
        self.jobs.insert(0 if first else len(self.jobs), (name, gen, load * 1.0))

    def _advance(self, cycles):
        self.lead += cycles
        while self.lead >= 6.0:
            self.zero = self.zero_ref[self.zero]
            self.lead -= 6.0

    def _tick(self, cycles):
        self.now += cycles
        self.delay += cycles
        while self.pending and self.pending[0][0] <= self.now:
            self.chain = self.pending.pop(0)[1] + self.chain
            self.delay -= 2.0
        n = int(self.delay / self.LINK)
        if n >= self.min_links:
            for _ in range(n):
                self.chain = pl.reciprocal(self.chain, approx=True)
            self.delay -= n * self.LINK

    def _step(self):
        item = next(self.jobs[0][1], None)
        if item is None:
            self.jobs.pop(0)
            return
        values, cycles, latency = (item + (0.0,))[:3]
        values = values if isinstance(values, list) else [values]
        values = [pltpu.bitcast(v, F32) for v in values]
        while len(values) > 1:
            values = [values[i] + values[i + 1] if i + 1 < len(values) else values[i]
                      for i in range(0, len(values), 2)]
        self.pending.append((self.now + latency, values[0]))
        self.pending.sort(key=lambda x: x[0])
        cycles = cycles / self.jobs[0][2]
        self.credit -= cycles
        self._advance(cycles)
        self._tick(self.stretch * cycles)

    def run(self, cycles):
        self.credit += cycles
        while self.jobs and self.credit > 0:
            self._step()
        if not self.jobs and self.credit > 0:
            self._tick(self.stretch * self.credit)
            self.credit = 0.0

    def finish(self, name):
        while any(job[0] == name for job in self.jobs):
            self._step()

    def close(self):
        while self.jobs:
            self._step()
        while self.pending:
            self.chain = self.pending.pop(0)[1] + self.chain
        self.sink[pl.ds(8 * self.blocks, 8), :] = self.chain
        self.blocks += 1
        self.credit = self.delay = 0.0


def _drain(gen):
    for _ in gen:
        pass


_W_COLS = ((0, 512), (512, 640), (1152, 576))


def _kernel(xa_hbm, wqkv_hbm, wo_hbm, xb_hbm, wr_hbm, wi_hbm, tab_hbm, zero_ref, out_hbm,
            tab, xb_raw, xa_raw, xa_rest, wq_raw, wo_raw, wr_raw, wi_raw, wlast,
            gmat, u_t, y_t, u_nat, x1_buf, t_buf, z_buf, x_nat, x_perm, wt_nat, wt_q, wt_k, wt_v,
            wo_nat, wo_perm, wo_tail, q_buf, k_buf, v_buf, o_t, o_nat, out0, a_tail, stage,
            sem_xa, sem_in, sem_out, sem_bar):
    side = _SideWork(zero_ref)
    zero = side.zero

    def now(ref):
        return ref.at[side.zero]

    tab_r, wr_r, wi_r = tab, wr_raw, wi_raw
    tab, wr_raw, wi_raw = tab.at[0], wr_raw.at[0], wi_raw.at[0]
    (u_r, y_r, t_r, wn_r, won_r, q_r, k_r, v_r, o_r) = (
        u_t, y_t, t_buf, wt_nat, wo_nat, q_buf, k_buf, v_buf, o_t)
    (gmat, u_t, y_t, x1_buf, t_buf, z_buf, x_perm, wt_nat, wt_q, wt_k, wt_v, wo_nat, wo_perm,
     wo_tail, q_buf, k_buf, v_buf, o_t, o_nat, out0, a_tail) = jax.tree.map(
        lambda r: r.at[zero],
        (gmat, u_t, y_t, x1_buf, t_buf, z_buf, x_perm, wt_nat, wt_q, wt_k, wt_v, wo_nat, wo_perm,
         wo_tail, q_buf, k_buf, v_buf, o_t, o_nat, out0, a_tail))
    wt = (wt_q, wt_k, wt_v)

    SEM_XB, SEM_TAB, SEM_WQ, SEM_WK, SEM_WV, SEM_WO, SEM_WR, SEM_WI, SEM_LAST = range(9)

    def cp_tab(row0, rows, z=0):
        return pltpu.make_async_copy(
            tab_hbm.at[pl.ds(row0, rows)], tab.at[pl.ds(pl.multiple_of(z + row0, 8), rows)],
            sem_in.at[SEM_TAB])

    def cp_xb(t, z=0):
        return pltpu.make_async_copy(
            xb_hbm.at[:, pl.ds(t * 128, 128)], xb_raw.at[z + t].bitcast(BF16), sem_in.at[SEM_XB])

    def cp_xa(t):
        return pltpu.make_async_copy(
            xa_hbm.at[pl.ds(0, 256), pl.ds(t * 128, 128)], xa_raw.at[t].bitcast(BF16),
            sem_xa.at[sum(t >= s for s in (6, 11, 14))])

    def cp_xa_rest():
        return pltpu.make_async_copy(xa_hbm.at[pl.ds(256, D - 256)], xa_rest, sem_xa.at[4])

    def cp_wq(part, row0=0, rows=D, z=0):
        cols = pl.ds(*_W_COLS[part])
        return pltpu.make_async_copy(
            wqkv_hbm.at[pl.ds(row0, rows), cols],
            wq_raw.at[pl.ds(pl.multiple_of(z + row0, 16), rows), cols], sem_in.at[SEM_WQ + part])

    def cp_wo(row0=0, rows=D, z=0):
        return pltpu.make_async_copy(
            wo_hbm.at[pl.ds(row0, rows)], wo_raw.at[pl.ds(pl.multiple_of(z + row0, 16), rows)],
            sem_in.at[SEM_WO])

    def cp_f(i, t, z=0):
        src, dst = ((wr_hbm, wr_raw), (wi_hbm, wi_raw))[i]
        return pltpu.make_async_copy(
            src.at[pl.ds(0, DF - 1), pl.ds(t * 128, 128)], dst.at[z + t].bitcast(BF16),
            sem_in.at[SEM_WR + i])

    def cp_flast(i):
        src = (wr_hbm, wi_hbm)[i]
        return pltpu.make_async_copy(src.at[pl.ds(DF - 1, 1), :], wlast.at[i], sem_in.at[SEM_LAST])

    def cp_out(ct, row0, rows):
        return pltpu.make_async_copy(
            stage.at[ct, pl.ds(row0, rows), :].bitcast(BF16),
            out_hbm.at[pl.ds(2 * row0, 2 * rows), pl.ds(ct * 128, 128)], sem_out)

    def fetch_xb(t, v):
        xb_raw[t, pl.ds(0, 8), :] = v
        cp_xb(t).start()

    def fetch_wq(part, piece, v):
        wq_raw[pl.ds(144 * piece, 16), pl.ds(_W_COLS[part][0], 128)] = _bf(v)
        cp_wq(part, 144 * piece, 144).start()

    def fetch_wo(piece, v):
        wo_raw[pl.ds(144 * piece, 16), pl.ds(0, 128)] = _bf(v)
        cp_wo(144 * piece, 144).start()

    def wo_settle(v):
        wo_raw[pl.ds(D, 16), pl.ds(0, 128)] = _bf(v)

    def fetch_tab(row0, rows, v):
        tab[pl.ds(row0, 8), :] = v
        cp_tab(row0, rows).start()

    def fetch_f(t, v):
        wr_raw[t, pl.ds(0, 8), :] = v
        cp_f(0, t).start()
        wi_raw[t, pl.ds(0, 8), :] = v
        cp_f(1, t).start()
        if t == 0:
            cp_flast(0).start()
            cp_flast(1).start()

    n_tab = _TABLE.shape[0]
    fetches = []

    def fetch_next(value):
        if fetches:
            for fetch in fetches.pop(0):
                fetch(pltpu.bitcast(value[:8, :128], U32))

    def store_pitched(dst, row0, vt):
        for r in range(16):
            dst[pl.ds(row0 + 17 * (r // 2) + 8 * (r % 2), 8), :] = vt[8 * r:8 * r + 8]

    def radix9(tau):
        for i in range(4):
            words = [[xb_raw[side.zero + 2 * tau + z, pl.ds(32 * j + 8 * i, 8), :] for j in range(9)]
                     for z in range(2)]
            for e in range(2):
                u = []
                for z in range(2):
                    u.append(_bfly9_fwd([_unpack(w, e) for w in words[z]]))
                    yield u[z][8], 14
                out = [_pack(u[0][o], u[1][o]) for o in range(9)]
                for o in range(9):
                    u_t[tau, pl.ds(64 * o + 32 * e + 8 * i, 8), :] = out[o]
                yield out, 5

    def u_to_token_major(gi, cost):
        g = _GROUPS[gi]
        for tau in range(8):
            if g:
                v = u_t[tau, pl.ds(64 * (2 * g - 1), 128), :]
            else:
                v = jnp.concatenate([u_t[tau, pl.ds(0, 64), :], _zeros_w(64)], axis=0)
            vt = v.T
            store_pitched(u_nat.at[gi], 136 * tau, vt)
            yield vt[120:], cost, 240

    def dft_matrix(a):
        twr = jnp.broadcast_to(pltpu.bitcast(tab[pl.ds(_OFF_TR + a, 1), :], F32), (8, 128))
        twi = jnp.broadcast_to(pltpu.bitcast(tab[pl.ds(_OFF_TI + a, 1), :], F32), (8, 128))
        for i in range(16):
            fr = pltpu.bitcast(now(tab_r)[pl.ds(_OFF_FR + 8 * i, 8), :], F32)
            fi = pltpu.bitcast(now(tab_r)[pl.ds(_OFF_FI + 8 * i, 8), :], F32)
            gr, gi = fr * twr - fi * twi, fr * twi + fi * twr
            gmat[a, 0, pl.ds(8 * i, 8), :] = gr
            out = [gr + gi, gi - gr]
            gmat[a, 1, pl.ds(8 * i, 8), :] = out[0]
            gmat[a, 2, pl.ds(8 * i, 8), :] = out[1]
            yield out, 3

    def filter_rows(row0, load_w):
        rows = pl.ds(row0, 8)
        y = [[None] * 4 for _ in range(4)]
        for a0 in range(4):
            src = now(t_r)
            z = _bfly4([(src[4 * a1 + a0, 0, rows, :], src[4 * a1 + a0, 1, rows, :])
                        for a1 in range(4)], False)
            for g0 in range(4):
                y[g0][a0] = _twiddle16(z[g0], a0 * g0, False)
            yield y[3][a0][0], 7
        for g0 in range(4):
            z = _bfly4(y[g0], False)
            yield z[3][1], 4
            for g1 in range(4):
                wr, wi = load_w(g0 + 4 * g1)
                zr, zi = z[g1]
                z[g1] = (zr * wr - zi * wi, zr * wi + zi * wr)
                if g1 % 2:
                    yield z[g1][1], 4
            z = _bfly4(z, True)
            for a0 in range(4):
                y[g0][a0] = _twiddle16(z[a0], a0 * g0, True)
            yield y[g0][3][0], 6
        for a0 in range(4):
            z = _bfly4([y[g0][a0] for g0 in range(4)], True)
            for a1 in range(4):
                t_buf[4 * a1 + a0, 0, rows, :] = z[a1][0]
                t_buf[4 * a1 + a0, 1, rows, :] = z[a1][1]
            yield [v for pair in z for v in pair], 6

    def filter_all():
        for n, (k0, h) in enumerate(_ROWGROUPS):
            rows = pl.ds(k0 // 2 + 72 * h, 8, stride=9)
            yield from filter_rows(8 * n, lambda f1: (
                _unpack(now(wr_r)[f1, rows, :], k0 % 2),
                _unpack(now(wi_r)[f1, rows, :], k0 % 2)))
        yield from filter_rows(NR - 8, lambda f1: tuple(
            jnp.broadcast_to(wlast[i, :, pl.ds(128 * f1, 128)].astype(F32), (8, 128))
            for i in range(2)))

    def radix9_inv(c):
        for i in range(8):
            y = []
            for e in range(2):
                y.append(_bfly9_inv(
                    [now(t_r)[2 * c + e, i // 4, pl.ds(256 + 8 * (i % 4), 8), :]]
                    + [now(t_r)[2 * c + e, o % 2, pl.ds(64 * (o // 2) + 8 * i, 8), :]
                       for o in range(8)]))
                yield (y[e] if 0 else y[e][8]), 12
            out = [_pack(y[0][j], y[1][j]) for j in range(9)]
            for j in range(9):
                y_t[c, pl.ds(64 * j + 8 * i, 8), :] = out[j]
            yield out, 5

    def y_to_token_major(c, cost):
        for q in range(4):
            vt = y_t[c, pl.ds(64 + 128 * q, 128), :].T
            stage[5 + q, pl.ds(c, 128, stride=8), :] = vt
            yield vt[120:], cost, 240

    def seam_to_token_major(c):
        top = _pack(a_tail[0, c], a_tail[1, c])
        stage[4, pl.ds(c, 128, stride=8), :] = jnp.concatenate(
            [top, y_t[c, pl.ds(0, 64), :]], axis=0).T

    def wo_tail_prep():
        for kt in range(5):
            vt = pltpu.bitcast(_bf(wo_perm[4, pl.ds(64 * kt, 64), :]).T, U32)
            wo_tail[kt] = vt[:32]
            yield vt[24:32], 22, 180

    def x_to_token_major(t, qs):
        lanes = pl.ds(128 * t, 128)
        for q in qs:
            if q == 0:
                v = xa_raw[t]
            elif q == 1:
                v = pltpu.bitcast(xa_rest[pl.ds(0, 256), lanes], U32)
            else:
                v = pltpu.bitcast(xa_rest[pl.ds(256, 64), lanes], U32)
                v = jnp.concatenate([v, _zeros_w(96)], axis=0)
            store_pitched(x_nat.at[q], 136 * t, v.T)

    def x_tile(a, qs):
        for q in qs:
            vt = x_nat[q, pl.ds(a, 128, stride=17), :].T
            n = 128 if q < 2 else 64
            x_perm[q][a] = vt[:n]
            yield vt[n - 8:n], 43, 240

    def w_prep(part, kts=range(5)):
        col0, _ = _W_COLS[part]
        first = 288 * part - col0 // 2
        for kt in kts:
            for nt in range(5):
                nn = min(128, 3 * D - col0 - 128 * nt)
                vt = wq_raw[pl.ds(128 * kt, 128), pl.ds(col0 + 128 * nt, nn)].T
                vt = pltpu.bitcast(vt, U32)
                wt_nat[kt, pl.ds(64 * nt, nn // 2), :] = vt
                yield vt[-8:], 22, 180
        for kt in kts:
            for i in range(2):
                for dl in range(9):
                    base = first + 144 * i + dl
                    wa = now(wn_r)[kt, pl.ds(base, 8, stride=18), :]
                    wb = now(wn_r)[kt, pl.ds(base + 9, 8, stride=18), :]
                    out = [_pack(_unpack(wa, e), _unpack(wb, e)) for e in range(2)]
                    for e in range(2):
                        wt[part][kt, pl.ds(16 * (2 * dl + e) + 8 * i, 8), :] = out[e]
                    yield out, 2

    def wo_prep():
        for nt in range(5):
            nn = min(128, D - 128 * nt)
            blk = wo_raw[pl.ds(0, D), pl.ds(128 * nt, nn)]
            if nn < 128:
                blk = jnp.concatenate([blk, jnp.zeros((D, 128 - nn), BF16)], axis=1)
            blk = pltpu.bitcast(blk, U32)
            wo_nat[nt] = blk
            wo_perm[nt, pl.ds(288, 32), :] = _zeros_w(32)
            yield blk[-8:], 20
            for i in range(2):
                for dl in range(9):
                    wa = now(won_r)[nt, pl.ds(144 * i + dl, 8, stride=18), :]
                    wb = now(won_r)[nt, pl.ds(144 * i + dl + 9, 8, stride=18), :]
                    out = [_pack(_unpack(wa, e), _unpack(wb, e)) for e in range(2)]
                    for e in range(2):
                        wo_perm[nt, pl.ds(16 * (2 * dl + e) + 8 * i, 8), :] = out[e]
                    yield out, 2

    scale = float(DH) ** -0.5
    QB = 6

    def attend(p, units):
        lane0 = lax.broadcasted_iota(jnp.int32, (8, 128), 1) == 0
        for unit in units:
            gam, hg = divmod(unit, 4)
            base = 2 * gam + 1
            acc = [[None] * W for _ in range(2)]
            for d0 in range(0, DH, QB):
                rows = [pl.ds(144 * hg + 8 * d, 8) for d in range(d0, d0 + QB)]
                q = [[now(q_r[4 * p + gam])[e, r, :] for r in rows] for e in range(2)]
                for l in range(9):
                    for n, r in enumerate(rows):
                        k = now(k_r[p])[base + l, r, :]
                        for e in range(2):
                            w = 7 + e - l
                            if 0 <= w < W:
                                t = q[e][n] * k
                                acc[e][w] = t if acc[e][w] is None else acc[e][w] + t
                    done = [acc[e][7 + e - l] for e in range(2) if 0 <= 7 + e - l < W]
                    yield done, QB / 2 * len(done)
            prob = []
            for e in range(2):
                lg = [jnp.where(lane0, -1e9 / scale, acc[e][w]) if 2 * gam + e < w else acc[e][w]
                      for w in range(W)]
                m = lg[0]
                for w in range(1, W):
                    m = jnp.maximum(m, lg[w])
                ex = [jnp.exp2((l_ - m) * (scale * float(np.log2(np.e)))) for l_ in lg]
                tot = ex[0]
                for w in range(1, W):
                    tot = tot + ex[w]
                inv = 1.0 / tot
                prob.append([x_ * inv for x_ in ex])
                yield prob[e][W - 1], 13, 30
            for d in range(DH):
                rows = pl.ds(32 * d + 8 * hg, 8)
                vv = [now(v_r[p])[base + l, pl.ds(144 * hg + 8 * d, 8), :] for l in range(9)]
                o = []
                for e in range(2):
                    t = prob[e][0] * vv[7 + e]
                    for w in range(1, W):
                        t = t + prob[e][w] * vv[7 + e - w]
                    o.append(t)
                word = _pack(o[0], o[1])
                o_t[p][gam, rows, :] = word
                yield word, 8

    def o_to_token_major(p, cost, gams):
        for gam in gams:
            for kt in range(5):
                if kt < 4:
                    v = (o_t[p] if 1 else now(o_r[p]))[gam, pl.ds(128 * kt, 128), :]
                else:
                    v = jnp.concatenate([(o_t[p] if 1 else now(o_r[p]))[gam, pl.ds(512, 64), :], _zeros_w(64)], axis=0)
                vt = v.T
                o_nat[p][kt, pl.ds(gam, 128, stride=4), :] = vt
                yield vt[120:], cost, 240

    def table(off, i):
        return _bf(tab[pl.ds(off[i], off[i + 1] - off[i]), :])

    def dft64(a, gi):
        x1 = _dot_nt(table(_OFF_LF, gi), _bf(u_nat[gi, pl.ds(a, 64, stride=17), :]))
        n = x1.shape[0] // 2
        side.run(n / 2)
        x1_buf[a, 0, pl.ds(64 * gi, n), :] = x1[:n]
        x1_buf[a, 1, pl.ds(64 * gi, n), :] = x1[n:]
        if a % 4 == 3:
            fetch_next(x1)

    def dft128(a):
        side.run(222)
        xr, xi = x1_buf[a, 0], x1_buf[a, 1]
        k1 = _dot(xr + xi, gmat[a, 0])
        t_buf[a, 0] = k1 - _dot(xi, gmat[a, 1])
        t_buf[a, 1] = k1 + _dot(xr, gmat[a, 2])

    def idft128(a):
        side.run(222)
        g = [jnp.concatenate([gmat[a, c, pl.ds(16 * tau + e, 8, stride=2), :]
                              for tau in range(8) for e in range(2)], axis=0) for c in range(3)]
        tr, ti = t_buf[a, 0], t_buf[a, 1]
        k1 = _dot_nt(tr + ti, g[0])
        z_buf[a % 2, 0] = k1 + _dot_nt(ti, g[2])
        z_buf[a % 2, 1] = k1 - _dot_nt(tr, g[1])

    def idft64(a):
        side.run(144)
        for gi in range(5):
            n = 64 if gi < 4 else NR - 256
            parts = [z_buf[a % 2, c, pl.ds(64 * gi, n), :] for c in range(2)]
            if n < 64:
                parts.append(jnp.zeros((128 - 2 * n, 128), F32))
            o = _dot(table(_OFF_LI, gi), jnp.concatenate(parts, axis=0))
            if gi < 4:
                t_buf[a, 0, pl.ds(64 * gi, 64), :] = o[:64]
                t_buf[a, 1, pl.ds(64 * gi, 64), :] = o[64:]
            else:
                t_buf[a, 0, pl.ds(256, 32), :] = o[:32]
                t_buf[a, 1, pl.ds(256, 32), :] = o[32:]

    def proj(part, p, gam, qs=(0, 1, 2), chunks=4, only=None):
        a = 4 * gam + p
        m = 288 // chunks
        kts = [kt for q in qs for kt in (2 * q, 2 * q + 1) if kt < 5]
        for ch in only or range(chunks):
            side.run(len(kts) * m)
            w = jnp.concatenate(
                [_bf(wt[part][kt, pl.ds(m * ch, m), :]) for kt in kts], axis=1)
            x = jnp.concatenate(
                [jnp.concatenate([_bf(x_perm[q][a + 2 * e]) for e in range(2)], axis=1)
                 for q in qs], axis=0)
            r = _dot(w, x)
            for e in range(2):
                c = 2 * gam + e
                buf, slot = (q_buf[4 * p + gam], e) if part == 0 else (
                    (k_buf, v_buf)[part - 1][p], 8 + c)
                rows = []
                for i in range(m // 4):
                    d, hg = divmod(m // 4 * ch + i, 4)
                    rows.append(pl.ds(144 * hg + 8 * d, 8))
                tile = r[:, 128 * e:128 * e + 128]
                if qs[0]:
                    tile = tile + jnp.concatenate([buf[slot, r_, :] for r_ in rows], axis=0)
                shifted = part and c and qs[-1] == 2
                rolled = pltpu.roll(tile, 1, 1) if shifted else None
                for i, r_ in enumerate(rows):
                    buf[slot, r_, :] = tile[8 * i:8 * i + 8]
                    if shifted:
                        buf[c, r_, :] = rolled[8 * i:8 * i + 8]
                        if part == 2:
                            lane0 = lax.broadcasted_iota(jnp.int32, (8, 128), 1) == 0
                            pltpu.store(buf.at[c, r_, :], v_buf[0][8, r_, :], mask=lane0)
            fetch_next(r)

    def out_proj(p, row0, cw):
        side.run(10 * cw)
        lhs = jnp.concatenate([_bf(o_nat[p][kt, pl.ds(row0, cw), :]) for kt in range(5)], axis=1)
        r = _dot(lhs, jnp.concatenate([_bf(wo_perm[nt]) for nt in range(4)], axis=1))
        rows = pl.ds(2 * row0, 2 * cw)
        for ct in range(4):
            tile = r[:, 128 * ct:128 * ct + 128]
            if p == 0:
                out0[ct, rows, :] = tile
            else:
                stage[ct, rows, :] = _pack(out0[ct, rows, :], tile)
                cp_out(ct, 2 * row0, 2 * cw).start()

    def out_tail(p, gam):
        side.run(160)
        words = o_t[p][gam]
        o = jnp.concatenate([_unpack(words, e) for e in range(2)], axis=1)
        o = jnp.concatenate([o, jnp.zeros((64, 256), F32)], axis=0)
        r = _dot(jnp.concatenate([_bf(wo_tail[kt]) for kt in range(5)], axis=1), o)
        for e in range(2):
            a_tail[p, 2 * gam + e] = r[:, 128 * e:128 * e + 128]

    cp_wq(1, 0, 256).start()
    for t in range(8):
        cp_xa(t).start()
    wq_raw[pl.ds(D, 64), :] = jnp.zeros((64, 3 * D), BF16)
    cp_wq(1, 0, 256).wait()
    _drain(w_prep(1, range(2)))

    for t0, t1 in ((0, 6), (6, 11), (11, 14), (14, 16)):
        if t0 == 0:
            for t in range(8, 16):
                cp_xa(t).start()
        elif t0 == 6:
            cp_wq(1, 256, D - 256).start()
        elif t0 == 11:
            cp_xa_rest().start()
        for t in range(t0, t1):
            cp_xa(t).wait()
        for t in range(t0, t1):
            x_to_token_major(t, (0,))

    _drain(x_tile(0, (0,)))
    _drain(x_tile(2, (0,)))

    side.start(xa_raw[0, pl.ds(0, 8), :], x1_buf.at[16, 0])
    pairs = [(p, gam) for p in range(2) for gam in range(4)]

    def barrier():
        side.close()
        _barrier(sem_bar)

    def pair_tiles(name, n, qs, load, first=False):
        p, gam = pairs[n]
        for e in (1, 0) if first else (0, 1):
            side.add(name, x_tile(4 * gam + p + 2 * e, qs), load, first=first)

    side.open(0.0)
    fetches += [[]] * 3
    fetches += [[partial(fetch_wq, 0, i)] for i in range(4)]
    fetches += [[partial(fetch_xb, t)] for t in range(16)]
    fetches += [[partial(fetch_wq, 2, i) for i in range(4)]]
    fetches += [[partial(fetch_tab, r, min(304, n_tab - r)) for r in range(0, n_tab, 304)]]
    fetches += [[partial(fetch_f, t) for t in range(4)]]
    n_a = 5
    for n in range(n_a):
        pair_tiles("next", n + 1, (0,), 0.5, first=True)
        if n + n_a + 1 < 8:
            pair_tiles("later", n + n_a + 1, (0,), 0.5)
        proj(1, *pairs[n], qs=(0,), chunks=2)
        side.finish("next")
    side.close()

    cp_xa_rest().wait()
    cp_wq(1, 256, D - 256).wait()
    side.open(0.0)
    for n in range(5, 8):
        proj(1, *pairs[n], qs=(0,), chunks=2)
    for q in (1, 2):
        for t in range(16):
            x_to_token_major(t, (q,))
        for n in range(2):
            pair_tiles("next", n, (q,), 0.6)
        side.add("next", w_prep(1, (2, 3) if q == 1 else (4,)), 0.6)
        if q == 2:
            pair_tiles("next", 2, (1, 2), 0.6)
        side.finish("next")
        for n in range(2):
            proj(1, *pairs[n], qs=(q,), chunks=2)
    for n in range(2, 5):
        pair_tiles("next", n + 1, (1, 2), 0.6)
        proj(1, *pairs[n], qs=(1, 2), chunks=3)
        side.finish("next")
    side.close()

    assert not fetches
    pltpu.make_async_copy(xb_raw, xb_raw, sem_in.at[SEM_XB]).wait()
    cp_wq(0).wait()
    side.open(0.9, 300.0)
    load = (8 * 264 + 2 * 172 + 730) / 4752
    side.add("w", w_prep(0), load)
    for tau in range(8):
        side.add("r9", radix9(tau), load)
    for n in range(5, 8):
        if n < 7:
            pair_tiles("next", n + 1, (1, 2), load, first=True)
        proj(1, *pairs[n], qs=(1, 2), chunks=3)
        side.finish("next")
    side.finish("w")
    proj(0, 0, 0)
    proj(0, 0, 1, chunks=4, only=(0, 1))
    side.close()

    cp_tab(0, n_tab).wait()
    cp_wq(2).wait()
    side.open(0.75)
    fetches += [[partial(fetch_f, t)] for t in range(4, 16)]
    fetches += [[partial(fetch_wo, i)] for i in range(4)]
    fetches.append([wo_settle])
    side.add("t", u_to_token_major(0, 43), 1.0)
    for a in range(16):
        side.add("g%d" % a, dft_matrix(a), 0.3)
    proj(0, 0, 1, chunks=4, only=(2, 3))
    side.finish("t")
    for gi in range(5):
        if gi < 4:
            side.add("t", u_to_token_major(gi + 1, 43), 1.0, first=True)
        for a in range(16):
            dft64(a, gi)
        side.finish("t")
    side.add("w", w_prep(2), 0.5)
    for a in range(16):
        side.finish("g%d" % a)
        dft128(a)
    side.close()

    n6, n8 = 8, 4

    pltpu.make_async_copy(wr_raw, wr_raw, sem_in.at[SEM_WR]).wait()
    pltpu.make_async_copy(wi_raw, wi_raw, sem_in.at[SEM_WI]).wait()
    cp_flast(0).wait()
    cp_flast(1).wait()
    cp_wo().wait()
    assert not fetches
    side.open(0.95, 400.0)
    load = (37 * 120 + 280) / 8640
    side.add("f", filter_all(), load)
    side.add("wo", wo_prep(), load)
    for gam in range(4):
        proj(2, 0, gam, chunks=1)
    proj(0, 0, 2, chunks=1)
    proj(0, 0, 3, chunks=1)
    side.finish("f")
    barrier()
    side.open()

    if -1 >= 0:
        side.open()

    side.add("att", attend(0, range(n6)), n6 * 319 / 5856)
    idft128(0)
    for a in range(16):
        if a < 15:
            idft128(a + 1)
        idft64(a)
    barrier()
    side.open()

    load = ((16 - n6) * 319 + 8 * 232) / 7200
    side.add("att", attend(0, range(n6, 16)), load)
    for c in range(8):
        side.add("r9", radix9_inv(c), load)
    for gam in range(4):
        proj(2, 1, gam, chunks=2)
    proj(0, 1, 0, chunks=2)
    side.finish("att")
    side.finish("r9")
    barrier()
    side.open()

    tc = 34.0
    side.add("att", attend(1, range(n8)), n8 * 319 / (4320 - 52 * tc))
    side.add("o", o_to_token_major(0, tc, range(4)), 1.0)
    for c in range(8):
        side.add("y", y_to_token_major(c, tc), 1.0)
    side.add("y", wo_tail_prep(), 1.0)
    for gam in range(1, 4):
        proj(0, 1, gam, chunks=1)
    side.close()
    for ct in range(5, 9):
        cp_out(ct, 0, S // 2).start()
    _barrier(sem_bar)
    side.open()

    side.add("att", attend(1, range(n8, 16)), (16 - n8) * 319 / 5120)
    for row0 in range(0, 512, 64):
        out_proj(0, row0, 64)
    side.finish("att")
    barrier()
    side.open()

    side.open(0.0)
    for p, gam in pairs:
        out_tail(p, gam)
    _drain(o_to_token_major(1, 0, range(4)))
    for c in range(8):
        seam_to_token_major(c)
    cp_out(4, 0, S // 2).start()
    row0 = 0
    for cw in (16, 32, 64, 128, 128, 64, 32, 32, 16):
        out_proj(1, row0, cw)
        row0 += cw
    pltpu.make_async_copy(out_hbm, out_hbm, sem_out).wait()


def _barrier(sem):
    pl.semaphore_signal(sem)
    pl.semaphore_wait(sem)


@jax.jit
def pallas_concat_heads__sliding_local_dilated__spectral_gfnet__prompt_kernel(
    A_x: jax.Array,
    A_wqkv: jax.Array,
    A_wo: jax.Array,
    B_x: jax.Array,
    B_w_r: jax.Array,
    B_w_i: jax.Array,
):
    assert A_x.shape == (1, S, D) and B_x.shape == (1, S, D)
    any_spec = pl.BlockSpec(memory_space=pl.ANY)
    scratch = [
        pltpu.VMEM((1,) + _TABLE.shape, U32),
        pltpu.VMEM((16, 288, 128), U32),
        pltpu.VMEM((16, 128, 128), U32),
        pltpu.VMEM((D - 256, S), BF16),
        pltpu.VMEM((D + 64, 3 * D), BF16),
        pltpu.VMEM((D + 64, D), BF16),
        pltpu.VMEM((1, 16, 144, 128), U32),
        pltpu.VMEM((1, 16, 144, 128), U32),
        pltpu.VMEM((2, 1, S), BF16),
        pltpu.VMEM((1, 16, 3, 128, 128), F32),
        pltpu.VMEM((1, 8, D, 128), U32),
        pltpu.VMEM((1, 8, D, 128), U32),
        pltpu.VMEM((5, 8 * 136, 128), U32),
        pltpu.VMEM((1, 18, 2, NR, 128), F32),
        pltpu.VMEM((1, 16, 2, NR, 128), F32),
        pltpu.VMEM((1, 2, 2, NR, 128), F32),
        pltpu.VMEM((3, 16 * 136, 128), U32),
        [pltpu.VMEM((1, 16, n, 128), U32) for n in (128, 128, 64)],
        pltpu.VMEM((1, 5, 320, 128), U32),
        pltpu.VMEM((1, 5, 288, 128), U32),
        pltpu.VMEM((1, 5, 288, 128), U32),
        pltpu.VMEM((1, 5, 288, 128), U32),
        pltpu.VMEM((1, 5, 288, 128), U32),
        pltpu.VMEM((1, 5, 320, 128), U32),
        pltpu.VMEM((1, 5, 32, 128), U32),
        [pltpu.VMEM((1, 2, D + 16, 128), F32)] * 8,
        [pltpu.VMEM((1, 16, D + 8, 128), F32)] * 2,
        [pltpu.VMEM((1, 16, D + 8, 128), F32)] * 2,
        [pltpu.VMEM((1, 4, D, 128), U32)] * 2,
        [pltpu.VMEM((1, 5, 512, 128), U32)] * 2,
        pltpu.VMEM((1, 4, S // 2, 128), F32),
        pltpu.VMEM((1, 2, 8, 64, 128), F32),
        pltpu.VMEM((9, S // 2, 128), U32),
        pltpu.SemaphoreType.DMA((5,)),
        pltpu.SemaphoreType.DMA((9,)),
        pltpu.SemaphoreType.DMA(()),
        pltpu.SemaphoreType.REGULAR,
    ]
    out = pl.pallas_call(
        _kernel,
        out_shape=jax.ShapeDtypeStruct((S, 2 * D), BF16),
        in_specs=[any_spec] * 7 + [pl.BlockSpec(memory_space=pltpu.SMEM)],
        out_specs=any_spec,
        scratch_shapes=scratch,
        compiler_params=pltpu.CompilerParams(vmem_limit_bytes=120 * 1024 * 1024),
        name="attn_gfnet",
    )(A_x[0].T, A_wqkv, A_wo, B_x[0].T, B_w_r.T, B_w_i.T, _TABLE, np.arange(2, dtype=np.int32))
    return out[None]
```

```python
from functools import partial

import numpy as np

import jax
import jax.numpy as jnp
from jax import lax
import jax.experimental.pallas as pl
import jax.experimental.pallas.tpu as pltpu

S = 2048
D = 576
H = 32
DH = 18
W = 8
DF = D // 2 + 1
NR = 296

F32 = jnp.float32
BF16 = jnp.bfloat16
U32 = jnp.uint32

_C3 = float(np.sqrt(3.0) / 2)
_C1, _S1 = float(np.cos(2 * np.pi / 9)), float(np.sin(2 * np.pi / 9))
_C2, _S2 = float(np.cos(4 * np.pi / 9)), float(np.sin(4 * np.pi / 9))


def _bfly9_fwd(x):
    a0, ar, ai = [], [], []
    for j in range(3):
        t = x[j + 3] + x[j + 6]
        a0.append(x[j] + t)
        ar.append(x[j] - 0.5 * t)
        ai.append(x[j + 6] - x[j + 3])
    t = a0[1] + a0[2]
    u0 = a0[0] + t
    u3r = a0[0] - 0.5 * t
    u3i = a0[2] - a0[1]
    b1r = ar[1] * _C1 + ai[1] * (_C3 * _S1)
    b1i = ai[1] * (_C3 * _C1) - ar[1] * _S1
    b2r = ar[2] * _C2 + ai[2] * (_C3 * _S2)
    b2i = ai[2] * (_C3 * _C2) - ar[2] * _S2
    a_r, a_i = ar[0], ai[0] * _C3
    tr, ti = b1r + b2r, b1i + b2i
    dr, di = (b1r - b2r) * _C3, (b1i - b2i) * _C3
    u1r, u1i = a_r + tr, a_i + ti
    mr, mi = a_r - 0.5 * tr, a_i - 0.5 * ti
    return [u0, u1r, u1i, mr - di, mi + dr, u3r, u3i, mr + di, mi - dr]


def _bfly9_inv(v):
    u0, u1r, u1i, u7r, u7i, u3r, u3i, u4r, u4i = v
    mr, mi = u4r + u7r, u4i + u7i
    di, dr = (u4r - u7r) * _C3, (u7i - u4i) * _C3
    a_r, a_i = u1r + mr, u1i + mi
    tr, ti = u1r - 0.5 * mr, u1i - 0.5 * mi
    b1r, b2r, b1i, b2i = tr + dr, tr - dr, ti + di, ti - di
    ar = [a_r, b1r * _C1 - b1i * _S1, b2r * _C2 - b2i * _S2]
    ai = [a_i * _C3, b1r * (_C3 * _S1) + b1i * (_C3 * _C1),
          b2r * (_C3 * _S2) + b2i * (_C3 * _C2)]
    t = u0 - 0.5 * u3r
    a0 = [u0 + u3r, t - u3i, t + u3i]
    y = [None] * 9
    for j in range(3):
        t = a0[j] - 0.5 * ar[j]
        y[j] = a0[j] + ar[j]
        y[j + 3] = t - ai[j]
        y[j + 6] = t + ai[j]
    return y


def _bfly4(x, inverse):
    (ar, ai), (br, bi), (cr, ci), (dr, di) = x
    pr, pi, qr, qi = ar + cr, ai + ci, ar - cr, ai - ci
    sr, si, tr, ti = br + dr, bi + di, br - dr, bi - di
    y1, y3 = (qr + ti, qi - tr), (qr - ti, qi + tr)
    if inverse:
        y1, y3 = y3, y1
    return [(pr + sr, pi + si), y1, (pr - sr, pi - si), y3]


def _twiddle16(z, e, inverse):
    zr, zi = z
    e = (-e if inverse else e) % 16
    h = float(np.sqrt(0.5))
    if e == 0:
        return z
    if e == 4:
        return zi, -zr
    if e == 12:
        return -zi, zr
    if e == 2:
        return (zr + zi) * h, (zi - zr) * h
    if e == 14:
        return (zr - zi) * h, (zr + zi) * h
    if e == 6:
        return (zi - zr) * h, (zr + zi) * (-h)
    if e == 10:
        return (zr + zi) * (-h), (zr - zi) * h
    c, s = float(np.cos(2 * np.pi * e / 16)), float(np.sin(2 * np.pi * e / 16))
    return zr * c + zi * s, zi * c - zr * s


_GROUPS = (1, 2, 3, 4, 0)


def _group_classes(g):
    return sorted({g, g + 9, 9 - g, 18 - g}) if g else [0, 9]


_ROWGROUPS = [(k0, h) for g in _GROUPS for k0 in _group_classes(g) for h in range(2)]


def _to_words(m):
    u = np.ascontiguousarray(m, dtype=np.float32).view(np.uint32)
    u = (u + 0x7FFF + ((u >> 16) & 1)) >> 16
    return (u[0::2] | (u[1::2] << 16)).astype(np.uint32)


def _coordinates(a, v):
    rhs = [np.sum(row * v) for row in a]
    if len(a) == 1:
        return [rhs[0] / np.sum(a[0] * a[0])]
    g00, g01, g11 = np.sum(a[0] * a[0]), np.sum(a[0] * a[1]), np.sum(a[1] * a[1])
    det = g00 * g11 - g01 * g01
    return [(g11 * rhs[0] - g01 * rhs[1]) / det, (g00 * rhs[1] - g01 * rhs[0]) / det]


def _make_tables():
    basis = np.array(_bfly9_fwd(list(np.eye(9))))
    m_fwd = np.array([2 * (r % 32) + r // 32 for r in range(64)])
    lf, li = [], []
    for g in _GROUPS:
        rows = [k0 + 18 * i for k0 in _group_classes(g) for i in range(16)]
        if g == 0:
            rows += [DF - 1] + [-1] * 7
        cols = [2 * g - 1, 2 * g] if g else [0]
        a = basis[cols]
        n = len(rows)
        f = np.zeros((2 * n, 128))
        b = np.zeros((64 * len(cols), 128))
        for r, k in enumerate(rows):
            if k < 0:
                continue
            ck = np.exp(-2j * np.pi * ((np.arange(9) * k) % 9) / 9)
            lam = _coordinates(a, ck)
            wk = (1.0 if k in (0, DF - 1) else 2.0) / (S * D)
            for c in range(len(cols)):
                e = lam[c] * np.exp(-2j * np.pi * ((m_fwd * k) % D) / D)
                f[r, 64 * c:64 * c + 64] = e.real
                f[n + r, 64 * c:64 * c + 64] = e.imag
                e = wk * lam[c] * np.exp(-2j * np.pi * ((np.arange(64) * k) % D) / D)
                b[64 * c:64 * c + 64, r] = e.real
                b[64 * c:64 * c + 64, n + r] = e.imag
        lf.append(_to_words(f))
        li.append(_to_words(b))
    n = np.arange(128)
    b_of_n = 16 * (n // 16) + 8 * (n % 2) + (n % 16) // 2
    f128 = np.exp(-2j * np.pi * (np.outer(b_of_n, n) % 128) / 128)
    tw = np.exp(-2j * np.pi * np.outer(np.arange(16), n) / S)
    f32w = lambda m: np.ascontiguousarray(m, dtype=np.float32).view(np.uint32)
    parts = [f32w(f128.real), f32w(f128.imag), f32w(tw.real), f32w(tw.imag)] + lf + li
    offs = np.cumsum([0] + [p.shape[0] for p in parts])
    parts.append(np.zeros((-offs[-1] % 32, 128), np.uint32))
    return np.concatenate(parts, axis=0), [int(o) for o in offs]


_TABLE, _OFF = _make_tables()
_OFF_FR, _OFF_FI, _OFF_TR, _OFF_TI = _OFF[0:4]
_OFF_LF = _OFF[4:10]
_OFF_LI = _OFF[9:15]
_ZERO = np.array([0, 5, 3], np.int32)


def _pack(lo, hi):
    return pltpu.pack_elementwise([lo, hi], packed_dtype=BF16)


def _unpack(w, index):
    return pltpu.unpack_elementwise(w, index=index, packed_dtype=BF16, unpacked_dtype=F32)


def _bf(words):
    return pltpu.bitcast(words, BF16)


def _dot(a, b):
    return lax.dot_general(a, b, (((1,), (0,)), ((), ())), preferred_element_type=F32)


def _dot_nt(a, b):
    return lax.dot_general(a, b, (((1,), (1,)), ((), ())), preferred_element_type=F32)


def _zeros_w(rows):
    return jnp.zeros((rows, 128), U32)


class _SideWork:
    LINK = 7.0
    HOP = 6.0

    def __init__(self, zero_ref):
        self.zero_ref = zero_ref
        self.zero = zero_ref[0]

    def start(self, seed, sink):
        self.chain = pltpu.bitcast(seed, F32)
        self.sink = sink
        self.jobs = []
        self.pending = []
        self.regions = 0
        self.credit = self.delay = self.clock = 0.0

    def open(self, stretch=1.0, slack=100.0):
        self.zero = self.zero_ref[0]
        self.lead = -slack
        self.stretch = stretch

    def add(self, name, job, load, first=False):
        self.jobs.insert(0 if first else len(self.jobs), (name, job, load))

    def _tick(self, cycles):
        self.clock += cycles
        self.delay += cycles
        while self.pending and self.pending[0][0] <= self.clock:
            self.chain = self.pending.pop(0)[1] + self.chain
            self.delay -= 2.0
        n = int(self.delay / self.LINK)
        if n >= 4:
            for _ in range(n):
                self.chain = pl.reciprocal(self.chain, approx=True)
            self.delay -= n * self.LINK

    def _step(self):
        item = next(self.jobs[0][1], None)
        if item is None:
            self.jobs.pop(0)
            return
        values, cycles, latency = (item + (0.0,))[:3]
        values = values if isinstance(values, list) else [values]
        values = [pltpu.bitcast(v, F32) for v in values]
        while len(values) > 1:
            values = [values[i] + values[i + 1] if i + 1 < len(values) else values[i]
                      for i in range(0, len(values), 2)]
        self.pending.append((self.clock + latency, values[0]))
        self.pending.sort(key=lambda x: x[0])
        cycles = cycles / self.jobs[0][2]
        self.credit -= cycles
        self.lead += cycles
        while self.lead >= self.HOP:
            self.zero = self.zero_ref[self.zero]
            self.lead -= self.HOP
        self._tick(self.stretch * cycles)

    def run(self, cycles):
        self.credit += cycles
        while self.jobs and self.credit > 0:
            self._step()
        if not self.jobs and self.credit > 0:
            self._tick(self.stretch * self.credit)
            self.credit = 0.0

    def finish(self, name):
        while any(job[0] == name for job in self.jobs):
            self._step()

    def close(self):
        while self.jobs:
            self._step()
        while self.pending:
            self.chain = self.pending.pop(0)[1] + self.chain
        self.sink[pl.ds(8 * self.regions, 8), :] = self.chain
        self.regions += 1
        self.credit = self.delay = 0.0


def _drain(gen):
    for _ in gen:
        pass


_W_COLS = ((0, 512), (512, 640), (1152, 576))


def _kernel(xa_hbm, wqkv_hbm, wo_hbm, xb_hbm, wr_hbm, wi_hbm, tab_hbm, zero_ref, out_hbm,
            tab, xb_raw, xa_raw, xa_rest, wq_raw, wo_raw, wr_raw, wi_raw, wlast,
            gmat, u_t, y_t, u_nat, x1_buf, t_buf, z_buf, x_nat, x_perm, wt_nat, wt_q, wt_k, wt_v,
            wo_nat, wo_perm, wo_tail, q_buf, k_buf, v_buf, o_t, o_nat, out0, a_tail, stage,
            sem_xa, sem_in, sem_out, sem_region):
    side = _SideWork(zero_ref)
    zero = side.zero

    def now(ref):
        return ref.at[side.zero]

    tab_r, wr_r, wi_r = tab, wr_raw, wi_raw
    tab, wr_raw, wi_raw = tab.at[0], wr_raw.at[0], wi_raw.at[0]
    t_r, wn_r, won_r, q_r, k_r, v_r = t_buf, wt_nat, wo_nat, q_buf, k_buf, v_buf
    (gmat, u_t, y_t, x1_buf, t_buf, z_buf, x_perm, wt_nat, wt_q, wt_k, wt_v, wo_nat, wo_perm,
     wo_tail, q_buf, k_buf, v_buf, o_t, o_nat, out0, a_tail) = jax.tree.map(
        lambda r: r.at[zero],
        (gmat, u_t, y_t, x1_buf, t_buf, z_buf, x_perm, wt_nat, wt_q, wt_k, wt_v, wo_nat, wo_perm,
         wo_tail, q_buf, k_buf, v_buf, o_t, o_nat, out0, a_tail))
    wt = (wt_q, wt_k, wt_v)

    SEM_XB, SEM_TAB, SEM_WQ, SEM_WK, SEM_WV, SEM_WO, SEM_WR, SEM_WI, SEM_LAST = range(9)

    def cp_tab(row0, rows):
        return pltpu.make_async_copy(
            tab_hbm.at[pl.ds(row0, rows)], tab.at[pl.ds(row0, rows)], sem_in.at[SEM_TAB])

    def cp_xb(t):
        return pltpu.make_async_copy(
            xb_hbm.at[:, pl.ds(t * 128, 128)], xb_raw.at[t].bitcast(BF16), sem_in.at[SEM_XB])

    def cp_xa(t):
        return pltpu.make_async_copy(
            xa_hbm.at[pl.ds(0, 256), pl.ds(t * 128, 128)], xa_raw.at[t].bitcast(BF16),
            sem_xa.at[sum(t >= s for s in (6, 11, 14))])

    def cp_xa_rest():
        return pltpu.make_async_copy(xa_hbm.at[pl.ds(256, D - 256)], xa_rest, sem_xa.at[4])

    def cp_wq(part, row0=0, rows=D):
        rows, cols = pl.ds(row0, rows), pl.ds(*_W_COLS[part])
        return pltpu.make_async_copy(
            wqkv_hbm.at[rows, cols], wq_raw.at[rows, cols], sem_in.at[SEM_WQ + part])

    def cp_wo(row0=0, rows=D):
        return pltpu.make_async_copy(
            wo_hbm.at[pl.ds(row0, rows)], wo_raw.at[pl.ds(row0, rows)], sem_in.at[SEM_WO])

    def cp_f(i, t):
        src, dst = ((wr_hbm, wr_raw), (wi_hbm, wi_raw))[i]
        return pltpu.make_async_copy(
            src.at[pl.ds(0, DF - 1), pl.ds(t * 128, 128)], dst.at[t].bitcast(BF16),
            sem_in.at[SEM_WR + i])

    def cp_flast(i):
        src = (wr_hbm, wi_hbm)[i]
        return pltpu.make_async_copy(src.at[pl.ds(DF - 1, 1), :], wlast.at[i], sem_in.at[SEM_LAST])

    def cp_out(ct, row0, rows):
        return pltpu.make_async_copy(
            stage.at[ct, pl.ds(row0, rows), :].bitcast(BF16),
            out_hbm.at[pl.ds(2 * row0, 2 * rows), pl.ds(ct * 128, 128)], sem_out)

    def fetch_xb(t, v):
        xb_raw[t, pl.ds(0, 8), :] = v
        cp_xb(t).start()

    def fetch_wq(part, piece, v):
        wq_raw[pl.ds(144 * piece, 16), pl.ds(_W_COLS[part][0], 128)] = _bf(v)
        cp_wq(part, 144 * piece, 144).start()

    def fetch_wo(piece, v):
        wo_raw[pl.ds(144 * piece, 16), pl.ds(0, 128)] = _bf(v)
        cp_wo(144 * piece, 144).start()

    def wo_settle(v):
        wo_raw[pl.ds(D, 16), pl.ds(0, 128)] = _bf(v)

    def fetch_tab(row0, rows, v):
        tab[pl.ds(row0, 8), :] = v
        cp_tab(row0, rows).start()

    def fetch_f(t, v):
        wr_raw[t, pl.ds(0, 8), :] = v
        cp_f(0, t).start()
        wi_raw[t, pl.ds(0, 8), :] = v
        cp_f(1, t).start()
        if t == 0:
            cp_flast(0).start()
            cp_flast(1).start()

    n_tab = _TABLE.shape[0]
    fetches = []

    def fetch_next(value):
        if fetches:
            for fetch in fetches.pop(0):
                fetch(pltpu.bitcast(value[:8, :128], U32))

    def store_pitched(dst, row0, vt):
        for r in range(16):
            dst[pl.ds(row0 + 17 * (r // 2) + 8 * (r % 2), 8), :] = vt[8 * r:8 * r + 8]

    def radix9(tau):
        for i in range(4):
            words = [[xb_raw[side.zero + 2 * tau + z, pl.ds(32 * j + 8 * i, 8), :]
                      for j in range(9)] for z in range(2)]
            for e in range(2):
                u = []
                for z in range(2):
                    u.append(_bfly9_fwd([_unpack(w, e) for w in words[z]]))
                    yield u[z][8], 14
                out = [_pack(u[0][o], u[1][o]) for o in range(9)]
                for o in range(9):
                    u_t[tau, pl.ds(64 * o + 32 * e + 8 * i, 8), :] = out[o]
                yield out, 5

    def u_to_token_major(gi, cost):
        g = _GROUPS[gi]
        for tau in range(8):
            if g:
                v = u_t[tau, pl.ds(64 * (2 * g - 1), 128), :]
            else:
                v = jnp.concatenate([u_t[tau, pl.ds(0, 64), :], _zeros_w(64)], axis=0)
            vt = v.T
            store_pitched(u_nat.at[gi], 136 * tau, vt)
            yield vt[120:], cost, 240

    def dft_matrix(a):
        twr = jnp.broadcast_to(pltpu.bitcast(tab[pl.ds(_OFF_TR + a, 1), :], F32), (8, 128))
        twi = jnp.broadcast_to(pltpu.bitcast(tab[pl.ds(_OFF_TI + a, 1), :], F32), (8, 128))
        for i in range(16):
            fr = pltpu.bitcast(now(tab_r)[pl.ds(_OFF_FR + 8 * i, 8), :], F32)
            fi = pltpu.bitcast(now(tab_r)[pl.ds(_OFF_FI + 8 * i, 8), :], F32)
            gr, gi = fr * twr - fi * twi, fr * twi + fi * twr
            gmat[a, 0, pl.ds(8 * i, 8), :] = gr
            out = [gr + gi, gi - gr]
            gmat[a, 1, pl.ds(8 * i, 8), :] = out[0]
            gmat[a, 2, pl.ds(8 * i, 8), :] = out[1]
            yield out, 3

    def filter_rows(row0, load_w):
        rows = pl.ds(row0, 8)
        y = [[None] * 4 for _ in range(4)]
        for a0 in range(4):
            src = now(t_r)
            z = _bfly4([(src[4 * a1 + a0, 0, rows, :], src[4 * a1 + a0, 1, rows, :])
                        for a1 in range(4)], False)
            for g0 in range(4):
                y[g0][a0] = _twiddle16(z[g0], a0 * g0, False)
            yield y[3][a0][0], 7
        for g0 in range(4):
            z = _bfly4(y[g0], False)
            yield z[3][1], 4
            for g1 in range(4):
                wr, wi = load_w(g0 + 4 * g1)
                zr, zi = z[g1]
                z[g1] = (zr * wr - zi * wi, zr * wi + zi * wr)
                if g1 % 2:
                    yield z[g1][1], 4
            z = _bfly4(z, True)
            for a0 in range(4):
                y[g0][a0] = _twiddle16(z[a0], a0 * g0, True)
            yield y[g0][3][0], 6
        for a0 in range(4):
            z = _bfly4([y[g0][a0] for g0 in range(4)], True)
            for a1 in range(4):
                t_buf[4 * a1 + a0, 0, rows, :] = z[a1][0]
                t_buf[4 * a1 + a0, 1, rows, :] = z[a1][1]
            yield [v for pair in z for v in pair], 6

    def filter_all():
        for n, (k0, h) in enumerate(_ROWGROUPS):
            rows = pl.ds(k0 // 2 + 72 * h, 8, stride=9)
            yield from filter_rows(8 * n, lambda f1: (
                _unpack(now(wr_r)[f1, rows, :], k0 % 2),
                _unpack(now(wi_r)[f1, rows, :], k0 % 2)))
        yield from filter_rows(NR - 8, lambda f1: tuple(
            jnp.broadcast_to(wlast[i, :, pl.ds(128 * f1, 128)].astype(F32), (8, 128))
            for i in range(2)))

    def radix9_inv(c):
        for i in range(8):
            y = []
            for e in range(2):
                y.append(_bfly9_inv(
                    [now(t_r)[2 * c + e, i // 4, pl.ds(256 + 8 * (i % 4), 8), :]]
                    + [now(t_r)[2 * c + e, o % 2, pl.ds(64 * (o // 2) + 8 * i, 8), :]
                       for o in range(8)]))
                yield y[e][8], 12
            out = [_pack(y[0][j], y[1][j]) for j in range(9)]
            for j in range(9):
                y_t[c, pl.ds(64 * j + 8 * i, 8), :] = out[j]
            yield out, 5

    def y_to_token_major(c, cost):
        for q in range(4):
            vt = y_t[c, pl.ds(64 + 128 * q, 128), :].T
            stage[5 + q, pl.ds(c, 128, stride=8), :] = vt
            yield vt[120:], cost, 240

    def seam_to_token_major(c):
        top = _pack(a_tail[0, c], a_tail[1, c])
        stage[4, pl.ds(c, 128, stride=8), :] = jnp.concatenate(
            [top, y_t[c, pl.ds(0, 64), :]], axis=0).T

    def wo_tail_prep():
        for kt in range(5):
            vt = pltpu.bitcast(_bf(wo_perm[4, pl.ds(64 * kt, 64), :]).T, U32)
            wo_tail[kt] = vt[:32]
            yield vt[24:32], 22, 180

    def x_to_token_major(t, qs):
        lanes = pl.ds(128 * t, 128)
        for q in qs:
            if q == 0:
                v = xa_raw[t]
            elif q == 1:
                v = pltpu.bitcast(xa_rest[pl.ds(0, 256), lanes], U32)
            else:
                v = pltpu.bitcast(xa_rest[pl.ds(256, 64), lanes], U32)
                v = jnp.concatenate([v, _zeros_w(96)], axis=0)
            store_pitched(x_nat.at[q], 136 * t, v.T)

    def x_tile(a, qs):
        for q in qs:
            vt = x_nat[q, pl.ds(a, 128, stride=17), :].T
            n = 128 if q < 2 else 64
            x_perm[q][a] = vt[:n]
            yield vt[n - 8:n], 43, 240

    def w_prep(part, kts=range(5)):
        col0, _ = _W_COLS[part]
        first = 288 * part - col0 // 2
        for kt in kts:
            for nt in range(5):
                nn = min(128, 3 * D - col0 - 128 * nt)
                vt = wq_raw[pl.ds(128 * kt, 128), pl.ds(col0 + 128 * nt, nn)].T
                vt = pltpu.bitcast(vt, U32)
                wt_nat[kt, pl.ds(64 * nt, nn // 2), :] = vt
                yield vt[-8:], 22, 180
        for kt in kts:
            for i in range(2):
                for dl in range(9):
                    base = first + 144 * i + dl
                    wa = now(wn_r)[kt, pl.ds(base, 8, stride=18), :]
                    wb = now(wn_r)[kt, pl.ds(base + 9, 8, stride=18), :]
                    out = [_pack(_unpack(wa, e), _unpack(wb, e)) for e in range(2)]
                    for e in range(2):
                        wt[part][kt, pl.ds(16 * (2 * dl + e) + 8 * i, 8), :] = out[e]
                    yield out, 2

    def wo_prep():
        for nt in range(5):
            nn = min(128, D - 128 * nt)
            blk = wo_raw[pl.ds(0, D), pl.ds(128 * nt, nn)]
            if nn < 128:
                blk = jnp.concatenate([blk, jnp.zeros((D, 128 - nn), BF16)], axis=1)
            blk = pltpu.bitcast(blk, U32)
            wo_nat[nt] = blk
            wo_perm[nt, pl.ds(288, 32), :] = _zeros_w(32)
            yield blk[-8:], 20
            for i in range(2):
                for dl in range(9):
                    wa = now(won_r)[nt, pl.ds(144 * i + dl, 8, stride=18), :]
                    wb = now(won_r)[nt, pl.ds(144 * i + dl + 9, 8, stride=18), :]
                    out = [_pack(_unpack(wa, e), _unpack(wb, e)) for e in range(2)]
                    for e in range(2):
                        wo_perm[nt, pl.ds(16 * (2 * dl + e) + 8 * i, 8), :] = out[e]
                    yield out, 2

    scale = float(DH) ** -0.5
    d_block = 6

    def attend(p, units):
        lane0 = lax.broadcasted_iota(jnp.int32, (8, 128), 1) == 0
        for unit in units:
            gam, hg = divmod(unit, 4)
            base = 2 * gam + 1
            acc = [[None] * W for _ in range(2)]
            for d0 in range(0, DH, d_block):
                rows = [pl.ds(144 * hg + 8 * d, 8) for d in range(d0, d0 + d_block)]
                q = [[now(q_r[4 * p + gam])[e, r, :] for r in rows] for e in range(2)]
                for l in range(9):
                    for n, r in enumerate(rows):
                        k = now(k_r[p])[base + l, r, :]
                        for e in range(2):
                            w = 7 + e - l
                            if 0 <= w < W:
                                t = q[e][n] * k
                                acc[e][w] = t if acc[e][w] is None else acc[e][w] + t
                    done = [acc[e][7 + e - l] for e in range(2) if 0 <= 7 + e - l < W]
                    yield done, d_block / 2 * len(done)
            prob = []
            for e in range(2):
                lg = [jnp.where(lane0, -1e9 / scale, acc[e][w]) if 2 * gam + e < w else acc[e][w]
                      for w in range(W)]
                m = lg[0]
                for w in range(1, W):
                    m = jnp.maximum(m, lg[w])
                ex = [jnp.exp2((l_ - m) * (scale * float(np.log2(np.e)))) for l_ in lg]
                tot = ex[0]
                for w in range(1, W):
                    tot = tot + ex[w]
                inv = 1.0 / tot
                prob.append([x_ * inv for x_ in ex])
                yield prob[e][W - 1], 13, 30
            for d in range(DH):
                rows = pl.ds(32 * d + 8 * hg, 8)
                vv = [now(v_r[p])[base + l, pl.ds(144 * hg + 8 * d, 8), :] for l in range(9)]
                o = []
                for e in range(2):
                    t = prob[e][0] * vv[7 + e]
                    for w in range(1, W):
                        t = t + prob[e][w] * vv[7 + e - w]
                    o.append(t)
                word = _pack(o[0], o[1])
                o_t[p][gam, rows, :] = word
                yield word, 8

    def o_to_token_major(p, cost):
        for gam in range(4):
            for kt in range(5):
                if kt < 4:
                    v = o_t[p][gam, pl.ds(128 * kt, 128), :]
                else:
                    v = jnp.concatenate([o_t[p][gam, pl.ds(512, 64), :], _zeros_w(64)], axis=0)
                vt = v.T
                o_nat[p][kt, pl.ds(gam, 128, stride=4), :] = vt
                yield vt[120:], cost, 240

    def table(off, i):
        return _bf(tab[pl.ds(off[i], off[i + 1] - off[i]), :])

    def dft64(a, gi):
        x1 = _dot_nt(table(_OFF_LF, gi), _bf(u_nat[gi, pl.ds(a, 64, stride=17), :]))
        n = x1.shape[0] // 2
        side.run(n / 2)
        x1_buf[a, 0, pl.ds(64 * gi, n), :] = x1[:n]
        x1_buf[a, 1, pl.ds(64 * gi, n), :] = x1[n:]
        if a % 4 == 3:
            fetch_next(x1)

    def dft128(a):
        side.run(222)
        xr, xi = x1_buf[a, 0], x1_buf[a, 1]
        k1 = _dot(xr + xi, gmat[a, 0])
        t_buf[a, 0] = k1 - _dot(xi, gmat[a, 1])
        t_buf[a, 1] = k1 + _dot(xr, gmat[a, 2])

    def idft128(a):
        side.run(222)
        g = [jnp.concatenate([gmat[a, c, pl.ds(16 * tau + e, 8, stride=2), :]
                              for tau in range(8) for e in range(2)], axis=0) for c in range(3)]
        tr, ti = t_buf[a, 0], t_buf[a, 1]
        k1 = _dot_nt(tr + ti, g[0])
        z_buf[a % 2, 0] = k1 + _dot_nt(ti, g[2])
        z_buf[a % 2, 1] = k1 - _dot_nt(tr, g[1])

    def idft64(a):
        side.run(144)
        for gi in range(5):
            n = 64 if gi < 4 else NR - 256
            parts = [z_buf[a % 2, c, pl.ds(64 * gi, n), :] for c in range(2)]
            if n < 64:
                parts.append(jnp.zeros((128 - 2 * n, 128), F32))
            o = _dot(table(_OFF_LI, gi), jnp.concatenate(parts, axis=0))
            if gi < 4:
                t_buf[a, 0, pl.ds(64 * gi, 64), :] = o[:64]
                t_buf[a, 1, pl.ds(64 * gi, 64), :] = o[64:]
            else:
                t_buf[a, 0, pl.ds(256, 32), :] = o[:32]
                t_buf[a, 1, pl.ds(256, 32), :] = o[32:]

    def proj(part, p, gam, qs=(0, 1, 2), chunks=4, only=None):
        a = 4 * gam + p
        m = 288 // chunks
        kts = [kt for q in qs for kt in (2 * q, 2 * q + 1) if kt < 5]
        for ch in only or range(chunks):
            side.run(len(kts) * m)
            w = jnp.concatenate(
                [_bf(wt[part][kt, pl.ds(m * ch, m), :]) for kt in kts], axis=1)
            x = jnp.concatenate(
                [jnp.concatenate([_bf(x_perm[q][a + 2 * e]) for e in range(2)], axis=1)
                 for q in qs], axis=0)
            r = _dot(w, x)
            for e in range(2):
                c = 2 * gam + e
                buf, slot = (q_buf[4 * p + gam], e) if part == 0 else (
                    (k_buf, v_buf)[part - 1][p], 8 + c)
                rows = []
                for i in range(m // 4):
                    d, hg = divmod(m // 4 * ch + i, 4)
                    rows.append(pl.ds(144 * hg + 8 * d, 8))
                tile = r[:, 128 * e:128 * e + 128]
                if qs[0]:
                    tile = tile + jnp.concatenate([buf[slot, r_, :] for r_ in rows], axis=0)
                shifted = part and c and qs[-1] == 2
                rolled = pltpu.roll(tile, 1, 1) if shifted else None
                for i, r_ in enumerate(rows):
                    buf[slot, r_, :] = tile[8 * i:8 * i + 8]
                    if shifted:
                        buf[c, r_, :] = rolled[8 * i:8 * i + 8]
                        if part == 2:
                            lane0 = lax.broadcasted_iota(jnp.int32, (8, 128), 1) == 0
                            pltpu.store(buf.at[c, r_, :], v_buf[0][8, r_, :], mask=lane0)
            fetch_next(r)

    def out_proj(p, row0, cw):
        side.run(10 * cw)
        lhs = jnp.concatenate([_bf(o_nat[p][kt, pl.ds(row0, cw), :]) for kt in range(5)], axis=1)
        r = _dot(lhs, jnp.concatenate([_bf(wo_perm[nt]) for nt in range(4)], axis=1))
        rows = pl.ds(2 * row0, 2 * cw)
        for ct in range(4):
            tile = r[:, 128 * ct:128 * ct + 128]
            if p == 0:
                out0[ct, rows, :] = tile
            else:
                stage[ct, rows, :] = _pack(out0[ct, rows, :], tile)
                cp_out(ct, 2 * row0, 2 * cw).start()

    def out_tail(p, gam):
        side.run(160)
        words = o_t[p][gam]
        o = jnp.concatenate([_unpack(words, e) for e in range(2)], axis=1)
        o = jnp.concatenate([o, jnp.zeros((64, 256), F32)], axis=0)
        r = _dot(jnp.concatenate([_bf(wo_tail[kt]) for kt in range(5)], axis=1), o)
        for e in range(2):
            a_tail[p, 2 * gam + e] = r[:, 128 * e:128 * e + 128]

    cp_wq(1, 0, 256).start()
    for t in range(8):
        cp_xa(t).start()
    wq_raw[pl.ds(D, 64), :] = jnp.zeros((64, 3 * D), BF16)
    cp_wq(1, 0, 256).wait()
    _drain(w_prep(1, range(2)))
    for t0, t1 in ((0, 6), (6, 11), (11, 14), (14, 16)):
        if t0 == 0:
            for t in range(8, 16):
                cp_xa(t).start()
        elif t0 == 6:
            cp_wq(1, 256, D - 256).start()
        elif t0 == 11:
            cp_xa_rest().start()
        for t in range(t0, t1):
            cp_xa(t).wait()
        for t in range(t0, t1):
            x_to_token_major(t, (0,))
    _drain(x_tile(0, (0,)))
    _drain(x_tile(2, (0,)))

    side.start(xa_raw[0, pl.ds(0, 8), :], x1_buf.at[16, 0])
    pairs = [(p, gam) for p in range(2) for gam in range(4)]
    unit = 319

    def end_region():
        pl.semaphore_signal(sem_region)
        pl.semaphore_wait(sem_region)

    def pair_tiles(name, n, qs, load, first=False):
        p, gam = pairs[n]
        for e in (1, 0) if first else (0, 1):
            side.add(name, x_tile(4 * gam + p + 2 * e, qs), load, first=first)

    side.open(0.0)
    fetches += [[]] * 3
    fetches += [[partial(fetch_wq, 0, i)] for i in range(4)]
    fetches += [[partial(fetch_xb, t)] for t in range(16)]
    fetches += [[partial(fetch_wq, 2, i) for i in range(4)]]
    fetches += [[partial(fetch_tab, r, min(304, n_tab - r)) for r in range(0, n_tab, 304)]]
    fetches += [[partial(fetch_f, t) for t in range(4)]]
    for n in range(5):
        pair_tiles("next", n + 1, (0,), 0.5, first=True)
        if n < 2:
            pair_tiles("later", n + 6, (0,), 0.5)
        proj(1, *pairs[n], qs=(0,), chunks=2)
        side.finish("next")
    side.close()

    cp_xa_rest().wait()
    cp_wq(1, 256, D - 256).wait()
    side.open(0.0)
    for n in range(5, 8):
        proj(1, *pairs[n], qs=(0,), chunks=2)
    for q in (1, 2):
        for t in range(16):
            x_to_token_major(t, (q,))
        for n in range(2):
            pair_tiles("next", n, (q,), 0.6)
        side.add("next", w_prep(1, (2, 3) if q == 1 else (4,)), 0.6)
        if q == 2:
            pair_tiles("next", 2, (1, 2), 0.6)
        side.finish("next")
        for n in range(2):
            proj(1, *pairs[n], qs=(q,), chunks=2)
    for n in range(2, 5):
        pair_tiles("next", n + 1, (1, 2), 0.6)
        proj(1, *pairs[n], qs=(1, 2), chunks=3)
        side.finish("next")
    side.close()

    assert not fetches
    pltpu.make_async_copy(xb_raw, xb_raw, sem_in.at[SEM_XB]).wait()
    cp_wq(0).wait()
    side.open(0.9, 300.0)
    load = (8 * 264 + 2 * 172 + 730) / 4752
    side.add("w", w_prep(0), load)
    for tau in range(8):
        side.add("r9", radix9(tau), load)
    for n in range(5, 8):
        if n < 7:
            pair_tiles("next", n + 1, (1, 2), load, first=True)
        proj(1, *pairs[n], qs=(1, 2), chunks=3)
        side.finish("next")
    side.finish("w")
    proj(0, 0, 0)
    proj(0, 0, 1, only=(0, 1))
    side.close()

    cp_tab(0, n_tab).wait()
    cp_wq(2).wait()
    side.open(0.75)
    fetches += [[partial(fetch_f, t)] for t in range(4, 16)]
    fetches += [[partial(fetch_wo, i)] for i in range(4)]
    fetches.append([wo_settle])
    side.add("t", u_to_token_major(0, 43), 1.0)
    for a in range(16):
        side.add("g%d" % a, dft_matrix(a), 0.3)
    proj(0, 0, 1, only=(2, 3))
    side.finish("t")
    for gi in range(5):
        if gi < 4:
            side.add("t", u_to_token_major(gi + 1, 43), 1.0, first=True)
        for a in range(16):
            dft64(a, gi)
        side.finish("t")
    side.add("w", w_prep(2), 0.5)
    for a in range(16):
        side.finish("g%d" % a)
        dft128(a)
    side.close()

    assert not fetches
    pltpu.make_async_copy(wr_raw, wr_raw, sem_in.at[SEM_WR]).wait()
    pltpu.make_async_copy(wi_raw, wi_raw, sem_in.at[SEM_WI]).wait()
    cp_flast(0).wait()
    cp_flast(1).wait()
    cp_wo().wait()
    side.open(0.95, 400.0)
    load = (37 * 120 + 280) / 8640
    side.add("f", filter_all(), load)
    side.add("wo", wo_prep(), load)
    for gam in range(4):
        proj(2, 0, gam, chunks=1)
    proj(0, 0, 2, chunks=1)
    proj(0, 0, 3, chunks=1)
    side.close()
    end_region()

    side.open()
    side.add("att", attend(0, range(8)), 8 * unit / 5856)
    idft128(0)
    for a in range(16):
        if a < 15:
            idft128(a + 1)
        idft64(a)
    side.close()
    end_region()

    side.open()
    load = (8 * unit + 8 * 232) / 7200
    side.add("att", attend(0, range(8, 16)), load)
    for c in range(8):
        side.add("r9", radix9_inv(c), load)
    for gam in range(4):
        proj(2, 1, gam, chunks=2)
    proj(0, 1, 0, chunks=2)
    side.close()
    end_region()

    side.open()
    tc = 34.0
    side.add("att", attend(1, range(4)), 4 * unit / (4320 - 52 * tc))
    side.add("o", o_to_token_major(0, tc), 1.0)
    for c in range(8):
        side.add("y", y_to_token_major(c, tc), 1.0)
    side.add("y", wo_tail_prep(), 1.0)
    for gam in range(1, 4):
        proj(0, 1, gam, chunks=1)
    side.close()
    for ct in range(5, 9):
        cp_out(ct, 0, S // 2).start()
    end_region()

    side.open()
    side.add("att", attend(1, range(4, 16)), 12 * unit / 5120)
    for row0 in range(0, 512, 64):
        out_proj(0, row0, 64)
    side.close()
    end_region()

    side.open(0.0)
    for p, gam in pairs:
        out_tail(p, gam)
    _drain(o_to_token_major(1, 0))
    for c in range(8):
        seam_to_token_major(c)
    cp_out(4, 0, S // 2).start()
    row0 = 0
    for cw in (16, 32, 64, 128, 128, 64, 32, 32, 16):
        out_proj(1, row0, cw)
        row0 += cw
    pltpu.make_async_copy(out_hbm, out_hbm, sem_out).wait()


@jax.jit
def pallas_concat_heads__sliding_local_dilated__spectral_gfnet__prompt_kernel(
    A_x: jax.Array,
    A_wqkv: jax.Array,
    A_wo: jax.Array,
    B_x: jax.Array,
    B_w_r: jax.Array,
    B_w_i: jax.Array,
):
    assert A_x.shape == (1, S, D) and B_x.shape == (1, S, D)
    any_spec = pl.BlockSpec(memory_space=pl.ANY)
    scratch = [
        pltpu.VMEM((1,) + _TABLE.shape, U32),
        pltpu.VMEM((16, 288, 128), U32),
        pltpu.VMEM((16, 128, 128), U32),
        pltpu.VMEM((D - 256, S), BF16),
        pltpu.VMEM((D + 64, 3 * D), BF16),
        pltpu.VMEM((D + 64, D), BF16),
        pltpu.VMEM((1, 16, 144, 128), U32),
        pltpu.VMEM((1, 16, 144, 128), U32),
        pltpu.VMEM((2, 1, S), BF16),
        pltpu.VMEM((1, 16, 3, 128, 128), F32),
        pltpu.VMEM((1, 8, D, 128), U32),
        pltpu.VMEM((1, 8, D, 128), U32),
        pltpu.VMEM((5, 8 * 136, 128), U32),
        pltpu.VMEM((1, 18, 2, NR, 128), F32),
        pltpu.VMEM((1, 16, 2, NR, 128), F32),
        pltpu.VMEM((1, 2, 2, NR, 128), F32),
        pltpu.VMEM((3, 16 * 136, 128), U32),
        [pltpu.VMEM((1, 16, n, 128), U32) for n in (128, 128, 64)],
        pltpu.VMEM((1, 5, 320, 128), U32),
        pltpu.VMEM((1, 5, 288, 128), U32),
        pltpu.VMEM((1, 5, 288, 128), U32),
        pltpu.VMEM((1, 5, 288, 128), U32),
        pltpu.VMEM((1, 5, 288, 128), U32),
        pltpu.VMEM((1, 5, 320, 128), U32),
        pltpu.VMEM((1, 5, 32, 128), U32),
        [pltpu.VMEM((1, 2, D + 16, 128), F32)] * 8,
        [pltpu.VMEM((1, 16, D + 8, 128), F32)] * 2,
        [pltpu.VMEM((1, 16, D + 8, 128), F32)] * 2,
        [pltpu.VMEM((1, 4, D, 128), U32)] * 2,
        [pltpu.VMEM((1, 5, 512, 128), U32)] * 2,
        pltpu.VMEM((1, 4, S // 2, 128), F32),
        pltpu.VMEM((1, 2, 8, 64, 128), F32),
        pltpu.VMEM((9, S // 2, 128), U32),
        pltpu.SemaphoreType.DMA((5,)),
        pltpu.SemaphoreType.DMA((9,)),
        pltpu.SemaphoreType.DMA(()),
        pltpu.SemaphoreType.REGULAR,
    ]
    out = pl.pallas_call(
        _kernel,
        out_shape=jax.ShapeDtypeStruct((S, 2 * D), BF16),
        in_specs=[any_spec] * 7 + [pl.BlockSpec(memory_space=pltpu.SMEM)],
        out_specs=any_spec,
        scratch_shapes=scratch,
        compiler_params=pltpu.CompilerParams(vmem_limit_bytes=120 * 1024 * 1024),
        name="attn_gfnet",
    )(A_x[0].T, A_wqkv, A_wo, B_x[0].T, B_w_r.T, B_w_i.T, _TABLE, _ZERO)
    return out[None]
```

```python
from functools import partial

import numpy as np

import jax
import jax.numpy as jnp
from jax import lax
import jax.experimental.pallas as pl
import jax.experimental.pallas.tpu as pltpu

S = 2048
D = 576
H = 32
DH = 18
W = 8
DF = D // 2 + 1
NR = 296

F32 = jnp.float32
BF16 = jnp.bfloat16
U32 = jnp.uint32

_C3 = float(np.sqrt(3.0) / 2)
_C1, _S1 = float(np.cos(2 * np.pi / 9)), float(np.sin(2 * np.pi / 9))
_C2, _S2 = float(np.cos(4 * np.pi / 9)), float(np.sin(4 * np.pi / 9))


def _bfly9_fwd(x):
    a0, ar, ai = [], [], []
    for j in range(3):
        t = x[j + 3] + x[j + 6]
        a0.append(x[j] + t)
        ar.append(x[j] - 0.5 * t)
        ai.append(x[j + 6] - x[j + 3])
    t = a0[1] + a0[2]
    u0 = a0[0] + t
    u3r = a0[0] - 0.5 * t
    u3i = a0[2] - a0[1]
    b1r = ar[1] * _C1 + ai[1] * (_C3 * _S1)
    b1i = ai[1] * (_C3 * _C1) - ar[1] * _S1
    b2r = ar[2] * _C2 + ai[2] * (_C3 * _S2)
    b2i = ai[2] * (_C3 * _C2) - ar[2] * _S2
    a_r, a_i = ar[0], ai[0] * _C3
    tr, ti = b1r + b2r, b1i + b2i
    dr, di = (b1r - b2r) * _C3, (b1i - b2i) * _C3
    u1r, u1i = a_r + tr, a_i + ti
    mr, mi = a_r - 0.5 * tr, a_i - 0.5 * ti
    return [u0, u1r, u1i, mr - di, mi + dr, u3r, u3i, mr + di, mi - dr]


def _bfly9_inv(v):
    u0, u1r, u1i, u7r, u7i, u3r, u3i, u4r, u4i = v
    mr, mi = u4r + u7r, u4i + u7i
    di, dr = (u4r - u7r) * _C3, (u7i - u4i) * _C3
    a_r, a_i = u1r + mr, u1i + mi
    tr, ti = u1r - 0.5 * mr, u1i - 0.5 * mi
    b1r, b2r, b1i, b2i = tr + dr, tr - dr, ti + di, ti - di
    ar = [a_r, b1r * _C1 - b1i * _S1, b2r * _C2 - b2i * _S2]
    ai = [a_i * _C3, b1r * (_C3 * _S1) + b1i * (_C3 * _C1),
          b2r * (_C3 * _S2) + b2i * (_C3 * _C2)]
    t = u0 - 0.5 * u3r
    a0 = [u0 + u3r, t - u3i, t + u3i]
    y = [None] * 9
    for j in range(3):
        t = a0[j] - 0.5 * ar[j]
        y[j] = a0[j] + ar[j]
        y[j + 3] = t - ai[j]
        y[j + 6] = t + ai[j]
    return y


def _bfly4(x, inverse):
    (ar, ai), (br, bi), (cr, ci), (dr, di) = x
    pr, pi, qr, qi = ar + cr, ai + ci, ar - cr, ai - ci
    sr, si, tr, ti = br + dr, bi + di, br - dr, bi - di
    y1, y3 = (qr + ti, qi - tr), (qr - ti, qi + tr)
    if inverse:
        y1, y3 = y3, y1
    return [(pr + sr, pi + si), y1, (pr - sr, pi - si), y3]


def _twiddle16(z, e, inverse):
    zr, zi = z
    e = (-e if inverse else e) % 16
    h = float(np.sqrt(0.5))
    if e == 0:
        return z
    if e == 4:
        return zi, -zr
    if e == 12:
        return -zi, zr
    if e == 2:
        return (zr + zi) * h, (zi - zr) * h
    if e == 14:
        return (zr - zi) * h, (zr + zi) * h
    if e == 6:
        return (zi - zr) * h, (zr + zi) * (-h)
    if e == 10:
        return (zr + zi) * (-h), (zr - zi) * h
    c, s = float(np.cos(2 * np.pi * e / 16)), float(np.sin(2 * np.pi * e / 16))
    return zr * c + zi * s, zi * c - zr * s


_GROUPS = (1, 2, 3, 4, 0)


def _group_classes(g):
    return sorted({g, g + 9, 9 - g, 18 - g}) if g else [0, 9]


_ROWGROUPS = [(k0, h) for g in _GROUPS for k0 in _group_classes(g) for h in range(2)]


def _to_words(m):
    u = np.ascontiguousarray(m, dtype=np.float32).view(np.uint32)
    u = (u + 0x7FFF + ((u >> 16) & 1)) >> 16
    return (u[0::2] | (u[1::2] << 16)).astype(np.uint32)


def _coordinates(a, v):
    rhs = [np.sum(row * v) for row in a]
    if len(a) == 1:
        return [rhs[0] / np.sum(a[0] * a[0])]
    g00, g01, g11 = np.sum(a[0] * a[0]), np.sum(a[0] * a[1]), np.sum(a[1] * a[1])
    det = g00 * g11 - g01 * g01
    return [(g11 * rhs[0] - g01 * rhs[1]) / det, (g00 * rhs[1] - g01 * rhs[0]) / det]


def _make_tables():
    basis = np.array(_bfly9_fwd(list(np.eye(9))))
    m_fwd = np.array([2 * (r % 32) + r // 32 for r in range(64)])
    lf, li = [], []
    for g in _GROUPS:
        rows = [k0 + 18 * i for k0 in _group_classes(g) for i in range(16)]
        if g == 0:
            rows += [DF - 1] + [-1] * 7
        cols = [2 * g - 1, 2 * g] if g else [0]
        a = basis[cols]
        n = len(rows)
        f = np.zeros((2 * n, 128))
        b = np.zeros((64 * len(cols), 128))
        for r, k in enumerate(rows):
            if k < 0:
                continue
            ck = np.exp(-2j * np.pi * ((np.arange(9) * k) % 9) / 9)
            lam = _coordinates(a, ck)
            wk = (1.0 if k in (0, DF - 1) else 2.0) / (S * D)
            for c in range(len(cols)):
                e = lam[c] * np.exp(-2j * np.pi * ((m_fwd * k) % D) / D)
                f[r, 64 * c:64 * c + 64] = e.real
                f[n + r, 64 * c:64 * c + 64] = e.imag
                e = wk * lam[c] * np.exp(-2j * np.pi * ((np.arange(64) * k) % D) / D)
                b[64 * c:64 * c + 64, r] = e.real
                b[64 * c:64 * c + 64, n + r] = e.imag
        lf.append(_to_words(f))
        li.append(_to_words(b))
    n = np.arange(128)
    b_of_n = 16 * (n // 16) + 8 * (n % 2) + (n % 16) // 2
    f128 = np.exp(-2j * np.pi * (np.outer(b_of_n, n) % 128) / 128)
    tw = np.exp(-2j * np.pi * np.outer(np.arange(16), n) / S)
    f32w = lambda m: np.ascontiguousarray(m, dtype=np.float32).view(np.uint32)
    parts = [f32w(f128.real), f32w(f128.imag), f32w(tw.real), f32w(tw.imag)] + lf + li
    offs = np.cumsum([0] + [p.shape[0] for p in parts])
    parts.append(np.zeros((-offs[-1] % 32, 128), np.uint32))
    return np.concatenate(parts, axis=0), [int(o) for o in offs]


_TABLE, _OFF = _make_tables()
_OFF_FR, _OFF_FI, _OFF_TR, _OFF_TI = _OFF[0:4]
_OFF_LF = _OFF[4:10]
_OFF_LI = _OFF[9:15]
_ZERO = np.array([0, 5, 3], np.int32)


def _pack(lo, hi):
    return pltpu.pack_elementwise([lo, hi], packed_dtype=BF16)


def _unpack(w, index):
    return pltpu.unpack_elementwise(w, index=index, packed_dtype=BF16, unpacked_dtype=F32)


def _bf(words):
    return pltpu.bitcast(words, BF16)


def _dot(a, b):
    return lax.dot_general(a, b, (((1,), (0,)), ((), ())), preferred_element_type=F32)


def _dot_nt(a, b):
    return lax.dot_general(a, b, (((1,), (1,)), ((), ())), preferred_element_type=F32)


def _zeros_w(rows):
    return jnp.zeros((rows, 128), U32)


class _SideWork:
    LINK = 7.0
    HOP = 6.0

    def __init__(self, zero_ref):
        self.zero_ref = zero_ref
        self.zero = zero_ref[0]

    def start(self, seed, sink):
        self.chain = pltpu.bitcast(seed, F32)
        self.sink = sink
        self.jobs = []
        self.pending = []
        self.regions = 0
        self.credit = self.delay = self.clock = 0.0

    def open(self, stretch=1.0, slack=100.0, links=4):
        self.links = links
        self.zero = self.zero_ref[0]
        self.lead = -slack
        self.stretch = stretch

    def add(self, name, job, load, first=False):
        self.jobs.insert(0 if first else len(self.jobs), (name, job, load))

    def _tick(self, cycles):
        self.clock += cycles
        self.delay += cycles
        while self.pending and self.pending[0][0] <= self.clock:
            self.chain = self.pending.pop(0)[1] + self.chain
            self.delay -= 2.0
        n = int(self.delay / self.LINK)
        if n >= self.links:
            for _ in range(n):
                self.chain = pl.reciprocal(self.chain, approx=True)
            self.delay -= n * self.LINK

    def _step(self):
        item = next(self.jobs[0][1], None)
        if item is None:
            self.jobs.pop(0)
            return
        values, cycles, latency = (item + (0.0,))[:3]
        values = values if isinstance(values, list) else [values]
        values = [pltpu.bitcast(v, F32) for v in values]
        while len(values) > 1:
            values = [values[i] + values[i + 1] if i + 1 < len(values) else values[i]
                      for i in range(0, len(values), 2)]
        self.pending.append((self.clock + latency, values[0]))
        self.pending.sort(key=lambda x: x[0])
        cycles = cycles / self.jobs[0][2]
        self.credit -= cycles
        self.lead += cycles
        while self.lead >= self.HOP:
            self.zero = self.zero_ref[self.zero]
            self.lead -= self.HOP
        self._tick(self.stretch * cycles)

    def run(self, cycles):
        self.credit += cycles
        while self.jobs and self.credit > 0:
            self._step()
        if not self.jobs and self.credit > 0:
            self._tick(self.stretch * self.credit)
            self.credit = 0.0

    def finish(self, name):
        while any(job[0] == name for job in self.jobs):
            self._step()

    def close(self):
        while self.jobs:
            self._step()
        while self.pending:
            self.chain = self.pending.pop(0)[1] + self.chain
        self.sink[pl.ds(8 * self.regions, 8), :] = self.chain
        self.regions += 1
        self.credit = self.delay = 0.0


def _drain(gen):
    for _ in gen:
        pass


_W_COLS = ((0, 512), (512, 640), (1152, 576))


def _kernel(xa_hbm, wqkv_hbm, wo_hbm, xb_hbm, wr_hbm, wi_hbm, tab_hbm, zero_ref, out_hbm,
            tab, xb_raw, xa_raw, xa_rest, wq_raw, wo_raw, wr_raw, wi_raw, wlast,
            gmat, u_t, y_t, u_nat, x1_buf, t_buf, z_buf, x_nat, x_perm, wt_nat, wt_q, wt_k, wt_v,
            wo_nat, wo_perm, wo_tail, q_buf, k_buf, v_buf, o_t, o_nat, out0, a_tail, stage,
            sem_xa, sem_in, sem_out, sem_region):
    side = _SideWork(zero_ref)
    zero = side.zero

    def now(ref):
        return ref.at[side.zero]

    tab_r, wr_r, wi_r = tab, wr_raw, wi_raw
    tab, wr_raw, wi_raw = tab.at[0], wr_raw.at[0], wi_raw.at[0]
    t_r, wn_r, won_r, q_r, k_r, v_r = t_buf, wt_nat, wo_nat, q_buf, k_buf, v_buf
    (gmat, u_t, y_t, x1_buf, t_buf, z_buf, x_perm, wt_nat, wt_q, wt_k, wt_v, wo_nat, wo_perm,
     wo_tail, q_buf, k_buf, v_buf, o_t, o_nat, out0, a_tail) = jax.tree.map(
        lambda r: r.at[zero],
        (gmat, u_t, y_t, x1_buf, t_buf, z_buf, x_perm, wt_nat, wt_q, wt_k, wt_v, wo_nat, wo_perm,
         wo_tail, q_buf, k_buf, v_buf, o_t, o_nat, out0, a_tail))
    wt = (wt_q, wt_k, wt_v)

    SEM_XB, SEM_TAB, SEM_WQ, SEM_WK, SEM_WV, SEM_WO, SEM_WR, SEM_WI, SEM_LAST = range(9)

    def cp_tab(row0, rows):
        return pltpu.make_async_copy(
            tab_hbm.at[pl.ds(row0, rows)], tab.at[pl.ds(row0, rows)], sem_in.at[SEM_TAB])

    def cp_xb(t):
        return pltpu.make_async_copy(
            xb_hbm.at[:, pl.ds(t * 128, 128)], xb_raw.at[t].bitcast(BF16), sem_in.at[SEM_XB])

    def cp_xa(t):
        return pltpu.make_async_copy(
            xa_hbm.at[pl.ds(0, 256), pl.ds(t * 128, 128)], xa_raw.at[t].bitcast(BF16),
            sem_xa.at[sum(t >= s for s in (6, 11, 14))])

    def cp_xa_rest():
        return pltpu.make_async_copy(xa_hbm.at[pl.ds(256, D - 256)], xa_rest, sem_xa.at[4])

    def cp_wq(part, row0=0, rows=D):
        rows, cols = pl.ds(row0, rows), pl.ds(*_W_COLS[part])
        return pltpu.make_async_copy(
            wqkv_hbm.at[rows, cols], wq_raw.at[rows, cols], sem_in.at[SEM_WQ + part])

    def cp_wo(row0=0, rows=D):
        return pltpu.make_async_copy(
            wo_hbm.at[pl.ds(row0, rows)], wo_raw.at[pl.ds(row0, rows)], sem_in.at[SEM_WO])

    def cp_f(i, t):
        src, dst = ((wr_hbm, wr_raw), (wi_hbm, wi_raw))[i]
        return pltpu.make_async_copy(
            src.at[pl.ds(0, DF - 1), pl.ds(t * 128, 128)], dst.at[t].bitcast(BF16),
            sem_in.at[SEM_WR + i])

    def cp_flast(i):
        src = (wr_hbm, wi_hbm)[i]
        return pltpu.make_async_copy(src.at[pl.ds(DF - 1, 1), :], wlast.at[i], sem_in.at[SEM_LAST])

    def cp_out(ct, row0, rows):
        return pltpu.make_async_copy(
            stage.at[ct, pl.ds(row0, rows), :].bitcast(BF16),
            out_hbm.at[pl.ds(2 * row0, 2 * rows), pl.ds(ct * 128, 128)], sem_out)

    def fetch_xb(t, v):
        xb_raw[t, pl.ds(0, 8), :] = v
        cp_xb(t).start()

    def fetch_wq(part, piece, v):
        wq_raw[pl.ds(144 * piece, 16), pl.ds(_W_COLS[part][0], 128)] = _bf(v)
        cp_wq(part, 144 * piece, 144).start()

    def fetch_wo(piece, v):
        wo_raw[pl.ds(144 * piece, 16), pl.ds(0, 128)] = _bf(v)
        cp_wo(144 * piece, 144).start()

    def wo_settle(v):
        wo_raw[pl.ds(D, 16), pl.ds(0, 128)] = _bf(v)

    def fetch_tab(row0, rows, v):
        tab[pl.ds(row0, 8), :] = v
        cp_tab(row0, rows).start()

    def fetch_f(t, v):
        wr_raw[t, pl.ds(0, 8), :] = v
        cp_f(0, t).start()
        wi_raw[t, pl.ds(0, 8), :] = v
        cp_f(1, t).start()
        if t == 0:
            cp_flast(0).start()
            cp_flast(1).start()

    n_tab = _TABLE.shape[0]
    fetches = []

    def fetch_next(value):
        if fetches:
            for fetch in fetches.pop(0):
                fetch(pltpu.bitcast(value[:8, :128], U32))

    def store_pitched(dst, row0, vt):
        for r in range(16):
            dst[pl.ds(row0 + 17 * (r // 2) + 8 * (r % 2), 8), :] = vt[8 * r:8 * r + 8]

    def radix9(tau):
        for i in range(4):
            words = [[xb_raw[side.zero + 2 * tau + z, pl.ds(32 * j + 8 * i, 8), :]
                      for j in range(9)] for z in range(2)]
            for e in range(2):
                u = []
                for z in range(2):
                    u.append(_bfly9_fwd([_unpack(w, e) for w in words[z]]))
                    yield u[z][8], 14
                out = [_pack(u[0][o], u[1][o]) for o in range(9)]
                for o in range(9):
                    u_t[tau, pl.ds(64 * o + 32 * e + 8 * i, 8), :] = out[o]
                yield out, 5

    def u_to_token_major(gi, cost):
        g = _GROUPS[gi]
        for tau in range(8):
            if g:
                v = u_t[tau, pl.ds(64 * (2 * g - 1), 128), :]
            else:
                v = jnp.concatenate([u_t[tau, pl.ds(0, 64), :], _zeros_w(64)], axis=0)
            vt = v.T
            store_pitched(u_nat.at[gi], 136 * tau, vt)
            yield vt[120:], cost, 240

    def dft_matrix(a):
        twr = jnp.broadcast_to(pltpu.bitcast(tab[pl.ds(_OFF_TR + a, 1), :], F32), (8, 128))
        twi = jnp.broadcast_to(pltpu.bitcast(tab[pl.ds(_OFF_TI + a, 1), :], F32), (8, 128))
        for i in range(16):
            fr = pltpu.bitcast(now(tab_r)[pl.ds(_OFF_FR + 8 * i, 8), :], F32)
            fi = pltpu.bitcast(now(tab_r)[pl.ds(_OFF_FI + 8 * i, 8), :], F32)
            gr, gi = fr * twr - fi * twi, fr * twi + fi * twr
            gmat[a, 0, pl.ds(8 * i, 8), :] = gr
            out = [gr + gi, gi - gr]
            gmat[a, 1, pl.ds(8 * i, 8), :] = out[0]
            gmat[a, 2, pl.ds(8 * i, 8), :] = out[1]
            yield out, 3

    def filter_rows(row0, load_w):
        rows = pl.ds(row0, 8)
        y = [[None] * 4 for _ in range(4)]
        for a0 in range(4):
            src = now(t_r)
            z = _bfly4([(src[4 * a1 + a0, 0, rows, :], src[4 * a1 + a0, 1, rows, :])
                        for a1 in range(4)], False)
            for g0 in range(4):
                y[g0][a0] = _twiddle16(z[g0], a0 * g0, False)
            yield y[3][a0][0], 7
        for g0 in range(4):
            z = _bfly4(y[g0], False)
            yield z[3][1], 4
            for g1 in range(4):
                wr, wi = load_w(g0 + 4 * g1)
                zr, zi = z[g1]
                z[g1] = (zr * wr - zi * wi, zr * wi + zi * wr)
                if g1 % 2:
                    yield z[g1][1], 4
            z = _bfly4(z, True)
            for a0 in range(4):
                y[g0][a0] = _twiddle16(z[a0], a0 * g0, True)
            yield y[g0][3][0], 6
        for a0 in range(4):
            z = _bfly4([y[g0][a0] for g0 in range(4)], True)
            for a1 in range(4):
                t_buf[4 * a1 + a0, 0, rows, :] = z[a1][0]
                t_buf[4 * a1 + a0, 1, rows, :] = z[a1][1]
            yield [v for pair in z for v in pair], 6

    def filter_all():
        for n, (k0, h) in enumerate(_ROWGROUPS):
            rows = pl.ds(k0 // 2 + 72 * h, 8, stride=9)
            yield from filter_rows(8 * n, lambda f1: (
                _unpack(now(wr_r)[f1, rows, :], k0 % 2),
                _unpack(now(wi_r)[f1, rows, :], k0 % 2)))
        yield from filter_rows(NR - 8, lambda f1: tuple(
            jnp.broadcast_to(wlast[i, :, pl.ds(128 * f1, 128)].astype(F32), (8, 128))
            for i in range(2)))

    def radix9_inv(c):
        for i in range(8):
            y = []
            for e in range(2):
                y.append(_bfly9_inv(
                    [now(t_r)[2 * c + e, i // 4, pl.ds(256 + 8 * (i % 4), 8), :]]
                    + [now(t_r)[2 * c + e, o % 2, pl.ds(64 * (o // 2) + 8 * i, 8), :]
                       for o in range(8)]))
                yield y[e][8], 12
            out = [_pack(y[0][j], y[1][j]) for j in range(9)]
            for j in range(9):
                y_t[c, pl.ds(64 * j + 8 * i, 8), :] = out[j]
            yield out, 5

    def y_to_token_major(c, cost):
        for q in range(4):
            vt = y_t[c, pl.ds(64 + 128 * q, 128), :].T
            stage[5 + q, pl.ds(c, 128, stride=8), :] = vt
            yield vt[120:], cost, 240

    def seam_to_token_major(c):
        top = _pack(a_tail[0, c], a_tail[1, c])
        stage[4, pl.ds(c, 128, stride=8), :] = jnp.concatenate(
            [top, y_t[c, pl.ds(0, 64), :]], axis=0).T

    def wo_tail_prep():
        for kt in range(5):
            vt = pltpu.bitcast(_bf(wo_perm[4, pl.ds(64 * kt, 64), :]).T, U32)
            wo_tail[kt] = vt[:32]
            yield vt[24:32], 22, 180

    def x_to_token_major(t, qs):
        lanes = pl.ds(128 * t, 128)
        for q in qs:
            if q == 0:
                v = xa_raw[t]
            elif q == 1:
                v = pltpu.bitcast(xa_rest[pl.ds(0, 256), lanes], U32)
            else:
                v = pltpu.bitcast(xa_rest[pl.ds(256, 64), lanes], U32)
                v = jnp.concatenate([v, _zeros_w(96)], axis=0)
            store_pitched(x_nat.at[q], 136 * t, v.T)

    def x_tile(a, qs):
        for q in qs:
            vt = x_nat[q, pl.ds(a, 128, stride=17), :].T
            n = 128 if q < 2 else 64
            x_perm[q][a] = vt[:n]
            yield vt[n - 8:n], 43, 240

    def w_prep(part, kts=range(5)):
        col0, _ = _W_COLS[part]
        first = 288 * part - col0 // 2
        for kt in kts:
            for nt in range(5):
                nn = min(128, 3 * D - col0 - 128 * nt)
                vt = wq_raw[pl.ds(128 * kt, 128), pl.ds(col0 + 128 * nt, nn)].T
                vt = pltpu.bitcast(vt, U32)
                wt_nat[kt, pl.ds(64 * nt, nn // 2), :] = vt
                yield vt[-8:], 22, 180
        for kt in kts:
            for i in range(2):
                for dl in range(9):
                    base = first + 144 * i + dl
                    wa = now(wn_r)[kt, pl.ds(base, 8, stride=18), :]
                    wb = now(wn_r)[kt, pl.ds(base + 9, 8, stride=18), :]
                    out = [_pack(_unpack(wa, e), _unpack(wb, e)) for e in range(2)]
                    for e in range(2):
                        wt[part][kt, pl.ds(16 * (2 * dl + e) + 8 * i, 8), :] = out[e]
                    yield out, 2

    def wo_prep():
        for nt in range(5):
            nn = min(128, D - 128 * nt)
            blk = wo_raw[pl.ds(0, D), pl.ds(128 * nt, nn)]
            if nn < 128:
                blk = jnp.concatenate([blk, jnp.zeros((D, 128 - nn), BF16)], axis=1)
            blk = pltpu.bitcast(blk, U32)
            wo_nat[nt] = blk
            wo_perm[nt, pl.ds(288, 32), :] = _zeros_w(32)
            yield blk[-8:], 20
            for i in range(2):
                for dl in range(9):
                    wa = now(won_r)[nt, pl.ds(144 * i + dl, 8, stride=18), :]
                    wb = now(won_r)[nt, pl.ds(144 * i + dl + 9, 8, stride=18), :]
                    out = [_pack(_unpack(wa, e), _unpack(wb, e)) for e in range(2)]
                    for e in range(2):
                        wo_perm[nt, pl.ds(16 * (2 * dl + e) + 8 * i, 8), :] = out[e]
                    yield out, 2

    scale = float(DH) ** -0.5

    def attend(p, units, d_block=6):
        lane0 = lax.broadcasted_iota(jnp.int32, (8, 128), 1) == 0
        for unit in units:
            gam, hg = divmod(unit, 4)
            base = 2 * gam + 1
            acc = [[None] * W for _ in range(2)]
            for d0 in range(0, DH, d_block):
                rows = [pl.ds(144 * hg + 8 * d, 8) for d in range(d0, d0 + d_block)]
                q = [[now(q_r[4 * p + gam])[e, r, :] for r in rows] for e in range(2)]
                for l in range(9):
                    for n, r in enumerate(rows):
                        k = now(k_r[p])[base + l, r, :]
                        for e in range(2):
                            w = 7 + e - l
                            if 0 <= w < W:
                                t = q[e][n] * k
                                acc[e][w] = t if acc[e][w] is None else acc[e][w] + t
                    done = [acc[e][7 + e - l] for e in range(2) if 0 <= 7 + e - l < W]
                    yield done, d_block / 2 * len(done)
            prob = []
            for e in range(2):
                lg = [jnp.where(lane0, -1e9 / scale, acc[e][w]) if 2 * gam + e < w else acc[e][w]
                      for w in range(W)]
                m = lg[0]
                for w in range(1, W):
                    m = jnp.maximum(m, lg[w])
                ex = [jnp.exp2((l_ - m) * (scale * float(np.log2(np.e)))) for l_ in lg]
                tot = ex[0]
                for w in range(1, W):
                    tot = tot + ex[w]
                inv = 1.0 / tot
                prob.append([x_ * inv for x_ in ex])
                yield prob[e][W - 1], 13, 30
            for d in range(DH):
                rows = pl.ds(32 * d + 8 * hg, 8)
                vv = [now(v_r[p])[base + l, pl.ds(144 * hg + 8 * d, 8), :] for l in range(9)]
                o = []
                for e in range(2):
                    t = prob[e][0] * vv[7 + e]
                    for w in range(1, W):
                        t = t + prob[e][w] * vv[7 + e - w]
                    o.append(t)
                word = _pack(o[0], o[1])
                o_t[p][gam, rows, :] = word
                yield word, 8

    def o_to_token_major(p, cost):
        for gam in range(4):
            for kt in range(5):
                if kt < 4:
                    v = o_t[p][gam, pl.ds(128 * kt, 128), :]
                else:
                    v = jnp.concatenate([o_t[p][gam, pl.ds(512, 64), :], _zeros_w(64)], axis=0)
                vt = v.T
                o_nat[p][kt, pl.ds(gam, 128, stride=4), :] = vt
                yield vt[120:], cost, 240

    def table(off, i):
        return _bf(tab[pl.ds(off[i], off[i + 1] - off[i]), :])

    def dft64(a, gi):
        x1 = _dot_nt(table(_OFF_LF, gi), _bf(u_nat[gi, pl.ds(a, 64, stride=17), :]))
        n = x1.shape[0] // 2
        side.run(n / 2)
        x1_buf[a, 0, pl.ds(64 * gi, n), :] = x1[:n]
        x1_buf[a, 1, pl.ds(64 * gi, n), :] = x1[n:]
        if a % 4 == 3:
            fetch_next(x1)

    def dft128(a):
        side.run(222)
        xr, xi = x1_buf[a, 0], x1_buf[a, 1]
        k1 = _dot(xr + xi, gmat[a, 0])
        t_buf[a, 0] = k1 - _dot(xi, gmat[a, 1])
        t_buf[a, 1] = k1 + _dot(xr, gmat[a, 2])

    def idft128(a):
        side.run(222)
        g = [jnp.concatenate([gmat[a, c, pl.ds(16 * tau + e, 8, stride=2), :]
                              for tau in range(8) for e in range(2)], axis=0) for c in range(3)]
        tr, ti = t_buf[a, 0], t_buf[a, 1]
        k1 = _dot_nt(tr + ti, g[0])
        z_buf[a % 2, 0] = k1 + _dot_nt(ti, g[2])
        z_buf[a % 2, 1] = k1 - _dot_nt(tr, g[1])

    def idft64(a):
        side.run(144)
        for gi in range(5):
            n = 64 if gi < 4 else NR - 256
            parts = [z_buf[a % 2, c, pl.ds(64 * gi, n), :] for c in range(2)]
            if n < 64:
                parts.append(jnp.zeros((128 - 2 * n, 128), F32))
            o = _dot(table(_OFF_LI, gi), jnp.concatenate(parts, axis=0))
            if gi < 4:
                t_buf[a, 0, pl.ds(64 * gi, 64), :] = o[:64]
                t_buf[a, 1, pl.ds(64 * gi, 64), :] = o[64:]
            else:
                t_buf[a, 0, pl.ds(256, 32), :] = o[:32]
                t_buf[a, 1, pl.ds(256, 32), :] = o[32:]

    def proj(part, p, gam, qs=(0, 1, 2), chunks=4, only=None):
        a = 4 * gam + p
        m = 288 // chunks
        kts = [kt for q in qs for kt in (2 * q, 2 * q + 1) if kt < 5]
        for ch in only or range(chunks):
            side.run(len(kts) * m)
            w = jnp.concatenate(
                [_bf(wt[part][kt, pl.ds(m * ch, m), :]) for kt in kts], axis=1)
            x = jnp.concatenate(
                [jnp.concatenate([_bf(x_perm[q][a + 2 * e]) for e in range(2)], axis=1)
                 for q in qs], axis=0)
            r = _dot(w, x)
            for e in range(2):
                c = 2 * gam + e
                buf, slot = (q_buf[4 * p + gam], e) if part == 0 else (
                    (k_buf, v_buf)[part - 1][p], 8 + c)
                rows = []
                for i in range(m // 4):
                    d, hg = divmod(m // 4 * ch + i, 4)
                    rows.append(pl.ds(144 * hg + 8 * d, 8))
                tile = r[:, 128 * e:128 * e + 128]
                if qs[0]:
                    tile = tile + jnp.concatenate([buf[slot, r_, :] for r_ in rows], axis=0)
                shifted = part and c and qs[-1] == 2
                rolled = pltpu.roll(tile, 1, 1) if shifted else None
                for i, r_ in enumerate(rows):
                    buf[slot, r_, :] = tile[8 * i:8 * i + 8]
                    if shifted:
                        buf[c, r_, :] = rolled[8 * i:8 * i + 8]
                        if part == 2:
                            lane0 = lax.broadcasted_iota(jnp.int32, (8, 128), 1) == 0
                            pltpu.store(buf.at[c, r_, :], v_buf[0][8, r_, :], mask=lane0)
            fetch_next(r)

    def out_proj(p, row0, cw):
        side.run(10 * cw)
        lhs = jnp.concatenate([_bf(o_nat[p][kt, pl.ds(row0, cw), :]) for kt in range(5)], axis=1)
        r = _dot(lhs, jnp.concatenate([_bf(wo_perm[nt]) for nt in range(4)], axis=1))
        rows = pl.ds(2 * row0, 2 * cw)
        for ct in range(4):
            tile = r[:, 128 * ct:128 * ct + 128]
            if p == 0:
                out0[ct, rows, :] = tile
            else:
                stage[ct, rows, :] = _pack(out0[ct, rows, :], tile)
                cp_out(ct, 2 * row0, 2 * cw).start()

    def out_tail(p, gam):
        side.run(160)
        words = o_t[p][gam]
        o = jnp.concatenate([_unpack(words, e) for e in range(2)], axis=1)
        o = jnp.concatenate([o, jnp.zeros((64, 256), F32)], axis=0)
        r = _dot(jnp.concatenate([_bf(wo_tail[kt]) for kt in range(5)], axis=1), o)
        for e in range(2):
            a_tail[p, 2 * gam + e] = r[:, 128 * e:128 * e + 128]

    cp_wq(1, 0, 256).start()
    for t in range(8):
        cp_xa(t).start()
    wq_raw[pl.ds(D, 64), :] = jnp.zeros((64, 3 * D), BF16)
    cp_wq(1, 0, 256).wait()
    _drain(w_prep(1, range(2)))
    for t0, t1 in ((0, 6), (6, 11), (11, 14), (14, 16)):
        if t0 == 0:
            for t in range(8, 16):
                cp_xa(t).start()
        elif t0 == 6:
            cp_wq(1, 256, D - 256).start()
        elif t0 == 11:
            cp_xa_rest().start()
        for t in range(t0, t1):
            cp_xa(t).wait()
        for t in range(t0, t1):
            x_to_token_major(t, (0,))
    _drain(x_tile(0, (0,)))
    _drain(x_tile(2, (0,)))

    side.start(xa_raw[0, pl.ds(0, 8), :], x1_buf.at[16, 0])
    pairs = [(p, gam) for p in range(2) for gam in range(4)]
    unit = 319

    def end_region():
        pl.semaphore_signal(sem_region)
        pl.semaphore_wait(sem_region)

    def pair_tiles(name, n, qs, load, first=False):
        p, gam = pairs[n]
        for e in (1, 0) if first else (0, 1):
            side.add(name, x_tile(4 * gam + p + 2 * e, qs), load, first=first)

    side.open(0.0)
    fetches += [[]] * 3
    fetches += [[partial(fetch_wq, 0, i)] for i in range(4)]
    fetches += [[partial(fetch_xb, t)] for t in range(16)]
    fetches += [[partial(fetch_wq, 2, i) for i in range(4)]]
    fetches += [[partial(fetch_tab, r, min(304, n_tab - r)) for r in range(0, n_tab, 304)]]
    fetches += [[partial(fetch_f, t) for t in range(4)]]
    for n in range(5):
        pair_tiles("next", n + 1, (0,), 0.5, first=True)
        if n < 2:
            pair_tiles("later", n + 6, (0,), 0.5)
        proj(1, *pairs[n], qs=(0,), chunks=2)
        side.finish("next")
    side.close()

    cp_xa_rest().wait()
    cp_wq(1, 256, D - 256).wait()
    side.open(0.0)
    for n in range(5, 8):
        proj(1, *pairs[n], qs=(0,), chunks=2)
    for q in (1, 2):
        for t in range(16):
            x_to_token_major(t, (q,))
        for n in range(2):
            pair_tiles("next", n, (q,), 0.6)
        side.add("next", w_prep(1, (2, 3) if q == 1 else (4,)), 0.6)
        if q == 2:
            pair_tiles("next", 2, (1, 2), 0.6)
        side.finish("next")
        for n in range(2):
            proj(1, *pairs[n], qs=(q,), chunks=2)
    for n in range(2, 5):
        pair_tiles("next", n + 1, (1, 2), 0.6)
        proj(1, *pairs[n], qs=(1, 2))
        side.finish("next")
    side.close()

    assert not fetches
    pltpu.make_async_copy(xb_raw, xb_raw, sem_in.at[SEM_XB]).wait()
    cp_wq(0).wait()
    side.open(0.85, 300.0, links=2)
    load = (8 * 264 + 2 * 172 + 730) / 4752 * 0.9
    side.add("w", w_prep(0), load)
    for tau in range(8):
        side.add("r9", radix9(tau), load)
    for n in range(5, 8):
        if n < 7:
            pair_tiles("next", n + 1, (1, 2), load, first=True)
        proj(1, *pairs[n], qs=(1, 2))
        side.finish("next")
    side.finish("w")
    proj(0, 0, 0, chunks=1)
    proj(0, 0, 1, only=(0, 1))
    side.close()

    cp_tab(0, n_tab).wait()
    cp_wq(2).wait()
    side.open(0.95, links=2)
    fetches += [[partial(fetch_f, t)] for t in range(4, 16)]
    fetches += [[partial(fetch_wo, i)] for i in range(4)]
    fetches.append([wo_settle])
    side.add("t", u_to_token_major(0, 43), 0.9)
    for a in range(16):
        side.add("g%d" % a, dft_matrix(a), 0.3 * 0.9)
    proj(0, 0, 1, only=(2, 3))
    side.finish("t")
    for gi in range(5):
        if gi < 4:
            side.add("t", u_to_token_major(gi + 1, 43), 0.9, first=True)
        for a in range(16):
            dft64(a, gi)
        side.finish("t")
    side.add("w", w_prep(2), 0.5 * 0.9)
    for a in range(16):
        side.finish("g%d" % a)
        dft128(a)
    side.close()

    assert not fetches
    pltpu.make_async_copy(wr_raw, wr_raw, sem_in.at[SEM_WR]).wait()
    pltpu.make_async_copy(wi_raw, wi_raw, sem_in.at[SEM_WI]).wait()
    cp_flast(0).wait()
    cp_flast(1).wait()
    cp_wo().wait()
    side.open(0.95, 400.0)
    load = (37 * 120 + 280) / 8640
    side.add("f", filter_all(), load)
    side.add("wo", wo_prep(), load)
    for gam in range(4):
        proj(2, 0, gam, chunks=2)
    proj(0, 0, 2, chunks=2)
    proj(0, 0, 3, chunks=2)
    side.close()
    end_region()

    side.open(0.95, 50.0, links=2)
    side.add("att", attend(0, range(8)), 8 * unit / 5856)
    idft128(0)
    for a in range(16):
        if a < 15:
            idft128(a + 1)
        idft64(a)
    side.close()
    end_region()

    side.open(0.85, 500.0, links=2)
    load = (8 * unit + 8 * 232) / 7200 * 0.95
    side.add("att", attend(0, range(8, 16)), load)
    for c in range(8):
        side.add("r9", radix9_inv(c), load)
    for gam in range(4):
        proj(2, 1, gam)
    proj(0, 1, 0)
    side.close()
    end_region()

    side.open(0.9)
    tc = 34.0
    side.add("att", attend(1, range(4), 9), 4 * unit / (4320 - 52 * tc) * 1.05)
    side.add("o", o_to_token_major(0, tc), 1.05)
    for c in range(8):
        side.add("y", y_to_token_major(c, tc), 1.05)
    side.add("y", wo_tail_prep(), 1.05)
    for gam in range(1, 4):
        proj(0, 1, gam, chunks=2)
    side.close()
    for ct in range(5, 9):
        cp_out(ct, 0, S // 2).start()
    end_region()

    side.open(1.05, 200.0, links=2)
    side.add("att", attend(1, range(4, 16), 9), 12 * unit / 5120)
    for row0 in range(0, 512, 64):
        out_proj(0, row0, 64)
    side.close()
    end_region()

    side.open(0.0)
    for p, gam in pairs:
        out_tail(p, gam)
    _drain(o_to_token_major(1, 0))
    for c in range(8):
        seam_to_token_major(c)
    cp_out(4, 0, S // 2).start()
    row0 = 0
    for cw in (16, 32, 64, 128, 128, 64, 32, 32, 16):
        out_proj(1, row0, cw)
        row0 += cw
    pltpu.make_async_copy(out_hbm, out_hbm, sem_out).wait()


@jax.jit
def pallas_concat_heads__sliding_local_dilated__spectral_gfnet__prompt_kernel(
    A_x: jax.Array,
    A_wqkv: jax.Array,
    A_wo: jax.Array,
    B_x: jax.Array,
    B_w_r: jax.Array,
    B_w_i: jax.Array,
):
    assert A_x.shape == (1, S, D) and B_x.shape == (1, S, D)
    any_spec = pl.BlockSpec(memory_space=pl.ANY)
    scratch = [
        pltpu.VMEM((1,) + _TABLE.shape, U32),
        pltpu.VMEM((16, 288, 128), U32),
        pltpu.VMEM((16, 128, 128), U32),
        pltpu.VMEM((D - 256, S), BF16),
        pltpu.VMEM((D + 64, 3 * D), BF16),
        pltpu.VMEM((D + 64, D), BF16),
        pltpu.VMEM((1, 16, 144, 128), U32),
        pltpu.VMEM((1, 16, 144, 128), U32),
        pltpu.VMEM((2, 1, S), BF16),
        pltpu.VMEM((1, 16, 3, 128, 128), F32),
        pltpu.VMEM((1, 8, D, 128), U32),
        pltpu.VMEM((1, 8, D, 128), U32),
        pltpu.VMEM((5, 8 * 136, 128), U32),
        pltpu.VMEM((1, 18, 2, NR, 128), F32),
        pltpu.VMEM((1, 16, 2, NR, 128), F32),
        pltpu.VMEM((1, 2, 2, NR, 128), F32),
        pltpu.VMEM((3, 16 * 136, 128), U32),
        [pltpu.VMEM((1, 16, n, 128), U32) for n in (128, 128, 64)],
        pltpu.VMEM((1, 5, 320, 128), U32),
        pltpu.VMEM((1, 5, 288, 128), U32),
        pltpu.VMEM((1, 5, 288, 128), U32),
        pltpu.VMEM((1, 5, 288, 128), U32),
        pltpu.VMEM((1, 5, 288, 128), U32),
        pltpu.VMEM((1, 5, 320, 128), U32),
        pltpu.VMEM((1, 5, 32, 128), U32),
        [pltpu.VMEM((1, 2, D + 16, 128), F32)] * 8,
        [pltpu.VMEM((1, 16, D + 8, 128), F32)] * 2,
        [pltpu.VMEM((1, 16, D + 8, 128), F32)] * 2,
        [pltpu.VMEM((1, 4, D, 128), U32)] * 2,
        [pltpu.VMEM((1, 5, 512, 128), U32)] * 2,
        pltpu.VMEM((1, 4, S // 2, 128), F32),
        pltpu.VMEM((1, 2, 8, 64, 128), F32),
        pltpu.VMEM((9, S // 2, 128), U32),
        pltpu.SemaphoreType.DMA((5,)),
        pltpu.SemaphoreType.DMA((9,)),
        pltpu.SemaphoreType.DMA(()),
        pltpu.SemaphoreType.REGULAR,
    ]
    out = pl.pallas_call(
        _kernel,
        out_shape=jax.ShapeDtypeStruct((S, 2 * D), BF16),
        in_specs=[any_spec] * 7 + [pl.BlockSpec(memory_space=pltpu.SMEM)],
        out_specs=any_spec,
        scratch_shapes=scratch,
        compiler_params=pltpu.CompilerParams(vmem_limit_bytes=120 * 1024 * 1024),
        name="attn_gfnet",
    )(A_x[0].T, A_wqkv, A_wo, B_x[0].T, B_w_r.T, B_w_i.T, _TABLE, _ZERO)
    return out[None]
```

```python
from functools import partial

import numpy as np

import jax
import jax.numpy as jnp
from jax import lax
import jax.experimental.pallas as pl
import jax.experimental.pallas.tpu as pltpu

S = 2048
D = 576
H = 32
DH = 18
W = 8
DF = D // 2 + 1
NR = 296

F32 = jnp.float32
BF16 = jnp.bfloat16
U32 = jnp.uint32

_C3 = float(np.sqrt(3.0) / 2)
_C1, _S1 = float(np.cos(2 * np.pi / 9)), float(np.sin(2 * np.pi / 9))
_C2, _S2 = float(np.cos(4 * np.pi / 9)), float(np.sin(4 * np.pi / 9))


def _bfly9_fwd(x):
    a0, ar, ai = [], [], []
    for j in range(3):
        t = x[j + 3] + x[j + 6]
        a0.append(x[j] + t)
        ar.append(x[j] - 0.5 * t)
        ai.append(x[j + 6] - x[j + 3])
    t = a0[1] + a0[2]
    u0 = a0[0] + t
    u3r = a0[0] - 0.5 * t
    u3i = a0[2] - a0[1]
    b1r = ar[1] * _C1 + ai[1] * (_C3 * _S1)
    b1i = ai[1] * (_C3 * _C1) - ar[1] * _S1
    b2r = ar[2] * _C2 + ai[2] * (_C3 * _S2)
    b2i = ai[2] * (_C3 * _C2) - ar[2] * _S2
    a_r, a_i = ar[0], ai[0] * _C3
    tr, ti = b1r + b2r, b1i + b2i
    dr, di = (b1r - b2r) * _C3, (b1i - b2i) * _C3
    u1r, u1i = a_r + tr, a_i + ti
    mr, mi = a_r - 0.5 * tr, a_i - 0.5 * ti
    return [u0, u1r, u1i, mr - di, mi + dr, u3r, u3i, mr + di, mi - dr]


def _bfly9_inv(v):
    u0, u1r, u1i, u7r, u7i, u3r, u3i, u4r, u4i = v
    mr, mi = u4r + u7r, u4i + u7i
    di, dr = (u4r - u7r) * _C3, (u7i - u4i) * _C3
    a_r, a_i = u1r + mr, u1i + mi
    tr, ti = u1r - 0.5 * mr, u1i - 0.5 * mi
    b1r, b2r, b1i, b2i = tr + dr, tr - dr, ti + di, ti - di
    ar = [a_r, b1r * _C1 - b1i * _S1, b2r * _C2 - b2i * _S2]
    ai = [a_i * _C3, b1r * (_C3 * _S1) + b1i * (_C3 * _C1),
          b2r * (_C3 * _S2) + b2i * (_C3 * _C2)]
    t = u0 - 0.5 * u3r
    a0 = [u0 + u3r, t - u3i, t + u3i]
    y = [None] * 9
    for j in range(3):
        t = a0[j] - 0.5 * ar[j]
        y[j] = a0[j] + ar[j]
        y[j + 3] = t - ai[j]
        y[j + 6] = t + ai[j]
    return y


def _bfly4(x, inverse):
    (ar, ai), (br, bi), (cr, ci), (dr, di) = x
    pr, pi, qr, qi = ar + cr, ai + ci, ar - cr, ai - ci
    sr, si, tr, ti = br + dr, bi + di, br - dr, bi - di
    y1, y3 = (qr + ti, qi - tr), (qr - ti, qi + tr)
    if inverse:
        y1, y3 = y3, y1
    return [(pr + sr, pi + si), y1, (pr - sr, pi - si), y3]


def _twiddle16(z, e, inverse):
    zr, zi = z
    e = (-e if inverse else e) % 16
    h = float(np.sqrt(0.5))
    if e == 0:
        return z
    if e == 4:
        return zi, -zr
    if e == 12:
        return -zi, zr
    if e == 2:
        return (zr + zi) * h, (zi - zr) * h
    if e == 14:
        return (zr - zi) * h, (zr + zi) * h
    if e == 6:
        return (zi - zr) * h, (zr + zi) * (-h)
    if e == 10:
        return (zr + zi) * (-h), (zr - zi) * h
    c, s = float(np.cos(2 * np.pi * e / 16)), float(np.sin(2 * np.pi * e / 16))
    return zr * c + zi * s, zi * c - zr * s


_GROUPS = (1, 2, 3, 4, 0)


def _group_classes(g):
    return sorted({g, g + 9, 9 - g, 18 - g}) if g else [0, 9]


_ROWGROUPS = [(k0, h) for g in _GROUPS for k0 in _group_classes(g) for h in range(2)]


def _to_words(m):
    u = np.ascontiguousarray(m, dtype=np.float32).view(np.uint32)
    u = (u + 0x7FFF + ((u >> 16) & 1)) >> 16
    return (u[0::2] | (u[1::2] << 16)).astype(np.uint32)


def _coordinates(a, v):
    rhs = [np.sum(row * v) for row in a]
    if len(a) == 1:
        return [rhs[0] / np.sum(a[0] * a[0])]
    g00, g01, g11 = np.sum(a[0] * a[0]), np.sum(a[0] * a[1]), np.sum(a[1] * a[1])
    det = g00 * g11 - g01 * g01
    return [(g11 * rhs[0] - g01 * rhs[1]) / det, (g00 * rhs[1] - g01 * rhs[0]) / det]


def _make_tables():
    basis = np.array(_bfly9_fwd(list(np.eye(9))))
    m_fwd = np.array([2 * (r % 32) + r // 32 for r in range(64)])
    lf, li = [], []
    for g in _GROUPS:
        rows = [k0 + 18 * i for k0 in _group_classes(g) for i in range(16)]
        if g == 0:
            rows += [DF - 1] + [-1] * 7
        cols = [2 * g - 1, 2 * g] if g else [0]
        a = basis[cols]
        n = len(rows)
        f = np.zeros((2 * n, 128))
        b = np.zeros((64 * len(cols), 128))
        for r, k in enumerate(rows):
            if k < 0:
                continue
            ck = np.exp(-2j * np.pi * ((np.arange(9) * k) % 9) / 9)
            lam = _coordinates(a, ck)
            wk = (1.0 if k in (0, DF - 1) else 2.0) / (S * D)
            for c in range(len(cols)):
                e = lam[c] * np.exp(-2j * np.pi * ((m_fwd * k) % D) / D)
                f[r, 64 * c:64 * c + 64] = e.real
                f[n + r, 64 * c:64 * c + 64] = e.imag
                e = wk * lam[c] * np.exp(-2j * np.pi * ((np.arange(64) * k) % D) / D)
                b[64 * c:64 * c + 64, r] = e.real
                b[64 * c:64 * c + 64, n + r] = e.imag
        lf.append(_to_words(f))
        li.append(_to_words(b))
    n = np.arange(128)
    b_of_n = 16 * (n // 16) + 8 * (n % 2) + (n % 16) // 2
    f128 = np.exp(-2j * np.pi * (np.outer(b_of_n, n) % 128) / 128)
    tw = np.exp(-2j * np.pi * np.outer(np.arange(16), n) / S)
    f32w = lambda m: np.ascontiguousarray(m, dtype=np.float32).view(np.uint32)
    parts = [f32w(f128.real), f32w(f128.imag), f32w(tw.real), f32w(tw.imag)] + lf + li
    offs = np.cumsum([0] + [p.shape[0] for p in parts])
    parts.append(np.zeros((-offs[-1] % 32, 128), np.uint32))
    return np.concatenate(parts, axis=0), [int(o) for o in offs]


_TABLE, _OFF = _make_tables()
_OFF_FR, _OFF_FI, _OFF_TR, _OFF_TI = _OFF[0:4]
_OFF_LF = _OFF[4:10]
_OFF_LI = _OFF[9:15]
_ZERO = np.array([0, 5, 3], np.int32)


def _pack(lo, hi):
    return pltpu.pack_elementwise([lo, hi], packed_dtype=BF16)


def _unpack(w, index):
    return pltpu.unpack_elementwise(w, index=index, packed_dtype=BF16, unpacked_dtype=F32)


def _bf(words):
    return pltpu.bitcast(words, BF16)


def _dot(a, b):
    return lax.dot_general(a, b, (((1,), (0,)), ((), ())), preferred_element_type=F32)


def _dot_nt(a, b):
    return lax.dot_general(a, b, (((1,), (1,)), ((), ())), preferred_element_type=F32)


def _zeros_w(rows):
    return jnp.zeros((rows, 128), U32)


class _SideWork:
    LINK = 7.0
    HOP = 6.0

    def __init__(self, zero_ref):
        self.zero_ref = zero_ref
        self.zero = zero_ref[0]

    def start(self, seed, sink):
        self.chain = pltpu.bitcast(seed, F32)
        self.sink = sink
        self.jobs = []
        self.paced = []
        self.pending = []
        self.regions = 0
        self.credit = self.delay = self.clock = 0.0

    def open(self, stretch=1.0, slack=100.0, links=4):
        self.links = links
        self.zero = self.zero_ref[0]
        self.lead = -slack
        self.stretch = stretch

    def add(self, name, job, load, first=False):
        self.jobs.insert(0 if first else len(self.jobs), (name, job, load))

    def add_paced(self, name, job, period):
        if not self.paced:
            self.due = self.clock
        self.paced.append((name, job, period))

    def _absorb(self, item):
        values, cycles, latency = (item + (0.0,))[:3]
        values = values if isinstance(values, list) else [values]
        values = [pltpu.bitcast(v, F32) for v in values]
        while len(values) > 1:
            values = [values[i] + values[i + 1] if i + 1 < len(values) else values[i]
                      for i in range(0, len(values), 2)]
        self.pending.append((self.clock + latency, values[0]))
        self.pending.sort(key=lambda x: x[0])
        return cycles

    def _step_paced(self):
        item = next(self.paced[0][1], None)
        if item is None:
            self.paced.pop(0)
        else:
            self._absorb(item)
            self.due += self.stretch * self.paced[0][2]

    def _tick(self, cycles):
        while self.paced and self.due <= self.clock:
            self._step_paced()
        self.clock += cycles
        self.delay += cycles
        while self.pending and self.pending[0][0] <= self.clock:
            self.chain = self.pending.pop(0)[1] + self.chain
            self.delay -= 2.0
        n = int(self.delay / self.LINK)
        if n >= self.links:
            for _ in range(n):
                self.chain = pl.reciprocal(self.chain, approx=True)
            self.delay -= n * self.LINK

    def _step(self):
        item = next(self.jobs[0][1], None)
        if item is None:
            self.jobs.pop(0)
            return
        cycles = self._absorb(item) / self.jobs[0][2]
        self.credit -= cycles
        self.lead += cycles
        while self.lead >= self.HOP:
            self.zero = self.zero_ref[self.zero]
            self.lead -= self.HOP
        self._tick(self.stretch * cycles)

    def run(self, cycles):
        self.credit += cycles
        while self.jobs and self.credit > 0:
            self._step()
        while not self.jobs and self.credit > 0:
            n = min(self.credit, 50.0) if self.paced else self.credit
            self._tick(self.stretch * n)
            self.credit -= n

    def finish(self, name):
        while any(job[0] == name for job in self.jobs):
            self._step()
        while any(job[0] == name for job in self.paced):
            self._step_paced()

    def close(self):
        while self.jobs:
            self._step()
        while self.paced:
            self._step_paced()
        while self.pending:
            self.chain = self.pending.pop(0)[1] + self.chain
        self.sink[pl.ds(8 * self.regions, 8), :] = self.chain
        self.regions += 1
        self.credit = self.delay = 0.0


def _drain(gen):
    for _ in gen:
        pass


_W_COLS = ((0, 512), (512, 640), (1152, 576))


def _kernel(xa_hbm, wqkv_hbm, wo_hbm, xb_hbm, wr_hbm, wi_hbm, tab_hbm, zero_ref, out_hbm,
            tab, xb_raw, xa_raw, xa_rest, wq_raw, wo_raw, wr_raw, wi_raw, wlast,
            gmat, u_t, y_t, u_nat, x1_buf, t_buf, z_buf, x_nat, x_perm, wt_nat, wt_q, wt_k, wt_v,
            wo_nat, wo_perm, wo_tail, q_buf, k_buf, v_buf, o_t, o_nat, out0, a_tail, stage,
            sem_xa, sem_in, sem_out, sem_region):
    side = _SideWork(zero_ref)
    zero = side.zero

    def now(ref):
        return ref.at[side.zero]

    tab_r, wr_r, wi_r = tab, wr_raw, wi_raw
    tab, wr_raw, wi_raw = tab.at[0], wr_raw.at[0], wi_raw.at[0]
    t_r, wn_r, won_r, q_r, k_r, v_r = t_buf, wt_nat, wo_nat, q_buf, k_buf, v_buf
    (gmat, u_t, y_t, x1_buf, t_buf, z_buf, x_perm, wt_nat, wt_q, wt_k, wt_v, wo_nat, wo_perm,
     wo_tail, q_buf, k_buf, v_buf, o_t, o_nat, out0, a_tail) = jax.tree.map(
        lambda r: r.at[zero],
        (gmat, u_t, y_t, x1_buf, t_buf, z_buf, x_perm, wt_nat, wt_q, wt_k, wt_v, wo_nat, wo_perm,
         wo_tail, q_buf, k_buf, v_buf, o_t, o_nat, out0, a_tail))
    wt = (wt_q, wt_k, wt_v)

    SEM_XB, SEM_TAB, SEM_WQ, SEM_WK, SEM_WV, SEM_WO, SEM_WR, SEM_WI, SEM_LAST = range(9)

    def cp_tab(row0, rows):
        return pltpu.make_async_copy(
            tab_hbm.at[pl.ds(row0, rows)], tab.at[pl.ds(row0, rows)], sem_in.at[SEM_TAB])

    def cp_xb(t):
        return pltpu.make_async_copy(
            xb_hbm.at[:, pl.ds(t * 128, 128)], xb_raw.at[t].bitcast(BF16), sem_in.at[SEM_XB])

    def cp_xa(t):
        return pltpu.make_async_copy(
            xa_hbm.at[pl.ds(0, 256), pl.ds(t * 128, 128)], xa_raw.at[t].bitcast(BF16),
            sem_xa.at[sum(t >= s for s in (6, 11, 14))])

    def cp_xa_rest():
        return pltpu.make_async_copy(xa_hbm.at[pl.ds(256, D - 256)], xa_rest, sem_xa.at[4])

    def cp_wq(part, row0=0, rows=D):
        rows, cols = pl.ds(row0, rows), pl.ds(*_W_COLS[part])
        return pltpu.make_async_copy(
            wqkv_hbm.at[rows, cols], wq_raw.at[rows, cols], sem_in.at[SEM_WQ + part])

    def cp_wo(row0=0, rows=D):
        return pltpu.make_async_copy(
            wo_hbm.at[pl.ds(row0, rows)], wo_raw.at[pl.ds(row0, rows)], sem_in.at[SEM_WO])

    def cp_f(i, t):
        src, dst = ((wr_hbm, wr_raw), (wi_hbm, wi_raw))[i]
        return pltpu.make_async_copy(
            src.at[pl.ds(0, DF - 1), pl.ds(t * 128, 128)], dst.at[t].bitcast(BF16),
            sem_in.at[SEM_WR + i])

    def cp_flast(i):
        src = (wr_hbm, wi_hbm)[i]
        return pltpu.make_async_copy(src.at[pl.ds(DF - 1, 1), :], wlast.at[i], sem_in.at[SEM_LAST])

    def cp_out(ct, row0, rows):
        return pltpu.make_async_copy(
            stage.at[ct, pl.ds(row0, rows), :].bitcast(BF16),
            out_hbm.at[pl.ds(2 * row0, 2 * rows), pl.ds(ct * 128, 128)], sem_out)

    def fetch_xb(t, v):
        xb_raw[t, pl.ds(0, 8), :] = v
        cp_xb(t).start()

    def fetch_wq(part, piece, v):
        wq_raw[pl.ds(144 * piece, 16), pl.ds(_W_COLS[part][0], 128)] = _bf(v)
        cp_wq(part, 144 * piece, 144).start()

    def fetch_wo(piece, v):
        wo_raw[pl.ds(144 * piece, 16), pl.ds(0, 128)] = _bf(v)
        cp_wo(144 * piece, 144).start()

    def wo_settle(v):
        wo_raw[pl.ds(D, 16), pl.ds(0, 128)] = _bf(v)

    def fetch_tab(row0, rows, v):
        tab[pl.ds(row0, 8), :] = v
        cp_tab(row0, rows).start()

    def fetch_f(t, v):
        wr_raw[t, pl.ds(0, 8), :] = v
        cp_f(0, t).start()
        wi_raw[t, pl.ds(0, 8), :] = v
        cp_f(1, t).start()
        if t == 0:
            cp_flast(0).start()
            cp_flast(1).start()

    n_tab = _TABLE.shape[0]
    fetches = []

    def fetch_next(value):
        if fetches:
            for fetch in fetches.pop(0):
                fetch(pltpu.bitcast(value[:8, :128], U32))

    def store_pitched(dst, row0, vt):
        for r in range(16):
            dst[pl.ds(row0 + 17 * (r // 2) + 8 * (r % 2), 8), :] = vt[8 * r:8 * r + 8]

    def radix9(tau):
        for i in range(4):
            words = [[xb_raw[side.zero + 2 * tau + z, pl.ds(32 * j + 8 * i, 8), :]
                      for j in range(9)] for z in range(2)]
            for e in range(2):
                u = []
                for z in range(2):
                    u.append(_bfly9_fwd([_unpack(w, e) for w in words[z]]))
                    yield u[z][8], 14
                out = [_pack(u[0][o], u[1][o]) for o in range(9)]
                for o in range(9):
                    u_t[tau, pl.ds(64 * o + 32 * e + 8 * i, 8), :] = out[o]
                yield out, 5

    def u_to_token_major(gi, cost):
        g = _GROUPS[gi]
        for tau in range(8):
            if g:
                v = u_t[tau, pl.ds(64 * (2 * g - 1), 128), :]
            else:
                v = jnp.concatenate([u_t[tau, pl.ds(0, 64), :], _zeros_w(64)], axis=0)
            vt = v.T
            store_pitched(u_nat.at[gi], 136 * tau, vt)
            yield vt[120:], cost, 240

    def dft_matrix(a):
        twr = jnp.broadcast_to(pltpu.bitcast(tab[pl.ds(_OFF_TR + a, 1), :], F32), (8, 128))
        twi = jnp.broadcast_to(pltpu.bitcast(tab[pl.ds(_OFF_TI + a, 1), :], F32), (8, 128))
        for i in range(16):
            fr = pltpu.bitcast(now(tab_r)[pl.ds(_OFF_FR + 8 * i, 8), :], F32)
            fi = pltpu.bitcast(now(tab_r)[pl.ds(_OFF_FI + 8 * i, 8), :], F32)
            gr, gi = fr * twr - fi * twi, fr * twi + fi * twr
            gmat[a, 0, pl.ds(8 * i, 8), :] = gr
            out = [gr + gi, gi - gr]
            gmat[a, 1, pl.ds(8 * i, 8), :] = out[0]
            gmat[a, 2, pl.ds(8 * i, 8), :] = out[1]
            yield out, 3

    def filter_rows(row0, load_w):
        rows = pl.ds(row0, 8)
        y = [[None] * 4 for _ in range(4)]
        for a0 in range(4):
            src = now(t_r)
            z = _bfly4([(src[4 * a1 + a0, 0, rows, :], src[4 * a1 + a0, 1, rows, :])
                        for a1 in range(4)], False)
            for g0 in range(4):
                y[g0][a0] = _twiddle16(z[g0], a0 * g0, False)
            yield y[3][a0][0], 7
        for g0 in range(4):
            z = _bfly4(y[g0], False)
            yield z[3][1], 4
            for g1 in range(4):
                wr, wi = load_w(g0 + 4 * g1)
                zr, zi = z[g1]
                z[g1] = (zr * wr - zi * wi, zr * wi + zi * wr)
                if g1 % 2:
                    yield z[g1][1], 4
            z = _bfly4(z, True)
            for a0 in range(4):
                y[g0][a0] = _twiddle16(z[a0], a0 * g0, True)
            yield y[g0][3][0], 6
        for a0 in range(4):
            z = _bfly4([y[g0][a0] for g0 in range(4)], True)
            for a1 in range(4):
                t_buf[4 * a1 + a0, 0, rows, :] = z[a1][0]
                t_buf[4 * a1 + a0, 1, rows, :] = z[a1][1]
            yield [v for pair in z for v in pair], 6

    def filter_all():
        for n, (k0, h) in enumerate(_ROWGROUPS):
            rows = pl.ds(k0 // 2 + 72 * h, 8, stride=9)
            yield from filter_rows(8 * n, lambda f1: (
                _unpack(now(wr_r)[f1, rows, :], k0 % 2),
                _unpack(now(wi_r)[f1, rows, :], k0 % 2)))
        yield from filter_rows(NR - 8, lambda f1: tuple(
            jnp.broadcast_to(wlast[i, :, pl.ds(128 * f1, 128)].astype(F32), (8, 128))
            for i in range(2)))

    def radix9_inv(c):
        for i in range(8):
            y = []
            for e in range(2):
                y.append(_bfly9_inv(
                    [now(t_r)[2 * c + e, i // 4, pl.ds(256 + 8 * (i % 4), 8), :]]
                    + [now(t_r)[2 * c + e, o % 2, pl.ds(64 * (o // 2) + 8 * i, 8), :]
                       for o in range(8)]))
                yield y[e][8], 12
            out = [_pack(y[0][j], y[1][j]) for j in range(9)]
            for j in range(9):
                y_t[c, pl.ds(64 * j + 8 * i, 8), :] = out[j]
            yield out, 5

    def y_to_token_major(c, cost):
        for q in range(4):
            vt = y_t[c, pl.ds(64 + 128 * q, 128), :].T
            stage[5 + q, pl.ds(c, 128, stride=8), :] = vt
            yield vt[120:], cost, 240

    def seam_to_token_major(c):
        top = _pack(a_tail[0, c], a_tail[1, c])
        stage[4, pl.ds(c, 128, stride=8), :] = jnp.concatenate(
            [top, y_t[c, pl.ds(0, 64), :]], axis=0).T

    def wo_tail_prep():
        for kt in range(5):
            vt = pltpu.bitcast(_bf(wo_perm[4, pl.ds(min(64 * kt, 224), 64), :]).T, U32)
            wo_tail[kt] = vt[:32]
            yield vt[24:32], 22, 180

    def x_to_token_major(t, qs):
        lanes = pl.ds(128 * t, 128)
        for q in qs:
            if q == 0:
                v = xa_raw[t]
            elif q == 1:
                v = pltpu.bitcast(xa_rest[pl.ds(0, 256), lanes], U32)
            else:
                v = pltpu.bitcast(xa_rest[pl.ds(256, 64), lanes], U32)
                v = jnp.concatenate([v, _zeros_w(96)], axis=0)
            store_pitched(x_nat.at[q], 136 * t, v.T)

    def difference(u, v):
        return _pack(_unpack(u, 0) - _unpack(v, 0), _unpack(u, 1) - _unpack(v, 1))

    def x_pair(p, gam, qs):
        a = 4 * gam + p
        for q in qs:
            vt = []
            for e in range(2):
                vt.append(x_nat[q, pl.ds(a + 2 * e, 128, stride=17), :].T)
                n = (128, 96, 0)[q]
                if n:
                    x_perm[q][a + 2 * e, pl.ds(0, n), :] = vt[e][:n]
                yield vt[e][max(n - 8, 0):max(n, 8)], 43, 240
            if q == 1:
                x_perm[1][a, pl.ds(96, 32), :] = difference(vt[0][96:], vt[1][96:])
                x_perm[2][4 * p + gam, pl.ds(0, 32), :] = vt[1][96:]
            if q == 2:
                x_perm[1][a + 2, pl.ds(96, 32), :] = difference(vt[1][:32], vt[0][:32])
                x_perm[2][4 * p + gam, pl.ds(32, 32), :] = vt[0][:32]

    def w_prep(part, kts=range(5)):
        col0, _ = _W_COLS[part]
        first = 288 * part - col0 // 2
        for kt in kts:
            for nt in range(5):
                nn = min(128, 3 * D - col0 - 128 * nt)
                vt = wq_raw[pl.ds(min(128 * kt, D - 128), 128), pl.ds(col0 + 128 * nt, nn)].T
                vt = pltpu.bitcast(vt, U32)
                wt_nat[kt, pl.ds(64 * nt, nn // 2), :] = vt
                yield vt[-8:], 22, 180
        low = lax.broadcasted_iota(jnp.int32, (8, 128), 1) < 64
        for kt in kts:
            for i in range(2):
                for dl in range(9):
                    base = first + 144 * i + dl
                    wa = now(wn_r)[kt, pl.ds(base, 8, stride=18), :]
                    wb = now(wn_r)[kt, pl.ds(base + 9, 8, stride=18), :]
                    out = [_pack(_unpack(wa, e), _unpack(wb, e)) for e in range(2)]
                    for e in range(2):
                        rows = pl.ds(16 * (2 * dl + e) + 8 * i, 8)
                        wt[part][kt, rows, :] = out[e]
                        if kt == 4:
                            wt[part][5, rows, :] = jnp.where(low, wt[part][3, rows, :], out[e])
                    yield out, 2 + 2 * (kt == 4)

    def wo_prep():
        for nt in range(5):
            nn = min(128, D - 128 * nt)
            blk = wo_raw[pl.ds(0, D), pl.ds(128 * nt, nn)]
            if nn < 128:
                blk = jnp.concatenate([blk, jnp.zeros((D, 128 - nn), BF16)], axis=1)
            blk = pltpu.bitcast(blk, U32)
            wo_nat[nt] = blk
            yield blk[-8:], 20
        for nts in ((0, 1), (2, 3), (4,)):
            for i in range(2):
                for dl in range(9):
                    wa = [now(won_r)[nt, pl.ds(144 * i + dl, 8, stride=18), :] for nt in nts]
                    wb = [now(won_r)[nt, pl.ds(144 * i + dl + 9, 8, stride=18), :] for nt in nts]
                    done = []
                    for e in range(2):
                        row = 16 * (2 * dl + e) + 8 * i
                        lo, hi = [[_unpack(w, e) for w in ws] for ws in (wa, wb)]
                        out = [(nt, row, _pack(lo[n], hi[n])) for n, nt in enumerate(nts)]
                        if len(nts) == 2 and dl >= 7:
                            n = dl - 7
                            out = [(nts[n], row - 32 * n,
                                    _pack(lo[n] - lo[1 - n], hi[n] - hi[1 - n])),
                                   (nts[1 - n], row + 32 * (1 - n), out[1 - n][2])]
                        for nt, r, word in out:
                            wo_perm[nt, pl.ds(r, 8), :] = word
                            done.append(word)
                    yield done, 2 * len(nts)

    scale = float(DH) ** -0.5

    def attend(p, units, d_block=6):
        lane0 = lax.broadcasted_iota(jnp.int32, (8, 128), 1) == 0
        for unit in units:
            gam, hg = divmod(unit, 4)
            base = 2 * gam + 1
            acc = [[None] * W for _ in range(2)]
            for d0 in range(0, DH, d_block):
                rows = [pl.ds(144 * hg + 8 * d, 8) for d in range(d0, d0 + d_block)]
                q = [[now(q_r[4 * p + gam])[e, r, :] for r in rows] for e in range(2)]
                for l in range(9):
                    for n, r in enumerate(rows):
                        k = now(k_r[p])[base + l, r, :]
                        for e in range(2):
                            w = 7 + e - l
                            if 0 <= w < W:
                                t = q[e][n] * k
                                acc[e][w] = t if acc[e][w] is None else acc[e][w] + t
                    done = [acc[e][7 + e - l] for e in range(2) if 0 <= 7 + e - l < W]
                    yield done, d_block / 2 * len(done)
            prob = []
            for e in range(2):
                lg = [jnp.where(lane0, -1e9 / scale, acc[e][w]) if 2 * gam + e < w else acc[e][w]
                      for w in range(W)]
                m = lg[0]
                for w in range(1, W):
                    m = jnp.maximum(m, lg[w])
                ex = [jnp.exp2((l_ - m) * (scale * float(np.log2(np.e)))) for l_ in lg]
                tot = ex[0]
                for w in range(1, W):
                    tot = tot + ex[w]
                inv = 1.0 / tot
                prob.append([x_ * inv for x_ in ex])
                yield prob[e][W - 1], 13, 30
            for d in range(DH):
                rows = pl.ds(32 * d + 8 * hg, 8)
                vv = [now(v_r[p])[base + l, pl.ds(144 * hg + 8 * d, 8), :] for l in range(9)]
                o = []
                for e in range(2):
                    t = prob[e][0] * vv[7 + e]
                    for w in range(1, W):
                        t = t + prob[e][w] * vv[7 + e - w]
                    o.append(t)
                word = _pack(o[0], o[1])
                o_t[p][gam, rows, :] = word
                yield word, 8

    def o_to_token_major(p, cost, gams=range(4)):
        for gam in gams:
            for kt in range(5):
                vt = o_t[p][gam, pl.ds(min(128 * kt, D - 128), 128), :].T
                o_nat[p][kt, pl.ds(gam, 128, stride=4), :] = vt
                yield vt[120:], cost, 240

    def table(off, i):
        return _bf(tab[pl.ds(off[i], off[i + 1] - off[i]), :])

    def dft64(a, gi):
        x1 = _dot_nt(table(_OFF_LF, gi), _bf(u_nat[gi, pl.ds(a, 64, stride=17), :]))
        n = x1.shape[0] // 2
        side.run(n / 2)
        x1_buf[a, 0, pl.ds(64 * gi, n), :] = x1[:n]
        x1_buf[a, 1, pl.ds(64 * gi, n), :] = x1[n:]
        if a % 4 == 3:
            fetch_next(x1)

    def dft128(a):
        side.run(222)
        xr, xi = x1_buf[a, 0], x1_buf[a, 1]
        k1 = _dot(xr + xi, gmat[a, 0])
        t_buf[a, 0] = k1 - _dot(xi, gmat[a, 1])
        t_buf[a, 1] = k1 + _dot(xr, gmat[a, 2])

    def idft128(a):
        side.run(222)
        g = [jnp.concatenate([gmat[a, c, pl.ds(16 * tau + e, 8, stride=2), :]
                              for tau in range(8) for e in range(2)], axis=0) for c in range(3)]
        tr, ti = t_buf[a, 0], t_buf[a, 1]
        k1 = _dot_nt(tr + ti, g[0])
        z_buf[a % 2, 0] = k1 + _dot_nt(ti, g[2])
        z_buf[a % 2, 1] = k1 - _dot_nt(tr, g[1])

    def idft64(a):
        side.run(144)
        for gi in range(5):
            n = 64 if gi < 4 else NR - 256
            parts = [z_buf[a % 2, c, pl.ds(64 * gi, n), :] for c in range(2)]
            if n < 64:
                parts.append(jnp.zeros((128 - 2 * n, 128), F32))
            o = _dot(table(_OFF_LI, gi), jnp.concatenate(parts, axis=0))
            if gi < 4:
                t_buf[a, 0, pl.ds(64 * gi, 64), :] = o[:64]
                t_buf[a, 1, pl.ds(64 * gi, 64), :] = o[64:]
            else:
                t_buf[a, 0, pl.ds(256, 32), :] = o[:32]
                t_buf[a, 1, pl.ds(256, 32), :] = o[32:]

    def proj(part, p, gam, qs=(0, 1, 2), chunks=4, only=None):
        a = 4 * gam + p
        m = 288 // chunks
        passes = [[(0, 0), (1, 1), (2, 2), (3, 3)], [(0, 0), (1, 1), (2, 2), (5, 3)]]
        passes = [[(kw, kx) for kw, kx in ps if kw // 2 in qs] for ps in passes]
        for ch in only or range(chunks):
            side.run((len(passes[0]) + len(passes[1]) + (2 in qs)) * m / 2)
            w = lambda kt: _bf(wt[part][kt, pl.ds(m * ch, m), :])
            r = [None, None]
            for e in range(2):
                if passes[e]:
                    r[e] = _dot(
                        jnp.concatenate([w(kw) for kw, _ in passes[e]], axis=1),
                        jnp.concatenate(
                            [_bf(x_perm[kx // 2][a + 2 * e, pl.ds(64 * (kx % 2), 64), :])
                             for _, kx in passes[e]], axis=0))
            if 2 in qs:
                both = _dot(w(4), _bf(x_perm[2][4 * p + gam]))
                r = [both if t is None else t + both for t in r]
            for e in range(2):
                c = 2 * gam + e
                buf, slot = (q_buf[4 * p + gam], e) if part == 0 else (
                    (k_buf, v_buf)[part - 1][p], 8 + c)
                rows = []
                for i in range(m // 4):
                    d, hg = divmod(m // 4 * ch + i, 4)
                    rows.append(pl.ds(144 * hg + 8 * d, 8))
                tile = r[e]
                if qs[0]:
                    tile = tile + jnp.concatenate([buf[slot, r_, :] for r_ in rows], axis=0)
                shifted = part and c and qs[-1] == 2
                rolled = pltpu.roll(tile, 1, 1) if shifted else None
                for i, r_ in enumerate(rows):
                    buf[slot, r_, :] = tile[8 * i:8 * i + 8]
                    if shifted:
                        buf[c, r_, :] = rolled[8 * i:8 * i + 8]
                        if part == 2:
                            lane0 = lax.broadcasted_iota(jnp.int32, (8, 128), 1) == 0
                            pltpu.store(buf.at[c, r_, :], v_buf[0][8, r_, :], mask=lane0)
            fetch_next(r[0])

    def out_proj(p, row0, cw):
        side.run(9 * cw)
        o = [o_nat[p][kt, pl.ds(row0, cw), :] for kt in range(5)]
        low = lax.broadcasted_iota(jnp.int32, (cw, 128), 1) < 64
        lhs = [jnp.concatenate([_bf(t) for t in o[:3] + [last]], axis=1)
               for last in (o[3], jnp.where(low, o[3], o[4]))]
        r = [_dot(lhs[n], jnp.concatenate(
            [_bf(wo_perm[nt, pl.ds(0, 256), :]) for nt in (n, n + 2)], axis=1)) for n in range(2)]
        both = _dot(_bf(o[4]), jnp.concatenate(
            [jnp.concatenate([_bf(wo_perm[nt + 1 - n, pl.ds(256, 32), :]) for n in range(2)], axis=0)
             for nt in (0, 2)], axis=1))
        rows = pl.ds(2 * row0, 2 * cw)
        for ct in range(4):
            cols = slice(128 * (ct // 2), 128 * (ct // 2) + 128)
            tile = r[ct % 2][:, cols] + both[:, cols]
            if p == 0:
                out0[ct, rows, :] = tile
            else:
                stage[ct, rows, :] = _pack(out0[ct, rows, :], tile)
                cp_out(ct, 2 * row0, 2 * cw).start()

    def out_tail(p, gam):
        side.run(144)
        words = o_t[p][gam]
        o = [_unpack(words, e) for e in range(2)]
        w = [wo_tail[kt] for kt in range(5)]
        low = lax.broadcasted_iota(jnp.int32, (32, 128), 1) < 64
        both = _dot(_bf(w[4]), jnp.concatenate([o[1][448:512], o[0][512:]], axis=0))
        for e, last in enumerate((w[3], jnp.where(low, w[3], w[4]))):
            rows = slice(448 + 64 * e, 512 + 64 * e)
            a_tail[p, 2 * gam + e] = both + _dot(
                jnp.concatenate([_bf(t) for t in w[:3] + [last]], axis=1),
                jnp.concatenate([o[e][:448], o[e][rows] - o[1 - e][rows]], axis=0))

    cp_wq(1, 0, 256).start()
    for t in range(8):
        cp_xa(t).start()
    cp_wq(1, 0, 256).wait()
    _drain(w_prep(1, range(2)))
    for t0, t1 in ((0, 6), (6, 11), (11, 14), (14, 16)):
        if t0 == 0:
            for t in range(8, 16):
                cp_xa(t).start()
        elif t0 == 6:
            cp_wq(1, 256, D - 256).start()
        elif t0 == 11:
            cp_xa_rest().start()
        for t in range(t0, t1):
            cp_xa(t).wait()
        for t in range(t0, t1):
            x_to_token_major(t, (0,))
    _drain(x_pair(0, 0, (0,)))

    side.start(xa_raw[0, pl.ds(0, 8), :], x1_buf.at[16, 0])
    pairs = [(p, gam) for p in range(2) for gam in range(4)]
    pair = 1296
    unit = 319

    def end_region():
        pl.semaphore_signal(sem_region)
        pl.semaphore_wait(sem_region)

    side.open(0.0)
    fetches += [[]] * 3
    fetches += [[partial(fetch_wq, 0, i)] for i in range(4)]
    fetches += [[partial(fetch_xb, t)] for t in range(16)]
    fetches += [[partial(fetch_wq, 2, i) for i in range(4)]]
    fetches += [[partial(fetch_tab, r, min(304, n_tab - r)) for r in range(0, n_tab, 304)]]
    fetches += [[partial(fetch_f, t) for t in range(4)]]
    for n in range(5):
        side.add("next", x_pair(*pairs[n + 1], (0,)), 0.5, first=True)
        if n < 2:
            side.add("later", x_pair(*pairs[n + 6], (0,)), 0.5)
        proj(1, *pairs[n], qs=(0,), chunks=2)
        side.finish("next")
    side.close()

    cp_xa_rest().wait()
    cp_wq(1, 256, D - 256).wait()
    side.open(0.0)
    for n in range(5, 8):
        proj(1, *pairs[n], qs=(0,), chunks=2)
    for q in (1, 2):
        for t in range(16):
            x_to_token_major(t, (q,))
        for n in range(2):
            side.add("next", x_pair(*pairs[n], (q,)), 0.6)
        side.add("next", w_prep(1, (2, 3) if q == 1 else (4,)), 0.6)
        if q == 2:
            side.add("next", x_pair(*pairs[2], (1, 2)), 0.6)
        side.finish("next")
        for n in range(2):
            proj(1, *pairs[n], qs=(q,), chunks=2)
    for n in range(2, 5):
        side.add("next", x_pair(*pairs[n + 1], (1, 2)), 0.6)
        proj(1, *pairs[n], qs=(1, 2))
        side.finish("next")
    side.close()

    assert not fetches
    pltpu.make_async_copy(xb_raw, xb_raw, sem_in.at[SEM_XB]).wait()
    cp_wq(0).wait()
    side.open(0.9, 300.0, links=2)
    load = (8 * 264 + 2 * 172 + 766) / (3 * 720 + 2 * pair) * 0.9
    side.add("w", w_prep(0), load)
    for tau in range(8):
        side.add("r9", radix9(tau), load)
    for n in range(5, 8):
        if n < 7:
            side.add("next", x_pair(*pairs[n + 1], (1, 2)), load, first=True)
        proj(1, *pairs[n], qs=(1, 2))
        side.finish("next")
    side.finish("w")
    proj(0, 0, 0, chunks=2)
    proj(0, 0, 1, chunks=2)
    side.close()

    cp_tab(0, n_tab).wait()
    cp_wq(2).wait()
    side.open(0.95, links=2)
    fetches += [[partial(fetch_f, t)] for t in range(4, 16)]
    fetches += [[partial(fetch_wo, i)] for i in range(4)]
    fetches.append([wo_settle])
    load = 0.9 * 0.95
    side.add("t", u_to_token_major(0, 43), load)
    for a in range(16):
        side.add("g%d" % a, dft_matrix(a), 0.3 * load)
    proj(0, 0, 2, chunks=2, only=(0,))
    side.finish("t")
    for gi in range(5):
        if gi < 4:
            side.add("t", u_to_token_major(gi + 1, 43), load, first=True)
        for a in range(16):
            dft64(a, gi)
        side.finish("t")
    side.add("w", w_prep(2), 0.5 * load)
    for a in range(16):
        side.finish("g%d" % a)
        dft128(a)
    side.close()

    assert not fetches
    pltpu.make_async_copy(wr_raw, wr_raw, sem_in.at[SEM_WR]).wait()
    pltpu.make_async_copy(wi_raw, wi_raw, sem_in.at[SEM_WI]).wait()
    cp_flast(0).wait()
    cp_flast(1).wait()
    cp_wo().wait()
    side.open(0.95, 400.0)
    load = (37 * 120 + 280) / (6 * pair)
    side.add("f", filter_all(), load)
    side.add("wo", wo_prep(), load)
    for gam in range(4):
        proj(2, 0, gam, chunks=2)
    proj(0, 0, 2, chunks=2, only=(1,))
    proj(0, 0, 3, chunks=2)
    proj(0, 1, 0, chunks=2, only=(0,))
    side.close()
    end_region()

    side.open(0.95, 50.0, links=2)
    side.add("att", attend(0, range(10)), 10 * unit / 5856)
    idft128(0)
    for a in range(16):
        if a < 15:
            idft128(a + 1)
        idft64(a)
    side.close()
    end_region()

    side.open(0.9, 500.0, links=2)
    load = (6 * unit + 8 * 232) / (4.5 * pair) * 0.95
    side.add("att", attend(0, range(10, 16)), load)
    for c in range(8):
        side.add("r9", radix9_inv(c), load)
    for gam in range(4):
        proj(2, 1, gam)
    proj(0, 1, 0, only=(2, 3))
    side.close()
    end_region()

    side.open(0.9, 200.0)
    period = 3 * pair / 57 * 0.9
    side.add_paced("o", o_to_token_major(0, 0), period)
    for c in range(8):
        side.add_paced("y", y_to_token_major(c, 0), period)
    side.add_paced("y", wo_tail_prep(), period)
    load = 7 * unit / (3 * pair) * 1.05 * 0.9
    side.add("att", attend(1, range(4)), load)
    proj(0, 1, 1)
    side.add("att", attend(1, range(4, 7)), load)
    proj(0, 1, 2)
    proj(0, 1, 3)
    side.close()
    for ct in range(5, 9):
        cp_out(ct, 0, S // 2).start()
    end_region()

    side.open(1.05, 200.0, links=2)
    side.add("att", attend(1, range(7, 16), 9), 9 * unit / (9 * 416 + 4 * 144))
    for gam in range(4):
        out_tail(0, gam)
    for row0 in range(0, 416, 64):
        out_proj(0, row0, min(64, 416 - row0))
    side.close()
    end_region()

    for gam in range(4):
        out_tail(1, gam)
    _drain(o_to_token_major(1, 0, range(1)))
    for c in range(8):
        seam_to_token_major(c)
    out_proj(0, 416, 32)
    cp_out(4, 0, S // 2).start()
    end_region()

    _drain(o_to_token_major(1, 0, range(1, 4)))
    out_proj(0, 448, 64)
    for row0 in range(0, 512, 16):
        out_proj(1, row0, 16)
    pltpu.make_async_copy(out_hbm, out_hbm, sem_out).wait()


@jax.jit
def pallas_concat_heads__sliding_local_dilated__spectral_gfnet__prompt_kernel(
    A_x: jax.Array,
    A_wqkv: jax.Array,
    A_wo: jax.Array,
    B_x: jax.Array,
    B_w_r: jax.Array,
    B_w_i: jax.Array,
):
    assert A_x.shape == (1, S, D) and B_x.shape == (1, S, D)
    any_spec = pl.BlockSpec(memory_space=pl.ANY)
    scratch = [
        pltpu.VMEM((1,) + _TABLE.shape, U32),
        pltpu.VMEM((16, 288, 128), U32),
        pltpu.VMEM((16, 128, 128), U32),
        pltpu.VMEM((D - 256, S), BF16),
        pltpu.VMEM((D, 3 * D), BF16),
        pltpu.VMEM((D + 64, D), BF16),
        pltpu.VMEM((1, 16, 144, 128), U32),
        pltpu.VMEM((1, 16, 144, 128), U32),
        pltpu.VMEM((2, 1, S), BF16),
        pltpu.VMEM((1, 16, 3, 128, 128), F32),
        pltpu.VMEM((1, 8, D, 128), U32),
        pltpu.VMEM((1, 8, D, 128), U32),
        pltpu.VMEM((5, 8 * 136, 128), U32),
        pltpu.VMEM((1, 18, 2, NR, 128), F32),
        pltpu.VMEM((1, 16, 2, NR, 128), F32),
        pltpu.VMEM((1, 2, 2, NR, 128), F32),
        pltpu.VMEM((3, 16 * 136, 128), U32),
        [pltpu.VMEM((1, n // 8, n, 128), U32) for n in (128, 128, 64)],
        pltpu.VMEM((1, 5, 320, 128), U32),
        pltpu.VMEM((1, 6, 288, 128), U32),
        pltpu.VMEM((1, 6, 288, 128), U32),
        pltpu.VMEM((1, 6, 288, 128), U32),
        pltpu.VMEM((1, 5, 288, 128), U32),
        pltpu.VMEM((1, 5, 288, 128), U32),
        pltpu.VMEM((1, 5, 32, 128), U32),
        [pltpu.VMEM((1, 2, D + 16, 128), F32)] * 8,
        [pltpu.VMEM((1, 16, D + 8, 128), F32)] * 2,
        [pltpu.VMEM((1, 16, D + 8, 128), F32)] * 2,
        [pltpu.VMEM((1, 4, D, 128), U32)] * 2,
        [pltpu.VMEM((1, 5, 512, 128), U32)] * 2,
        pltpu.VMEM((1, 4, S // 2, 128), F32),
        pltpu.VMEM((1, 2, 8, 64, 128), F32),
        pltpu.VMEM((9, S // 2, 128), U32),
        pltpu.SemaphoreType.DMA((5,)),
        pltpu.SemaphoreType.DMA((9,)),
        pltpu.SemaphoreType.DMA(()),
        pltpu.SemaphoreType.REGULAR,
    ]
    out = pl.pallas_call(
        _kernel,
        out_shape=jax.ShapeDtypeStruct((S, 2 * D), BF16),
        in_specs=[any_spec] * 7 + [pl.BlockSpec(memory_space=pltpu.SMEM)],
        out_specs=any_spec,
        scratch_shapes=scratch,
        compiler_params=pltpu.CompilerParams(vmem_limit_bytes=120 * 1024 * 1024),
        name="attn_gfnet",
    )(A_x[0].T, A_wqkv, A_wo, B_x[0].T, B_w_r.T, B_w_i.T, _TABLE, _ZERO)
    return out[None]
```

```python
from functools import partial

import numpy as np

import jax
import jax.numpy as jnp
from jax import lax
import jax.experimental.pallas as pl
import jax.experimental.pallas.tpu as pltpu

S = 2048
D = 576
H = 32
DH = 18
W = 8
DF = D // 2 + 1
NR = 296

F32 = jnp.float32
BF16 = jnp.bfloat16
U32 = jnp.uint32

_R9 = float(2 * np.cos(2 * np.pi / 9))
_S9 = float(np.sin(2 * np.pi / 3) / np.sin(2 * np.pi / 9))


def _bfly9_fwd(x):
    tot = [x[j] + x[j + 3] + x[j + 6] for j in range(3)]
    re = [x[j] - x[j + 6] for j in range(3)]
    im = [x[j + 3] - x[j + 6] for j in range(3)]
    ar, ai = re[0] * (_R9 - 1) + im[0], im[0] * _R9 - re[0]
    br, bi = re[1] * _S9, im[1] * _S9
    cr, ci = re[2] * _R9 - im[2], im[2] * (_R9 - 1) + re[2]
    pr, pi, qr, qi = ar - cr, ai - ci, br - cr, bi - ci
    t = pr - qr
    return [tot[0] + tot[1] + tot[2], ar + br + cr, ai + bi + ci, qr - pi, qi + t,
            tot[0] - tot[2], tot[1] - tot[2], pr - qi, pi - t]


def _bfly9_inv(v):
    u0, u1r, u1i, u2r, u2i, u3r, u3i, u4r, u4i = v
    t = u2i - u4i
    pr, pi, qr, qi = u4r + t, u4i - u2r, u2r - t, u2i - u4r
    ar, ai, br, bi = u1r + pr, u1i + pi, u1r + qr, u1i + qi
    cr, ci = u1r - pr - qr, u1i - pi - qi
    re = [ar * (_R9 - 1) - ai, br * _S9, cr * _R9 + ci]
    im = [ai * _R9 + ar, bi * _S9, ci * (_R9 - 1) - cr]
    tot = [u0 + u3r, u0 + u3i, u0 - u3r - u3i]
    return ([tot[j] + re[j] for j in range(3)] + [tot[j] + im[j] for j in range(3)]
            + [tot[j] - re[j] - im[j] for j in range(3)])


def _bfly4(x, inverse):
    (ar, ai), (br, bi), (cr, ci), (dr, di) = x
    pr, pi, qr, qi = ar + cr, ai + ci, ar - cr, ai - ci
    sr, si, tr, ti = br + dr, bi + di, br - dr, bi - di
    y1, y3 = (qr + ti, qi - tr), (qr - ti, qi + tr)
    if inverse:
        y1, y3 = y3, y1
    return [(pr + sr, pi + si), y1, (pr - sr, pi - si), y3]


def _twiddle16(z, e, inverse):
    zr, zi = z
    e = (-e if inverse else e) % 16
    h = float(np.sqrt(0.5))
    if e == 0:
        return z
    if e == 4:
        return zi, -zr
    if e == 12:
        return -zi, zr
    if e == 2:
        return (zr + zi) * h, (zi - zr) * h
    if e == 14:
        return (zr - zi) * h, (zr + zi) * h
    if e == 6:
        return (zi - zr) * h, (zr + zi) * (-h)
    if e == 10:
        return (zr + zi) * (-h), (zr - zi) * h
    c, s = float(np.cos(2 * np.pi * e / 16)), float(np.sin(2 * np.pi * e / 16))
    return zr * c + zi * s, zi * c - zr * s


_GROUPS = (1, 2, 3, 4, 0)


def _group_classes(g):
    return sorted({g, g + 9, 9 - g, 18 - g}) if g else [0, 9]


_ROWGROUPS = [(k0, h) for g in _GROUPS for k0 in _group_classes(g) for h in range(2)]


def _to_words(m):
    u = np.ascontiguousarray(m, dtype=np.float32).view(np.uint32)
    u = (u + 0x7FFF + ((u >> 16) & 1)) >> 16
    return (u[0::2] | (u[1::2] << 16)).astype(np.uint32)


def _coordinates(a, v):
    rhs = [np.sum(row * v) for row in a]
    if len(a) == 1:
        return [rhs[0] / np.sum(a[0] * a[0])]
    g00, g01, g11 = np.sum(a[0] * a[0]), np.sum(a[0] * a[1]), np.sum(a[1] * a[1])
    det = g00 * g11 - g01 * g01
    return [(g11 * rhs[0] - g01 * rhs[1]) / det, (g00 * rhs[1] - g01 * rhs[0]) / det]


def _make_tables():
    basis = np.array(_bfly9_fwd(list(np.eye(9))))
    m_fwd = np.array([2 * (r % 32) + r // 32 for r in range(64)])
    lf, li = [], []
    for g in _GROUPS:
        rows = [k0 + 18 * i for k0 in _group_classes(g) for i in range(16)]
        if g == 0:
            rows += [DF - 1] + [-1] * 7
        cols = [2 * g - 1, 2 * g] if g else [0]
        a = basis[cols]
        n = len(rows)
        f = np.zeros((2 * n, 128))
        b = np.zeros((64 * len(cols), 128))
        for r, k in enumerate(rows):
            if k < 0:
                continue
            ck = np.exp(-2j * np.pi * ((np.arange(9) * k) % 9) / 9)
            lam = _coordinates(a, ck)
            wk = (1.0 if k in (0, DF - 1) else 2.0) / (S * D)
            for c in range(len(cols)):
                e = lam[c] * np.exp(-2j * np.pi * ((m_fwd * k) % D) / D)
                f[r, 64 * c:64 * c + 64] = e.real
                f[n + r, 64 * c:64 * c + 64] = e.imag
                e = wk * lam[c] * np.exp(-2j * np.pi * ((np.arange(64) * k) % D) / D)
                b[64 * c:64 * c + 64, r] = e.real
                b[64 * c:64 * c + 64, n + r] = e.imag
        lf.append(_to_words(f))
        li.append(_to_words(b))
    n = np.arange(128)
    b_of_n = 16 * (n // 16) + 8 * (n % 2) + (n % 16) // 2
    f128 = np.exp(-2j * np.pi * (np.outer(b_of_n, n) % 128) / 128)
    tw = np.exp(-2j * np.pi * np.outer(np.arange(16), n) / S)
    f32w = lambda m: np.ascontiguousarray(m, dtype=np.float32).view(np.uint32)
    parts = [f32w(f128.real), f32w(f128.imag), f32w(tw.real), f32w(tw.imag)] + lf + li
    offs = np.cumsum([0] + [p.shape[0] for p in parts])
    parts.append(np.zeros((-offs[-1] % 32, 128), np.uint32))
    return np.concatenate(parts, axis=0), [int(o) for o in offs]


_TABLE, _OFF = _make_tables()
_OFF_FR, _OFF_FI, _OFF_TR, _OFF_TI = _OFF[0:4]
_OFF_LF = _OFF[4:10]
_OFF_LI = _OFF[9:15]


def _pack(lo, hi):
    return pltpu.pack_elementwise([lo, hi], packed_dtype=BF16)


def _unpack(w, index):
    return pltpu.unpack_elementwise(w, index=index, packed_dtype=BF16, unpacked_dtype=F32)


def _bf(words):
    return pltpu.bitcast(words, BF16)


def _dot(a, b):
    return lax.dot_general(a, b, (((1,), (0,)), ((), ())), preferred_element_type=F32)


def _dot_nt(a, b):
    return lax.dot_general(a, b, (((1,), (1,)), ((), ())), preferred_element_type=F32)


def _zeros_w(rows):
    return jnp.zeros((rows, 128), U32)


class _SideWork:
    LINK = 7.0
    HOP = 6.0

    def __init__(self, zero_ref):
        self.zero_ref = zero_ref
        self.zero = zero_ref[0]

    def start(self, seed, sink):
        self.chain = pltpu.bitcast(seed, F32)
        self.sink = sink
        self.jobs = []
        self.paced = []
        self.pending = []
        self.regions = 0
        self.credit = self.delay = self.clock = 0.0

    def open(self, stretch=0.0, slack=100.0, links=4):
        self.links = links
        self.zero = self.zero_ref[0]
        self.lead = -slack
        self.stretch = stretch

    def add(self, name, job, load, first=False):
        self.jobs.insert(0 if first else len(self.jobs), (name, job, load))

    def add_paced(self, job, period):
        if not self.paced:
            self.due = self.clock
        self.paced.append((job, period))

    def _absorb(self, item):
        values, cycles, latency = (item + (0.0,))[:3]
        values = values if isinstance(values, list) else [values]
        values = [pltpu.bitcast(v, F32) for v in values]
        while len(values) > 1:
            values = [values[i] + values[i + 1] if i + 1 < len(values) else values[i]
                      for i in range(0, len(values), 2)]
        self.pending.append((self.clock + latency, values[0]))
        self.pending.sort(key=lambda x: x[0])
        return cycles

    def _step_paced(self):
        item = next(self.paced[0][0], None)
        if item is None:
            self.paced.pop(0)
        else:
            self._absorb(item)
            self.due += self.stretch * self.paced[0][1]

    def _tick(self, cycles):
        while self.paced and self.due <= self.clock:
            self._step_paced()
        self.clock += cycles
        self.delay += cycles
        while self.pending and self.pending[0][0] <= self.clock:
            self.chain = self.pending.pop(0)[1] + self.chain
            self.delay -= 2.0
        n = int(self.delay / self.LINK)
        if n >= self.links:
            for _ in range(n):
                self.chain = pl.reciprocal(self.chain, approx=True)
            self.delay -= n * self.LINK

    def _step(self):
        item = next(self.jobs[0][1], None)
        if item is None:
            self.jobs.pop(0)
            return
        cycles = self._absorb(item) / self.jobs[0][2]
        self.credit -= cycles
        self.lead += cycles
        while self.lead >= self.HOP:
            self.zero = self.zero_ref[self.zero]
            self.lead -= self.HOP
        self._tick(self.stretch * cycles)

    def run(self, cycles):
        self.credit += cycles
        while self.jobs and self.credit > 0:
            self._step()
        while not self.jobs and self.credit > 0:
            n = min(self.credit, 50.0) if self.paced else self.credit
            self._tick(self.stretch * n)
            self.credit -= n

    def finish(self, name):
        while any(job[0] == name for job in self.jobs):
            self._step()

    def close(self):
        while self.jobs:
            self._step()
        while self.paced:
            self._step_paced()
        while self.pending:
            self.chain = self.pending.pop(0)[1] + self.chain
        self.sink[pl.ds(8 * self.regions, 8), :] = self.chain
        self.regions += 1
        self.credit = self.delay = 0.0


def _drain(gen):
    for _ in gen:
        pass


_W_COLS = ((0, 512), (512, 640), (1152, 576))


def _kernel(xa_hbm, wqkv_hbm, wo_hbm, xb_hbm, wr_hbm, wi_hbm, tab_hbm, out_hbm,
            tab, xb_raw, xa_raw, wq_raw, wo_raw, wr_raw, wi_raw, wlast,
            gmat, u_t, y_t, u_nat, x1_buf, t_buf, z_buf, x_nat, x_seam, wt_nat, wt_q, wt_k, wt_v,
            wo_diff, wo_tail, q_buf, k_buf, v_buf, p_buf, o_t, o_nat, y_seam, stage,
            zero_ref, sem, sem_region):
    zero_ref[0] = pl.semaphore_read(sem_region)
    side = _SideWork(zero_ref)
    zero = side.zero

    def now(ref):
        return ref.at[side.zero]

    tab_r, wr_r, wi_r = tab, wr_raw, wi_raw
    tab, wr_raw, wi_raw = tab.at[0], wr_raw.at[0], wi_raw.at[0]
    t_r, wn_r, q_r, k_r, v_r, p_r = t_buf, wt_nat, q_buf, k_buf, v_buf, p_buf
    u_r, y_r, g_r = u_t, y_t, gmat
    (gmat, u_t, y_t, x1_buf, t_buf, z_buf, x_nat, x_seam, wt_nat, wt_q, wt_k, wt_v, wo_diff,
     wo_tail, q_buf, k_buf, v_buf, p_buf, o_t, o_nat, y_seam) = jax.tree.map(
        lambda r: r.at[zero],
        (gmat, u_t, y_t, x1_buf, t_buf, z_buf, x_nat, x_seam, wt_nat, wt_q, wt_k, wt_v, wo_diff,
         wo_tail, q_buf, k_buf, v_buf, p_buf, o_t, o_nat, y_seam))
    wt = (wt_q, wt_k, wt_v)

    sem_xb, sem_tab, sem_f, sem_out, sem_k = (sem.at[i] for i in range(5))

    def cp_tab(row0, rows):
        return pltpu.make_async_copy(
            tab_hbm.at[pl.ds(row0, rows)], tab.at[pl.ds(row0, rows)], sem_tab)

    def cp_xb(t):
        return pltpu.make_async_copy(
            xb_hbm.at[:, pl.ds(t * 128, 128)], xb_raw.at[t].bitcast(BF16), sem_xb)

    def cp_xa(half, row0, rows, sem_):
        rows, cols = pl.ds(row0, rows), pl.ds(S // 2 * half, S // 2)
        return pltpu.make_async_copy(xa_hbm.at[rows, cols], xa_raw.at[rows, cols], sem_)

    def cp_wq(part, row0, rows, sem_):
        rows, cols = pl.ds(row0, rows), pl.ds(*_W_COLS[part])
        return pltpu.make_async_copy(wqkv_hbm.at[rows, cols], wq_raw.at[rows, cols], sem_)

    def cp_wo(row0=0, rows=D):
        return pltpu.make_async_copy(
            wo_hbm.at[pl.ds(row0, rows)], wo_raw.at[pl.ds(row0, rows)], sem_f)

    def cp_f(i, t):
        src, dst = ((wr_hbm, wr_raw), (wi_hbm, wi_raw))[i]
        return pltpu.make_async_copy(
            src.at[pl.ds(0, DF - 1), pl.ds(t * 128, 128)], dst.at[t].bitcast(BF16),
            sem_f)

    def cp_flast(i):
        src = (wr_hbm, wi_hbm)[i]
        return pltpu.make_async_copy(src.at[pl.ds(DF - 1, 1), :], wlast.at[i], sem_f)

    def cp_out(ct, row0, rows):
        return pltpu.make_async_copy(
            stage.at[ct, pl.ds(row0, rows), :].bitcast(BF16),
            out_hbm.at[pl.ds(2 * row0, 2 * rows), pl.ds(ct * 128, 128)], sem_out)

    def fetch_xb(t, v):
        xb_raw[t, pl.ds(0, 8), :] = v
        cp_xb(t).start()

    def fetch_wq(part, row0, rows, sem_, v):
        wq_raw[pl.ds(row0, 16), pl.ds(_W_COLS[part][0], 128)] = _bf(v)
        cp_wq(part, row0, rows, sem_).start()

    def fetch_xa(half, row0, rows, sem_, v):
        xa_raw[pl.ds(row0, 16), pl.ds(S // 2 * half, 128)] = _bf(v)
        cp_xa(half, row0, rows, sem_).start()

    def fetch_wo(piece, v):
        wo_raw[pl.ds(144 * piece, 16), pl.ds(0, 128)] = _bf(v)
        cp_wo(144 * piece, 144).start()

    def wo_settle(v):
        wo_raw[pl.ds(D, 16), pl.ds(0, 128)] = _bf(v)

    def fetch_tab(row0, rows, v):
        tab[pl.ds(row0, 8), :] = v
        cp_tab(row0, rows).start()

    def fetch_f(t, v):
        wr_raw[t, pl.ds(0, 8), :] = v
        cp_f(0, t).start()
        wi_raw[t, pl.ds(0, 8), :] = v
        cp_f(1, t).start()
        if t == 0:
            cp_flast(0).start()
            cp_flast(1).start()

    n_tab = _TABLE.shape[0]
    fetches = []

    def fetch_next(value):
        if fetches:
            for fetch in fetches.pop(0):
                fetch(pltpu.bitcast(value[:8, :128], U32))

    def store_pitched(dst, row0, vt):
        for r in range(16):
            dst[pl.ds(row0 + 17 * (r // 2) + 8 * (r % 2), 8), :] = vt[8 * r:8 * r + 8]

    def radix9(tau):
        for i in range(4):
            words = [[xb_raw[side.zero + 2 * tau + z, pl.ds(32 * j + 8 * i, 8), :]
                      for j in range(9)] for z in range(2)]
            for e in range(2):
                u = []
                for z in range(2):
                    u.append(_bfly9_fwd([_unpack(w, e) for w in words[z]]))
                    yield u[z][8], 12
                out = [_pack(u[0][o], u[1][o]) for o in range(9)]
                for o in range(9):
                    u_t[tau, pl.ds(64 * o + 32 * e + 8 * i, 8), :] = out[o]
                if tau == i == e == 0:
                    out[8] = now(u_r)[0, pl.ds(512, 8), :]
                yield out, 5

    def u_to_token_major(gi):
        g = _GROUPS[gi]
        for tau in range(8):
            if g:
                v = u_t[tau, pl.ds(64 * (2 * g - 1), 128), :]
            else:
                v = jnp.concatenate([u_t[tau, pl.ds(0, 64), :], _zeros_w(64)], axis=0)
            vt = v.T
            store_pitched(u_nat.at[gi], 136 * tau, vt)
            yield vt[120:], 43, 240

    def dft_matrix(a):
        twr = jnp.broadcast_to(pltpu.bitcast(tab[pl.ds(_OFF_TR + a, 1), :], F32), (8, 128))
        twi = jnp.broadcast_to(pltpu.bitcast(tab[pl.ds(_OFF_TI + a, 1), :], F32), (8, 128))
        for i in range(16):
            fr = pltpu.bitcast(now(tab_r)[pl.ds(_OFF_FR + 8 * i, 8), :], F32)
            fi = pltpu.bitcast(now(tab_r)[pl.ds(_OFF_FI + 8 * i, 8), :], F32)
            gr, gi = fr * twr - fi * twi, fr * twi + fi * twr
            gmat[a, 0, pl.ds(8 * i, 8), :] = gr
            out = [gr + gi, gi - gr]
            gmat[a, 1, pl.ds(8 * i, 8), :] = out[0]
            gmat[a, 2, pl.ds(8 * i, 8), :] = out[1]
            if a == i == 0:
                out[1] = now(g_r)[0, 2, pl.ds(0, 8), :]
            yield out, 3

    def filter_rows(row0, load_w):
        rows = pl.ds(row0, 8)
        y = [[None] * 4 for _ in range(4)]
        for a0 in range(4):
            src = now(t_r)
            z = _bfly4([(src[4 * a1 + a0, 0, rows, :], src[4 * a1 + a0, 1, rows, :])
                        for a1 in range(4)], False)
            for g0 in range(4):
                y[g0][a0] = _twiddle16(z[g0], a0 * g0, False)
            yield y[3][a0][0], 7
        for g0 in range(4):
            z = _bfly4(y[g0], False)
            yield z[3][1], 4
            for g1 in range(4):
                wr, wi = load_w(g0 + 4 * g1)
                zr, zi = z[g1]
                z[g1] = (zr * wr - zi * wi, zr * wi + zi * wr)
                if g1 % 2:
                    yield z[g1][1], 4
            z = _bfly4(z, True)
            for a0 in range(4):
                y[g0][a0] = _twiddle16(z[a0], a0 * g0, True)
            yield y[g0][3][0], 6
        for a0 in range(4):
            z = _bfly4([y[g0][a0] for g0 in range(4)], True)
            for a1 in range(4):
                t_buf[4 * a1 + a0, 0, rows, :] = z[a1][0]
                t_buf[4 * a1 + a0, 1, rows, :] = z[a1][1]
            yield [v for pair in z for v in pair], 6

    def filter_all():
        for n, (k0, h) in enumerate(_ROWGROUPS):
            rows = pl.ds(k0 // 2 + 72 * h, 8, stride=9)
            yield from filter_rows(8 * n, lambda f1: (
                _unpack(now(wr_r)[f1, rows, :], k0 % 2),
                _unpack(now(wi_r)[f1, rows, :], k0 % 2)))
        yield from filter_rows(NR - 8, lambda f1: tuple(
            jnp.broadcast_to(wlast[i, :, pl.ds(128 * f1, 128)].astype(F32), (8, 128))
            for i in range(2)))

    def radix9_inv(c):
        for i in range(8):
            y = []
            for e in range(2):
                y.append(_bfly9_inv(
                    [now(t_r)[2 * c + e, i // 4, pl.ds(256 + 8 * (i % 4), 8), :]]
                    + [now(t_r)[2 * c + e, o % 2, pl.ds(64 * (o // 2) + 8 * i, 8), :]
                       for o in range(8)]))
                yield y[e][8], 10
            out = [_pack(y[0][j], y[1][j]) for j in range(9)]
            for j in range(9):
                y_t[c, pl.ds(64 * j + 8 * i, 8), :] = out[j]
            if c == i == 0:
                out[8] = now(y_r)[0, pl.ds(512, 8), :]
            yield out, 5

    def y_to_token_major(c):
        for q in range(4):
            vt = y_t[c, pl.ds(64 + 128 * q, 128), :].T
            stage[5 + q, pl.ds(c, 128, stride=8), :] = vt
            yield vt[120:], 43, 240

    def y_seam_to_token_major():
        for c in range(8):
            vt = jnp.concatenate([_zeros_w(64), y_t[c, pl.ds(0, 64), :]], axis=0).T
            y_seam[c] = vt
            yield vt[120:], 43, 240

    def k_rows(kt):
        return min(128 * kt, D - 128)

    def x_to_token_major(half, kts):
        for kt in kts:
            for t in range(8 * half, 8 * half + 8):
                vt = xa_raw[pl.ds(k_rows(kt), 128), pl.ds(128 * t, 128)].T
                vt = pltpu.bitcast(vt, U32)
                for u in range(8):
                    x_nat[kt][pl.ds(72 * t + 9 * u, 8), :] = vt[8 * u:8 * u + 8]
                yield vt[56:], 22, 180

    def x_rows(half, c, i=0, n=64):
        return pl.ds(576 * half + 9 * i + c, n, stride=9)

    def difference(u, v):
        return _pack(_unpack(u, 0) - _unpack(v, 0), _unpack(u, 1) - _unpack(v, 1))

    def low_lanes(rows, n=64):
        return lax.broadcasted_iota(jnp.int32, (rows, 128), 1) < n

    def x_prep(half, gam):
        for i in range(0, 64, 8):
            (a3, a4), (b3, b4) = [[x_nat[kt][x_rows(half, 2 * gam + e, i, 8), :] for kt in (3, 4)]
                                  for e in range(2)]
            out = [jnp.where(low_lanes(8), lo, hi) for lo, hi in
                   ((a3, difference(a3, b3)), (b3, difference(b4, a4)), (b4, a4))]
            for j in range(3):
                x_seam[4 * half + gam, j, pl.ds(i, 8), :] = out[j]
            yield out, 5

    def w_prep(part, kts=range(5)):
        col0, _ = _W_COLS[part]
        first = 288 * part - col0 // 2
        for kt in kts:
            for nt in range(5):
                nn = min(128, 3 * D - col0 - 128 * nt)
                vt = wq_raw[pl.ds(k_rows(kt), 128), pl.ds(col0 + 128 * nt, nn)].T
                vt = pltpu.bitcast(vt, U32)
                wt_nat[kt, pl.ds(64 * nt, nn // 2), :] = vt
                yield vt[-8:], 22, 180
        for kt in kts:
            for i in range(2):
                for dl in range(9):
                    base = first + 144 * i + dl
                    wa = now(wn_r)[kt, pl.ds(base, 8, stride=18), :]
                    wb = now(wn_r)[kt, pl.ds(base + 9, 8, stride=18), :]
                    out = [_pack(_unpack(wa, e), _unpack(wb, e)) for e in range(2)]
                    for e in range(2):
                        rows = pl.ds(16 * (2 * dl + e) + 8 * i, 8)
                        wt[part][kt, rows, :] = out[e]
                        if kt == 4:
                            wt[part][5, rows, :] = jnp.where(
                                low_lanes(8), wt[part][3, rows, :], out[e])
                    yield out, 2 + 2 * (kt == 4)

    def wo_tile(row0, rows, ct):
        return wo_raw[pl.ds(row0, rows), pl.ds(128 * ct, 128)]

    def wo_prep():
        for ct in range(4):
            words = [pltpu.bitcast(wo_tile(448 + 64 * (ct % 2), 64, c), U32) for c in (ct, ct ^ 1)]
            wo_diff[ct] = difference(*words)
        for kt in range(5):
            vt = wo_raw[pl.ds(k_rows(kt), 128), pl.ds(512, 64)].T
            vt = pltpu.bitcast(vt, U32)
            wo_tail[kt] = vt
            yield vt[24:], 22, 180

    scale = float(DH) ** -0.5

    def softmax(unit, d_block):
        half, gam, hg = unit // 16, unit // 4 % 4, unit % 4
        base = 2 * gam + 1
        acc = [[None] * W for _ in range(2)]
        for d0 in range(0, DH, d_block):
            rows = [pl.ds(144 * hg + 8 * d, 8) for d in range(d0, d0 + d_block)]
            q = [[now(q_r[4 * half + gam])[e, r, :] for r in rows] for e in range(2)]
            for l in range(9):
                for n, r in enumerate(rows):
                    k = now(k_r[half])[base + l, r, :]
                    for e in range(2):
                        w = 7 + e - l
                        if 0 <= w < W:
                            t = q[e][n] * k
                            acc[e][w] = t if acc[e][w] is None else acc[e][w] + t
                done = [acc[e][7 + e - l] for e in range(2) if 0 <= 7 + e - l < W]
                yield done, d_block / 2 * len(done)
        prob = []
        for e in range(2):
            lg = [jnp.where(low_lanes(8, 2), -1e9 / scale, acc[e][w])
                  if half == 0 and 2 * gam + e < w else acc[e][w] for w in range(W)]
            m = lg[0]
            for w in range(1, W):
                m = jnp.maximum(m, lg[w])
            ex = [jnp.exp2((l_ - m) * (scale * float(np.log2(np.e)))) for l_ in lg]
            tot = ex[0]
            for w in range(1, W):
                tot = tot + ex[w]
            inv = pl.reciprocal(tot, approx=True)
            inv = inv + inv * (1.0 - tot * inv)
            prob.append([x_ * inv for x_ in ex])
            yield prob[e][W - 1], 11, 30
        return prob

    def weigh_values(unit, prob):
        half, gam, hg = unit // 16, unit // 4 % 4, unit % 4
        base = 2 * gam + 1
        for d in range(DH):
            vv = [now(v_r[half])[base + l, pl.ds(144 * hg + 8 * d, 8), :] for l in range(9)]
            o = []
            for e in range(2):
                t = prob[e][0] * vv[7 + e]
                for w in range(1, W):
                    t = t + prob[e][w] * vv[7 + e - w]
                o.append(t)
            if d % 2:
                o = [_pack(even[e], o[e]) for e in range(2)]
                for e in range(2):
                    o_t[half][2 * gam + e, pl.ds(72 * hg + d // 2, 8, stride=DH // 2), :] = o[e]
            even = o
            yield o, 8

    def attend(units, d_block):
        for n in units:
            prob = yield from softmax(n, d_block)
            yield from weigh_values(n, prob)

    def softmax_ahead(units, d_block):
        for n in units:
            prob = yield from softmax(n, d_block)
            for e in range(2):
                for w in range(W):
                    p_buf[n, pl.ds(8 * (W * e + w), 8), :] = prob[e][w]

    def weigh_values_later(units):
        for n in units:
            prob = [[now(p_r)[n, pl.ds(8 * (W * e + w), 8), :] for w in range(W)]
                    for e in range(2)]
            yield from weigh_values(n, prob)

    def o_to_token_major(half, gams):
        for c in [2 * gam + e for gam in gams for e in range(2)]:
            for kt in range(5):
                vt = pltpu.bitcast(_bf(o_t[half][c, pl.ds(k_rows(kt) // 2, 64), :]).T, U32)
                o_nat[half][kt, pl.ds(c, 64, stride=9), :] = vt
                yield vt[56:], 22, 180

    def table(off, i):
        return _bf(tab[pl.ds(off[i], off[i + 1] - off[i]), :])

    def dft64(a, gi):
        x1 = _dot_nt(table(_OFF_LF, gi), _bf(u_nat[gi, pl.ds(a, 64, stride=17), :]))
        n = x1.shape[0] // 2
        side.run(n / 2)
        x1_buf[a, 0, pl.ds(64 * gi, n), :] = x1[:n]
        x1_buf[a, 1, pl.ds(64 * gi, n), :] = x1[n:]
        if a % 4 == 3:
            fetch_next(x1)

    def dft128(a):
        side.run(222)
        xr, xi = x1_buf[a, 0], x1_buf[a, 1]
        k1 = _dot(xr + xi, gmat[a, 0])
        t_buf[a, 0] = k1 - _dot(xi, gmat[a, 1])
        t_buf[a, 1] = k1 + _dot(xr, gmat[a, 2])

    def idft128(a):
        side.run(222)
        g = [jnp.concatenate([gmat[a, c, pl.ds(16 * tau + e, 8, stride=2), :]
                              for tau in range(8) for e in range(2)], axis=0) for c in range(3)]
        tr, ti = t_buf[a, 0], t_buf[a, 1]
        k1 = _dot_nt(tr + ti, g[0])
        z_buf[a % 2, 0] = k1 + _dot_nt(ti, g[2])
        z_buf[a % 2, 1] = k1 - _dot_nt(tr, g[1])

    def idft64(a):
        side.run(144)
        for gi in range(5):
            n = 64 if gi < 4 else NR - 256
            parts = [z_buf[a % 2, c, pl.ds(64 * gi, n), :] for c in range(2)]
            if n < 64:
                parts.append(jnp.zeros((128 - 2 * n, 128), F32))
            o = _dot(table(_OFF_LI, gi), jnp.concatenate(parts, axis=0))
            if gi < 4:
                t_buf[a, 0, pl.ds(64 * gi, 64), :] = o[:64]
                t_buf[a, 1, pl.ds(64 * gi, 64), :] = o[64:]
            else:
                t_buf[a, 0, pl.ds(256, 32), :] = o[:32]
                t_buf[a, 1, pl.ds(256, 32), :] = o[32:]

    def proj(part, half, gam, kts=(0, 1, 2, 3), chunks=4, only=None):
        m = 288 // chunks
        last = kts[-1] == 3
        for ch in only or range(chunks):
            side.run((len(kts) + last / 2) * m)
            w = lambda kt: _bf(wt[part][kt, pl.ds(m * ch, m), :])
            both = _dot_nt(w(4), _bf(x_seam[4 * half + gam, 2])) if last else None
            for e in range(2):
                c = 2 * gam + e
                tile = _dot_nt(
                    jnp.concatenate([w(3 + 2 * e if kt == 3 else kt) for kt in kts], axis=1),
                    jnp.concatenate([_bf(x_seam[4 * half + gam, e] if kt == 3
                                         else x_nat[kt][x_rows(half, c), :]) for kt in kts], axis=1))
                if last:
                    tile = tile + both
                if part == 0:
                    buf, slot = q_buf[4 * half + gam], e
                else:
                    buf, slot = (k_buf if part == 1 and last else v_buf)[half], 8 + c
                rows = []
                for i in range(m // 4):
                    d, hg = divmod(m // 4 * ch + i, 4)
                    rows.append(pl.ds(144 * hg + 8 * d, 8))
                if kts[0]:
                    tile = tile + jnp.concatenate([v_buf[half][slot, r, :] for r in rows], axis=0)
                for i, r in enumerate(rows):
                    buf[slot, r, :] = tile[8 * i:8 * i + 8]
                if part == 0 or not last:
                    continue
                if c:
                    if half:
                        before = (k_buf, v_buf)[part - 1][0]
                        tile = jnp.where(low_lanes(2 * m, 126), tile, jnp.concatenate(
                            [before[slot, r, :] for r in rows], axis=0))
                    tile = pltpu.roll(tile, 2, 1)
                    for i, r in enumerate(rows):
                        buf[c, r, :] = tile[8 * i:8 * i + 8]
                        if part == 2 and half == 0:
                            pltpu.store(buf.at[c, r, :], buf[0, r, :], mask=low_lanes(8, 2))
                elif part == 2 and half == 0:
                    tile = jnp.where(low_lanes(2 * m, 1), tile, pltpu.roll(tile, 1, 1))
                    for i, r in enumerate(rows):
                        buf[0, r, :] = tile[8 * i:8 * i + 8]
            fetch_next(tile)

    def out_proj(half, row0, cw):
        side.run(9 * cw)
        o = [jnp.concatenate([o_nat[half][kt, pl.ds(9 * b, 8), :]
                              for b in range(row0 // 8, (row0 + cw) // 8)], axis=0)
             for kt in range(5)]
        lhs = [jnp.concatenate([_bf(t) for t in o[:3] + [last]], axis=1)
               for last in (o[3], jnp.where(low_lanes(cw), o[3], o[4]))]
        both = _dot(_bf(o[4]), jnp.concatenate(
            [jnp.concatenate([wo_tile(448, 64, ct + 1), wo_tile(512, 64, ct)], axis=0)
             for ct in (0, 2)], axis=1))
        r = [_dot(lhs[n], jnp.concatenate(
            [jnp.concatenate([wo_tile(0, 448, ct), _bf(wo_diff[ct])], axis=0)
             for ct in (n, n + 2)], axis=1)) for n in range(2)]
        for ct in (0, 2, 1, 3):
            cols = slice(128 * (ct // 2), 128 * (ct // 2) + 128)
            tile = (r[ct % 2][:, cols] + both[:, cols]).astype(BF16)
            stage[ct, pl.ds(512 * half + row0, cw), :] = pltpu.bitcast(tile, U32)
            cp_out(ct, 512 * half + row0, cw).start()

    def out_tail(half, gam):
        side.run(144)
        o = [o_t[half][2 * gam + e] for e in range(2)]
        w = [wo_tail[kt] for kt in range(5)]
        both = _dot(_bf(w[4]), _bf(jnp.concatenate([o[1][224:256], o[0][256:]], axis=0)))
        for e, last in enumerate((w[3], jnp.where(low_lanes(32), w[3], w[4]))):
            c, rows = 2 * gam + e, slice(224 + 32 * e, 256 + 32 * e)
            tile = both + _dot(
                jnp.concatenate([_bf(t) for t in w[:3] + [last]], axis=1),
                _bf(jnp.concatenate([o[e][:224], difference(o[e][rows], o[1 - e][rows])], axis=0)))
            tile = jnp.concatenate([tile.astype(BF16), jnp.zeros((64, 128), BF16)], axis=0)
            stage[4, pl.ds(512 * half + c, 64, stride=8), :] = jnp.where(
                low_lanes(64), pltpu.bitcast(tile.T, U32), y_seam[c, pl.ds(64 * half, 64), :])

    pair = 1296
    unit = 315

    def end_region():
        pl.semaphore_signal(sem_region)
        pl.semaphore_wait(sem_region)

    def queries(i0, i1, chunks=4):
        for i in range(i0, i1, 4 // chunks):
            proj(0, i // 16, i // 4 % 4, chunks=chunks, only=(i % 4 * chunks // 4,))

    blocks = ((0, 128, (0,)), (128, 256, (1, 2)), (384, D - 384, (3,)))

    def fetch_block(i):
        cp_wq(1, *blocks[i][:2], sem.at[i]).start()
        cp_xa(0, *blocks[i][:2], sem.at[i]).start()

    cp_wq(1, 0, 128, sem_k).start()
    cp_xa(0, 0, 128, sem.at[0]).start()
    fetch_block(1)
    cp_wq(1, 0, 128, sem_k).wait()
    fetch_block(2)
    _drain(w_prep(1, (0,)))
    side.start(pltpu.bitcast(wq_raw[pl.ds(0, 16), pl.ds(512, 128)], U32), x1_buf.at[16, 0])
    fetches += [[partial(fetch_xa, 1, r, 192, sem_k)] for r in range(0, D, 192)]
    for i, (row0, rows, kts) in enumerate(blocks):
        if i:
            cp_wq(1, row0, rows, sem.at[i]).wait()
        cp_xa(0, row0, rows, sem.at[i]).wait()
        if i == 1:
            fetches += [[partial(fetch_wq, 0, r, 144, sem_xb)] for r in range(0, D, 144)]
            fetches += [[partial(fetch_xb, t)] for t in range(16)]
        if i == 2:
            fetches += [[partial(fetch_wq, 2, r, 144, sem_tab) for r in range(0, D, 144)]]
            fetches += [[partial(fetch_tab, r, min(304, n_tab - r)) for r in range(0, n_tab, 304)]]
        side.open()
        tiles = kts + (4,) * (i == 2)
        if i:
            side.add("prep", w_prep(1, tiles), 0.8)
        side.add("prep", x_to_token_major(0, tiles), 0.8)
        if i == 2:
            side.add("prep", x_prep(0, 0), 0.8)
        if i:
            for gam in (2, 3):
                proj(1, 0, gam, blocks[i - 1][2])
        side.finish("prep")
        for gam in (0, 1):
            if i == 2:
                side.add("next", x_prep(0, gam + 1), 0.5)
            proj(1, 0, gam, kts)
            side.finish("next")
        if i == 2:
            side.add("next", x_prep(0, 3), 0.5)
        side.close()

    cp_xa(1, 0, D, sem_k).wait()
    side.open()
    fetches += [[partial(fetch_f, t) for t in range(4)]]
    side.add("prep", x_to_token_major(1, range(5)), 0.8)
    side.add("prep", x_prep(1, 0), 0.8)
    for gam in (2, 3):
        proj(1, 0, gam, blocks[2][2])
    side.finish("prep")
    for gam in range(3):
        side.add("next", x_prep(1, gam + 1), 0.5)
        proj(1, 1, gam)
        side.finish("next")
    side.close()

    assert not fetches
    pltpu.make_async_copy(xb_raw, xb_raw, sem_xb).wait()
    cp_wq(0, 0, D, sem_xb).wait()
    side.open(0.95, 20.0, links=2)
    load = (8 * 232 + 766) / (pair + 8 * pair / 4) * 0.9 * 1.05
    side.add("w", w_prep(0), load)
    for tau in range(8):
        side.add("r9", radix9(tau), load)
    proj(1, 1, 3)
    side.finish("w")
    queries(0, 8, 4)
    side.close()

    cp_tab(0, n_tab).wait()
    cp_wq(2, 0, D, sem_tab).wait()
    side.open(0.95, 50.0, links=2)
    fetches += [[partial(fetch_f, t)] for t in range(4, 16)]
    fetches += [[partial(fetch_wo, i)] for i in range(4)]
    fetches.append([wo_settle])
    side.add("t", u_to_token_major(0), 0.9 * 0.95)
    load = (768 + 766 + 2 * 168) / (5920 + (10 - 8) * pair / 4 - 2000.0) * 1.0 * 0.95
    for a in range(16):
        side.add("g%d" % a, dft_matrix(a), load)
    queries(8, 10)
    side.finish("t")
    for gi in range(5):
        if gi < 4:
            side.add("t", u_to_token_major(gi + 1), 0.9 * 0.95, first=True)
        for a in range(16):
            dft64(a, gi)
        side.finish("t")
    side.add("w", w_prep(2), load)
    side.add("att", softmax_ahead(range(2), 6), load)
    for a in range(16):
        side.finish("g%d" % a)
        dft128(a)
    side.close()

    assert not fetches
    pltpu.make_async_copy(wr_raw, wr_raw, sem_f).wait()
    pltpu.make_async_copy(wi_raw, wi_raw, sem_f).wait()
    cp_flast(0).wait()
    cp_flast(1).wait()
    cp_wo().wait()
    side.open(1.0, 300.0, links=2)
    side.add("f", filter_all(), 37 * 120 / (4 * pair + (18 - 10) * pair / 4) * 1.0)
    for gam in range(4):
        proj(2, 0, gam, chunks=2)
    queries(10, 18, 2)
    side.close()
    end_region()

    side.open(0.95, 20.0, links=3)
    load = (10 * unit - 2 * 168) / 5856 * 1.0
    side.add("att", weigh_values_later(range(2)), load)
    side.add("att", attend(range(2, 10), 9), load)
    idft128(0)
    for a in range(16):
        if a < 15:
            idft128(a + 1)
        idft64(a)
    side.close()
    end_region()

    side.open(0.9, 400.0, links=3)
    load = ((16 - 10) * unit + 8 * 200) / (4 * pair + (20 - 18) * pair / 4) * 0.95 * 1.0
    side.add("att", attend(range(10, 16), 6), load)
    for c in range(8):
        side.add("r9", radix9_inv(c), load)
    for gam in range(4):
        proj(2, 1, gam, chunks=4)
    queries(18, 20)
    side.close()
    end_region()

    side.open(0.9, 100.0, links=3)
    period = 3 * pair / 63 * 0.95
    side.add_paced(o_to_token_major(0, range(4)), period / 2)
    for c in range(8):
        side.add_paced(y_to_token_major(c), period)
    side.add_paced(y_seam_to_token_major(), period)
    side.add_paced(wo_prep(), period / 2)
    load = 7 * unit / (3 * pair) * 1.05 * 0.95
    side.add("att", attend(range(16, 20), 9), load)
    queries(20, 24, 4)
    side.add("att", attend(range(20, 16 + 7), 9), load)
    queries(24, 32, 4)
    side.close()
    for ct in range(5, 9):
        cp_out(ct, 0, S // 2).start()
    end_region()

    side.open(1.05, 500.0, links=2)
    side.add_paced(o_to_token_major(1, range(1)), 60.0)
    load = (16 - 7) * unit / (9 * 496 + 4 * 144) * 1.0
    side.add("att", attend(range(16 + 7, 32), 9), load)
    for gam in range(4):
        out_tail(0, gam)
    for row0 in range(0, 496, 64):
        out_proj(0, row0, min(64, 496 - row0))
    cp_out(4, 0, 512).start()
    side.close()
    end_region()

    _drain(o_to_token_major(1, range(1, 4)))
    for gam in range(4):
        out_tail(1, gam)
    cp_out(4, 512, 512).start()
    out_proj(0, 496, 512 - 496)
    row0 = 0
    for cw in (64,)*6+(32,)*3+(16,16):
        out_proj(1, row0, cw)
        row0 += cw
    pltpu.make_async_copy(out_hbm, out_hbm, sem_out).wait()


@jax.jit
def pallas_concat_heads__sliding_local_dilated__spectral_gfnet__prompt_kernel(
    A_x: jax.Array,
    A_wqkv: jax.Array,
    A_wo: jax.Array,
    B_x: jax.Array,
    B_w_r: jax.Array,
    B_w_i: jax.Array,
):
    assert A_x.shape == (1, S, D) and B_x.shape == (1, S, D)
    any_spec = pl.BlockSpec(memory_space=pl.ANY)
    scratch = [
        pltpu.VMEM((1,) + _TABLE.shape, U32),
        pltpu.VMEM((16, 288, 128), U32),
        pltpu.VMEM((D, S), BF16),
        pltpu.VMEM((D, 3 * D), BF16),
        pltpu.VMEM((D + 64, D), BF16),
        pltpu.VMEM((1, 16, 144, 128), U32),
        pltpu.VMEM((1, 16, 144, 128), U32),
        pltpu.VMEM((2, 1, S), BF16),
        pltpu.VMEM((1, 16, 3, 128, 128), F32),
        pltpu.VMEM((1, 8, D, 128), U32),
        pltpu.VMEM((1, 8, D, 128), U32),
        pltpu.VMEM((5, 8 * 136, 128), U32),
        pltpu.VMEM((1, 18, 2, NR, 128), F32),
        pltpu.VMEM((1, 16, 2, NR, 128), F32),
        pltpu.VMEM((1, 2, 2, NR, 128), F32),
        [pltpu.VMEM((1, 9 * 128, 128), U32)] * 5,
        pltpu.VMEM((1, 8, 3, 64, 128), U32),
        pltpu.VMEM((1, 5, 320, 128), U32),
        pltpu.VMEM((1, 6, 288, 128), U32),
        pltpu.VMEM((1, 6, 288, 128), U32),
        pltpu.VMEM((1, 6, 288, 128), U32),
        pltpu.VMEM((1, 4, 32, 128), U32),
        pltpu.VMEM((1, 5, 32, 128), U32),
        [pltpu.VMEM((1, 2, D + 16, 128), F32)] * 8,
        [pltpu.VMEM((1, 16, D + 8, 128), F32)] * 2,
        [pltpu.VMEM((1, 16, D + 8, 128), F32)] * 2,
        pltpu.VMEM((1, 4, 2 * W * 8, 128), F32),
        [pltpu.VMEM((1, 8, D // 2, 128), U32)] * 2,
        [pltpu.VMEM((1, 5, 9 * 64, 128), U32)] * 2,
        pltpu.VMEM((1, 8, 128, 128), U32),
        pltpu.VMEM((9, S // 2, 128), U32),
        pltpu.SMEM((4,), jnp.int32),
        pltpu.SemaphoreType.DMA((5,)),
        pltpu.SemaphoreType.REGULAR,
    ]
    out = pl.pallas_call(
        _kernel,
        out_shape=jax.ShapeDtypeStruct((S, 2 * D), BF16),
        in_specs=[any_spec] * 7,
        out_specs=any_spec,
        scratch_shapes=scratch,
        compiler_params=pltpu.CompilerParams(vmem_limit_bytes=120 * 1024 * 1024),
        name="attn_gfnet",
    )(A_x[0].T, A_wqkv, A_wo, B_x[0].T, B_w_r.T, B_w_i.T, _TABLE)
    return out[None]
```

```python
from functools import partial

import numpy as np

import jax
import jax.numpy as jnp
from jax import lax
import jax.experimental.pallas as pl
import jax.experimental.pallas.tpu as pltpu

S = 2048
D = 576
H = 32
DH = 18
W = 8
DF = D // 2 + 1
NR = 296

F32 = jnp.float32
BF16 = jnp.bfloat16
U32 = jnp.uint32

_R9 = float(2 * np.cos(2 * np.pi / 9))
_S9 = float(np.sin(2 * np.pi / 3) / np.sin(2 * np.pi / 9))


def _bfly9_fwd(x):
    tot = [x[j] + x[j + 3] + x[j + 6] for j in range(3)]
    re = [x[j] - x[j + 6] for j in range(3)]
    im = [x[j + 3] - x[j + 6] for j in range(3)]
    ar, ai = re[0] * (_R9 - 1) + im[0], im[0] * _R9 - re[0]
    br, bi = re[1] * _S9, im[1] * _S9
    cr, ci = re[2] * _R9 - im[2], im[2] * (_R9 - 1) + re[2]
    pr, pi, qr, qi = ar - cr, ai - ci, br - cr, bi - ci
    t = pr - qr
    return [tot[0] + tot[1] + tot[2], ar + br + cr, ai + bi + ci, qr - pi, qi + t,
            tot[0] - tot[2], tot[1] - tot[2], pr - qi, pi - t]


def _bfly9_inv(v):
    u0, u1r, u1i, u2r, u2i, u3r, u3i, u4r, u4i = v
    t = u2i - u4i
    pr, pi, qr, qi = u4r + t, u4i - u2r, u2r - t, u2i - u4r
    ar, ai, br, bi = u1r + pr, u1i + pi, u1r + qr, u1i + qi
    cr, ci = u1r - pr - qr, u1i - pi - qi
    re = [ar * (_R9 - 1) - ai, br * _S9, cr * _R9 + ci]
    im = [ai * _R9 + ar, bi * _S9, ci * (_R9 - 1) - cr]
    tot = [u0 + u3r, u0 + u3i, u0 - u3r - u3i]
    return ([tot[j] + re[j] for j in range(3)] + [tot[j] + im[j] for j in range(3)]
            + [tot[j] - re[j] - im[j] for j in range(3)])


def _bfly4(x, inverse):
    (ar, ai), (br, bi), (cr, ci), (dr, di) = x
    pr, pi, qr, qi = ar + cr, ai + ci, ar - cr, ai - ci
    sr, si, tr, ti = br + dr, bi + di, br - dr, bi - di
    y1, y3 = (qr + ti, qi - tr), (qr - ti, qi + tr)
    if inverse:
        y1, y3 = y3, y1
    return [(pr + sr, pi + si), y1, (pr - sr, pi - si), y3]


def _twiddle16(z, e, inverse):
    zr, zi = z
    e = (-e if inverse else e) % 16
    h = float(np.sqrt(0.5))
    if e == 0:
        return z
    if e == 4:
        return zi, -zr
    if e == 12:
        return -zi, zr
    if e == 2:
        return (zr + zi) * h, (zi - zr) * h
    if e == 14:
        return (zr - zi) * h, (zr + zi) * h
    if e == 6:
        return (zi - zr) * h, (zr + zi) * (-h)
    if e == 10:
        return (zr + zi) * (-h), (zr - zi) * h
    c, s = float(np.cos(2 * np.pi * e / 16)), float(np.sin(2 * np.pi * e / 16))
    return zr * c + zi * s, zi * c - zr * s


_GROUPS = (1, 2, 3, 4, 0)


def _group_classes(g):
    return sorted({g, g + 9, 9 - g, 18 - g}) if g else [0, 9]


_ROWGROUPS = [(k0, h) for g in _GROUPS for k0 in _group_classes(g) for h in range(2)]


def _to_words(m):
    u = np.ascontiguousarray(m, dtype=np.float32).view(np.uint32)
    u = (u + 0x7FFF + ((u >> 16) & 1)) >> 16
    return (u[0::2] | (u[1::2] << 16)).astype(np.uint32)


def _coordinates(a, v):
    rhs = [np.sum(row * v) for row in a]
    if len(a) == 1:
        return [rhs[0] / np.sum(a[0] * a[0])]
    g00, g01, g11 = np.sum(a[0] * a[0]), np.sum(a[0] * a[1]), np.sum(a[1] * a[1])
    det = g00 * g11 - g01 * g01
    return [(g11 * rhs[0] - g01 * rhs[1]) / det, (g00 * rhs[1] - g01 * rhs[0]) / det]


def _make_tables():
    basis = np.array(_bfly9_fwd(list(np.eye(9))))
    m_fwd = np.array([2 * (r % 32) + r // 32 for r in range(64)])
    lf, li = [], []
    for g in _GROUPS:
        rows = [k0 + 18 * i for k0 in _group_classes(g) for i in range(16)]
        if g == 0:
            rows += [DF - 1] + [-1] * 7
        cols = [2 * g - 1, 2 * g] if g else [0]
        a = basis[cols]
        n = len(rows)
        f = np.zeros((2 * n, 128))
        b = np.zeros((64 * len(cols), 128))
        for r, k in enumerate(rows):
            if k < 0:
                continue
            ck = np.exp(-2j * np.pi * ((np.arange(9) * k) % 9) / 9)
            lam = _coordinates(a, ck)
            wk = (1.0 if k in (0, DF - 1) else 2.0) / (S * D)
            for c in range(len(cols)):
                e = lam[c] * np.exp(-2j * np.pi * ((m_fwd * k) % D) / D)
                f[r, 64 * c:64 * c + 64] = e.real
                f[n + r, 64 * c:64 * c + 64] = e.imag
                e = wk * lam[c] * np.exp(-2j * np.pi * ((np.arange(64) * k) % D) / D)
                b[64 * c:64 * c + 64, r] = e.real
                b[64 * c:64 * c + 64, n + r] = e.imag
        lf.append(_to_words(f))
        li.append(_to_words(b))
    n = np.arange(128)
    b_of_n = 16 * (n // 16) + 8 * (n % 2) + (n % 16) // 2
    f128 = np.exp(-2j * np.pi * (np.outer(b_of_n, n) % 128) / 128)
    tw = np.exp(-2j * np.pi * np.outer(np.arange(16), n) / S)
    f32w = lambda m: np.ascontiguousarray(m, dtype=np.float32).view(np.uint32)
    parts = [f32w(f128.real), f32w(f128.imag), f32w(tw.real), f32w(tw.imag)] + lf + li
    offs = np.cumsum([0] + [p.shape[0] for p in parts])
    parts.append(np.zeros((-offs[-1] % 32, 128), np.uint32))
    return np.concatenate(parts, axis=0), [int(o) for o in offs]


_TABLE, _OFF = _make_tables()
_OFF_FR, _OFF_FI, _OFF_TR, _OFF_TI = _OFF[0:4]
_OFF_LF = _OFF[4:10]
_OFF_LI = _OFF[9:15]


def _pack(lo, hi):
    return pltpu.pack_elementwise([lo, hi], packed_dtype=BF16)


def _unpack(w, index):
    return pltpu.unpack_elementwise(w, index=index, packed_dtype=BF16, unpacked_dtype=F32)


def _bf(words):
    return pltpu.bitcast(words, BF16)


def _dot(a, b):
    return lax.dot_general(a, b, (((1,), (0,)), ((), ())), preferred_element_type=F32)


def _dot_nt(a, b):
    return lax.dot_general(a, b, (((1,), (1,)), ((), ())), preferred_element_type=F32)


def _zeros_w(rows):
    return jnp.zeros((rows, 128), U32)


class _SideWork:
    LINK = 7.0
    HOP = 6.0

    def __init__(self, zero_ref):
        self.zero_ref = zero_ref
        self.zero = zero_ref[0]

    def start(self, seed, sink):
        self.chain = pltpu.bitcast(seed, F32)
        self.sink = sink
        self.jobs = []
        self.paced = []
        self.pending = []
        self.regions = 0
        self.credit = self.delay = self.clock = 0.0

    def open(self, stretch=0.0, slack=100.0, links=4):
        self.links = links
        self.zero = self.zero_ref[0]
        self.lead = -slack
        self.stretch = stretch

    def add(self, name, job, load, first=False):
        self.jobs.insert(0 if first else len(self.jobs), (name, job, load))

    def add_paced(self, job, period):
        if not self.paced:
            self.due = self.clock
        self.paced.append((job, period))

    def _absorb(self, item):
        values, cycles, latency = (item + (0.0,))[:3]
        values = values if isinstance(values, list) else [values]
        values = [pltpu.bitcast(v, F32) for v in values]
        while len(values) > 1:
            values = [values[i] + values[i + 1] if i + 1 < len(values) else values[i]
                      for i in range(0, len(values), 2)]
        self.pending.append((self.clock + latency, values[0]))
        self.pending.sort(key=lambda x: x[0])
        return cycles

    def _step_paced(self):
        item = next(self.paced[0][0], None)
        if item is None:
            self.paced.pop(0)
        else:
            self._absorb(item)
            self.due += self.stretch * self.paced[0][1]

    def _tick(self, cycles):
        while self.paced and self.due <= self.clock:
            self._step_paced()
        self.clock += cycles
        self.delay += cycles
        while self.pending and self.pending[0][0] <= self.clock:
            self.chain = self.pending.pop(0)[1] + self.chain
            self.delay -= 2.0
        n = int(self.delay / self.LINK)
        if n >= self.links:
            for _ in range(n):
                self.chain = pl.reciprocal(self.chain, approx=True)
            self.delay -= n * self.LINK

    def _step(self):
        item = next(self.jobs[0][1], None)
        if item is None:
            self.jobs.pop(0)
            return
        cycles = self._absorb(item) / self.jobs[0][2]
        self.credit -= cycles
        self.lead += cycles
        while self.lead >= self.HOP:
            self.zero = self.zero_ref[self.zero]
            self.lead -= self.HOP
        self._tick(self.stretch * cycles)

    def run(self, cycles):
        self.credit += cycles
        while self.jobs and self.credit > 0:
            self._step()
        while not self.jobs and self.credit > 0:
            n = min(self.credit, 50.0) if self.paced else self.credit
            self._tick(self.stretch * n)
            self.credit -= n

    def finish(self, name):
        while any(job[0] == name for job in self.jobs):
            self._step()

    def close(self):
        while self.jobs:
            self._step()
        while self.paced:
            self._step_paced()
        while self.pending:
            self.chain = self.pending.pop(0)[1] + self.chain
        self.sink[pl.ds(8 * self.regions, 8), :] = self.chain
        self.regions += 1
        self.credit = self.delay = 0.0


def _drain(gen):
    for _ in gen:
        pass


_W_COLS = ((0, 512), (512, 640), (1152, 576))


def _kernel(xa_hbm, wqkv_hbm, wo_hbm, xb_hbm, wr_hbm, wi_hbm, tab_hbm, out_hbm,
            tab, xb_raw, xa_raw, wq_raw, wo_raw, wr_raw, wi_raw, wlast,
            gmat, u_t, y_t, u_nat, x1_buf, t_buf, z_buf, x_nat, x_seam, wt_nat, wt_q, wt_k, wt_v,
            wo_diff, wo_tail, q_buf, k_buf, v_buf, p_buf, o_t, o_nat, y_seam, stage,
            zero_ref, sem, sem_region):
    zero_ref[0] = pl.semaphore_read(sem_region)
    side = _SideWork(zero_ref)
    zero = side.zero

    def now(ref):
        return ref.at[side.zero]

    tab_r, wr_r, wi_r = tab, wr_raw, wi_raw
    tab, wr_raw, wi_raw = tab.at[0], wr_raw.at[0], wi_raw.at[0]
    t_r, wn_r, q_r, k_r, v_r, p_r = t_buf, wt_nat, q_buf, k_buf, v_buf, p_buf
    u_r, y_r, g_r = u_t, y_t, gmat
    (gmat, u_t, y_t, x1_buf, t_buf, z_buf, x_nat, x_seam, wt_nat, wt_q, wt_k, wt_v, wo_diff,
     wo_tail, q_buf, k_buf, v_buf, p_buf, o_t, o_nat, y_seam) = jax.tree.map(
        lambda r: r.at[zero],
        (gmat, u_t, y_t, x1_buf, t_buf, z_buf, x_nat, x_seam, wt_nat, wt_q, wt_k, wt_v, wo_diff,
         wo_tail, q_buf, k_buf, v_buf, p_buf, o_t, o_nat, y_seam))
    wt = (wt_q, wt_k, wt_v)

    sem_xb, sem_tab, sem_f, sem_out, sem_k = (sem.at[i] for i in range(5))

    def cp_tab(row0, rows):
        return pltpu.make_async_copy(
            tab_hbm.at[pl.ds(row0, rows)], tab.at[pl.ds(row0, rows)], sem_tab)

    def cp_xb(t):
        return pltpu.make_async_copy(
            xb_hbm.at[:, pl.ds(t * 128, 128)], xb_raw.at[t].bitcast(BF16), sem_xb)

    def cp_xa(half, row0, rows, sem_):
        rows, cols = pl.ds(row0, rows), pl.ds(S // 2 * half, S // 2)
        return pltpu.make_async_copy(xa_hbm.at[rows, cols], xa_raw.at[rows, cols], sem_)

    def cp_wq(part, row0, rows, sem_):
        rows, cols = pl.ds(row0, rows), pl.ds(*_W_COLS[part])
        return pltpu.make_async_copy(wqkv_hbm.at[rows, cols], wq_raw.at[rows, cols], sem_)

    def cp_wo(row0=0, rows=D):
        return pltpu.make_async_copy(
            wo_hbm.at[pl.ds(row0, rows)], wo_raw.at[pl.ds(row0, rows)], sem_f)

    def cp_f(i, t):
        src, dst = ((wr_hbm, wr_raw), (wi_hbm, wi_raw))[i]
        return pltpu.make_async_copy(
            src.at[pl.ds(0, DF - 1), pl.ds(t * 128, 128)], dst.at[t].bitcast(BF16),
            sem_f)

    def cp_flast(i):
        src = (wr_hbm, wi_hbm)[i]
        return pltpu.make_async_copy(src.at[pl.ds(DF - 1, 1), :], wlast.at[i], sem_f)

    def cp_out(ct, row0, rows):
        return pltpu.make_async_copy(
            stage.at[ct, pl.ds(row0, rows), :].bitcast(BF16),
            out_hbm.at[pl.ds(2 * row0, 2 * rows), pl.ds(ct * 128, 128)], sem_out)

    def fetch_xb(t, v):
        xb_raw[t, pl.ds(0, 8), :] = v
        cp_xb(t).start()

    def fetch_wq(part, row0, rows, sem_, v):
        wq_raw[pl.ds(row0, 16), pl.ds(_W_COLS[part][0], 128)] = _bf(v)
        cp_wq(part, row0, rows, sem_).start()

    def fetch_xa(half, row0, rows, sem_, v):
        xa_raw[pl.ds(row0, 16), pl.ds(S // 2 * half, 128)] = _bf(v)
        cp_xa(half, row0, rows, sem_).start()

    def fetch_wo(piece, v):
        wo_raw[pl.ds(144 * piece, 16), pl.ds(0, 128)] = _bf(v)
        cp_wo(144 * piece, 144).start()

    def wo_settle(v):
        wo_raw[pl.ds(D, 16), pl.ds(0, 128)] = _bf(v)

    def fetch_tab(row0, rows, v):
        tab[pl.ds(row0, 8), :] = v
        cp_tab(row0, rows).start()

    def fetch_f(t, v):
        wr_raw[t, pl.ds(0, 8), :] = v
        cp_f(0, t).start()
        wi_raw[t, pl.ds(0, 8), :] = v
        cp_f(1, t).start()
        if t == 0:
            cp_flast(0).start()
            cp_flast(1).start()

    n_tab = _TABLE.shape[0]
    fetches = []

    def fetch_next(value):
        if fetches:
            for fetch in fetches.pop(0):
                fetch(pltpu.bitcast(value[:8, :128], U32))

    def store_pitched(dst, row0, vt):
        for r in range(16):
            dst[pl.ds(row0 + 17 * (r // 2) + 8 * (r % 2), 8), :] = vt[8 * r:8 * r + 8]

    def radix9(tau):
        for i in range(4):
            words = [[xb_raw[side.zero + 2 * tau + z, pl.ds(32 * j + 8 * i, 8), :]
                      for j in range(9)] for z in range(2)]
            for e in range(2):
                u = []
                for z in range(2):
                    u.append(_bfly9_fwd([_unpack(w, e) for w in words[z]]))
                    yield u[z][8], 12
                out = [_pack(u[0][o], u[1][o]) for o in range(9)]
                for o in range(9):
                    u_t[tau, pl.ds(64 * o + 32 * e + 8 * i, 8), :] = out[o]
                if tau == i == e == 0:
                    out[8] = now(u_r)[0, pl.ds(512, 8), :]
                yield out, 5

    def u_to_token_major(gi):
        g = _GROUPS[gi]
        for tau in range(8):
            if g:
                v = u_t[tau, pl.ds(64 * (2 * g - 1), 128), :]
            else:
                v = jnp.concatenate([u_t[tau, pl.ds(0, 64), :], _zeros_w(64)], axis=0)
            vt = v.T
            store_pitched(u_nat.at[gi], 136 * tau, vt)
            yield vt[120:], 43, 240

    def dft_matrix(a):
        twr = jnp.broadcast_to(pltpu.bitcast(tab[pl.ds(_OFF_TR + a, 1), :], F32), (8, 128))
        twi = jnp.broadcast_to(pltpu.bitcast(tab[pl.ds(_OFF_TI + a, 1), :], F32), (8, 128))
        for i in range(16):
            fr = pltpu.bitcast(now(tab_r)[pl.ds(_OFF_FR + 8 * i, 8), :], F32)
            fi = pltpu.bitcast(now(tab_r)[pl.ds(_OFF_FI + 8 * i, 8), :], F32)
            gr, gi = fr * twr - fi * twi, fr * twi + fi * twr
            gmat[a, 0, pl.ds(8 * i, 8), :] = gr
            out = [gr + gi, gi - gr]
            gmat[a, 1, pl.ds(8 * i, 8), :] = out[0]
            gmat[a, 2, pl.ds(8 * i, 8), :] = out[1]
            if a == i == 0:
                out[1] = now(g_r)[0, 2, pl.ds(0, 8), :]
            yield out, 3

    def filter_rows(row0, load_w):
        rows = pl.ds(row0, 8)
        y = [[None] * 4 for _ in range(4)]
        for a0 in range(4):
            src = now(t_r)
            z = _bfly4([(src[4 * a1 + a0, 0, rows, :], src[4 * a1 + a0, 1, rows, :])
                        for a1 in range(4)], False)
            for g0 in range(4):
                y[g0][a0] = _twiddle16(z[g0], a0 * g0, False)
            yield y[3][a0][0], 7
        for g0 in range(4):
            z = _bfly4(y[g0], False)
            yield z[3][1], 4
            for g1 in range(4):
                wr, wi = load_w(g0 + 4 * g1)
                zr, zi = z[g1]
                z[g1] = (zr * wr - zi * wi, zr * wi + zi * wr)
                if g1 % 2:
                    yield z[g1][1], 4
            z = _bfly4(z, True)
            for a0 in range(4):
                y[g0][a0] = _twiddle16(z[a0], a0 * g0, True)
            yield y[g0][3][0], 6
        for a0 in range(4):
            z = _bfly4([y[g0][a0] for g0 in range(4)], True)
            for a1 in range(4):
                t_buf[4 * a1 + a0, 0, rows, :] = z[a1][0]
                t_buf[4 * a1 + a0, 1, rows, :] = z[a1][1]
            yield [v for pair in z for v in pair], 6

    def filter_all():
        for n, (k0, h) in enumerate(_ROWGROUPS):
            rows = pl.ds(k0 // 2 + 72 * h, 8, stride=9)
            yield from filter_rows(8 * n, lambda f1: (
                _unpack(now(wr_r)[f1, rows, :], k0 % 2),
                _unpack(now(wi_r)[f1, rows, :], k0 % 2)))
        yield from filter_rows(NR - 8, lambda f1: tuple(
            jnp.broadcast_to(wlast[i, :, pl.ds(128 * f1, 128)].astype(F32), (8, 128))
            for i in range(2)))

    def radix9_inv(c):
        for i in range(8):
            y = []
            for e in range(2):
                y.append(_bfly9_inv(
                    [now(t_r)[2 * c + e, i // 4, pl.ds(256 + 8 * (i % 4), 8), :]]
                    + [now(t_r)[2 * c + e, o % 2, pl.ds(64 * (o // 2) + 8 * i, 8), :]
                       for o in range(8)]))
                yield y[e][8], 10
            out = [_pack(y[0][j], y[1][j]) for j in range(9)]
            for j in range(9):
                y_t[c, pl.ds(64 * j + 8 * i, 8), :] = out[j]
            if c == i == 0:
                out[8] = now(y_r)[0, pl.ds(512, 8), :]
            yield out, 5

    def y_to_token_major(c):
        for q in range(4):
            vt = y_t[c, pl.ds(64 + 128 * q, 128), :].T
            stage[5 + q, pl.ds(c, 128, stride=8), :] = vt
            yield vt[120:], 43, 240

    def y_seam_to_token_major():
        for c in range(8):
            vt = jnp.concatenate([_zeros_w(64), y_t[c, pl.ds(0, 64), :]], axis=0).T
            y_seam[c] = vt
            yield vt[120:], 43, 240

    def k_rows(kt):
        return min(128 * kt, D - 128)

    def x_to_token_major(half, kts):
        for kt in kts:
            for t in range(8 * half, 8 * half + 8):
                vt = xa_raw[pl.ds(k_rows(kt), 128), pl.ds(128 * t, 128)].T
                vt = pltpu.bitcast(vt, U32)
                for u in range(8):
                    x_nat[kt][pl.ds(72 * t + 9 * u, 8), :] = vt[8 * u:8 * u + 8]
                yield vt[56:], 22, 180

    def x_rows(half, c, i=0, n=64):
        return pl.ds(576 * half + 9 * i + c, n, stride=9)

    def difference(u, v):
        return _pack(_unpack(u, 0) - _unpack(v, 0), _unpack(u, 1) - _unpack(v, 1))

    def low_lanes(rows, n=64):
        return lax.broadcasted_iota(jnp.int32, (rows, 128), 1) < n

    def x_prep(half, gam):
        for i in range(0, 64, 8):
            (a3, a4), (b3, b4) = [[x_nat[kt][x_rows(half, 2 * gam + e, i, 8), :] for kt in (3, 4)]
                                  for e in range(2)]
            out = [jnp.where(low_lanes(8), lo, hi) for lo, hi in
                   ((a3, difference(a3, b3)), (b3, difference(b4, a4)), (b4, a4))]
            for j in range(3):
                x_seam[4 * half + gam, j, pl.ds(i, 8), :] = out[j]
            yield out, 5

    def w_prep(part, kts=range(5)):
        col0, _ = _W_COLS[part]
        first = 288 * part - col0 // 2
        for kt in kts:
            for nt in range(5):
                nn = min(128, 3 * D - col0 - 128 * nt)
                vt = wq_raw[pl.ds(k_rows(kt), 128), pl.ds(col0 + 128 * nt, nn)].T
                vt = pltpu.bitcast(vt, U32)
                wt_nat[kt, pl.ds(64 * nt, nn // 2), :] = vt
                yield vt[-8:], 22, 180
        for kt in kts:
            for i in range(2):
                for dl in range(9):
                    base = first + 144 * i + dl
                    wa = now(wn_r)[kt, pl.ds(base, 8, stride=18), :]
                    wb = now(wn_r)[kt, pl.ds(base + 9, 8, stride=18), :]
                    out = [_pack(_unpack(wa, e), _unpack(wb, e)) for e in range(2)]
                    for e in range(2):
                        rows = pl.ds(16 * (2 * dl + e) + 8 * i, 8)
                        wt[part][kt, rows, :] = out[e]
                        if kt == 4:
                            wt[part][5, rows, :] = jnp.where(
                                low_lanes(8), wt[part][3, rows, :], out[e])
                    yield out, 2 + 2 * (kt == 4)

    def wo_tile(row0, rows, ct):
        return wo_raw[pl.ds(row0, rows), pl.ds(128 * ct, 128)]

    def wo_prep():
        for ct in range(4):
            words = [pltpu.bitcast(wo_tile(448 + 64 * (ct % 2), 64, c), U32) for c in (ct, ct ^ 1)]
            wo_diff[ct] = difference(*words)
        for kt in range(5):
            vt = wo_raw[pl.ds(k_rows(kt), 128), pl.ds(512, 64)].T
            vt = pltpu.bitcast(vt, U32)
            wo_tail[kt] = vt
            yield vt[24:], 22, 180

    scale = float(DH) ** -0.5

    def softmax(unit, d_block):
        half, gam, hg = unit // 16, unit // 4 % 4, unit % 4
        base = 2 * gam + 1
        acc = [[None] * W for _ in range(2)]
        for d0 in range(0, DH, d_block):
            rows = [pl.ds(144 * hg + 8 * d, 8) for d in range(d0, d0 + d_block)]
            q = [[now(q_r[4 * half + gam])[e, r, :] for r in rows] for e in range(2)]
            for l in range(9):
                for n, r in enumerate(rows):
                    k = now(k_r[half])[base + l, r, :]
                    for e in range(2):
                        w = 7 + e - l
                        if 0 <= w < W:
                            t = q[e][n] * k
                            acc[e][w] = t if acc[e][w] is None else acc[e][w] + t
                done = [acc[e][7 + e - l] for e in range(2) if 0 <= 7 + e - l < W]
                yield done, d_block / 2 * len(done)
        prob = []
        for e in range(2):
            lg = [jnp.where(low_lanes(8, 2), -1e9 / scale, acc[e][w])
                  if half == 0 and 2 * gam + e < w else acc[e][w] for w in range(W)]
            m = lg[0]
            for w in range(1, W):
                m = jnp.maximum(m, lg[w])
            ex = [jnp.exp2((l_ - m) * (scale * float(np.log2(np.e)))) for l_ in lg]
            tot = ex[0]
            for w in range(1, W):
                tot = tot + ex[w]
            inv = pl.reciprocal(tot, approx=True)
            inv = inv + inv * (1.0 - tot * inv)
            prob.append([x_ * inv for x_ in ex])
            yield prob[e][W - 1], 11, 30
        return prob

    def weigh_values(unit, prob):
        half, gam, hg = unit // 16, unit // 4 % 4, unit % 4
        base = 2 * gam + 1
        for d in range(DH):
            vv = [now(v_r[half])[base + l, pl.ds(144 * hg + 8 * d, 8), :] for l in range(9)]
            o = []
            for e in range(2):
                t = prob[e][0] * vv[7 + e]
                for w in range(1, W):
                    t = t + prob[e][w] * vv[7 + e - w]
                o.append(t)
            if d % 2:
                o = [_pack(even[e], o[e]) for e in range(2)]
                for e in range(2):
                    o_t[half][2 * gam + e, pl.ds(72 * hg + d // 2, 8, stride=DH // 2), :] = o[e]
            even = o
            yield o, 8

    def attend(units, d_block):
        for n in units:
            prob = yield from softmax(n, d_block)
            yield from weigh_values(n, prob)

    def softmax_ahead(units, d_block):
        for n in units:
            prob = yield from softmax(n, d_block)
            for e in range(2):
                for w in range(W):
                    p_buf[n, pl.ds(8 * (W * e + w), 8), :] = prob[e][w]

    def weigh_values_later(units):
        for n in units:
            prob = [[now(p_r)[n, pl.ds(8 * (W * e + w), 8), :] for w in range(W)]
                    for e in range(2)]
            yield from weigh_values(n, prob)

    def o_to_token_major(half, gams):
        for c in [2 * gam + e for gam in gams for e in range(2)]:
            for kt in range(5):
                vt = pltpu.bitcast(_bf(o_t[half][c, pl.ds(k_rows(kt) // 2, 64), :]).T, U32)
                o_nat[half][kt, pl.ds(c, 64, stride=9), :] = vt
                yield vt[56:], 22, 180

    def table(off, i):
        return _bf(tab[pl.ds(off[i], off[i + 1] - off[i]), :])

    def dft64(a, gi):
        x1 = _dot_nt(table(_OFF_LF, gi), _bf(u_nat[gi, pl.ds(a, 64, stride=17), :]))
        n = x1.shape[0] // 2
        side.run(n / 2)
        x1_buf[a, 0, pl.ds(64 * gi, n), :] = x1[:n]
        x1_buf[a, 1, pl.ds(64 * gi, n), :] = x1[n:]
        if a % 4 == 3:
            fetch_next(x1)

    def dft128(a):
        side.run(222)
        xr, xi = x1_buf[a, 0], x1_buf[a, 1]
        k1 = _dot(xr + xi, gmat[a, 0])
        t_buf[a, 0] = k1 - _dot(xi, gmat[a, 1])
        t_buf[a, 1] = k1 + _dot(xr, gmat[a, 2])

    def idft128(a):
        side.run(222)
        g = [jnp.concatenate([gmat[a, c, pl.ds(16 * tau + e, 8, stride=2), :]
                              for tau in range(8) for e in range(2)], axis=0) for c in range(3)]
        tr, ti = t_buf[a, 0], t_buf[a, 1]
        k1 = _dot_nt(tr + ti, g[0])
        z_buf[a % 2, 0] = k1 + _dot_nt(ti, g[2])
        z_buf[a % 2, 1] = k1 - _dot_nt(tr, g[1])

    def idft64(a):
        side.run(144)
        for gi in range(5):
            n = 64 if gi < 4 else NR - 256
            parts = [z_buf[a % 2, c, pl.ds(64 * gi, n), :] for c in range(2)]
            if n < 64:
                parts.append(jnp.zeros((128 - 2 * n, 128), F32))
            o = _dot(table(_OFF_LI, gi), jnp.concatenate(parts, axis=0))
            if gi < 4:
                t_buf[a, 0, pl.ds(64 * gi, 64), :] = o[:64]
                t_buf[a, 1, pl.ds(64 * gi, 64), :] = o[64:]
            else:
                t_buf[a, 0, pl.ds(256, 32), :] = o[:32]
                t_buf[a, 1, pl.ds(256, 32), :] = o[32:]

    def proj(part, half, gam, kts=(0, 1, 2, 3), chunks=4, only=None):
        m = 288 // chunks
        last = kts[-1] == 3
        for ch in only or range(chunks):
            side.run((len(kts) + last / 2) * m)
            w = lambda kt: _bf(wt[part][kt, pl.ds(m * ch, m), :])
            both = _dot_nt(w(4), _bf(x_seam[4 * half + gam, 2])) if last else None
            for e in range(2):
                c = 2 * gam + e
                tile = _dot_nt(
                    jnp.concatenate([w(3 + 2 * e if kt == 3 else kt) for kt in kts], axis=1),
                    jnp.concatenate([_bf(x_seam[4 * half + gam, e] if kt == 3
                                         else x_nat[kt][x_rows(half, c), :]) for kt in kts], axis=1))
                if last:
                    tile = tile + both
                if part == 0:
                    buf, slot = q_buf[4 * half + gam], e
                else:
                    buf, slot = (k_buf if part == 1 and last else v_buf)[half], 8 + c
                rows = []
                for i in range(m // 4):
                    d, hg = divmod(m // 4 * ch + i, 4)
                    rows.append(pl.ds(144 * hg + 8 * d, 8))
                if kts[0]:
                    sums = v_buf[half] if part else buf
                    tile = tile + jnp.concatenate([sums[slot, r, :] for r in rows], axis=0)
                for i, r in enumerate(rows):
                    buf[slot, r, :] = tile[8 * i:8 * i + 8]
                if part == 0 or not last:
                    continue
                if c:
                    if half:
                        before = (k_buf, v_buf)[part - 1][0]
                        tile = jnp.where(low_lanes(2 * m, 126), tile, jnp.concatenate(
                            [before[slot, r, :] for r in rows], axis=0))
                    tile = pltpu.roll(tile, 2, 1)
                    for i, r in enumerate(rows):
                        buf[c, r, :] = tile[8 * i:8 * i + 8]
                        if part == 2 and half == 0:
                            pltpu.store(buf.at[c, r, :], buf[0, r, :], mask=low_lanes(8, 2))
                elif part == 2 and half == 0:
                    tile = jnp.where(low_lanes(2 * m, 1), tile, pltpu.roll(tile, 1, 1))
                    for i, r in enumerate(rows):
                        buf[0, r, :] = tile[8 * i:8 * i + 8]
            fetch_next(tile)

    def out_proj(half, row0, cw):
        side.run(9 * cw)
        o = [jnp.concatenate([o_nat[half][kt, pl.ds(9 * b, 8), :]
                              for b in range(row0 // 8, (row0 + cw) // 8)], axis=0)
             for kt in range(5)]
        lhs = [jnp.concatenate([_bf(t) for t in o[:3] + [last]], axis=1)
               for last in (o[3], jnp.where(low_lanes(cw), o[3], o[4]))]
        both = _dot(_bf(o[4]), jnp.concatenate(
            [jnp.concatenate([wo_tile(448, 64, ct + 1), wo_tile(512, 64, ct)], axis=0)
             for ct in (0, 2)], axis=1))
        r = [_dot(lhs[n], jnp.concatenate(
            [jnp.concatenate([wo_tile(0, 448, ct), _bf(wo_diff[ct])], axis=0)
             for ct in (n, n + 2)], axis=1)) for n in range(2)]
        for ct in (0, 2, 1, 3):
            cols = slice(128 * (ct // 2), 128 * (ct // 2) + 128)
            tile = (r[ct % 2][:, cols] + both[:, cols]).astype(BF16)
            stage[ct, pl.ds(512 * half + row0, cw), :] = pltpu.bitcast(tile, U32)
            cp_out(ct, 512 * half + row0, cw).start()

    def out_tail(half, gam):
        side.run(144)
        o = [o_t[half][2 * gam + e] for e in range(2)]
        w = [wo_tail[kt] for kt in range(5)]
        both = _dot(_bf(w[4]), _bf(jnp.concatenate([o[1][224:256], o[0][256:]], axis=0)))
        for e, last in enumerate((w[3], jnp.where(low_lanes(32), w[3], w[4]))):
            c, rows = 2 * gam + e, slice(224 + 32 * e, 256 + 32 * e)
            tile = both + _dot(
                jnp.concatenate([_bf(t) for t in w[:3] + [last]], axis=1),
                _bf(jnp.concatenate([o[e][:224], difference(o[e][rows], o[1 - e][rows])], axis=0)))
            tile = jnp.concatenate([tile.astype(BF16), jnp.zeros((64, 128), BF16)], axis=0)
            stage[4, pl.ds(512 * half + c, 64, stride=8), :] = jnp.where(
                low_lanes(64), pltpu.bitcast(tile.T, U32), y_seam[c, pl.ds(64 * half, 64), :])

    pair = 1296
    unit = 315

    def end_region():
        pl.semaphore_signal(sem_region)
        pl.semaphore_wait(sem_region)

    def queries(i0, i1, chunks=4):
        while i0 < i1:
            n = chunks if i0 % (4 // chunks) == 0 and i0 + 4 // chunks <= i1 else 4
            proj(0, i0 // 16, i0 // 4 % 4, (1, 2, 3) if i0 < 4 * 3 else (0, 1, 2, 3),
                 chunks=n, only=(i0 % 4 * n // 4,))
            i0 += 4 // n

    def cycles(i0, i1):
        return sum(pair / 4 - 72 * (i < 4 * 3) for i in range(i0, i1))

    blocks = ((0,128,(0,)),(128,256,(1,2)),(384,D-384,(3,)))

    def fetch_block(i):
        cp_wq(1, *blocks[i][:2], sem.at[i]).start()
        cp_xa(0, *blocks[i][:2], sem.at[i]).start()

    cp_xa(0, 0, 128, sem.at[0]).start()
    cp_wq(1, 0, 128, sem_k).start()
    cp_wq(0, 0, 128, sem_out).start()
    fetch_block(1)
    cp_xa(0, 0, 128, sem.at[0]).wait()
    fetch_block(2)
    _drain(x_to_token_major(0, (0,)))
    cp_wq(1, 0, 128, sem_k).wait()
    _drain(w_prep(1, (0,)))
    cp_wq(0, 0, 128, sem_out).wait()
    side.start(pltpu.bitcast(wq_raw[pl.ds(0, 16), pl.ds(512, 128)], U32), x1_buf.at[16, 0])
    fetches += [[partial(fetch_xa, 1, r, 192, sem_k)] for r in range(0, D, 192)]
    for i, (row0, rows, kts) in enumerate(blocks):
        if i:
            cp_wq(1, row0, rows, sem.at[i]).wait()
            cp_xa(0, row0, rows, sem.at[i]).wait()
        if i == 1:
            fetches += [[partial(fetch_wq, 0, r, 224, sem_xb)] for r in range(128, D, 224)]
            fetches += [[partial(fetch_xb, t)] for t in range(16)]
        if i == 2:
            fetches += [[partial(fetch_wq, 2, r, 144, sem_tab) for r in range(0, D, 144)]]
            fetches += [[partial(fetch_tab, r, min(304, n_tab - r)) for r in range(0, n_tab, 304)]]
        side.open()
        tiles = kts + (4,) * (i == 2)
        if i:
            side.add("prep", w_prep(1, tiles), 0.8)
            side.add("prep", x_to_token_major(0, tiles), 0.8)
        if i == 2:
            side.add("prep", x_prep(0, 0), 0.8)
        if i:
            for gam in range((4,2,2)[i - 1], 4):
                proj(1, 0, gam, blocks[i - 1][2])
        if i == 1:
            for gam in range(0, 3):
                proj(0, 0, gam, (0,))
        side.finish("prep")
        if i == 0 and not 0:
            side.add("q", w_prep(0, (0,)), 0.5)
        for gam in range((4,2,2)[i]):
            if i == 2:
                side.add("next", x_prep(0, gam + 1), 0.5)
            proj(1, 0, gam, kts)
            side.finish("next")
        if i == 0:
            side.finish("q")
            for gam in range(0):
                proj(0, 0, gam, (0,))
        if i == 2:
            for gam in range((4,2,2)[i] + 1, 4):
                side.add("next", x_prep(0, gam), 0.5)
        side.close()

    cp_xa(1, 0, D, sem_k).wait()
    side.open()
    fetches += [[partial(fetch_f, t) for t in range(4)]]
    side.add("prep", x_to_token_major(1, range(5)), 0.8)
    side.add("prep", x_prep(1, 0), 0.8)
    for gam in range((4,2,2)[2], 4):
        proj(1, 0, gam, blocks[2][2])
    side.finish("prep")
    for gam in range(3):
        side.add("next", x_prep(1, gam + 1), 0.5)
        proj(1, 1, gam, only=range(4 - 2 * (gam == 2)))
        side.finish("next")
    side.close()

    assert not fetches
    pltpu.make_async_copy(xb_raw, xb_raw, sem_xb).wait()
    cp_wq(0, 128, D - 128, sem_xb).wait()
    side.open(0.95, 20.0, links=4)
    load = (8 * 232 + 620) / (pair * (4 + 2) / 4 + cycles(0, 7)) * 0.9 * 1.05
    side.add("w", w_prep(0, range(1, 5)), load)
    for tau in range(8):
        side.add("r9", radix9(tau), load)
    if 2:
        proj(1, 1, 2, only=range(4 - 2, 4))
    proj(1, 1, 3)
    side.finish("w")
    queries(0, 7, 4)
    side.close()

    cp_tab(0, n_tab).wait()
    cp_wq(2, 0, D, sem_tab).wait()
    side.open(0.95, 50.0, links=2)
    fetches += [[partial(fetch_f, t)] for t in range(4, 16)]
    fetches += [[partial(fetch_wo, i)] for i in range(4)]
    fetches.append([wo_settle])
    side.add("t", u_to_token_major(0), 0.9 * 0.95)
    load = (768 + 766 + 3 * 168) / (5920 + cycles(7, 10) - 2000.0) * 1.0 * 0.95
    for a in range(16):
        side.add("g%d" % a, dft_matrix(a), load)
    queries(7, 10)
    side.finish("t")
    for gi in range(5):
        if gi < 4:
            side.add("t", u_to_token_major(gi + 1), 0.9 * 0.95, first=True)
        for a in range(16):
            dft64(a, gi)
        side.finish("t")
    side.add("w", w_prep(2), load)
    side.add("att", softmax_ahead(range(3), 6), load)
    for a in range(16):
        side.finish("g%d" % a)
        dft128(a)
    side.close()

    assert not fetches
    pltpu.make_async_copy(wr_raw, wr_raw, sem_f).wait()
    pltpu.make_async_copy(wi_raw, wi_raw, sem_f).wait()
    cp_flast(0).wait()
    cp_flast(1).wait()
    cp_wo().wait()
    side.open(1.0, 300.0, links=2)
    side.add("f", filter_all(), 37 * 120 / (4 * pair + cycles(10, 19)) * 1.0)
    for gam in range(4):
        proj(2, 0, gam, chunks=4)
    queries(10, 19, 4)
    side.close()
    end_region()

    side.open(0.95, 400.0, links=2)
    load = (16 * unit - 3 * 168 + 8 * 200) / (5856 + 4 * pair + cycles(19, 20)) * 1.0
    side.add("att", weigh_values_later(range(3)), load)
    side.add("att", attend(range(3, 16), 9), load)
    idft128(0)
    for a in range(16):
        if a < 15:
            idft128(a + 1)
        idft64(a)
    for c in range(8):
        side.add("r9", radix9_inv(c), load * 1.05)
    for gam in range(4):
        proj(2, 1, gam, chunks=1)
    queries(19, 20)
    side.close()
    end_region()

    side.open(0.9, 100.0, links=2)
    period = 3 * pair / 63 * 0.95
    side.add_paced(o_to_token_major(0, range(4)), period / 2)
    for c in range(8):
        side.add_paced(y_to_token_major(c), period)
    side.add_paced(y_seam_to_token_major(), period)
    side.add_paced(wo_prep(), period / 2)
    load = 7 * unit / (3 * pair) * 1.05 * 0.9
    side.add("att", attend(range(16, 20), 6), load)
    queries(20, 24, 4)
    side.add("att", attend(range(20, 16 + 7), 6), load)
    queries(24, 32, 4)
    side.close()
    for ct in range(5, 9):
        cp_out(ct, 0, S // 2).start()
    end_region()

    side.open(1.05, 100.0, links=2)
    side.add_paced(o_to_token_major(1, range(1)), 60.0)
    load = (16 - 7) * unit / (9 * 496 + 4 * 144) * 1.0
    side.add("att", attend(range(16 + 7, 32), 9), load)
    for gam in range(4):
        out_tail(0, gam)
    for row0 in range(0, 496, 64):
        out_proj(0, row0, min(64, 496 - row0))
    cp_out(4, 0, 512).start()
    side.close()
    end_region()

    _drain(o_to_token_major(1, range(1, 4)))
    for gam in range(4):
        out_tail(1, gam)
    cp_out(4, 512, 512).start()
    out_proj(0, 496, 512 - 496)
    row0 = 0
    for cw in (64,)*6+(32,)*3+(16,16):
        out_proj(1, row0, cw)
        row0 += cw
    pltpu.make_async_copy(out_hbm, out_hbm, sem_out).wait()


@jax.jit
def pallas_concat_heads__sliding_local_dilated__spectral_gfnet__prompt_kernel(
    A_x: jax.Array,
    A_wqkv: jax.Array,
    A_wo: jax.Array,
    B_x: jax.Array,
    B_w_r: jax.Array,
    B_w_i: jax.Array,
):
    assert A_x.shape == (1, S, D) and B_x.shape == (1, S, D)
    any_spec = pl.BlockSpec(memory_space=pl.ANY)
    scratch = [
        pltpu.VMEM((1,) + _TABLE.shape, U32),
        pltpu.VMEM((16, 288, 128), U32),
        pltpu.VMEM((D, S), BF16),
        pltpu.VMEM((D, 3 * D), BF16),
        pltpu.VMEM((D + 64, D), BF16),
        pltpu.VMEM((1, 16, 144, 128), U32),
        pltpu.VMEM((1, 16, 144, 128), U32),
        pltpu.VMEM((2, 1, S), BF16),
        pltpu.VMEM((1, 16, 3, 128, 128), F32),
        pltpu.VMEM((1, 8, D, 128), U32),
        pltpu.VMEM((1, 8, D, 128), U32),
        pltpu.VMEM((5, 8 * 136, 128), U32),
        pltpu.VMEM((1, 18, 2, NR, 128), F32),
        pltpu.VMEM((1, 16, 2, NR, 128), F32),
        pltpu.VMEM((1, 2, 2, NR, 128), F32),
        [pltpu.VMEM((1, 9 * 128, 128), U32)] * 5,
        pltpu.VMEM((1, 8, 3, 64, 128), U32),
        pltpu.VMEM((1, 5, 320, 128), U32),
        pltpu.VMEM((1, 6, 288, 128), U32),
        pltpu.VMEM((1, 6, 288, 128), U32),
        pltpu.VMEM((1, 6, 288, 128), U32),
        pltpu.VMEM((1, 4, 32, 128), U32),
        pltpu.VMEM((1, 5, 32, 128), U32),
        [pltpu.VMEM((1, 2, D + 16, 128), F32)] * 8,
        [pltpu.VMEM((1, 16, D + 8, 128), F32)] * 2,
        [pltpu.VMEM((1, 16, D + 8, 128), F32)] * 2,
        pltpu.VMEM((1, 4, 2 * W * 8, 128), F32),
        [pltpu.VMEM((1, 8, D // 2, 128), U32)] * 2,
        [pltpu.VMEM((1, 5, 9 * 64, 128), U32)] * 2,
        pltpu.VMEM((1, 8, 128, 128), U32),
        pltpu.VMEM((9, S // 2, 128), U32),
        pltpu.SMEM((4,), jnp.int32),
        pltpu.SemaphoreType.DMA((5,)),
        pltpu.SemaphoreType.REGULAR,
    ]
    out = pl.pallas_call(
        _kernel,
        out_shape=jax.ShapeDtypeStruct((S, 2 * D), BF16),
        in_specs=[any_spec] * 7,
        out_specs=any_spec,
        scratch_shapes=scratch,
        compiler_params=pltpu.CompilerParams(vmem_limit_bytes=120 * 1024 * 1024),
        name="attn_gfnet",
    )(A_x[0].T, A_wqkv, A_wo, B_x[0].T, B_w_r.T, B_w_i.T, _TABLE)
    return out[None]
```

```python
from functools import partial

import numpy as np

import jax
import jax.numpy as jnp
from jax import lax
import jax.experimental.pallas as pl
import jax.experimental.pallas.tpu as pltpu

S = 2048
D = 576
H = 32
DH = 18
W = 8
DF = D // 2 + 1
NR = DF - 1

F32 = jnp.float32
BF16 = jnp.bfloat16
U32 = jnp.uint32

_R9 = float(2 * np.cos(2 * np.pi / 9))
_S9 = float(np.sin(2 * np.pi / 3) / np.sin(2 * np.pi / 9))


def _bfly9_fwd(x):
    tot = [x[j] + x[j + 3] + x[j + 6] for j in range(3)]
    re = [x[j] - x[j + 6] for j in range(3)]
    im = [x[j + 3] - x[j + 6] for j in range(3)]
    ar, ai = re[0] * (_R9 - 1) + im[0], im[0] * _R9 - re[0]
    br, bi = re[1] * _S9, im[1] * _S9
    cr, ci = re[2] * _R9 - im[2], im[2] * (_R9 - 1) + re[2]
    pr, pi, qr, qi = ar - cr, ai - ci, br - cr, bi - ci
    t = pr - qr
    return [tot[0] + tot[1] + tot[2], ar + br + cr, ai + bi + ci, qr - pi, qi + t,
            tot[0] - tot[2], tot[1] - tot[2], pr - qi, pi - t]


def _bfly9_inv(v):
    u0, u1r, u1i, u2r, u2i, u3r, u3i, u4r, u4i = v
    t = u2i - u4i
    pr, pi, qr, qi = u4r + t, u4i - u2r, u2r - t, u2i - u4r
    ar, ai, br, bi = u1r + pr, u1i + pi, u1r + qr, u1i + qi
    cr, ci = u1r - pr - qr, u1i - pi - qi
    re = [ar * (_R9 - 1) - ai, br * _S9, cr * _R9 + ci]
    im = [ai * _R9 + ar, bi * _S9, ci * (_R9 - 1) - cr]
    tot = [u0 + u3r, u0 + u3i, u0 - u3r - u3i]
    return ([tot[j] + re[j] for j in range(3)] + [tot[j] + im[j] for j in range(3)]
            + [tot[j] - re[j] - im[j] for j in range(3)])


def _bfly4(x, inverse):
    (ar, ai), (br, bi), (cr, ci), (dr, di) = x
    pr, pi, qr, qi = ar + cr, ai + ci, ar - cr, ai - ci
    sr, si, tr, ti = br + dr, bi + di, br - dr, bi - di
    y1, y3 = (qr + ti, qi - tr), (qr - ti, qi + tr)
    if inverse:
        y1, y3 = y3, y1
    return [(pr + sr, pi + si), y1, (pr - sr, pi - si), y3]


def _twiddle16(z, e, inverse):
    zr, zi = z
    e = (-e if inverse else e) % 16
    h = float(np.sqrt(0.5))
    if e == 0:
        return z
    if e == 4:
        return zi, -zr
    if e == 12:
        return -zi, zr
    if e == 2:
        return (zr + zi) * h, (zi - zr) * h
    if e == 14:
        return (zr - zi) * h, (zr + zi) * h
    if e == 6:
        return (zi - zr) * h, (zr + zi) * (-h)
    if e == 10:
        return (zr + zi) * (-h), (zr - zi) * h
    c, s = float(np.cos(2 * np.pi * e / 16)), float(np.sin(2 * np.pi * e / 16))
    return zr * c + zi * s, zi * c - zr * s


_GROUPS = (1, 2, 3, 4, 0)


def _group_classes(g):
    return sorted({g, g + 9, 9 - g, 18 - g}) if g else [0, 9]


_ROWGROUPS = [(k0, h) for g in _GROUPS for k0 in _group_classes(g) for h in range(2)]


def _to_words(m):
    u = np.ascontiguousarray(m, dtype=np.float32).view(np.uint32)
    u = (u + 0x7FFF + ((u >> 16) & 1)) >> 16
    return (u[0::2] | (u[1::2] << 16)).astype(np.uint32)


def _coordinates(a, v):
    rhs = [np.sum(row * v) for row in a]
    if len(a) == 1:
        return [rhs[0] / np.sum(a[0] * a[0])]
    g00, g01, g11 = np.sum(a[0] * a[0]), np.sum(a[0] * a[1]), np.sum(a[1] * a[1])
    det = g00 * g11 - g01 * g01
    return [(g11 * rhs[0] - g01 * rhs[1]) / det, (g00 * rhs[1] - g01 * rhs[0]) / det]


def _make_tables():
    basis = np.array(_bfly9_fwd(list(np.eye(9))))
    m_fwd = np.array([2 * (r % 32) + r // 32 for r in range(64)])
    lf, li = [], []
    for g in _GROUPS:
        rows = [k0 + 18 * i for k0 in _group_classes(g) for i in range(16)]
        cols = [2 * g - 1, 2 * g] if g else [0]
        a = basis[cols]
        n = len(rows)
        f = np.zeros((2 * n, 128))
        b = np.zeros((64 * len(cols), 128))
        for r, k in enumerate(rows):
            ck = np.exp(-2j * np.pi * ((np.arange(9) * k) % 9) / 9)
            lam = _coordinates(a, ck)
            wk = (2.0 if k else 1.0) / (S * D)
            for c in range(len(cols)):
                e = lam[c] * np.exp(-2j * np.pi * ((m_fwd * k) % D) / D)
                f[r, 64 * c:64 * c + 64] = e.real
                f[n + r, 64 * c:64 * c + 64] = e.imag
                e = wk * lam[c] * np.exp(-2j * np.pi * ((np.arange(64) * k) % D) / D)
                b[64 * c:64 * c + 64, r] = e.real
                b[64 * c:64 * c + 64, n + r] = e.imag
        if g == 0:
            f = np.concatenate([f, np.zeros((8, 128))])
            f[2 * n:, :64] = 1 - 2 * (m_fwd % 2)
        lf.append(_to_words(f))
        li.append(_to_words(b))
    n = np.arange(128)
    b_of_n = 16 * (n // 16) + 8 * (n % 2) + (n % 16) // 2
    f128 = np.exp(-2j * np.pi * (np.outer(b_of_n, n) % 128) / 128)
    tw = np.exp(-2j * np.pi * np.outer(np.arange(16), n) / S)
    f32w = lambda m: np.ascontiguousarray(m, dtype=np.float32).view(np.uint32)
    f16 = np.exp(-2j * np.pi * np.outer(n[:16], n[:16]) / 16)
    f16 = np.block([[f16.real, -f16.imag], [f16.imag, f16.real]])
    f16 = [_to_words(np.concatenate([m, np.zeros((32, 96))], axis=1)) for m in (f16, f16.T)]
    parts = [f32w(f128.real), f32w(f128.imag), f32w(tw.real), f32w(tw.imag)] + f16 + lf + li
    parts = [np.concatenate([p, np.zeros((-len(p) % 8, 128), np.uint32)]) for p in parts]
    offs = np.cumsum([0] + [p.shape[0] for p in parts])
    parts.append(np.zeros((-offs[-1] % 32, 128), np.uint32))
    return np.concatenate(parts, axis=0), [int(o) for o in offs]


_TABLE, _OFF = _make_tables()
_OFF_FR, _OFF_FI, _OFF_TR, _OFF_TI = _OFF[0:4]
_OFF_16, _OFF_LF, _OFF_LI = _OFF[4:7], _OFF[6:12], _OFF[11:17]


def _pack(lo, hi):
    return pltpu.pack_elementwise([lo, hi], packed_dtype=BF16)


def _unpack(w, index):
    return pltpu.unpack_elementwise(w, index=index, packed_dtype=BF16, unpacked_dtype=F32)


def _bf(words):
    return pltpu.bitcast(words, BF16)


def _dot(a, b):
    return lax.dot_general(a, b, (((1,), (0,)), ((), ())), preferred_element_type=F32)


def _dot_nt(a, b):
    return lax.dot_general(a, b, (((1,), (1,)), ((), ())), preferred_element_type=F32)


def _zeros_w(rows):
    return jnp.zeros((rows, 128), U32)


class _SideWork:
    LINK = 7.0
    HOP = 6.0

    def __init__(self, zero_ref):
        self.zero_ref = zero_ref
        self.zero = zero_ref[0]

    def start(self, seed, sink):
        self.chain = pltpu.bitcast(seed, F32)
        self.sink = sink
        self.jobs = []
        self.paced = []
        self.pending = []
        self.regions = 0
        self.credit = self.delay = self.clock = 0.0

    def open(self, stretch=0.0, slack=100.0, links=4):
        self.links = links
        self.zero = self.zero_ref[0]
        self.lead = -slack
        self.stretch = stretch

    def add(self, name, job, load, first=False):
        self.jobs.insert(0 if first else len(self.jobs), (name, job, load))

    def add_paced(self, job, period):
        if not self.paced:
            self.due = self.clock
        self.paced.append((job, period))

    def absorb(self, item):
        values, cycles, latency = (item + (0.0,))[:3]
        values = values if isinstance(values, list) else [values]
        values = [pltpu.bitcast(v, F32) for v in values]
        while len(values) > 1:
            values = [values[i] + values[i + 1] if i + 1 < len(values) else values[i]
                      for i in range(0, len(values), 2)]
        self.pending.append((self.clock + latency, values[0]))
        self.pending.sort(key=lambda x: x[0])
        return cycles

    def _step_paced(self):
        item = next(self.paced[0][0], None)
        if item is None:
            self.paced.pop(0)
        else:
            self.absorb(item)
            self.due += self.stretch * self.paced[0][1]

    def _tick(self, cycles):
        while self.paced and self.due <= self.clock:
            self._step_paced()
        self.clock += cycles
        self.delay += cycles
        while self.pending and self.pending[0][0] <= self.clock:
            self.chain = self.pending.pop(0)[1] + self.chain
            self.delay -= 2.0
        n = int(self.delay / self.LINK)
        if n >= self.links:
            for _ in range(n):
                self.chain = pl.reciprocal(self.chain, approx=True)
            self.delay -= n * self.LINK

    def _step(self):
        item = next(self.jobs[0][1], None)
        if item is None:
            self.jobs.pop(0)
            return
        cycles = self.absorb(item) / self.jobs[0][2]
        self.credit -= cycles
        self.lead += cycles
        while self.lead >= self.HOP:
            self.zero = self.zero_ref[self.zero]
            self.lead -= self.HOP
        self._tick(self.stretch * cycles)

    def run(self, cycles):
        self.credit += cycles
        while self.jobs and self.credit > 0:
            self._step()
        while not self.jobs and self.credit > 0:
            n = min(self.credit, 50.0) if self.paced else self.credit
            self._tick(self.stretch * n)
            self.credit -= n

    def finish(self, name):
        while any(job[0] == name for job in self.jobs):
            self._step()

    def close(self):
        while self.jobs:
            self._step()
        while self.paced:
            self._step_paced()
        while self.pending:
            self.chain = self.pending.pop(0)[1] + self.chain
        self.sink[pl.ds(8 * self.regions, 8), :] = self.chain
        self.regions += 1
        self.credit = self.delay = 0.0


def _drain(gen):
    for _ in gen:
        pass


_W_COLS = ((0, 512), (512, 640), (1152, 576))


def _kernel(xa_hbm, wqkv_hbm, wo_hbm, xb_hbm, wr_hbm, wi_hbm, tab_hbm, out_hbm,
            tab, xb_raw, xa_raw, wq_raw, wo_raw, wr_raw, wi_raw, wlast,
            gmat, u_t, y_t, u_nat, x1_buf, t_buf, z_buf, nyq, x_nat, x_seam, wt_nat, wt_q, wt_k, wt_v,
            wo_diff, wo_tail, q_buf, k_buf, v_buf, p_buf, o_t, o_nat, y_seam, stage,
            zero_ref, sem, sem_region):
    zero_ref[0] = pl.semaphore_read(sem_region)
    side = _SideWork(zero_ref)
    zero = side.zero

    def now(ref):
        return ref.at[side.zero]

    tab_r, wr_r, wi_r = tab, wr_raw, wi_raw
    tab, wr_raw, wi_raw = tab.at[0], wr_raw.at[0], wi_raw.at[0]
    t_r, wn_r, q_r, k_r, v_r, p_r = t_buf, wt_nat, q_buf, k_buf, v_buf, p_buf
    u_r, y_r, g_r, nyq_r = u_t, y_t, gmat, nyq
    (gmat, u_t, y_t, x1_buf, t_buf, z_buf, nyq, x_nat, x_seam, wt_nat, wt_q, wt_k, wt_v, wo_diff,
     wo_tail, q_buf, k_buf, v_buf, p_buf, o_t, o_nat, y_seam) = jax.tree.map(
        lambda r: r.at[zero],
        (gmat, u_t, y_t, x1_buf, t_buf, z_buf, nyq, x_nat, x_seam, wt_nat, wt_q, wt_k, wt_v, wo_diff,
         wo_tail, q_buf, k_buf, v_buf, p_buf, o_t, o_nat, y_seam))
    wt = (wt_q, wt_k, wt_v)

    sem_xb, sem_tab, sem_f, sem_out, sem_k = (sem.at[i] for i in range(5))

    def cp_tab(row0, rows):
        return pltpu.make_async_copy(
            tab_hbm.at[pl.ds(row0, rows)], tab.at[pl.ds(row0, rows)], sem_tab)

    def cp_xb(t):
        return pltpu.make_async_copy(
            xb_hbm.at[:, pl.ds(t * 128, 128)], xb_raw.at[t].bitcast(BF16), sem_xb)

    def cp_xa(half, row0, rows, sem_):
        rows, cols = pl.ds(row0, rows), pl.ds(S // 2 * half, S // 2)
        return pltpu.make_async_copy(xa_hbm.at[rows, cols], xa_raw.at[rows, cols], sem_)

    def cp_wq(part, row0, rows, sem_):
        rows, cols = pl.ds(row0, rows), pl.ds(*_W_COLS[part])
        return pltpu.make_async_copy(wqkv_hbm.at[rows, cols], wq_raw.at[rows, cols], sem_)

    def cp_wo(row0=0, rows=D):
        return pltpu.make_async_copy(
            wo_hbm.at[pl.ds(row0, rows)], wo_raw.at[pl.ds(row0, rows)], sem_f)

    def cp_f(i, t):
        src, dst = ((wr_hbm, wr_raw), (wi_hbm, wi_raw))[i]
        return pltpu.make_async_copy(
            src.at[pl.ds(0, DF - 1), pl.ds(t * 128, 128)], dst.at[t].bitcast(BF16),
            sem_f)

    def cp_flast(i):
        src = (wr_hbm, wi_hbm)[i]
        return pltpu.make_async_copy(src.at[pl.ds(DF - 1, 1), :], wlast.at[i], sem_f)

    def cp_out(ct, row0, rows):
        return pltpu.make_async_copy(
            stage.at[ct, pl.ds(row0, rows), :].bitcast(BF16),
            out_hbm.at[pl.ds(2 * row0, 2 * rows), pl.ds(ct * 128, 128)], sem_out)

    def fetch_xb(t, v):
        xb_raw[t, pl.ds(0, 8), :] = v
        cp_xb(t).start()

    def fetch_wq(part, row0, rows, sem_, v):
        wq_raw[pl.ds(row0, 16), pl.ds(_W_COLS[part][0], 128)] = _bf(v)
        cp_wq(part, row0, rows, sem_).start()

    def fetch_xa(half, row0, rows, sem_, v):
        xa_raw[pl.ds(row0, 16), pl.ds(S // 2 * half, 128)] = _bf(v)
        cp_xa(half, row0, rows, sem_).start()

    def fetch_wo(piece, v):
        wo_raw[pl.ds(144 * piece, 16), pl.ds(0, 128)] = _bf(v)
        cp_wo(144 * piece, 144).start()

    def wo_settle(v):
        wo_raw[pl.ds(D, 16), pl.ds(0, 128)] = _bf(v)

    def fetch_tab(row0, rows, v):
        tab[pl.ds(row0, 8), :] = v
        cp_tab(row0, rows).start()

    def fetch_f(t, v):
        wr_raw[t, pl.ds(0, 8), :] = v
        cp_f(0, t).start()
        wi_raw[t, pl.ds(0, 8), :] = v
        cp_f(1, t).start()
        if t == 0:
            cp_flast(0).start()
            cp_flast(1).start()

    n_tab = _TABLE.shape[0]
    fetches = []

    def fetch_next(value):
        if fetches:
            for fetch in fetches.pop(0):
                fetch(pltpu.bitcast(value[:8, :128], U32))

    def store_pitched(dst, row0, vt):
        for r in range(16):
            dst[pl.ds(row0 + 17 * (r // 2) + 8 * (r % 2), 8), :] = vt[8 * r:8 * r + 8]

    def radix9(tau):
        for i in range(4):
            words = [[xb_raw[side.zero + 2 * tau + z, pl.ds(32 * j + 8 * i, 8), :]
                      for j in range(9)] for z in range(2)]
            for e in range(2):
                u = []
                for z in range(2):
                    u.append(_bfly9_fwd([_unpack(w, e) for w in words[z]]))
                    yield u[z][8], 12
                out = [_pack(u[0][o], u[1][o]) for o in range(9)]
                for o in range(9):
                    u_t[tau, pl.ds(64 * o + 32 * e + 8 * i, 8), :] = out[o]
                if tau == i == e == 0:
                    out[8] = now(u_r)[0, pl.ds(512, 8), :]
                yield out, 5

    def u_to_token_major(gi):
        g = _GROUPS[gi]
        for tau in range(8):
            if g:
                v = u_t[tau, pl.ds(64 * (2 * g - 1), 128), :]
            else:
                v = jnp.concatenate([u_t[tau, pl.ds(0, 64), :], _zeros_w(64)], axis=0)
            vt = v.T
            store_pitched(u_nat.at[gi], 136 * tau, vt)
            yield vt[120:], 43, 240

    def dft_matrix(a):
        twr = jnp.broadcast_to(pltpu.bitcast(tab[pl.ds(_OFF_TR + a, 1), :], F32), (8, 128))
        twi = jnp.broadcast_to(pltpu.bitcast(tab[pl.ds(_OFF_TI + a, 1), :], F32), (8, 128))
        for i in range(16):
            fr = pltpu.bitcast(now(tab_r)[pl.ds(_OFF_FR + 8 * i, 8), :], F32)
            fi = pltpu.bitcast(now(tab_r)[pl.ds(_OFF_FI + 8 * i, 8), :], F32)
            gr, gi = fr * twr - fi * twi, fr * twi + fi * twr
            gmat[a, 0, pl.ds(8 * i, 8), :] = gr
            out = [gr + gi, gi - gr]
            gmat[a, 1, pl.ds(8 * i, 8), :] = out[0]
            gmat[a, 2, pl.ds(8 * i, 8), :] = out[1]
            if a == i == 0:
                out[1] = now(g_r)[0, 2, pl.ds(0, 8), :]
            yield out, 3

    def filter_rows(row0, load_w):
        rows = pl.ds(row0, 8)
        y = [[None] * 4 for _ in range(4)]
        for a0 in range(4):
            src = now(t_r)
            z = _bfly4([(src[4 * a1 + a0, 0, rows, :], src[4 * a1 + a0, 1, rows, :])
                        for a1 in range(4)], False)
            for g0 in range(4):
                y[g0][a0] = _twiddle16(z[g0], a0 * g0, False)
            yield y[3][a0][0], 7
        for g0 in range(4):
            z = _bfly4(y[g0], False)
            yield z[3][1], 4
            for g1 in range(4):
                wr, wi = load_w(g0 + 4 * g1)
                zr, zi = z[g1]
                z[g1] = (zr * wr - zi * wi, zr * wi + zi * wr)
                if g1 % 2:
                    yield z[g1][1], 4
            z = _bfly4(z, True)
            for a0 in range(4):
                y[g0][a0] = _twiddle16(z[a0], a0 * g0, True)
            yield y[g0][3][0], 6
        for a0 in range(4):
            z = _bfly4([y[g0][a0] for g0 in range(4)], True)
            for a1 in range(4):
                t_buf[4 * a1 + a0, 0, rows, :] = z[a1][0]
                t_buf[4 * a1 + a0, 1, rows, :] = z[a1][1]
            yield [v for pair in z for v in pair], 6

    def filter_all():
        for n, (k0, h) in enumerate(_ROWGROUPS):
            rows = pl.ds(k0 // 2 + 72 * h, 8, stride=9)
            yield from filter_rows(8 * n, lambda f1: (
                _unpack(now(wr_r)[f1, rows, :], k0 % 2),
                _unpack(now(wi_r)[f1, rows, :], k0 % 2)))

    def radix9_inv(c):
        odd = lax.broadcasted_iota(jnp.int32, (8, 128), 0) & 1
        sign = jnp.where(odd == 1, -1.0 / (S * D), 1.0 / (S * D))
        last = [sign * now(nyq_r)[pl.ds(2 * c + e, 1), :] for e in range(2)]
        for i in range(8):
            y = []
            for e in range(2):
                y.append(_bfly9_inv(
                    [now(t_r)[2 * c + e, i // 4, pl.ds(256 + 8 * (i % 4), 8), :] + last[e]]
                    + [now(t_r)[2 * c + e, o % 2, pl.ds(64 * (o // 2) + 8 * i, 8), :]
                       for o in range(8)]))
                yield y[e][8], 10
            out = [_pack(y[0][j], y[1][j]) for j in range(9)]
            for j in range(9):
                y_t[c, pl.ds(64 * j + 8 * i, 8), :] = out[j]
            if c == i == 0:
                out[8] = now(y_r)[0, pl.ds(512, 8), :]
            yield out, 5

    def y_to_token_major(c):
        for q in range(4):
            vt = y_t[c, pl.ds(64 + 128 * q, 128), :].T
            stage[5 + q, pl.ds(c, 128, stride=8), :] = vt
            yield vt[120:], 43, 240

    def y_seam_to_token_major():
        for c in range(8):
            vt = jnp.concatenate([_zeros_w(64), y_t[c, pl.ds(0, 64), :]], axis=0).T
            y_seam[c] = vt
            yield vt[120:], 43, 240

    def k_rows(kt):
        return min(128 * kt, D - 128)

    def x_to_token_major(half, kts):
        for kt in kts:
            for t in range(8 * half, 8 * half + 8):
                vt = xa_raw[pl.ds(k_rows(kt), 128), pl.ds(128 * t, 128)].T
                vt = pltpu.bitcast(vt, U32)
                for u in range(8):
                    x_nat[kt][pl.ds(72 * t + 9 * u, 8), :] = vt[8 * u:8 * u + 8]
                yield vt[56:], 22, 180

    def x_rows(half, c, i=0, n=64):
        return pl.ds(576 * half + 9 * i + c, n, stride=9)

    def difference(u, v):
        return _pack(_unpack(u, 0) - _unpack(v, 0), _unpack(u, 1) - _unpack(v, 1))

    def low_lanes(rows, n=64):
        return lax.broadcasted_iota(jnp.int32, (rows, 128), 1) < n

    def x_prep(half, gam):
        for i in range(0, 64, 8):
            (a3, a4), (b3, b4) = [[x_nat[kt][x_rows(half, 2 * gam + e, i, 8), :] for kt in (3, 4)]
                                  for e in range(2)]
            out = [jnp.where(low_lanes(8), lo, hi) for lo, hi in
                   ((a3, difference(a3, b3)), (b3, difference(b4, a4)), (b4, a4))]
            for j in range(3):
                x_seam[4 * half + gam, j, pl.ds(i, 8), :] = out[j]
            yield out, 5

    def w_prep(part, kts=range(5)):
        col0, _ = _W_COLS[part]
        first = 288 * part - col0 // 2
        for kt in kts:
            for nt in range(5):
                nn = min(128, 3 * D - col0 - 128 * nt)
                vt = wq_raw[pl.ds(k_rows(kt), 128), pl.ds(col0 + 128 * nt, nn)].T
                vt = pltpu.bitcast(vt, U32)
                wt_nat[kt, pl.ds(64 * nt, nn // 2), :] = vt
                yield vt[-8:], 22, 180
        for kt in kts:
            for i in range(2):
                for dl in range(9):
                    base = first + 144 * i + dl
                    wa = now(wn_r)[kt, pl.ds(base, 8, stride=18), :]
                    wb = now(wn_r)[kt, pl.ds(base + 9, 8, stride=18), :]
                    out = [_pack(_unpack(wa, e), _unpack(wb, e)) for e in range(2)]
                    for e in range(2):
                        rows = pl.ds(16 * (2 * dl + e) + 8 * i, 8)
                        wt[part][kt, rows, :] = out[e]
                        if kt == 4:
                            wt[part][5, rows, :] = jnp.where(
                                low_lanes(8), wt[part][3, rows, :], out[e])
                    yield out, 2 + 2 * (kt == 4)

    def wo_tile(row0, rows, ct):
        return wo_raw[pl.ds(row0, rows), pl.ds(128 * ct, 128)]

    def wo_prep():
        for ct in range(4):
            words = [pltpu.bitcast(wo_tile(448 + 64 * (ct % 2), 64, c), U32) for c in (ct, ct ^ 1)]
            wo_diff[ct] = difference(*words)
        for kt in range(5):
            vt = wo_raw[pl.ds(k_rows(kt), 128), pl.ds(512, 64)].T
            vt = pltpu.bitcast(vt, U32)
            wo_tail[kt] = vt
            yield vt[24:], 22, 180

    scale = float(DH) ** -0.5

    def softmax(unit, d_block):
        half, gam, hg = unit // 16, unit // 4 % 4, unit % 4
        base = 2 * gam + 1
        acc = [[None] * W for _ in range(2)]
        for d0 in range(0, DH, d_block):
            rows = [pl.ds(144 * hg + 8 * d, 8) for d in range(d0, d0 + d_block)]
            q = [[now(q_r[4 * half + gam])[e, r, :] for r in rows] for e in range(2)]
            for l in range(9):
                for n, r in enumerate(rows):
                    k = now(k_r[half])[base + l, r, :]
                    for e in range(2):
                        w = 7 + e - l
                        if 0 <= w < W:
                            t = q[e][n] * k
                            acc[e][w] = t if acc[e][w] is None else acc[e][w] + t
                done = [acc[e][7 + e - l] for e in range(2) if 0 <= 7 + e - l < W]
                yield done, d_block / 2 * len(done)
        prob = []
        for e in range(2):
            lg = [jnp.where(low_lanes(8, 2), -1e9 / scale, acc[e][w])
                  if half == 0 and 2 * gam + e < w else acc[e][w] for w in range(W)]
            m = lg[0]
            for w in range(1, W):
                m = jnp.maximum(m, lg[w])
            ex = [jnp.exp2((l_ - m) * (scale * float(np.log2(np.e)))) for l_ in lg]
            tot = ex[0]
            for w in range(1, W):
                tot = tot + ex[w]
            inv = pl.reciprocal(tot, approx=True)
            inv = inv + inv * (1.0 - tot * inv)
            prob.append([x_ * inv for x_ in ex])
            yield prob[e][W - 1], 11, 30
        return prob

    def weigh_values(unit, prob):
        half, gam, hg = unit // 16, unit // 4 % 4, unit % 4
        base = 2 * gam + 1
        for d in range(DH):
            vv = [now(v_r[half])[base + l, pl.ds(144 * hg + 8 * d, 8), :] for l in range(9)]
            o = []
            for e in range(2):
                t = prob[e][0] * vv[7 + e]
                for w in range(1, W):
                    t = t + prob[e][w] * vv[7 + e - w]
                o.append(t)
            if d % 2:
                o = [_pack(even[e], o[e]) for e in range(2)]
                for e in range(2):
                    o_t[half][2 * gam + e, pl.ds(72 * hg + d // 2, 8, stride=DH // 2), :] = o[e]
            even = o
            yield o, 8

    def attend(units, d_block):
        for n in units:
            prob = yield from softmax(n, d_block)
            yield from weigh_values(n, prob)

    def softmax_ahead(units, d_block):
        for n in units:
            prob = yield from softmax(n, d_block)
            for e in range(2):
                for w in range(W):
                    p_buf[n, pl.ds(8 * (W * e + w), 8), :] = prob[e][w]

    def weigh_values_later(units):
        for n in units:
            prob = [[now(p_r)[n, pl.ds(8 * (W * e + w), 8), :] for w in range(W)]
                    for e in range(2)]
            yield from weigh_values(n, prob)

    def o_to_token_major(half, gams):
        for c in [2 * gam + e for gam in gams for e in range(2)]:
            for kt in range(5):
                vt = pltpu.bitcast(_bf(o_t[half][c, pl.ds(k_rows(kt) // 2, 64), :]).T, U32)
                o_nat[half][kt, pl.ds(c, 64, stride=9), :] = vt
                yield vt[56:], 22, 180

    def table(off, i):
        return _bf(tab[pl.ds(off[i], off[i + 1] - off[i]), :])

    def dft64(a, gi):
        x1 = _dot_nt(table(_OFF_LF, gi)[:128 if gi < 4 else 72],
                     _bf(u_nat[gi, pl.ds(a, 64, stride=17), :]))
        n = 64 if gi < 4 else NR - 256
        side.run(x1.shape[0] / 4)
        x1_buf[a, 0, pl.ds(64 * gi, n), :] = x1[:n]
        x1_buf[a, 1, pl.ds(64 * gi, n), :] = x1[n:2 * n]
        if gi == 4:
            nyq[pl.ds(a, 1), :] = x1[2 * n + a % 8:2 * n + a % 8 + 1]
        if a % 4 == 3:
            fetch_next(x1)

    def dft128(a):
        side.run(216)
        xr, xi = x1_buf[a, 0, pl.ds(0, NR), :], x1_buf[a, 1, pl.ds(0, NR), :]
        k1 = _dot(xr + xi, gmat[a, 0])
        t_buf[a, 0, pl.ds(0, NR), :] = k1 - _dot(xi, gmat[a, 1])
        t_buf[a, 1, pl.ds(0, NR), :] = k1 + _dot(xr, gmat[a, 2])

    def gmat_rows(a, c):
        return jnp.concatenate([gmat[a, c, pl.ds(16 * tau + e, 8, stride=2), :]
                                for tau in range(8) for e in range(2)], axis=0)

    def nyquist(step):
        twr, twi = [pltpu.bitcast(tab[pl.ds(off, 16), :], F32) for off in (_OFF_TR, _OFF_TI)]
        if step == 0:
            re = _dot(nyq[pl.ds(0, 16), :], gmat[0, 0])
            im = re + _dot(nyq[pl.ds(0, 16), :], gmat[0, 2])
            re, im = re * twr - im * twi, re * twi + im * twr
        elif step == 2:
            row = lax.broadcasted_iota(jnp.int32, (8, 128), 0)
            w = []
            for i in range(2):
                for f8 in (0, 8):
                    t = jnp.zeros((8, 128), F32)
                    for f in range(8):
                        t = jnp.where(row == f, wlast[i, :, pl.ds(128 * (f8 + f), 128)].astype(F32), t)
                    w.append(t)
            wr, wi = jnp.concatenate(w[:2], axis=0), jnp.concatenate(w[2:], axis=0)
            re, im = nyq[pl.ds(0, 16), :], nyq[pl.ds(16, 16), :]
            re, im = re * wr - im * wi, re * wi + im * wr
        elif step == 4:
            re, im = nyq[pl.ds(0, 16), :], nyq[pl.ds(16, 16), :]
            re = _dot_nt(re + im, gmat_rows(0, 0)) + _dot_nt(im, gmat_rows(0, 2))
        else:
            x = _dot(table(_OFF_16, step // 2),
                     jnp.concatenate([nyq[...], jnp.zeros((96, 128), F32)], axis=0))
            re, im = x[:16], x[16:]
            if step == 3:
                re, im = re * twr + im * twi, im * twr - re * twi
        nyq[pl.ds(0, 16), :] = re
        nyq[pl.ds(16, 16), :] = im
        side.absorb(([re[:8], re[8:], im[:8], im[8:]], 0, 200))

    def idft128(a):
        side.run(216)
        g = [gmat_rows(a, c) for c in range(3)]
        tr, ti = t_buf[a, 0, pl.ds(0, NR), :], t_buf[a, 1, pl.ds(0, NR), :]
        k1 = _dot_nt(tr + ti, g[0])
        z_buf[a % 2, 0, pl.ds(0, NR), :] = k1 + _dot_nt(ti, g[2])
        z_buf[a % 2, 1, pl.ds(0, NR), :] = k1 - _dot_nt(tr, g[1])

    def idft64(a):
        side.run(144)
        for gi in range(5):
            n = 64 if gi < 4 else NR - 256
            parts = [z_buf[a % 2, c, pl.ds(64 * gi, n), :] for c in range(2)]
            if n < 64:
                parts.append(jnp.zeros((128 - 2 * n, 128), F32))
            o = _dot(table(_OFF_LI, gi), jnp.concatenate(parts, axis=0))
            if gi < 4:
                t_buf[a, 0, pl.ds(64 * gi, 64), :] = o[:64]
                t_buf[a, 1, pl.ds(64 * gi, 64), :] = o[64:]
            else:
                t_buf[a, 0, pl.ds(256, 32), :] = o[:32]
                t_buf[a, 1, pl.ds(256, 32), :] = o[32:]

    def proj(part, half, gam, kts=(0, 1, 2, 3), chunks=4, only=None):
        m = 288 // chunks
        last = kts[-1] == 3
        for ch in only or range(chunks):
            side.run((len(kts) + last / 2) * m)
            w = lambda kt: _bf(wt[part][kt, pl.ds(m * ch, m), :])
            both = _dot_nt(w(4), _bf(x_seam[4 * half + gam, 2])) if last else None
            for e in range(2):
                c = 2 * gam + e
                tile = _dot_nt(
                    jnp.concatenate([w(3 + 2 * e if kt == 3 else kt) for kt in kts], axis=1),
                    jnp.concatenate([_bf(x_seam[4 * half + gam, e] if kt == 3
                                         else x_nat[kt][x_rows(half, c), :]) for kt in kts], axis=1))
                if last:
                    tile = tile + both
                if part == 0:
                    buf, slot = q_buf[4 * half + gam], e
                else:
                    buf, slot = (k_buf if part == 1 and last else v_buf)[half], 8 + c
                rows = []
                for i in range(m // 4):
                    d, hg = divmod(m // 4 * ch + i, 4)
                    rows.append(pl.ds(144 * hg + 8 * d, 8))
                if kts[0]:
                    sums = v_buf[half] if part else buf
                    tile = tile + jnp.concatenate([sums[slot, r, :] for r in rows], axis=0)
                for i, r in enumerate(rows):
                    buf[slot, r, :] = tile[8 * i:8 * i + 8]
                if part == 0 or not last:
                    continue
                if c:
                    if half:
                        before = (k_buf, v_buf)[part - 1][0]
                        tile = jnp.where(low_lanes(2 * m, 126), tile, jnp.concatenate(
                            [before[slot, r, :] for r in rows], axis=0))
                    tile = pltpu.roll(tile, 2, 1)
                    for i, r in enumerate(rows):
                        buf[c, r, :] = tile[8 * i:8 * i + 8]
                        if part == 2 and half == 0:
                            pltpu.store(buf.at[c, r, :], buf[0, r, :], mask=low_lanes(8, 2))
                elif part == 2 and half == 0:
                    tile = jnp.where(low_lanes(2 * m, 1), tile, pltpu.roll(tile, 1, 1))
                    for i, r in enumerate(rows):
                        buf[0, r, :] = tile[8 * i:8 * i + 8]
            fetch_next(tile)

    def out_proj(half, row0, cw):
        side.run(9 * cw)
        o = [jnp.concatenate([o_nat[half][kt, pl.ds(9 * b, 8), :]
                              for b in range(row0 // 8, (row0 + cw) // 8)], axis=0)
             for kt in range(5)]
        lhs = [jnp.concatenate([_bf(t) for t in o[:3] + [last]], axis=1)
               for last in (o[3], jnp.where(low_lanes(cw), o[3], o[4]))]
        both = _dot(_bf(o[4]), jnp.concatenate(
            [jnp.concatenate([wo_tile(448, 64, ct + 1), wo_tile(512, 64, ct)], axis=0)
             for ct in (0, 2)], axis=1))
        r = [_dot(lhs[n], jnp.concatenate(
            [jnp.concatenate([wo_tile(0, 448, ct), _bf(wo_diff[ct])], axis=0)
             for ct in (n, n + 2)], axis=1)) for n in range(2)]
        for ct in (0, 2, 1, 3):
            cols = slice(128 * (ct // 2), 128 * (ct // 2) + 128)
            tile = (r[ct % 2][:, cols] + both[:, cols]).astype(BF16)
            stage[ct, pl.ds(512 * half + row0, cw), :] = pltpu.bitcast(tile, U32)
            cp_out(ct, 512 * half + row0, cw).start()

    def out_tail(half, gam):
        side.run(144)
        o = [o_t[half][2 * gam + e] for e in range(2)]
        w = [wo_tail[kt] for kt in range(5)]
        both = _dot(_bf(w[4]), _bf(jnp.concatenate([o[1][224:256], o[0][256:]], axis=0)))
        for e, last in enumerate((w[3], jnp.where(low_lanes(32), w[3], w[4]))):
            c, rows = 2 * gam + e, slice(224 + 32 * e, 256 + 32 * e)
            tile = both + _dot(
                jnp.concatenate([_bf(t) for t in w[:3] + [last]], axis=1),
                _bf(jnp.concatenate([o[e][:224], difference(o[e][rows], o[1 - e][rows])], axis=0)))
            tile = jnp.concatenate([tile.astype(BF16), jnp.zeros((64, 128), BF16)], axis=0)
            stage[4, pl.ds(512 * half + c, 64, stride=8), :] = jnp.where(
                low_lanes(64), pltpu.bitcast(tile.T, U32), y_seam[c, pl.ds(64 * half, 64), :])

    pair = 1296
    unit = 315

    def end_region():
        pl.semaphore_signal(sem_region)
        pl.semaphore_wait(sem_region)

    def queries(i0, i1, chunks=4):
        while i0 < i1:
            n = chunks if i0 % (4 // chunks) == 0 and i0 + 4 // chunks <= i1 else 4
            proj(0, i0 // 16, i0 // 4 % 4, (1, 2, 3) if i0 < 4 * 3 else (0, 1, 2, 3),
                 chunks=n, only=(i0 % 4 * n // 4,))
            i0 += 4 // n

    def cycles(i0, i1):
        return sum(pair / 4 - 72 * (i < 4 * 3) for i in range(i0, i1))

    blocks = ((0,128,(0,)),(128,256,(1,2)),(384,D-384,(3,)))

    def fetch_block(i):
        cp_wq(1, *blocks[i][:2], sem.at[i]).start()
        cp_xa(0, *blocks[i][:2], sem.at[i]).start()

    cp_xa(0, 0, 128, sem.at[0]).start()
    cp_wq(1, 0, 128, sem_k).start()
    cp_wq(0, 0, 128, sem_out).start()
    fetch_block(1)
    cp_xa(0, 0, 128, sem.at[0]).wait()
    fetch_block(2)
    _drain(x_to_token_major(0, (0,)))
    cp_wq(1, 0, 128, sem_k).wait()
    _drain(w_prep(1, (0,)))
    cp_wq(0, 0, 128, sem_out).wait()
    side.start(pltpu.bitcast(wq_raw[pl.ds(0, 16), pl.ds(512, 128)], U32), x1_buf.at[16, 0])
    fetches += [[partial(fetch_xa, 1, r, 192, sem_k)] for r in range(0, D, 192)]
    for i, (row0, rows, kts) in enumerate(blocks):
        if i:
            cp_wq(1, row0, rows, sem.at[i]).wait()
            cp_xa(0, row0, rows, sem.at[i]).wait()
        if i == 1:
            fetches += [[partial(fetch_wq, 0, r, 224, sem_xb)] for r in range(128, D, 224)]
            fetches += [[partial(fetch_xb, t)] for t in range(16)]
        if i == 2:
            fetches += [[partial(fetch_wq, 2, r, 144, sem_tab) for r in range(0, D, 144)]]
            fetches += [[partial(fetch_tab, r, min(304, n_tab - r)) for r in range(0, n_tab, 304)]]
        side.open((0,0,0,0)[i])
        tiles = kts + (4,) * (i == 2)
        if i and not 1:
            side.add("prep", w_prep(1, tiles), 0.8)
        if i:
            side.add("prep", x_to_token_major(0, tiles), 0.8)
        if i == 2:
            side.add("prep", x_prep(0, 0), 0.8)
        if i and 1:
            for kt in tiles:
                side.add("prep", w_prep(1, (kt,)), 0.8)
        if i:
            for gam in range((4,2,0)[i - 1], 4):
                proj(1, 0, gam, blocks[i - 1][2])
        if i == 1:
            for gam in range(0, 3):
                proj(0, 0, gam, (0,))
        side.finish("prep")
        if i == 0 and not 0:
            side.add("q", w_prep(0, (0,)), 0.5)
        for gam in range((4,2,0)[i]):
            if i == 2:
                side.add("next", x_prep(0, gam + 1), 0.5)
            proj(1, 0, gam, kts)
            side.finish("next")
        if i == 0:
            side.finish("q")
            for gam in range(0):
                proj(0, 0, gam, (0,))
        if i == 2:
            for gam in range((4,2,0)[i] + 1, 4):
                side.add("next", x_prep(0, gam), 0.5)
        side.close()

    cp_xa(1, 0, D, sem_k).wait()
    side.open((0,0,0,0)[3])
    fetches += [[partial(fetch_f, t) for t in range(4)]]
    side.add("prep", x_to_token_major(1, range(5)), 0.6)
    side.add("prep", x_prep(1, 0), 0.6)
    for gam in range((4,2,0)[2], 4):
        proj(1, 0, gam, blocks[2][2])
    side.finish("prep")
    for gam in range(3):
        side.add("next", x_prep(1, gam + 1), 0.5)
        proj(1, 1, gam, only=range(4 - 2 * (gam == 2)))
        side.finish("next")
    side.close()

    assert not fetches
    pltpu.make_async_copy(xb_raw, xb_raw, sem_xb).wait()
    cp_wq(0, 128, D - 128, sem_xb).wait()
    side.open(0.95, 20.0, links=4)
    load = (8 * 232 + 620) / (pair * (4 + 2) / 4 + cycles(0, 7)) * 0.9 * 1.05
    side.add("w", w_prep(0, range(1, 5)), load)
    for tau in range(8):
        side.add("r9", radix9(tau), load)
    if 2:
        proj(1, 1, 2, only=range(4 - 2, 4))
    proj(1, 1, 3)
    side.finish("w")
    queries(0, 7, 4)
    side.close()

    cp_tab(0, n_tab).wait()
    cp_wq(2, 0, D, sem_tab).wait()
    side.open(0.95, 50.0, links=2)
    fetches += [[partial(fetch_f, t)] for t in range(4, 16)]
    fetches += [[partial(fetch_wo, i)] for i in range(4)]
    fetches.append([wo_settle])
    side.add("t", u_to_token_major(0), 0.9 * 0.95)
    load = (768 + 766 + 4 * 168) / (5792 + cycles(7, 10) - 2000.0) * 1.0 * 0.95
    for a in range(16):
        side.add("g%d" % a, dft_matrix(a), load)
    queries(7, 10)
    side.finish("t")
    for gi in range(5):
        if gi < 4:
            side.add("t", u_to_token_major(gi + 1), 0.9 * 0.95, first=True)
        for a in range(16):
            dft64(a, gi)
        side.finish("t")
    side.add("w", w_prep(2), load)
    side.add("att", softmax_ahead(range(4), 6), load)
    for a in range(16):
        side.finish("g%d" % a)
        dft128(a)
        if a in (2, 6):
            nyquist(a // 4)
    side.close()

    assert not fetches
    pltpu.make_async_copy(wr_raw, wr_raw, sem_f).wait()
    pltpu.make_async_copy(wi_raw, wi_raw, sem_f).wait()
    cp_flast(0).wait()
    cp_flast(1).wait()
    cp_wo().wait()
    side.open(1.0, 100.0, links=2)
    side.add("f", filter_all(), 36 * 120 / (4 * pair + cycles(10, 18)) * 1.0)
    for gam in range(4):
        proj(2, 0, gam, chunks=1)
    queries(10, 18, 1)
    side.close()
    end_region()

    side.open(0.95, 20.0, links=2)
    load = (16 * unit - 4 * 168 + 8 * 200) / (5760 + 4 * pair + cycles(18, 20)) * 1.0
    side.add("att", weigh_values_later(range(4)), load)
    side.add("att", attend(range(4, 16), 9), load)
    idft128(0)
    for a in range(16):
        if a < 15:
            idft128(a + 1)
        idft64(a)
        if a in (2, 6, 10):
            nyquist(2 + a // 4)
    for c in range(8):
        side.add("r9", radix9_inv(c), load * 1.05)
    for gam in range(4):
        proj(2, 1, gam, chunks=2)
    queries(18, 20)
    side.close()
    end_region()

    side.open(0.9, 100.0, links=3)
    period = 3 * pair / 63 * 0.95
    side.add_paced(o_to_token_major(0, range(4)), period / 2)
    for c in range(8):
        side.add_paced(y_to_token_major(c), period)
    side.add_paced(y_seam_to_token_major(), period)
    side.add_paced(wo_prep(), period / 2)
    load = 7 * unit / (3 * pair) * 1.05 * 0.9
    side.add("att", attend(range(16, 20), 6), load)
    queries(20, 24, 4)
    side.add("att", attend(range(20, 16 + 7), 6), load)
    queries(24, 32, 4)
    side.close()
    for ct in range(5, 9):
        cp_out(ct, 0, S // 2).start()
    end_region()

    side.open(1.05, 20.0, links=2)
    side.add_paced(o_to_token_major(1, range(1)), 60.0)
    load = (16 - 7) * unit / (9 * 496 + 4 * 144) * 1.0
    side.add("att", attend(range(16 + 7, 32), 9), load)
    for gam in range(4):
        out_tail(0, gam)
    for row0 in range(0, 496, 64):
        out_proj(0, row0, min(64, 496 - row0))
    cp_out(4, 0, 512).start()
    side.close()
    end_region()

    _drain(o_to_token_major(1, range(1, 4)))
    for gam in range(4):
        out_tail(1, gam)
    cp_out(4, 512, 512).start()
    out_proj(0, 496, 512 - 496)
    row0 = 0
    for cw in (64,)*6+(32,)*3+(16,16):
        out_proj(1, row0, cw)
        row0 += cw
    pltpu.make_async_copy(out_hbm, out_hbm, sem_out).wait()


@jax.jit
def pallas_concat_heads__sliding_local_dilated__spectral_gfnet__prompt_kernel(
    A_x: jax.Array,
    A_wqkv: jax.Array,
    A_wo: jax.Array,
    B_x: jax.Array,
    B_w_r: jax.Array,
    B_w_i: jax.Array,
):
    assert A_x.shape == (1, S, D) and B_x.shape == (1, S, D)
    any_spec = pl.BlockSpec(memory_space=pl.ANY)
    scratch = [
        pltpu.VMEM((1,) + _TABLE.shape, U32),
        pltpu.VMEM((16, 288, 128), U32),
        pltpu.VMEM((D, S), BF16),
        pltpu.VMEM((D, 3 * D), BF16),
        pltpu.VMEM((D + 64, D), BF16),
        pltpu.VMEM((1, 16, 144, 128), U32),
        pltpu.VMEM((1, 16, 144, 128), U32),
        pltpu.VMEM((2, 1, S), BF16),
        pltpu.VMEM((1, 16, 3, 128, 128), F32),
        pltpu.VMEM((1, 8, D, 128), U32),
        pltpu.VMEM((1, 8, D, 128), U32),
        pltpu.VMEM((5, 8 * 136, 128), U32),
        pltpu.VMEM((1, 18, 2, 288, 128), F32),
        pltpu.VMEM((1, 16, 2, 296, 128), F32),
        pltpu.VMEM((1, 2, 2, 288, 128), F32),
        pltpu.VMEM((1, 32, 128), F32),
        [pltpu.VMEM((1, 9 * 128, 128), U32)] * 5,
        pltpu.VMEM((1, 8, 3, 64, 128), U32),
        pltpu.VMEM((1, 5, 320, 128), U32),
        pltpu.VMEM((1, 6, 288, 128), U32),
        pltpu.VMEM((1, 6, 288, 128), U32),
        pltpu.VMEM((1, 6, 288, 128), U32),
        pltpu.VMEM((1, 4, 32, 128), U32),
        pltpu.VMEM((1, 5, 32, 128), U32),
        [pltpu.VMEM((1, 2, D + 16, 128), F32)] * 8,
        [pltpu.VMEM((1, 16, D + 8, 128), F32)] * 2,
        [pltpu.VMEM((1, 16, D + 8, 128), F32)] * 2,
        pltpu.VMEM((1, 4, 2 * W * 8, 128), F32),
        [pltpu.VMEM((1, 8, D // 2, 128), U32)] * 2,
        [pltpu.VMEM((1, 5, 9 * 64, 128), U32)] * 2,
        pltpu.VMEM((1, 8, 128, 128), U32),
        pltpu.VMEM((9, S // 2, 128), U32),
        pltpu.SMEM((4,), jnp.int32),
        pltpu.SemaphoreType.DMA((5,)),
        pltpu.SemaphoreType.REGULAR,
    ]
    out = pl.pallas_call(
        _kernel,
        out_shape=jax.ShapeDtypeStruct((S, 2 * D), BF16),
        in_specs=[any_spec] * 7,
        out_specs=any_spec,
        scratch_shapes=scratch,
        compiler_params=pltpu.CompilerParams(vmem_limit_bytes=120 * 1024 * 1024),
        name="attn_gfnet",
    )(A_x[0].T, A_wqkv, A_wo, B_x[0].T, B_w_r.T, B_w_i.T, _TABLE)
    return out[None]
```

```python
from functools import partial

import numpy as np

import jax
import jax.numpy as jnp
from jax import lax
import jax.experimental.pallas as pl
import jax.experimental.pallas.tpu as pltpu

S = 2048
D = 576
H = 32
DH = 18
W = 8
DF = D // 2 + 1
NR = DF - 1

F32 = jnp.float32
BF16 = jnp.bfloat16
U32 = jnp.uint32

_R9 = float(2 * np.cos(2 * np.pi / 9))
_S9 = float(np.sin(2 * np.pi / 3) / np.sin(2 * np.pi / 9))


def _bfly9_fwd(x):
    tot = [x[j] + x[j + 3] + x[j + 6] for j in range(3)]
    re = [x[j] - x[j + 6] for j in range(3)]
    im = [x[j + 3] - x[j + 6] for j in range(3)]
    ar, ai = re[0] * (_R9 - 1) + im[0], im[0] * _R9 - re[0]
    br, bi = re[1] * _S9, im[1] * _S9
    cr, ci = re[2] * _R9 - im[2], im[2] * (_R9 - 1) + re[2]
    pr, pi, qr, qi = ar - cr, ai - ci, br - cr, bi - ci
    t = pr - qr
    return [tot[0] + tot[1] + tot[2], ar + br + cr, ai + bi + ci, qr - pi, qi + t,
            tot[0] - tot[2], tot[1] - tot[2], pr - qi, pi - t]


def _bfly9_inv(v):
    u0, u1r, u1i, u2r, u2i, u3r, u3i, u4r, u4i = v
    t = u2i - u4i
    pr, pi, qr, qi = u4r + t, u4i - u2r, u2r - t, u2i - u4r
    ar, ai, br, bi = u1r + pr, u1i + pi, u1r + qr, u1i + qi
    cr, ci = u1r - pr - qr, u1i - pi - qi
    re = [ar * (_R9 - 1) - ai, br * _S9, cr * _R9 + ci]
    im = [ai * _R9 + ar, bi * _S9, ci * (_R9 - 1) - cr]
    tot = [u0 + u3r, u0 + u3i, u0 - u3r - u3i]
    return ([tot[j] + re[j] for j in range(3)] + [tot[j] + im[j] for j in range(3)]
            + [tot[j] - re[j] - im[j] for j in range(3)])


def _bfly4(x, inverse):
    (ar, ai), (br, bi), (cr, ci), (dr, di) = x
    pr, pi, qr, qi = ar + cr, ai + ci, ar - cr, ai - ci
    sr, si, tr, ti = br + dr, bi + di, br - dr, bi - di
    y1, y3 = (qr + ti, qi - tr), (qr - ti, qi + tr)
    if inverse:
        y1, y3 = y3, y1
    return [(pr + sr, pi + si), y1, (pr - sr, pi - si), y3]


def _twiddle16(z, e, inverse):
    zr, zi = z
    e = (-e if inverse else e) % 16
    h = float(np.sqrt(0.5))
    if e == 0:
        return z
    if e == 4:
        return zi, -zr
    if e == 12:
        return -zi, zr
    if e == 2:
        return (zr + zi) * h, (zi - zr) * h
    if e == 14:
        return (zr - zi) * h, (zr + zi) * h
    if e == 6:
        return (zi - zr) * h, (zr + zi) * (-h)
    if e == 10:
        return (zr + zi) * (-h), (zr - zi) * h
    c, s = float(np.cos(2 * np.pi * e / 16)), float(np.sin(2 * np.pi * e / 16))
    return zr * c + zi * s, zi * c - zr * s


_GROUPS = (1, 2, 3, 4, 0)


def _group_classes(g):
    return sorted({g, g + 9, 9 - g, 18 - g}) if g else [0, 9]


_ROWGROUPS = [(k0, h) for g in _GROUPS for k0 in _group_classes(g) for h in range(2)]


def _to_words(m):
    u = np.ascontiguousarray(m, dtype=np.float32).view(np.uint32)
    u = (u + 0x7FFF + ((u >> 16) & 1)) >> 16
    return (u[0::2] | (u[1::2] << 16)).astype(np.uint32)


def _coordinates(a, v):
    rhs = [np.sum(row * v) for row in a]
    if len(a) == 1:
        return [rhs[0] / np.sum(a[0] * a[0])]
    g00, g01, g11 = np.sum(a[0] * a[0]), np.sum(a[0] * a[1]), np.sum(a[1] * a[1])
    det = g00 * g11 - g01 * g01
    return [(g11 * rhs[0] - g01 * rhs[1]) / det, (g00 * rhs[1] - g01 * rhs[0]) / det]


def _make_tables():
    basis = np.array(_bfly9_fwd(list(np.eye(9))))
    m_fwd = np.array([2 * (r % 32) + r // 32 for r in range(64)])
    lf, li = [], []
    for g in _GROUPS:
        rows = [k0 + 18 * i for k0 in _group_classes(g) for i in range(16)]
        cols = [2 * g - 1, 2 * g] if g else [0]
        a = basis[cols]
        n = len(rows)
        f = np.zeros((2 * n, 128))
        b = np.zeros((64 * len(cols), 128))
        for r, k in enumerate(rows):
            ck = np.exp(-2j * np.pi * ((np.arange(9) * k) % 9) / 9)
            lam = _coordinates(a, ck)
            wk = (2.0 if k else 1.0) / (S * D)
            for c in range(len(cols)):
                e = lam[c] * np.exp(-2j * np.pi * ((m_fwd * k) % D) / D)
                f[r, 64 * c:64 * c + 64] = e.real
                f[n + r, 64 * c:64 * c + 64] = e.imag
                e = wk * lam[c] * np.exp(-2j * np.pi * ((np.arange(64) * k) % D) / D)
                b[64 * c:64 * c + 64, r] = e.real
                b[64 * c:64 * c + 64, n + r] = e.imag
        if g == 0:
            f = np.concatenate([f, np.zeros((8, 128))])
            f[2 * n:, :64] = 1 - 2 * (m_fwd % 2)
        lf.append(_to_words(f))
        li.append(_to_words(b))
    n = np.arange(128)
    b_of_n = 16 * (n // 16) + 8 * (n % 2) + (n % 16) // 2
    f128 = np.exp(-2j * np.pi * (np.outer(b_of_n, n) % 128) / 128)
    tw = np.exp(-2j * np.pi * np.outer(np.arange(16), n) / S)
    f32w = lambda m: np.ascontiguousarray(m, dtype=np.float32).view(np.uint32)
    f16 = np.exp(-2j * np.pi * np.outer(n[:16], n[:16]) / 16)
    f16 = np.block([[f16.real, -f16.imag], [f16.imag, f16.real]])
    f16 = [_to_words(np.concatenate([m, np.zeros((32, 96))], axis=1)) for m in (f16, f16.T)]
    parts = [f32w(f128.real), f32w(f128.imag), f32w(tw.real), f32w(tw.imag)] + f16 + lf + li
    parts = [np.concatenate([p, np.zeros((-len(p) % 8, 128), np.uint32)]) for p in parts]
    offs = np.cumsum([0] + [p.shape[0] for p in parts])
    parts.append(np.zeros((-offs[-1] % 32, 128), np.uint32))
    return np.concatenate(parts, axis=0), [int(o) for o in offs]


_TABLE, _OFF = _make_tables()
_OFF_FR, _OFF_FI, _OFF_TR, _OFF_TI = _OFF[0:4]
_OFF_16, _OFF_LF, _OFF_LI = _OFF[4:7], _OFF[6:12], _OFF[11:17]


def _pack(lo, hi):
    return pltpu.pack_elementwise([lo, hi], packed_dtype=BF16)


def _unpack(w, index):
    return pltpu.unpack_elementwise(w, index=index, packed_dtype=BF16, unpacked_dtype=F32)


def _bf(words):
    return pltpu.bitcast(words, BF16)


def _dot(a, b):
    return lax.dot_general(a, b, (((1,), (0,)), ((), ())), preferred_element_type=F32)


def _dot_nt(a, b):
    return lax.dot_general(a, b, (((1,), (1,)), ((), ())), preferred_element_type=F32)


def _zeros_w(rows):
    return jnp.zeros((rows, 128), U32)


class _SideWork:
    LINK = 7.0
    HOP = 6.0

    def __init__(self, zero_ref):
        self.zero_ref = zero_ref
        self.zero = zero_ref[0]

    def start(self, seed, sink):
        self.chain = pltpu.bitcast(seed, F32)
        self.sink = sink
        self.jobs = []
        self.paced = []
        self.pending = []
        self.regions = 0
        self.credit = self.delay = self.clock = 0.0

    def open(self, stretch=0.0, slack=100.0, links=4):
        self.links = links
        self.zero = self.zero_ref[0]
        self.lead = -slack
        self.stretch = stretch

    def add(self, name, job, load, first=False):
        self.jobs.insert(0 if first else len(self.jobs), (name, job, load))

    def add_paced(self, job, period):
        if not self.paced:
            self.due = self.clock
        self.paced.append((job, period))

    def absorb(self, item):
        values, cycles, latency = (item + (0.0,))[:3]
        values = values if isinstance(values, list) else [values]
        values = [pltpu.bitcast(v, F32) for v in values]
        while len(values) > 1:
            values = [values[i] + values[i + 1] if i + 1 < len(values) else values[i]
                      for i in range(0, len(values), 2)]
        self.pending.append((self.clock + latency, values[0]))
        self.pending.sort(key=lambda x: x[0])
        return cycles

    def _step_paced(self):
        item = next(self.paced[0][0], None)
        if item is None:
            self.paced.pop(0)
        else:
            self.absorb(item)
            self.due += self.stretch * self.paced[0][1]

    def _tick(self, cycles):
        while self.paced and self.due <= self.clock:
            self._step_paced()
        self.clock += cycles
        self.delay += cycles
        while self.pending and self.pending[0][0] <= self.clock:
            self.chain = self.pending.pop(0)[1] + self.chain
            self.delay -= 2.0
        n = int(self.delay / self.LINK)
        if n >= self.links:
            for _ in range(n):
                self.chain = pl.reciprocal(self.chain, approx=True)
            self.delay -= n * self.LINK

    def _step(self):
        item = next(self.jobs[0][1], None)
        if item is None:
            self.jobs.pop(0)
            return
        cycles = self.absorb(item) / self.jobs[0][2]
        self.credit -= cycles
        self.lead += cycles
        while self.lead >= self.HOP:
            self.zero = self.zero_ref[self.zero]
            self.lead -= self.HOP
        self._tick(self.stretch * cycles)

    def run(self, cycles):
        self.credit += cycles
        while self.jobs and self.credit > 0:
            self._step()
        while not self.jobs and self.credit > 0:
            n = min(self.credit, 50.0) if self.paced else self.credit
            self._tick(self.stretch * n)
            self.credit -= n

    def finish(self, name):
        while any(job[0] == name for job in self.jobs):
            self._step()

    def close(self):
        while self.jobs:
            self._step()
        while self.paced:
            self._step_paced()
        while self.pending:
            self.chain = self.pending.pop(0)[1] + self.chain
        self.sink[pl.ds(8 * self.regions, 8), :] = self.chain
        self.regions += 1
        self.credit = self.delay = 0.0


def _drain(gen):
    for _ in gen:
        pass


_W_COLS = ((0, 512), (512, 640), (1152, 576))


def _kernel(xa_hbm, wqkv_hbm, wo_hbm, xb_hbm, wr_hbm, wi_hbm, tab_hbm, out_hbm,
            tab, xb_raw, xa_raw, wq_raw, wo_raw, wo_last, wr_raw, wi_raw, wlast,
            gmat, u_t, y_t, u_nat, x1_buf, t_buf, z_buf, nyq, x_nat, x_seam, wt_nat, wt,
            wo_diff, wo_tail, q_buf, k_buf, v_buf, p_buf, o_t, o_nat, y_seam, stage, stage_seam,
            zero_ref, sem, sem_region):
    zero_ref[0] = pl.semaphore_read(sem_region)
    side = _SideWork(zero_ref)
    zero = side.zero

    def now(ref):
        return ref.at[side.zero]

    tab_r, wr_r, wi_r = tab, wr_raw, wi_raw
    tab, wr_raw, wi_raw = tab.at[0], wr_raw.at[0], wi_raw.at[0]
    t_r, wn_r, q_r, k_r, v_r, p_r = t_buf, wt_nat, q_buf, k_buf, v_buf, p_buf
    u_r, y_r, g_r, nyq_r = u_t, y_t, gmat, nyq
    (gmat, u_t, y_t, x1_buf, t_buf, z_buf, nyq, x_nat, x_seam, wt_nat, wt, wo_diff, wo_tail,
     q_buf, k_buf, v_buf, p_buf, o_t, o_nat, y_seam) = jax.tree.map(
        lambda r: r.at[zero],
        (gmat, u_t, y_t, x1_buf, t_buf, z_buf, nyq, x_nat, x_seam, wt_nat, wt, wo_diff, wo_tail,
         q_buf, k_buf, v_buf, p_buf, o_t, o_nat, y_seam))

    sem_xb, sem_tab, sem_f, sem_out, sem_k = (sem.at[i] for i in range(5))

    def cp_tab(row0, rows):
        return pltpu.make_async_copy(
            tab_hbm.at[pl.ds(row0, rows)], tab.at[pl.ds(row0, rows)], sem_tab)

    def cp_xb(t):
        return pltpu.make_async_copy(
            xb_hbm.at[:, pl.ds(t * 128, 128)], xb_raw.at[t].bitcast(BF16), sem_xb)

    def cp_xa(tiles, row0, rows, sem_):
        rows, cols = pl.ds(row0, rows), pl.ds(128 * tiles[0], 128 * len(tiles))
        return pltpu.make_async_copy(xa_hbm.at[rows, cols], xa_raw.at[rows, cols], sem_)

    def cp_wq(part, row0, rows, sem_):
        rows, cols = pl.ds(row0, rows), pl.ds(*_W_COLS[part])
        return pltpu.make_async_copy(wqkv_hbm.at[rows, cols], wq_raw.at[rows, cols], sem_)

    def cp_wo(ct):
        cols, dst = (128, wo_raw.at[ct].bitcast(BF16)) if ct < 4 else (D - 512, wo_last)
        return pltpu.make_async_copy(wo_hbm.at[:, pl.ds(128 * ct, cols)], dst, sem_f)

    def cp_f(i, t):
        src, dst = ((wr_hbm, wr_raw), (wi_hbm, wi_raw))[i]
        return pltpu.make_async_copy(
            src.at[pl.ds(0, DF - 1), pl.ds(t * 128, 128)], dst.at[t].bitcast(BF16), sem_f)

    def cp_flast(i):
        src = (wr_hbm, wi_hbm)[i]
        return pltpu.make_async_copy(src.at[pl.ds(DF - 1, 1), :], wlast.at[i], sem_f)

    def cp_out(ct, row0, rows):
        src = stage_seam if ct == 4 else stage.at[ct - (ct > 4)]
        return pltpu.make_async_copy(
            src.at[pl.ds(row0, rows)].bitcast(BF16),
            out_hbm.at[pl.ds(2 * row0, 2 * rows), pl.ds(ct * 128, 128)], sem_out)

    def fetch_xb(t, v):
        xb_raw[t, pl.ds(0, 8), :] = v
        cp_xb(t).start()

    def fetch_wq(part, row0, rows, sem_, v):
        wq_raw[pl.ds(row0, 16), pl.ds(_W_COLS[part][0], 128)] = _bf(v)
        cp_wq(part, row0, rows, sem_).start()

    def fetch_xa(tiles, row0, rows, sem_, v):
        xa_raw[pl.ds(row0, 16), pl.ds(128 * tiles[0], 128)] = _bf(v)
        cp_xa(tiles, row0, rows, sem_).start()

    def fetch_wo(ct, v):
        wo_raw[ct, pl.ds(0, 8), :] = v
        cp_wo(ct).start()
        if ct == 0:
            cp_wo(4).start()

    def wo_settle(v):
        wo_raw[4, pl.ds(0, 8), :] = v

    def fetch_tab(row0, rows, v):
        tab[pl.ds(row0, 8), :] = v
        cp_tab(row0, rows).start()

    def fetch_f(t, v):
        wr_raw[t, pl.ds(0, 8), :] = v
        cp_f(0, t).start()
        wi_raw[t, pl.ds(0, 8), :] = v
        cp_f(1, t).start()
        if t == 0:
            cp_flast(0).start()
            cp_flast(1).start()

    n_tab = _TABLE.shape[0]
    fetches = []

    def fetch_next(value):
        if fetches:
            for fetch in fetches.pop(0):
                fetch(pltpu.bitcast(value[:8, :128], U32))

    def store_pitched(dst, row0, vt):
        for r in range(16):
            dst[pl.ds(row0 + 17 * (r // 2) + 8 * (r % 2), 8), :] = vt[8 * r:8 * r + 8]

    def radix9(tau):
        for i in range(4):
            words = [[xb_raw[side.zero + 2 * tau + z, pl.ds(32 * j + 8 * i, 8), :]
                      for j in range(9)] for z in range(2)]
            for e in range(2):
                u = []
                for z in range(2):
                    u.append(_bfly9_fwd([_unpack(w, e) for w in words[z]]))
                    yield u[z][8], 12
                out = [_pack(u[0][o], u[1][o]) for o in range(9)]
                for o in range(9):
                    u_t[tau, pl.ds(64 * o + 32 * e + 8 * i, 8), :] = out[o]
                if tau == i == e == 0:
                    out[8] = now(u_r)[0, pl.ds(512, 8), :]
                yield out, 5

    def u_to_token_major(gi):
        g = _GROUPS[gi]
        for tau in range(8):
            if g:
                v = u_t[tau, pl.ds(64 * (2 * g - 1), 128), :]
            else:
                v = jnp.concatenate([u_t[tau, pl.ds(0, 64), :], _zeros_w(64)], axis=0)
            vt = v.T
            store_pitched(u_nat.at[gi], 136 * tau, vt)
            yield vt[120:], 43, 240

    def dft_matrix(a):
        twr = jnp.broadcast_to(pltpu.bitcast(tab[pl.ds(_OFF_TR + a, 1), :], F32), (8, 128))
        twi = jnp.broadcast_to(pltpu.bitcast(tab[pl.ds(_OFF_TI + a, 1), :], F32), (8, 128))
        for i in range(16):
            fr = pltpu.bitcast(now(tab_r)[pl.ds(_OFF_FR + 8 * i, 8), :], F32)
            fi = pltpu.bitcast(now(tab_r)[pl.ds(_OFF_FI + 8 * i, 8), :], F32)
            gr, gi = fr * twr - fi * twi, fr * twi + fi * twr
            gmat[a, 0, pl.ds(8 * i, 8), :] = gr
            out = [gr + gi, gi - gr]
            gmat[a, 1, pl.ds(8 * i, 8), :] = out[0]
            gmat[a, 2, pl.ds(8 * i, 8), :] = out[1]
            if a == i == 0:
                out[1] = now(g_r)[0, 2, pl.ds(0, 8), :]
            yield out, 3

    def filter_rows(row0, load_w):
        rows = pl.ds(row0, 8)
        y = [[None] * 4 for _ in range(4)]
        for a0 in range(4):
            src = now(t_r)
            z = _bfly4([(src[4 * a1 + a0, 0, rows, :], src[4 * a1 + a0, 1, rows, :])
                        for a1 in range(4)], False)
            for g0 in range(4):
                y[g0][a0] = _twiddle16(z[g0], a0 * g0, False)
            yield y[3][a0][0], 7
        for g0 in range(4):
            z = _bfly4(y[g0], False)
            yield z[3][1], 4
            for g1 in range(4):
                wr, wi = load_w(g0 + 4 * g1)
                zr, zi = z[g1]
                z[g1] = (zr * wr - zi * wi, zr * wi + zi * wr)
                if g1 % 2:
                    yield z[g1][1], 4
            z = _bfly4(z, True)
            for a0 in range(4):
                y[g0][a0] = _twiddle16(z[a0], a0 * g0, True)
            yield y[g0][3][0], 6
        for a0 in range(4):
            z = _bfly4([y[g0][a0] for g0 in range(4)], True)
            for a1 in range(4):
                t_buf[4 * a1 + a0, 0, rows, :] = z[a1][0]
                t_buf[4 * a1 + a0, 1, rows, :] = z[a1][1]
            yield [v for pair in z for v in pair], 6

    def filter_all():
        for n, (k0, h) in enumerate(_ROWGROUPS):
            rows = pl.ds(k0 // 2 + 72 * h, 8, stride=9)
            yield from filter_rows(8 * n, lambda f1: (
                _unpack(now(wr_r)[f1, rows, :], k0 % 2),
                _unpack(now(wi_r)[f1, rows, :], k0 % 2)))

    def radix9_inv(c):
        odd = lax.broadcasted_iota(jnp.int32, (8, 128), 0) & 1
        sign = jnp.where(odd == 1, -1.0 / (S * D), 1.0 / (S * D))
        last = [sign * now(nyq_r)[pl.ds(2 * c + e, 1), :] for e in range(2)]
        for i in range(8):
            y = []
            for e in range(2):
                y.append(_bfly9_inv(
                    [now(t_r)[2 * c + e, i // 4, pl.ds(256 + 8 * (i % 4), 8), :] + last[e]]
                    + [now(t_r)[2 * c + e, o % 2, pl.ds(64 * (o // 2) + 8 * i, 8), :]
                       for o in range(8)]))
                yield y[e][8], 10
            out = [_pack(y[0][j], y[1][j]) for j in range(9)]
            for j in range(9):
                y_t[c, pl.ds(64 * j + 8 * i, 8), :] = out[j]
            if c == i == 0:
                out[8] = now(y_r)[0, pl.ds(512, 8), :]
            yield out, 5

    def y_to_token_major(c):
        for q in range(4):
            vt = y_t[c, pl.ds(64 + 128 * q, 128), :].T
            stage[4 + q, pl.ds(c, 128, stride=8), :] = vt
            yield vt[120:], 43, 240

    def y_seam_to_token_major():
        for c in range(8):
            vt = jnp.concatenate([_zeros_w(64), y_t[c, pl.ds(0, 64), :]], axis=0).T
            y_seam[c] = vt
            yield vt[120:], 43, 240

    def k_rows(kt):
        return min(128 * kt, D - 128)

    def x_to_token_major(tiles, kts):
        for kt in kts:
            for t in tiles:
                vt = xa_raw[pl.ds(k_rows(kt), 128), pl.ds(128 * t, 128)].T
                vt = pltpu.bitcast(vt, U32)
                for u in range(8):
                    x_nat[kt][pl.ds(72 * t + 9 * u, 8), :] = vt[8 * u:8 * u + 8]
                yield vt[56:], 22, 180

    def x_rows(half, c, i=0, n=64):
        return pl.ds(576 * half + 9 * i + c, n, stride=9)

    def difference(u, v):
        return _pack(_unpack(u, 0) - _unpack(v, 0), _unpack(u, 1) - _unpack(v, 1))

    def low_lanes(rows, n=64):
        return lax.broadcasted_iota(jnp.int32, (rows, 128), 1) < n

    def x_prep(half, gam):
        for i in range(0, 64, 8):
            (a3, a4), (b3, b4) = [[x_nat[kt][x_rows(half, 2 * gam + e, i, 8), :] for kt in (3, 4)]
                                  for e in range(2)]
            out = [jnp.where(low_lanes(8), lo, hi) for lo, hi in
                   ((a3, difference(a3, b3)), (b3, difference(b4, a4)), (b4, a4))]
            for j in range(3):
                x_seam[4 * half + gam, j, pl.ds(i, 8), :] = out[j]
            yield out, 5

    def w_prep(part, kts=range(5)):
        col0, _ = _W_COLS[part]
        first = 288 * part - col0 // 2
        for kt in kts:
            for nt in range(5):
                nn = min(128, 3 * D - col0 - 128 * nt)
                vt = wq_raw[pl.ds(k_rows(kt), 128), pl.ds(col0 + 128 * nt, nn)].T
                vt = pltpu.bitcast(vt, U32)
                wt_nat[kt, pl.ds(64 * nt, nn // 2), :] = vt
                yield vt[-8:], 22, 180
        for kt in kts:
            for i in range(2):
                for dl in range(9):
                    base = first + 144 * i + dl
                    wa = now(wn_r)[kt, pl.ds(base, 8, stride=18), :]
                    wb = now(wn_r)[kt, pl.ds(base + 9, 8, stride=18), :]
                    out = [_pack(_unpack(wa, e), _unpack(wb, e)) for e in range(2)]
                    for e in range(2):
                        rows = pl.ds(16 * (2 * dl + e) + 8 * i, 8)
                        wt[part][kt, rows, :] = out[e]
                        if kt == 4:
                            wt[part][5, rows, :] = jnp.where(
                                low_lanes(8), wt[part][3, rows, :], out[e])
                    yield out, 2 + 2 * (kt == 4)

    def wo_prep():
        for ct in range(4):
            rows = pl.ds(224 + 32 * (ct % 2), 32)
            wo_diff[ct] = difference(wo_raw[ct, rows, :], wo_raw[ct ^ 1, rows, :])
        for kt in range(5):
            vt = pltpu.bitcast(wo_last[pl.ds(k_rows(kt), 128), :].T, U32)
            wo_tail[kt] = vt
            yield vt[24:], 22, 180

    scale = float(DH) ** -0.5

    def softmax(unit, d_block):
        half, gam, hg = unit // 16, unit // 4 % 4, unit % 4
        base = 2 * gam + 1
        acc = [[None] * W for _ in range(2)]
        for d0 in range(0, DH, d_block):
            rows = [pl.ds(144 * hg + 8 * d, 8) for d in range(d0, d0 + d_block)]
            q = [[now(q_r[4 * half + gam])[e, r, :] for r in rows] for e in range(2)]
            for l in range(9):
                for n, r in enumerate(rows):
                    k = now(k_r[half])[base + l, r, :]
                    for e in range(2):
                        w = 7 + e - l
                        if 0 <= w < W:
                            t = q[e][n] * k
                            acc[e][w] = t if acc[e][w] is None else acc[e][w] + t
                done = [acc[e][7 + e - l] for e in range(2) if 0 <= 7 + e - l < W]
                yield done, d_block / 2 * len(done)
        prob = []
        for e in range(2):
            lg = [jnp.where(low_lanes(8, 2), -1e9 / scale, acc[e][w])
                  if half == 0 and 2 * gam + e < w else acc[e][w] for w in range(W)]
            m = lg[0]
            for w in range(1, W):
                m = jnp.maximum(m, lg[w])
            ex = [jnp.exp2((l_ - m) * (scale * float(np.log2(np.e)))) for l_ in lg]
            tot = ex[0]
            for w in range(1, W):
                tot = tot + ex[w]
            inv = pl.reciprocal(tot, approx=True)
            inv = inv + inv * (1.0 - tot * inv)
            prob.append([x_ * inv for x_ in ex])
            yield prob[e][W - 1], 11, 30
        return prob

    def weigh_values(unit, prob):
        half, gam, hg = unit // 16, unit // 4 % 4, unit % 4
        base = 2 * gam + 1
        for d in range(DH):
            vv = [now(v_r[half])[base + l, pl.ds(144 * hg + 8 * d, 8), :] for l in range(9)]
            o = []
            for e in range(2):
                t = prob[e][0] * vv[7 + e]
                for w in range(1, W):
                    t = t + prob[e][w] * vv[7 + e - w]
                o.append(t)
            if d % 2:
                o = [_pack(even[e], o[e]) for e in range(2)]
                for e in range(2):
                    o_t[half][2 * gam + e, pl.ds(72 * hg + d // 2, 8, stride=DH // 2), :] = o[e]
            even = o
            yield o, 8

    def attend(units, d_block):
        for n in units:
            prob = yield from softmax(n, d_block)
            yield from weigh_values(n, prob)

    def softmax_ahead(units, d_block):
        for n in units:
            prob = yield from softmax(n, d_block)
            for e in range(2):
                for w in range(W):
                    p_buf[n, pl.ds(8 * (W * e + w), 8), :] = prob[e][w]

    def weigh_values_later(units):
        for n in units:
            prob = [[now(p_r)[n, pl.ds(8 * (W * e + w), 8), :] for w in range(W)]
                    for e in range(2)]
            yield from weigh_values(n, prob)

    def o_to_token_major(half, gams):
        for c in [2 * gam + e for gam in gams for e in range(2)]:
            for kt in range(5):
                vt = pltpu.bitcast(_bf(o_t[half][c, pl.ds(k_rows(kt) // 2, 64), :]).T, U32)
                o_nat[half][kt, pl.ds(c, 64, stride=9), :] = vt
                yield vt[56:], 22, 180

    def table(off, i):
        return _bf(tab[pl.ds(off[i], off[i + 1] - off[i]), :])

    def dft64(a, gi):
        x1 = _dot_nt(table(_OFF_LF, gi)[:128 if gi < 4 else 72],
                     _bf(u_nat[gi, pl.ds(a, 64, stride=17), :]))
        n = 64 if gi < 4 else NR - 256
        side.run(x1.shape[0] / 4)
        x1_buf[a, 0, pl.ds(64 * gi, n), :] = x1[:n]
        x1_buf[a, 1, pl.ds(64 * gi, n), :] = x1[n:2 * n]
        if gi == 4:
            nyq[pl.ds(a, 1), :] = x1[2 * n + a % 8:2 * n + a % 8 + 1]
        if a % 4 == 3:
            fetch_next(x1)

    def dft128(a):
        side.run(216)
        xr, xi = x1_buf[a, 0], x1_buf[a, 1]
        k1 = _dot(xr + xi, gmat[a, 0])
        t_buf[a, 0, pl.ds(0, NR), :] = k1 - _dot(xi, gmat[a, 1])
        t_buf[a, 1, pl.ds(0, NR), :] = k1 + _dot(xr, gmat[a, 2])

    def gmat_rows(a, c):
        return jnp.concatenate([gmat[a, c, pl.ds(16 * tau + e, 8, stride=2), :]
                                for tau in range(8) for e in range(2)], axis=0)

    def nyquist(step):
        twr, twi = [pltpu.bitcast(tab[pl.ds(off, 16), :], F32) for off in (_OFF_TR, _OFF_TI)]
        if step == 0:
            re = _dot(nyq[pl.ds(0, 16), :], gmat[0, 0])
            im = re + _dot(nyq[pl.ds(0, 16), :], gmat[0, 2])
            re, im = re * twr - im * twi, re * twi + im * twr
        elif step == 2:
            row = lax.broadcasted_iota(jnp.int32, (8, 128), 0)
            w = []
            for i in range(2):
                for f8 in (0, 8):
                    t = jnp.zeros((8, 128), F32)
                    for f in range(8):
                        v = wlast[i, :, pl.ds(128 * (f8 + f), 128)].astype(F32)
                        t = jnp.where(row == f, v, t)
                    w.append(t)
            wr, wi = jnp.concatenate(w[:2], axis=0), jnp.concatenate(w[2:], axis=0)
            re, im = nyq[pl.ds(0, 16), :], nyq[pl.ds(16, 16), :]
            re, im = re * wr - im * wi, re * wi + im * wr
        elif step == 4:
            re, im = nyq[pl.ds(0, 16), :], nyq[pl.ds(16, 16), :]
            re = _dot_nt(re + im, gmat_rows(0, 0)) + _dot_nt(im, gmat_rows(0, 2))
        else:
            x = _dot(table(_OFF_16, step // 2),
                     jnp.concatenate([nyq[...], jnp.zeros((96, 128), F32)], axis=0))
            re, im = x[:16], x[16:]
            if step == 3:
                re, im = re * twr + im * twi, im * twr - re * twi
        nyq[pl.ds(0, 16), :] = re
        nyq[pl.ds(16, 16), :] = im
        side.absorb(([re[:8], re[8:], im[:8], im[8:]], 0, 200))

    def idft128(a):
        side.run(216)
        g = [gmat_rows(a, c) for c in range(3)]
        tr, ti = t_buf[a, 0, pl.ds(0, NR), :], t_buf[a, 1, pl.ds(0, NR), :]
        k1 = _dot_nt(tr + ti, g[0])
        z_buf[a % 2, 0] = k1 + _dot_nt(ti, g[2])
        z_buf[a % 2, 1] = k1 - _dot_nt(tr, g[1])

    def idft64(a):
        side.run(144)
        for gi in range(5):
            n = 64 if gi < 4 else NR - 256
            parts = [z_buf[a % 2, c, pl.ds(64 * gi, n), :] for c in range(2)]
            if n < 64:
                parts.append(jnp.zeros((128 - 2 * n, 128), F32))
            o = _dot(table(_OFF_LI, gi), jnp.concatenate(parts, axis=0))
            if gi < 4:
                t_buf[a, 0, pl.ds(64 * gi, 64), :] = o[:64]
                t_buf[a, 1, pl.ds(64 * gi, 64), :] = o[64:]
            else:
                t_buf[a, 0, pl.ds(256, 32), :] = o[:32]
                t_buf[a, 1, pl.ds(256, 32), :] = o[32:]

    def proj(part, half, gam, kts=(0, 1, 2, 3), chunks=4, only=None):
        m = 288 // chunks
        last = kts[-1] == 3
        for ch in only or range(chunks):
            side.run((len(kts) + last / 2) * m)
            w = lambda kt: _bf(wt[part][kt, pl.ds(m * ch, m), :])
            both = _dot_nt(w(4), _bf(x_seam[4 * half + gam, 2])) if last else None
            for e in range(2):
                c = 2 * gam + e
                x = [x_seam[4 * half + gam, e] if kt == 3 else x_nat[kt][x_rows(half, c), :]
                     for kt in kts]
                tile = _dot_nt(
                    jnp.concatenate([w(3 + 2 * e if kt == 3 else kt) for kt in kts], axis=1),
                    jnp.concatenate([_bf(x_) for x_ in x], axis=1))
                if last:
                    tile = tile + both
                if part == 0:
                    buf, slot = q_buf[4 * half + gam], e
                else:
                    buf, slot = (k_buf if part == 1 and last else v_buf)[half], 8 + c
                rows = []
                for i in range(m // 4):
                    d, hg = divmod(m // 4 * ch + i, 4)
                    rows.append(pl.ds(144 * hg + 8 * d, 8))
                if kts[0]:
                    sums = v_buf[half] if part else buf
                    tile = tile + jnp.concatenate([sums[slot, r, :] for r in rows], axis=0)
                for i, r in enumerate(rows):
                    buf[slot, r, :] = tile[8 * i:8 * i + 8]
                if part == 0 or not last:
                    continue
                if c:
                    if half:
                        before = (k_buf, v_buf)[part - 1][0]
                        tile = jnp.where(low_lanes(2 * m, 126), tile, jnp.concatenate(
                            [before[slot, r, :] for r in rows], axis=0))
                    tile = pltpu.roll(tile, 2, 1)
                    for i, r in enumerate(rows):
                        buf[c, r, :] = tile[8 * i:8 * i + 8]
                        if part == 2 and half == 0:
                            pltpu.store(buf.at[c, r, :], buf[0, r, :], mask=low_lanes(8, 2))
                elif part == 2 and half == 0:
                    tile = jnp.where(low_lanes(2 * m, 1), tile, pltpu.roll(tile, 1, 1))
                    for i, r in enumerate(rows):
                        buf[0, r, :] = tile[8 * i:8 * i + 8]
            fetch_next(tile)

    def out_proj(half, row0, cw):
        side.run(9 * cw)
        o = [jnp.concatenate([o_nat[half][kt, pl.ds(9 * b, 8), :]
                              for b in range(row0 // 8, (row0 + cw) // 8)], axis=0)
             for kt in range(5)]
        lhs = [jnp.concatenate([_bf(t) for t in o[:3] + [last]], axis=1)
               for last in (o[3], jnp.where(low_lanes(cw), o[3], o[4]))]
        both = _dot(_bf(o[4]), jnp.concatenate(
            [_bf(jnp.concatenate([wo_raw[ct + 1, pl.ds(224, 32), :],
                                  wo_raw[ct, pl.ds(256, 32), :]], axis=0))
             for ct in (0, 2)], axis=1))
        r = [_dot(lhs[n], jnp.concatenate(
            [_bf(jnp.concatenate([wo_raw[ct, pl.ds(0, 224), :], wo_diff[ct]], axis=0))
             for ct in (n, n + 2)], axis=1)) for n in range(2)]
        for ct in (0, 2, 1, 3):
            cols = slice(128 * (ct // 2), 128 * (ct // 2) + 128)
            tile = (r[ct % 2][:, cols] + both[:, cols]).astype(BF16)
            stage[ct, pl.ds(512 * half + row0, cw), :] = pltpu.bitcast(tile, U32)
            cp_out(ct, 512 * half + row0, cw).start()

    def out_tail(half, gam):
        side.run(144)
        o = [o_t[half][2 * gam + e] for e in range(2)]
        w = [wo_tail[kt] for kt in range(5)]
        both = _dot(_bf(w[4]), _bf(jnp.concatenate([o[1][224:256], o[0][256:]], axis=0)))
        for e, last in enumerate((w[3], jnp.where(low_lanes(32), w[3], w[4]))):
            c, rows = 2 * gam + e, slice(224 + 32 * e, 256 + 32 * e)
            tile = both + _dot(
                jnp.concatenate([_bf(t) for t in w[:3] + [last]], axis=1),
                _bf(jnp.concatenate([o[e][:224], difference(o[e][rows], o[1 - e][rows])], axis=0)))
            tile = jnp.concatenate([tile, jnp.zeros((64, 128), F32)], axis=0).astype(BF16)
            stage_seam[pl.ds(512 * half + c, 64, stride=8), :] = jnp.where(
                low_lanes(64), pltpu.bitcast(tile.T, U32), y_seam[c, pl.ds(64 * half, 64), :])

    pair = 1296
    unit = 315
    early = 3

    def end_region():
        pl.semaphore_signal(sem_region)
        pl.semaphore_wait(sem_region)

    def queries(i0, i1, chunks=4):
        while i0 < i1:
            n = chunks if i0 % (4 // chunks) == 0 and i0 + 4 // chunks <= i1 else 4
            proj(0, i0 // 16, i0 // 4 % 4, (1, 2, 3) if i0 < 4 * early else (0, 1, 2, 3),
                 chunks=n, only=(i0 % 4 * n // 4,))
            i0 += 4 // n

    def cycles(i0, i1):
        return sum(pair / 4 - 72 * (i < 4 * early) for i in range(i0, i1))

    def block(i):
        row0, rows = ((128, 256), (384, D - 384))[i - 1]
        return cp_wq(1, row0, rows, sem.at[i]), cp_xa(range(8), row0, rows, sem.at[i])

    first = cp_xa(range(8), 0, 128, sem_xb), cp_wq(1, 0, 128, sem_k), cp_wq(0, 0, 128, sem_out)
    for cp in first + block(1):
        cp.start()
    first[0].wait()
    for cp in block(2):
        cp.start()
    _drain(x_to_token_major(range(8), (0,)))
    first[1].wait()
    _drain(w_prep(1, (0,)))
    first[2].wait()
    side.start(pltpu.bitcast(wq_raw[pl.ds(0, 16), pl.ds(512, 128)], U32), x1_buf.at[16, 0])
    side.open()
    fetches += [[partial(fetch_xa, range(8, 16), r, 192, sem_k)] for r in range(0, D, 192)]
    side.add("prep", w_prep(0, (0,)), 0.5)
    for gam in range(4):
        proj(1, 0, gam, (0,))
    side.close()

    for cp in block(1):
        cp.wait()
    side.open()
    fetches += [[partial(fetch_wq, 0, r, 224, sem_xb)] for r in range(128, D, 224)]
    fetches += [[partial(fetch_xb, t)] for t in range(16)]
    side.add("prep", x_to_token_major(range(8), (1, 2)), 0.8)
    for kt in (1, 2):
        side.add("prep", w_prep(1, (kt,)), 0.8)
    for gam in range(early):
        proj(0, 0, gam, (0,))
    side.finish("prep")
    for gam in (0, 1):
        proj(1, 0, gam, (1, 2))
    side.close()

    for cp in block(2):
        cp.wait()
    side.open()
    fetches += [[partial(fetch_wq, 2, r, 144, sem_tab) for r in range(0, D, 144)]]
    fetches += [[partial(fetch_tab, r, min(304, n_tab - r)) for r in range(0, n_tab, 304)]]
    side.add("prep", x_to_token_major(range(8), (3, 4)), 0.8)
    side.add("prep", x_prep(0, 0), 0.8)
    for kt in (3, 4):
        side.add("prep", w_prep(1, (kt,)), 0.8)
    for gam in (2, 3):
        proj(1, 0, gam, (1, 2))
    for gam in range(1, 4):
        side.add("prep", x_prep(0, gam), 0.5)
    side.close()

    cp_xa(range(8, 16), 0, D, sem_k).wait()
    side.open()
    fetches += [[partial(fetch_f, t) for t in range(4)]]
    side.add("prep", x_to_token_major(range(8, 16), range(5)), 0.6)
    side.add("prep", x_prep(1, 0), 0.6)
    for gam in range(4):
        proj(1, 0, gam, (3,))
    side.finish("prep")
    for gam in range(3):
        side.add("prep", x_prep(1, gam + 1), 0.5)
        proj(1, 1, gam, only=range(4 - (gam == 2)))
        side.finish("prep")
    side.close()

    assert not fetches
    pltpu.make_async_copy(xb_raw, xb_raw, sem_xb).wait()
    cp_wq(0, 128, D - 128, sem_xb).wait()
    side.open(0.85, 20.0)
    load = (8 * 232 + 620) / (1.25 * pair + cycles(0, 7)) * 0.9
    side.add("w", w_prep(0, range(1, 5)), load)
    for tau in range(8):
        side.add("r9", radix9(tau), load)
    proj(1, 1, 2, only=(3,))
    proj(1, 1, 3)
    side.finish("w")
    queries(0, 7)
    side.close()

    cp_tab(0, n_tab).wait()
    cp_wq(2, 0, D, sem_tab).wait()
    side.open(0.95, 50.0, links=3)
    fetches += [[partial(fetch_f, t)] for t in range(4, 16)]
    fetches += [[partial(fetch_wo, i)] for i in range(4)]
    fetches.append([wo_settle])
    side.add("t", u_to_token_major(0), 0.855)
    load = (768 + 766 + 4 * 168) / (5792 + cycles(7, 10) - 2000) * 0.95
    for a in range(16):
        side.add("g%d" % a, dft_matrix(a), load)
    queries(7, 10)
    side.finish("t")
    for gi in range(5):
        if gi < 4:
            side.add("t", u_to_token_major(gi + 1), 0.855, first=True)
        for a in range(16):
            dft64(a, gi)
        side.finish("t")
    side.add("w", w_prep(2), load)
    side.add("att", softmax_ahead(range(4), 6), load)
    for a in range(16):
        side.finish("g%d" % a)
        dft128(a)
        if a in (2, 6):
            nyquist(a // 4)
    side.close()

    assert not fetches
    pltpu.make_async_copy(wr_raw, wr_raw, sem_f).wait()
    pltpu.make_async_copy(wi_raw, wi_raw, sem_f).wait()
    for cp in [cp_flast(0), cp_flast(1)] + [cp_wo(ct) for ct in range(5)]:
        cp.wait()
    side.open(1.0, links=2)
    side.add("f", filter_all(), 36 * 120 / (4 * pair + cycles(10, 18)))
    for gam in range(4):
        proj(2, 0, gam, chunks=1)
    queries(10, 18, 1)
    side.close()
    end_region()

    side.open(0.9, 20.0, links=2)
    load = (16 * unit - 4 * 168 + 8 * 200) / (5760 + 4 * pair + cycles(18, 20)) * 0.95
    side.add("att", weigh_values_later(range(4)), load)
    side.add("att", attend(range(4, 16), 9), load)
    idft128(0)
    for a in range(16):
        if a < 15:
            idft128(a + 1)
        idft64(a)
        if a in (2, 6, 10):
            nyquist(2 + a // 4)
    for c in range(8):
        side.add("r9", radix9_inv(c), load * 1.1)
    for gam in range(4):
        proj(2, 1, gam, chunks=2)
    queries(18, 20)
    side.close()
    end_region()

    side.open(0.9, links=2)
    period = 3 * pair / 63 * 0.85
    side.add_paced(o_to_token_major(0, range(4)), period / 2)
    for c in range(8):
        side.add_paced(y_to_token_major(c), period)
    side.add_paced(y_seam_to_token_major(), period)
    side.add_paced(wo_prep(), period / 2)
    load = 7 * unit / (3 * pair) * 0.945
    side.add("att", attend(range(16, 20), 6), load)
    queries(20, 24)
    side.add("att", attend(range(20, 23), 6), load)
    queries(24, 32)
    side.close()
    for ct in range(5, 9):
        cp_out(ct, 0, S // 2).start()
    end_region()

    side.open(1.0, 700.0, links=2)
    side.add_paced(o_to_token_major(1, range(1)), 60.0)
    side.add("att", attend(range(23, 32), 9), 9 * unit / (9 * 496 + 4 * 144))
    for gam in range(4):
        out_tail(0, gam)
    for row0 in range(0, 496, 64):
        out_proj(0, row0, min(64, 496 - row0))
    cp_out(4, 0, 512).start()
    side.close()
    end_region()

    _drain(o_to_token_major(1, range(1, 4)))
    for gam in range(4):
        out_tail(1, gam)
    cp_out(4, 512, 512).start()
    out_proj(0, 496, 16)
    row0 = 0
    for cw in (64,) * 7 + (32, 16, 16):
        out_proj(1, row0, cw)
        row0 += cw
    pltpu.make_async_copy(out_hbm, out_hbm, sem_out).wait()


@jax.jit
def pallas_concat_heads__sliding_local_dilated__spectral_gfnet__prompt_kernel(
    A_x: jax.Array,
    A_wqkv: jax.Array,
    A_wo: jax.Array,
    B_x: jax.Array,
    B_w_r: jax.Array,
    B_w_i: jax.Array,
):
    assert A_x.shape == (1, S, D) and B_x.shape == (1, S, D)
    any_spec = pl.BlockSpec(memory_space=pl.ANY)
    scratch = [
        pltpu.VMEM((1,) + _TABLE.shape, U32),
        pltpu.VMEM((16, 288, 128), U32),
        pltpu.VMEM((D, S), BF16),
        pltpu.VMEM((D, 3 * D), BF16),
        pltpu.VMEM((5, D // 2, 128), U32),
        pltpu.VMEM((D, D - 512), BF16),
        pltpu.VMEM((1, 16, 144, 128), U32),
        pltpu.VMEM((1, 16, 144, 128), U32),
        pltpu.VMEM((2, 1, S), BF16),
        pltpu.VMEM((1, 16, 3, 128, 128), F32),
        pltpu.VMEM((1, 8, D, 128), U32),
        pltpu.VMEM((1, 8, D, 128), U32),
        pltpu.VMEM((5, 8 * 136, 128), U32),
        pltpu.VMEM((1, 18, 2, NR, 128), F32),
        pltpu.VMEM((1, 16, 2, NR + 8, 128), F32),
        pltpu.VMEM((1, 2, 2, NR, 128), F32),
        pltpu.VMEM((1, 32, 128), F32),
        [pltpu.VMEM((1, 9 * 128, 128), U32)] * 5,
        pltpu.VMEM((1, 8, 3, 64, 128), U32),
        pltpu.VMEM((1, 5, 320, 128), U32),
        [pltpu.VMEM((1, 6, 288, 128), U32)] * 3,
        pltpu.VMEM((1, 4, 32, 128), U32),
        pltpu.VMEM((1, 5, 32, 128), U32),
        [pltpu.VMEM((1, 2, D + 16, 128), F32)] * 8,
        [pltpu.VMEM((1, 16, D + 8, 128), F32)] * 2,
        [pltpu.VMEM((1, 16, D + 8, 128), F32)] * 2,
        pltpu.VMEM((1, 4, 2 * W * 8, 128), F32),
        [pltpu.VMEM((1, 8, D // 2, 128), U32)] * 2,
        [pltpu.VMEM((1, 5, 9 * 64, 128), U32)] * 2,
        pltpu.VMEM((1, 8, 128, 128), U32),
        pltpu.VMEM((8, S // 2, 128), U32),
        pltpu.VMEM((S // 2, 128), U32),
        pltpu.SMEM((4,), jnp.int32),
        pltpu.SemaphoreType.DMA((5,)),
        pltpu.SemaphoreType.REGULAR,
    ]
    out = pl.pallas_call(
        _kernel,
        out_shape=jax.ShapeDtypeStruct((S, 2 * D), BF16),
        in_specs=[any_spec] * 7,
        out_specs=any_spec,
        scratch_shapes=scratch,
        compiler_params=pltpu.CompilerParams(vmem_limit_bytes=120 * 1024 * 1024),
        name="attn_gfnet",
    )(A_x[0].T, A_wqkv, A_wo, B_x[0].T, B_w_r.T, B_w_i.T, _TABLE)
    return out[None]
```
